```python
import jax
import jax.numpy as jnp

def _softmax(x, axis=-1):
    return jax.nn.softmax(x, axis=axis)

def _gelu(x):
    return jax.nn.gelu(x, approximate=True)

def _silu(x):
    return jax.nn.silu(x)

def _sigmoid(x):
    return jax.nn.sigmoid(x)

def _layernorm(x, axis=-1, eps=1e-05):
    m = jnp.mean(x, axis=axis, keepdims=True)
    v = jnp.var(x, axis=axis, keepdims=True)
    return (x - m) / jnp.sqrt(v + eps)

def _scatter_add(tgt, idx, src, axis=0):
    return tgt.at[idx].add(src)

def _segment_sum(src, seg, n):
    return jax.ops.segment_sum(src, seg, n)

class _Rng:

    def __init__(self, key):
        self._k = key

    def _next(self):
        self._k, sub = jax.random.split(self._k)
        return sub

    def normal(self, shape):
        return jax.random.normal(self._next(), shape, dtype=jnp.bfloat16)

    def randint(self, lo, hi, shape):
        return jax.random.randint(self._next(), shape, lo, hi, dtype=jnp.int32)

    def uniform(self, shape, lo=0.0, hi=1.0):
        return jax.random.uniform(self._next(), shape, jnp.bfloat16, lo, hi)

    def permutation(self, n):
        return jax.random.permutation(self._next(), n)
kernel_name = 'adaLN_cond__linear_kernel_hedgehog__moe_arch_mod__prompt'

def setup_inputs():
    _rng = _Rng(jax.random.key(int.from_bytes(__import__("os").urandom(4), "little")))
    _w = lambda a: (lambda t: t.astype(jnp.bfloat16) if jnp.issubdtype(t.dtype, jnp.floating) else t)(jnp.asarray(a))

    def _A_setup():
        B, S, D, H = (1, 2048, 1024, 32)
        Dh = D // H
        return {'x': _w((lambda *s: _rng.normal(s) * 0.05)(B, S, D)), 'wqkv': _w((lambda *s: _rng.normal(s) * 0.05)(D, 3 * D)), 'w_phi': _w((lambda *s: _rng.normal(s) * 0.05)(H, Dh, Dh) * Dh ** (-0.5)), 'wo': _w((lambda *s: _rng.normal(s) * 0.05)(D, D))}
    _A_in = _A_setup()

    def _B_setup():
        B, S, D, F, C = (1, 2048, 1024, 3584, 2)
        return {'x': _w((lambda *s: _rng.normal(s) * 0.05)(B, S, D)), 'w_r': _w((lambda *s: _rng.normal(s) * 0.05)(D)), 'w_gate': _w((lambda *s: _rng.normal(s) * 0.05)(D, F)), 'w_up': _w((lambda *s: _rng.normal(s) * 0.05)(D, F)), 'w_down': _w((lambda *s: _rng.normal(s) * 0.05)(F, D))}
    _B_in = _B_setup()
    return {'A_x': _A_in['x'], 'A_wqkv': _A_in['wqkv'], 'A_w_phi': _A_in['w_phi'], 'A_wo': _A_in['wo'], 'B_x': _B_in['x'], 'B_w_r': _B_in['w_r'], 'B_w_gate': _B_in['w_gate'], 'B_w_up': _B_in['w_up'], 'B_w_down': _B_in['w_down'], 'c': _w((lambda *s: _rng.normal(s) * 0.05)(1, 1024)), 'w_mod': _w((lambda *s: _rng.normal(s) * 0.05)(1024, 6 * 1024) * 1024 ** (-0.5))}

def reference(A_x, A_wqkv, A_w_phi, A_wo, B_x, B_w_r, B_w_gate, B_w_up, B_w_down, c, w_mod):

    def _A_ref(x, wqkv, w_phi, wo):
        B, S, D = x.shape
        H = 32
        Dh = D // H
        qkv = (lambda x, *d: x.transpose(*d))((x @ wqkv).reshape(B, S, 3, H, Dh), 2, 0, 3, 1, 4)
        q, k, v = (qkv[0], qkv[1], qkv[2])
        pq = jnp.einsum('bhsd,hdf->bhsf', q, w_phi)
        pk = jnp.einsum('bhsd,hdf->bhsf', k, w_phi)
        phi_q = jnp.concatenate([_softmax(pq, axis=-1), _softmax(-pq, axis=-1)], axis=-1)
        phi_k = jnp.concatenate([_softmax(pk, axis=-1), _softmax(-pk, axis=-1)], axis=-1)
        kv = jnp.einsum('bhsf,bhsd->bhfd', phi_k, v)
        z = jnp.einsum('bhsf->bhf', phi_k)
        num = jnp.einsum('bhqf,bhfd->bhqd', phi_q, kv)
        den = jnp.einsum('bhqf,bhf->bhq', phi_q, z)[..., None] + 1e-06
        o = num / den
        return (lambda x, *d: x.transpose(*d))(o, 0, 2, 1, 3).reshape(B, S, D) @ wo

    def _B_ref(x, w_r, w_gate, w_up, w_down):
        B, S, D = x.shape
        C = 2
        r = x @ w_r
        idx = jnp.argsort(-r, axis=-1)[:, :C]
        idx_e = jnp.repeat(idx.reshape(B, C, 1), D, axis=2)
        x_sel = jnp.take_along_axis(x, idx_e, axis=1)
        g = _silu(x_sel @ w_gate)
        u = x_sel @ w_up
        y = g * u @ w_down
        r_sel = _sigmoid(jnp.take_along_axis(r, idx, axis=1))
        y = y * r_sel.reshape(B, C, 1)
        b_off = (jnp.arange(B) * S).reshape(B, 1)
        flat_idx = (idx + b_off).reshape(B * C)
        zero = (x * 0.0).reshape(B * S, D)
        upd = _scatter_add(zero, flat_idx, y.reshape(B * C, D), axis=0)
        return x + upd.reshape(B, S, D)
    x = A_x
    mod = (_silu(c) @ w_mod).reshape(c.shape[0], 6, 1, -1)
    sa, ca, ga, sb, cb, gb = (mod[:, 0].copy(), mod[:, 1].copy(), mod[:, 2].copy(), mod[:, 3].copy(), mod[:, 4].copy(), mod[:, 5].copy())
    h = _layernorm(x, axis=-1) * (1 + ca) + sa
    x = x + ga * _A_ref(h, A_wqkv, A_w_phi, A_wo)
    h = _layernorm(x, axis=-1) * (1 + cb) + sb
    x = x + gb * _B_ref(h, B_w_r, B_w_gate, B_w_up, B_w_down)
    return x
```

```python
import collections
import functools

import jax
import jax.numpy as jnp
import numpy as np
import jax.experimental.pallas as pl
import jax.experimental.pallas.tpu as pltpu

F32, BF16, I32, U32 = jnp.float32, jnp.bfloat16, jnp.int32, jnp.uint32
S, D, H, DH, FF = 2048, 1024, 32, 32, 3584
HD = D // 2
NPAIR = H // 2
EPS = 1e-5
LOG2E = float(np.log2(np.e))
NN = (((1,), (0,)), ((), ()))
NT = (((1,), (1,)), ((), ()))
TN = (((0,), (0,)), ((), ()))


def _dot(a, b, dn=NN):
    return jax.lax.dot_general(a, b, dn, preferred_element_type=F32)


def _pack(x):
    return pltpu.bitcast(x.astype(BF16), U32)


def _unpack(w):
    return pltpu.bitcast(w, BF16)


def _recip(x):
    r = pl.reciprocal(x, approx=True)
    return r * (2.0 - x * r)


def _lhs_terms(a11, a12, a21, a22):
    return (a11 + a22, a21 + a22, a11, a22, a11 + a12, a21 - a11, a12 - a22)


def _rhs_terms(b11, b12, b21, b22):
    return (b11 + b22, b11, b12 - b22, b21 - b11, b22, b11 + b12, b21 + b22)


_USES = (((0, 1), (3, 1)), ((2, 1), (3, -1)), ((1, 1), (3, 1)), ((0, 1), (2, 1)),
         ((0, -1), (1, 1)), ((3, 1),), ((0, 1),))


def _layernorm(x):
    d = x - jnp.mean(x, axis=-1, keepdims=True)
    v = jnp.mean(d * d, axis=-1, keepdims=True)
    return d * jax.lax.rsqrt(v + EPS)


def _features(p):
    rows, n = p.shape
    p3 = p.reshape(rows // DH, DH, n)
    e_pos = jnp.exp2(p3 - jnp.max(p3, axis=1, keepdims=True))
    e_neg = jnp.exp2(jnp.min(p3, axis=1, keepdims=True) - p3)
    pos = e_pos * _recip(jnp.sum(e_pos, axis=1, keepdims=True))
    neg = e_neg * _recip(jnp.sum(e_neg, axis=1, keepdims=True))
    pos = pos.reshape(rows // (2 * DH), 2 * DH, n)
    neg = neg.reshape(rows // (2 * DH), 2 * DH, n)
    return jnp.concatenate([pos, neg], axis=1)


class _Interleaver:
    def __init__(self, ratio):
        self.queue = collections.deque()
        self.ratio = ratio
        self.credit = 0.0

    def defer(self, cost, fn):
        self.queue.append((cost, fn))

    def spent(self, cycles):
        self.credit += cycles * self.ratio
        while self.queue and self.credit >= self.queue[0][0]:
            cost, fn = self.queue.popleft()
            self.credit -= cost
            fn()
        if not self.queue:
            self.credit = 0.0

    def drain(self):
        while self.queue:
            self.queue.popleft()[1]()
        self.credit = 0.0


def make(RC=128, LNC=16, FC=512, EC=16, ratio=0.55, ratio2=0.75, lag=1, vlimit=120, flags=None, S=S,
         att_cost=45, fin_cost=64):
    T = 512
    HT = T // 2
    NTILE = S // T
    G = 128

    def kernel(x_hbm, wqkv_hbm, wphi_hbm, wo_hbm, wr_hbm, wg_hbm, wu_hbm, wd_hbm, c_hbm, wmod_hbm,
               out_hbm,
               x_v, wqkv_v, wphi_v, wo_v, wr_v, wg_v, wu_v, wd_v, c_v, wmod_v,
               mod_v, bd_v, wt_v, wot_v, ht_v, phiq_v, phik_v, vt_v, kv_v, kvb_v, z_v, zb_v, ot_v,
               y_v, xn_v, out_v, r_v, fix_v, sems, xsems, osems):

        side = _Interleaver(ratio)
        copies = {}

        def add_copy(name, src, dst):
            copies[name] = pltpu.make_async_copy(src, dst, sems.at[len(copies)])

        cols = lambda i: pl.ds(i * D, D)
        add_copy("c", c_hbm, c_v)
        add_copy("wphi", wphi_hbm, wphi_v)
        add_copy("wr", wr_hbm, wr_v)
        for i in range(6):
            add_copy(("mod", i), wmod_hbm.at[:, cols(i)], wmod_v.at[i])
        for i in range(3):
            add_copy(("w", i), wqkv_hbm.at[:, cols(i)], wqkv_v.at[i])
        add_copy("wo", wo_hbm, wo_v)
        add_copy("wg", wg_hbm, wg_v)
        add_copy("wu", wu_hbm, wu_v)
        add_copy("wd", wd_hbm, wd_v)

        def start(*names):
            for n in names:
                copies[n].start()

        def wait(*names):
            for n in names:
                copies[n].wait()

        def rows_at(base, size):
            return pl.ds(base if isinstance(base, int) else pl.multiple_of(base, 16), size)

        def x_copy(t):
            return pltpu.make_async_copy(x_hbm.at[rows_at(t * T, T)], x_v.at[rows_at(t * T, T)], xsems.at[t])

        def out_copy(n):
            if isinstance(n, int):
                lo, hi = max(n * T - 2 * G, 0), min((n + 1) * T - 2 * G, S)
                rows = pl.ds(lo, hi - lo)
            else:
                rows = rows_at(n * T - 2 * G, T)
            return pltpu.make_async_copy(out_v.at[rows], out_hbm.at[rows], osems.at[n])

        def silu_c():
            cc = c_v[...].astype(F32)
            return (cc * jax.nn.sigmoid(cc)).astype(BF16)

        def modulation(i):
            m = _dot(jnp.broadcast_to(silu_c(), (16, D)), wmod_v[i])[:8]
            mod_v[i] = m + 1.0 if i in (1, 4) else m

        def router_weights():
            w = wr_v[...].astype(F32)
            mod_v[6] = jnp.concatenate(
                [jnp.broadcast_to(w[j:j + 1], (8, 128)) for j in range(D // 128)], axis=1)

        def block_diag_phi():
            row = jax.lax.broadcasted_iota(I32, (128, DH), 0)
            col = jax.lax.broadcasted_iota(I32, (128, DH), 1)
            sel = jnp.where(row % DH == col, 1.0, 0.0).astype(BF16)
            r2 = jax.lax.broadcasted_iota(I32, (128, 128), 0) // DH
            c2 = jax.lax.broadcasted_iota(I32, (128, 128), 1) // DH
            for g in range(D // 128):
                tiled = _dot(sel, wphi_v[pl.ds(g * 128, 128), :], NT)
                bd_v[g] = _pack(jnp.where(r2 == c2, tiled, 0.0))

        def prep_weight(i):
            def group(g, carry):
                eye = jnp.where(jax.lax.broadcasted_iota(I32, (128, 128), 0)
                                == jax.lax.broadcasted_iota(I32, (128, 128), 1), 1.0, 0.0).astype(BF16)
                parts = []
                for gg in (g, g + HD // 128):
                    for half in range(2):
                        w = wqkv_v[i, pl.ds(half * HD, HD), pl.ds(pl.multiple_of(gg * 128, 128), 128)]
                        if i == 2:
                            parts.append(_dot(eye, w, NT))
                        else:
                            parts.append(_dot(_unpack(bd_v[gg]), w, NT) * LOG2E)
                for j, term in enumerate(_lhs_terms(*parts)):
                    wt_v[i, j, pl.ds(pl.multiple_of(g * 64, 64), 64), :] = _pack(term)
                return carry

            jax.lax.fori_loop(0, HD // 128, group, 0)

        def prep_wo():
            for r in range(0, HD, 32):
                lo = wo_v[pl.ds(r, 32), :].astype(F32)
                hi = wo_v[pl.ds(HD + r, 32), :].astype(F32)
                terms = _rhs_terms(lo[:, :HD], lo[:, HD:], hi[:, :HD], hi[:, HD:])
                for j, term in enumerate(terms):
                    wot_v[j, pl.ds(r // 2, 16), :] = _pack(term)

        start("c", "wphi", "wr", ("w", 1), ("mod", 1), ("mod", 0))
        x_copy(0).start()
        wait("c")
        bits = pltpu.bitcast(jnp.broadcast_to(c_v[:, :128].astype(F32), (8, 128)), I32)
        zero = jnp.minimum(jnp.max(bits & 0xFF), 0)
        latest = {}

        def hold_rows():
            back = jnp.minimum(zero & 255, S // 16) * 16
            x_v[pl.ds(pl.multiple_of(S - back, 16), 16), pl.ds(0, 128)] = latest["m"].astype(BF16)

        def norm1_unit(t, slot, n):
            r = n * LNC
            half = n * (LNC // 2)
            half = half if isinstance(half, int) else pl.multiple_of(half, LNC // 2)
            hs = []
            for offset in (r, HT + r):
                xx = x_v[rows_at(t * T + offset, LNC), :].astype(F32)
                hh = _layernorm(xx).reshape(LNC // 8, 8, D) * mod_v[1] + mod_v[0]
                hs.append(hh.reshape(LNC, D))
            a, b = hs
            terms = _rhs_terms(a[:, :HD], b[:, :HD], a[:, HD:], b[:, HD:])
            for j, term in enumerate(terms):
                ht_v[slot, j, pl.ds(half, LNC // 2), :] = _pack(term)

        def strassen(product, cycles, extra):
            quads = [None] * 4
            waiting = collections.deque()

            def absorb():
                j, m = waiting.popleft()
                for q, sign in _USES[j]:
                    if quads[q] is None:
                        quads[q] = m
                    else:
                        quads[q] = quads[q] + m if sign > 0 else quads[q] - m

            for j in range(7):
                m = product(j)
                latest["m"] = m[-16:, -128:]
                waiting.append((j, m))
                if len(waiting) > lag:
                    absorb()
                side.spent(cycles)
                extra()
            while waiting:
                absorb()
            return quads

        def project(i, slot, r, extra):
            return strassen(
                lambda j: _dot(_unpack(wt_v[i, j, pl.ds(r // 2, RC // 2), :]), _unpack(ht_v[slot, j]), NT),
                RC * HT // 128, extra)

        def keys(slot, extra):
            for r in range(0, HD, RC):
                quads = project(1, slot, r, extra)

                def unit(half, o, quads=quads, r=r):
                    pair = (half * HD + r + o) // 64
                    acc = z_v[pair]
                    for part in range(2):
                        phi = _features(quads[2 * half + part][o:o + 64])[0]
                        phik_v[pair, :, pl.ds(part * HT, HT)] = _pack(phi)
                        for l in range(0, HT, 128):
                            acc = acc + phi[:, l:l + 128]
                    z_v[pair] = acc

                for half in range(2):
                    for o in range(0, RC, 64):
                        side.defer(T // 16 * 20 / 4, functools.partial(unit, half, o))

        def queries(t, slot, extra):
            for r in range(0, HD, RC):
                quads = project(0, slot, r, extra)

                def unit(half, o, quads=quads, r=r):
                    pair = (half * HD + r + o) // 64
                    for part in range(2):
                        phi = _features(quads[2 * half + part][o:o + 64])[0]
                        phiq_v[t, pair, :, pl.ds(part * HT, HT)] = _pack(phi)

                for half in range(2):
                    for o in range(0, RC, 64):
                        side.defer(T // 16 * 18 / 4, functools.partial(unit, half, o))

        def values(slot, extra):
            for r in range(0, HD, RC):
                quads = project(2, slot, r, extra)
                for half in range(2):
                    for part in range(2):
                        vt_v[pl.ds((half * HD + r) // 2, RC // 2), pl.ds(part * HT, HT)] = _pack(
                            quads[2 * half + part])

        def accumulate_kv(j):
            kv_v[j] += _dot(_unpack(vt_v[pl.ds(j * 32, 32), :]), _unpack(phik_v[j]), NT)
            side.spent(T // 8)

        def finish_kv(j):
            rh = jax.lax.broadcasted_iota(I32, (64, 128), 0) // DH
            ch = (jax.lax.broadcasted_iota(I32, (64, 128), 1) % 64) // DH
            kvb_v[j] = _pack(jnp.where(rh == ch, kv_v[j], 0.0))
            zb_v[j] = jnp.broadcast_to(jnp.sum(z_v[j], axis=-1, keepdims=True), (128, 128))

        def attend(t, part, slot, i):
            lanes = pl.ds(part * HT, HT)
            outs = {}
            for half in range(2):
                for k in range(2):
                    p = half * (NPAIR // 2) + 2 * i + k
                    num = _dot(_unpack(kvb_v[p]), _unpack(phiq_v[t, p, :, lanes]))

                    def unit(p=p, num=num, key=(half, k)):
                        w = _unpack(phiq_v[t, p, :, lanes]).astype(F32) * jnp.concatenate([zb_v[p]] * 2, axis=1)
                        w = (w[:64] + w[64:]).reshape(2, DH, HT)
                        den = jnp.sum(w, axis=1, keepdims=True) + 1e-6
                        outs[key] = (num.reshape(2, DH, HT) * _recip(den)).reshape(64, HT)

                    side.defer(att_cost, unit)
                    side.spent(32)

            def terms_unit():
                lo, hi = (jnp.concatenate([outs[half, 0], outs[half, 1]], axis=0).T for half in range(2))
                for q, term in enumerate(_lhs_terms(lo[:G], hi[:G], lo[G:], hi[G:])):
                    w = _pack(jnp.concatenate([term[:G // 2], term[G // 2:]], axis=1))
                    ot_v[slot, q, pl.ds(0, G // 4), pl.ds(i * 128, 128)] = w[:, :128]
                    ot_v[slot, q, pl.ds(G // 4, G // 4), pl.ds(i * 128, 128)] = w[:, 128:]

            side.defer(att_cost, terms_unit)

        def norm2(xn):
            n = xn.shape[0]
            return _layernorm(xn).reshape(n // 8, 8, D) * mod_v[4] + mod_v[3]

        def finish_rows(base, y):
            rows = rows_at(base, EC)
            xn = x_v[rows, :].astype(F32).reshape(EC // 8, 8, D) + mod_v[2] * y.reshape(EC // 8, 8, D)
            xn2 = xn.reshape(EC, D)
            xn_v[rows, :] = xn2
            h2 = norm2(xn2)
            out_v[rows, :] = (xn + mod_v[5] * h2).reshape(EC, D).astype(BF16)
            score = jnp.sum((h2 * mod_v[6]).reshape(EC, D), axis=-1, keepdims=True)
            lane = jax.lax.broadcasted_iota(I32, (8, 128), 1)
            acc = r_v[base // 1024]
            for o in range(0, EC, 8):
                acc = jnp.where(lane == (base % 1024 + o) // 8, score[o:o + 8], acc)
            r_v[base // 1024] = acc

        def mix(slot, extra):
            return strassen(lambda j: _dot(_unpack(ot_v[slot, j]), _unpack(wot_v[j])), 4 * G, extra)

        def defer_finish(base, rows_of, hold=True):
            def unit(o):
                if hold and latest:
                    hold_rows()
                finish_rows(base + o, rows_of(o))

            for o in range(0, 2 * G, EC):
                side.defer(fin_cost, functools.partial(unit, o))

        def quad_rows(quads):
            def rows_of(o):
                part, o = divmod(o, G)
                return jnp.concatenate([quads[2 * part][o:o + EC], quads[2 * part + 1][o:o + EC]], axis=1)
            return rows_of

        def top2():
            shape = (S // 1024, 8, 128)
            idx = (jax.lax.broadcasted_iota(I32, shape, 0) * 1024 + jax.lax.broadcasted_iota(I32, shape, 2) * 8
                   + jax.lax.broadcasted_iota(I32, shape, 1)).astype(F32)
            m = r_v[...]
            reduce = lambda op, v: op(op(op(v, axis=0), axis=0, keepdims=True), axis=1, keepdims=True)
            picks = []
            for _ in range(2):
                top = reduce(jnp.max, m)
                first = reduce(jnp.min, jnp.where(m == top, idx, float(S - 1)))
                picks.append((jnp.max(first.astype(I32)), top))
                m = jnp.where(idx == first, -jnp.inf, m)
            return picks

        def experts():
            (i1, m1), (i2, m2) = top2()
            bases = [pl.multiple_of(jnp.clip(i // 16, 0, S // 16 - 1) * 16, 16) for i in (i1, i2)]
            sub = jax.lax.broadcasted_iota(I32, (16, D), 0)
            groups = []
            sel = jnp.zeros((16, D), F32)
            for n, (i, base) in enumerate(zip((i1, i2), bases)):
                xn = xn_v[pl.ds(base, 16), :]
                h2 = norm2(xn).reshape(16, D)
                groups.append((xn, h2))
                row = jnp.sum(jnp.where(sub == i - base, h2, 0.0), axis=0, keepdims=True)
                sel = jnp.where(sub == n, row, sel)
            sel = sel.astype(BF16)
            y = None
            acts = collections.deque()

            def down():
                nonlocal y
                f, g, u = acts.popleft()
                act = (g * jax.nn.sigmoid(g) * u).astype(BF16)
                part = _dot(act, wd_v[pl.ds(f, FC), :])
                y = part if y is None else y + part

            for f in range(0, FF, FC):
                acts.append((f, _dot(sel, wg_v[:, pl.ds(f, FC)]), _dot(sel, wu_v[:, pl.ds(f, FC)])))
                if len(acts) > 1:
                    down()
            down()
            y1, y2 = y[0:1] * jax.nn.sigmoid(m1), y[1:2] * jax.nn.sigmoid(m2)
            for n, (base, (xn, h2)) in enumerate(zip(bases, groups)):
                upd = jnp.where(sub == i1 - base, y1, 0.0) + jnp.where(sub == i2 - base, y2, 0.0)
                full = xn.reshape(2, 8, D) + mod_v[5] * (h2 + upd).reshape(2, 8, D)
                fix_v[n] = full.reshape(16, D).astype(BF16)
            return bases

        kv_v[...] = jnp.zeros(kv_v.shape, F32)
        z_v[...] = jnp.zeros(z_v.shape, F32)
        y_v[...] = jnp.zeros(y_v.shape, F32)
        r_v[...] = jnp.full(r_v.shape, -jnp.inf, F32)
        wait("wphi")
        block_diag_phi()
        wait(("w", 1))
        start(("w", 2), ("w", 0))
        prep_weight(1)
        wait(("mod", 1), ("mod", 0))
        x_copy(0).wait()
        modulation(1)
        modulation(0)

        def first_norm(n, carry):
            norm1_unit(0, 0, n)
            return carry

        jax.lax.fori_loop(0, HT // LNC, first_norm, 0, unroll=4)
        for t in range(1, NTILE):
            x_copy(t).start()
        wait(("w", 2))
        prep_weight(2)
        wait(("w", 0))
        start("wo", *[("mod", i) for i in range(2, 6)])
        prep_weight(0)

        def first_pass(t, carry):
            @pl.when(t + 1 < NTILE)
            def _():
                x_copy(t + 1).wait()

            @pl.when(t == 1)
            def _():
                start("wg", "wu", "wd")

            slot = t % 2
            norms = collections.deque(range(HT // LNC))
            every = (3 * 7 * HD // RC - 1) // len(norms)
            count = [0]

            def extra():
                count[0] += 1
                if count[0] % every == 1:
                    if norms and count[0] > 1:
                        norm1_unit(jnp.minimum(t + 1, NTILE - 1), 1 - slot, norms.popleft())
                    if norms:
                        hold_rows()

            keys(slot, extra)
            values(slot, extra)
            queries(t, slot, extra)
            assert not norms
            for j in range(NPAIR):
                accumulate_kv(j)
            side.drain()
            return carry

        jax.lax.fori_loop(0, NTILE, first_pass, 0)

        wait("wo", "wr", *[("mod", i) for i in range(2, 6)])
        side.ratio = ratio2
        for j in range(NPAIR):
            finish_kv(j)
        modulation(2)
        modulation(3)
        for i in range(4):
            attend(0, 0, 0, i)
        modulation(4)
        modulation(5)
        router_weights()
        prep_wo()
        side.drain()

        def second_pass(t, last=False):
            latest.clear()
            slot = 2 * (t % 2)
            defer_finish(jnp.maximum(t * T - 2 * G, 0), lambda o: y_v[pl.ds(o, EC), :])
            todo = collections.deque(range(4))
            quads = mix(slot, lambda: todo and attend(t, 1, slot + 1, todo.popleft()))
            side.drain()
            defer_finish(t * T, quad_rows(quads))
            todo = collections.deque(() if last else range(4))
            quads = mix(slot + 1, lambda: todo and attend(t + 1, 0, 2 - slot, todo.popleft()))
            side.drain()
            if last:
                defer_finish(t * T + 2 * G, quad_rows(quads), hold=False)
                side.drain()
            else:
                for part in range(2):
                    for half in range(2):
                        y_v[pl.ds(part * G, G), pl.ds(half * HD, HD)] = quads[2 * part + half]

        def second_step(t, carry):
            second_pass(t)

            @pl.when(t == 0)
            def _():
                out_copy(0).start()

            @pl.when(t > 0)
            def _():
                out_copy(t).start()

            return carry

        jax.lax.fori_loop(0, NTILE - 1, second_step, 0)
        second_pass(NTILE - 1, last=True)
        out_copy(NTILE - 1).start()
        out_copy(NTILE).start()
        wait("wg", "wu", "wd")
        b1, b2 = experts()
        for n in range(NTILE + 1):
            out_copy(n).wait()
        fix = [pltpu.make_async_copy(fix_v.at[n], out_hbm.at[pl.ds(b, 16)], osems.at[n])
               for n, b in enumerate((b1, b2))]
        fix[0].start()

        @pl.when(b1 != b2)
        def _():
            fix[1].start()
            fix[1].wait()

        fix[0].wait()

    nsem = 3 + 6 + 3 + 4
    scratch = [
        pltpu.VMEM((S + 16, D), BF16), pltpu.VMEM((3, D, D), BF16), pltpu.VMEM((D, DH), BF16),
        pltpu.VMEM((D, D), BF16), pltpu.VMEM((8, 128), BF16),
        pltpu.VMEM((D, FF), BF16), pltpu.VMEM((D, FF), BF16), pltpu.VMEM((FF, D), BF16),
        pltpu.VMEM((1, D), BF16), pltpu.VMEM((6, D, D), BF16),
        pltpu.VMEM((7, 8, D), F32),
        pltpu.VMEM((D // 128, 64, 128), U32),
        pltpu.VMEM((3, 7, HD // 2, HD), U32),
        pltpu.VMEM((7, HD // 2, HD), U32),
        pltpu.VMEM((2, 7, HT // 2, HD), U32),
        pltpu.VMEM((NTILE, NPAIR, 64, T), U32),
        pltpu.VMEM((NPAIR, 64, T), U32),
        pltpu.VMEM((D // 2, T), U32),
        pltpu.VMEM((NPAIR, 64, 128), F32),
        pltpu.VMEM((NPAIR, 32, 128), U32),
        pltpu.VMEM((NPAIR, 128, 128), F32),
        pltpu.VMEM((NPAIR, 128, 128), F32),
        pltpu.VMEM((4, 7, G // 2, HD), U32),
        pltpu.VMEM((2 * G, D), F32),
        pltpu.VMEM((S, D), F32),
        pltpu.VMEM((S, D), BF16),
        pltpu.VMEM((S // 1024, 8, 128), F32),
        pltpu.VMEM((2, 16, D), BF16),
        pltpu.SemaphoreType.DMA((nsem,)),
        pltpu.SemaphoreType.DMA((NTILE,)),
        pltpu.SemaphoreType.DMA((NTILE + 1,)),
    ]

    def fn(A_x, A_wqkv, A_w_phi, A_wo, B_x, B_w_r, B_w_gate, B_w_up, B_w_down, c, w_mod):
        del B_x
        out = pl.pallas_call(
            kernel,
            out_shape=jax.ShapeDtypeStruct((S, D), A_x.dtype),
            in_specs=[pl.BlockSpec(memory_space=pl.ANY)] * 10,
            out_specs=pl.BlockSpec(memory_space=pl.ANY),
            scratch_shapes=scratch,
            compiler_params=pltpu.CompilerParams(vmem_limit_bytes=vlimit * 2**20, flags=flags),
        )(A_x.reshape(S, D), A_wqkv, A_w_phi.reshape(D, DH), A_wo, B_w_r.reshape(8, 128),
          B_w_gate, B_w_up, B_w_down, c, w_mod)
        return out.reshape(A_x.shape)

    return fn


@jax.jit
def pallas_adaLN_cond__linear_kernel_hedgehog__moe_arch_mod__prompt_kernel(
    A_x, A_wqkv, A_w_phi, A_wo, B_x, B_w_r, B_w_gate, B_w_up, B_w_down, c, w_mod
):
    return make()(A_x, A_wqkv, A_w_phi, A_wo, B_x, B_w_r, B_w_gate, B_w_up, B_w_down, c, w_mod)
```

```python
import collections
import contextlib
import functools

import jax
import jax.numpy as jnp
import numpy as np
import jax.experimental.pallas as pl
import jax.experimental.pallas.tpu as pltpu

F32, BF16, I32, U32 = jnp.float32, jnp.bfloat16, jnp.int32, jnp.uint32
S, D, H, DH, FF = 2048, 1024, 32, 32, 3584
HD = D // 2
NPAIR = H // 2
EPS = 1e-5
LOG2E = float(np.log2(np.e))
NN = (((1,), (0,)), ((), ()))
NT = (((1,), (1,)), ((), ()))


def _dot(a, b, dn=NN):
    return jax.lax.dot_general(a, b, dn, preferred_element_type=F32)


def _pack(x):
    n = x.shape[0] // 2
    if x.shape[1] > 128:
        return pltpu.bitcast(x.astype(BF16), U32)
    w = pltpu.bitcast(jnp.concatenate([x[:n], x[n:]], axis=1).astype(BF16), U32)
    return jnp.concatenate([w[:, :128], w[:, 128:]], axis=0)


def _unpack(w):
    return pltpu.bitcast(w, BF16)


def _recip(x):
    r = pl.reciprocal(x, approx=True)
    return r * (2.0 - x * r)


def _lhs_terms(a11, a12, a21, a22):
    return (a11 + a22, a21 + a22, a11, a22, a11 + a12, a21 - a11, a12 - a22)


def _rhs_terms(b11, b12, b21, b22):
    return (b11 + b22, b11, b12 - b22, b21 - b11, b22, b11 + b12, b21 + b22)


_QUADRANTS = (((0, 1), (3, 1), (4, -1), (6, 1)), ((2, 1), (4, 1)), ((1, 1), (3, 1)),
              ((0, 1), (1, -1), (2, 1), (5, 1)))


def _quadrant(q, product):
    total = None
    for j, sign in _QUADRANTS[q]:
        m = product(j)
        total = m if total is None else (total + m if sign > 0 else total - m)
    return total


def _layernorm(x):
    d = x - jnp.mean(x, axis=-1, keepdims=True)
    v = jnp.mean(d * d, axis=-1, keepdims=True)
    return d * jax.lax.rsqrt(v + EPS)


def _per_head(op, p):
    parts = [p[r:r + 8] for r in range(0, p.shape[0], 8)]
    while len(parts) > 1:
        parts = [op(a, b) for a, b in zip(parts[::2], parts[1::2])]
    out = op(parts[0], pltpu.roll(parts[0], 4, 0))
    return op(out, pltpu.roll(out, 2, 0))


def _apply(op, p, stat):
    n = p.shape[0] // 8
    return op(p.reshape(n, 8, p.shape[1]), stat).reshape(p.shape)


def _features(p):
    e_pos = jnp.exp2(_apply(jnp.subtract, p, _per_head(jnp.maximum, p)))
    e_neg = jnp.exp2(_apply(lambda a, low: low - a, p, _per_head(jnp.minimum, p)))
    pos = _apply(jnp.multiply, e_pos, _recip(_per_head(jnp.add, e_pos)))
    neg = _apply(jnp.multiply, e_neg, _recip(_per_head(jnp.add, e_neg)))
    return jnp.concatenate([pos, neg], axis=0)


def _interleaved_source(row):
    return (row & ~63) + ((row & 1) << 5) + ((row & 63) >> 1)


class _Interleaver:
    def __init__(self, ratio):
        self.queue = collections.deque()
        self.ratio = ratio
        self.credit = 0.0

    def defer(self, cost, fn):
        self.queue.append((cost, fn))

    def spent(self, cycles):
        self.credit += cycles * self.ratio
        while self.queue and self.credit >= self.queue[0][0]:
            cost, fn = self.queue.popleft()
            self.credit -= cost
            fn()
        if not self.queue:
            self.credit = 0.0

    def drain(self):
        while self.queue:
            self.queue.popleft()[1]()
        self.credit = 0.0


def make(RC=256, VC=256, LW=512, lfirst=15, FC=512, EC=32, ratio=0.55, vlimit=120, flags=None, S=S,
         prof=False, only=0, cdelay=3, spread=(2, 2, 2, 2, 2, 4, 2), last_rows=128, marks=(),
         vcost=256, split=True, kcost=150, lnv=True, ne=5, close2=False, mfirst=1, mlast=42, order='kqv', llast=28, pfirst=29, plast=42):
    scope = lambda n: jax.named_scope(n) if prof is True or (prof and n in prof) else contextlib.nullcontext()
    T = 512
    HT = T // 2
    NTILE = S // T
    G = 128
    MC = 256
    MT = pl.cdiv(4 * D // 128, NTILE - 1)
    nk, nv = 7 * HD // RC, 7 * HD // VC

    def kernel(x_hbm, wqkv_hbm, wphi_hbm, wo_hbm, wr_hbm, wg_hbm, wu_hbm, wd_hbm, c_hbm, wmod_hbm,
               out_hbm,
               x_v, wqkv_v, wphi_v, wo_v, wr_v, wg_v, wu_v, wd_v, c_v, wmod_v,
               act_v, raw_v, mod_v, stat_v, bd_v, wt_v, wot_v, ht_v, phiq_v, phik_v, vt_v, kv_v, kvb_v, ot_v,
               y_v, xn_v, out_v, r_v, fix_v, sems, osems):

        side = _Interleaver(ratio)
        copies = {}

        def add_copy(name, src, dst):
            copies[name] = pltpu.make_async_copy(src, dst, sems.at[NTILE + len(copies)])

        add_copy("c", c_hbm, c_v)
        add_copy("wphi", wphi_hbm, wphi_v)
        add_copy("wr", wr_hbm, wr_v)
        def add_columns(name, hbm, vmem, lo, n):
            add_copy(name, hbm.at[:, pl.ds(lo, n)], vmem.at[:, pl.ds(lo, n)])

        for i in range(2):
            for n in range(D // MC):
                add_columns(("mod", i, n), wmod_hbm, wmod_v, i * D + n * MC, MC)
        for n in range(NTILE - 1):
            add_columns(("mod", n), wmod_hbm, wmod_v, 2 * D + n * MT * 128, min(MT * 128, 4 * D - n * MT * 128))
        for i in (0, 2):
            add_columns(("w", i), wqkv_hbm, wqkv_v, i * D, D)
        for n in range(8):
            add_columns(("wk", n), wqkv_hbm, wqkv_v, D + n * 128, 128)
        add_copy("wo", wo_hbm, wo_v)
        add_copy("wg", wg_hbm, wg_v)
        add_copy("wu", wu_hbm, wu_v)
        add_copy("wd", wd_hbm, wd_v)

        def start(*names):
            for n in names:
                copies[n].start()

        def wait(*names):
            with scope("w_" + "_".join(str(n) for n in names)[:20].replace("'", "").replace(" ", "")):
                for n in names:
                    copies[n].wait()

        def rows_at(base, size):
            return pl.ds(base if isinstance(base, int) else pl.multiple_of(base, 8), size)

        def x_copy(t):
            return pltpu.make_async_copy(x_hbm.at[rows_at(t * T, T)], x_v.at[rows_at(t * T, T)], sems.at[t])

        def out_copy(n):
            if isinstance(n, int):
                lo, hi = max(n * T - 2 * G, 0), min((n + 1) * T - 2 * G, S)
                rows = pl.ds(lo, hi - lo)
            else:
                rows = rows_at(n * T - 2 * G, T)
            return pltpu.make_async_copy(out_v.at[rows], out_hbm.at[rows], osems.at[n])

        def modulation(lo, n, half=None):
            rows = pl.ds(0, D) if half is None else pl.ds(half * HD, HD)
            lanes = pl.ds(lo if isinstance(lo, int) else pl.multiple_of(lo, 128), n)
            m = _dot(_unpack(act_v[:, rows]), wmod_v[rows, lanes])[:8]
            raw_v[:, lanes] = m if not half else raw_v[:, lanes] + m

        raw = lambda i: raw_v[:, pl.ds(i * D, D)]

        def block_diag_phi():
            row = _interleaved_source(jax.lax.broadcasted_iota(I32, (128, DH), 0))
            col = jax.lax.broadcasted_iota(I32, (128, DH), 1)
            sel = jnp.where((row & (DH - 1)) == col, 1.0, 0.0).astype(BF16)
            r2 = _interleaved_source(jax.lax.broadcasted_iota(I32, (128, 128), 0)) >> 5
            c2 = jax.lax.broadcasted_iota(I32, (128, 128), 1) >> 5
            for g in range(D // 128):
                tiled = _dot(sel, wphi_v[pl.ds(g * 128, 128), :], NT)
                bd_v[g] = _pack(jnp.where(r2 == c2, tiled, 0.0))

        def prep_scores(i, g):
            parts = []
            for gg in (g, g + HD // 128):
                for half in range(2):
                    w = wqkv_v[pl.ds(half * HD, HD), pl.ds(i * D + gg * 128, 128)]
                    parts.append(_dot(_unpack(bd_v[gg]), w, NT) * LOG2E)
            for j, term in enumerate(_lhs_terms(*parts)):
                wt_v[7 * i + j, pl.ds(g * 64, 64), :] = _pack(term)

        def prep_values(n):
            lo = wqkv_v[pl.ds(n * 32, 32), pl.ds(2 * D, D)].astype(F32)
            hi = wqkv_v[pl.ds(HD + n * 32, 32), pl.ds(2 * D, D)].astype(F32)
            for j, term in enumerate(_lhs_terms(lo[:, :HD], hi[:, :HD], lo[:, HD:], hi[:, HD:])):
                wt_v[14 + j, pl.ds(n * 16, 16), :] = _pack(term)

        def prep_output(n):
            lo = wo_v[rows_at(n * 32, 32), :].astype(F32)
            hi = wo_v[rows_at(HD + n * 32, 32), :].astype(F32)
            for j, term in enumerate(_rhs_terms(lo[:, :HD], lo[:, HD:], hi[:, :HD], hi[:, HD:])):
                wot_v[j, rows_at(n * 16, 16), :] = _pack(term)

        start("c", "wphi")
        x_copy(0).start()
        start(*[("mod", i, n) for i in (1, 0) for n in range(D // MC)])
        start(*[("wk", g + 4 * k) for g in range(4) for k in range(2)], ("w", 0), ("w", 2))
        x_copy(1).start()
        start("wo")
        for t in range(1, NTILE):
            start(("mod", t - 1))
            if t + 1 < NTILE:
                x_copy(t + 1).start()
        start("wr")
        wait("c")
        bits = pltpu.bitcast(jnp.broadcast_to(c_v[:, :128].astype(F32), (8, 128)), I32)
        zero = jnp.minimum(jnp.max(bits & 0xFF), 0)
        latest = {}

        class Chain:
            def __init__(self, strands):
                self.tokens = collections.deque([None] * strands)

            def enter(self, value):
                token = self.tokens.popleft()
                if token is None:
                    return value
                head = pltpu.bitcast(pltpu.bitcast(value[:8, :128], I32) | token, F32)
                if value.shape[1] > 128:
                    head = jnp.concatenate([head, value[:8, 128:]], axis=1)
                return jnp.concatenate([head, value[8:]], axis=0) if value.shape[0] > 8 else head

            def leave(self, *values):
                token = None
                for value in values:
                    value = pltpu.bitcast(value, I32)
                    token = value if token is None else token | value
                self.tokens.append(token & zero)

            def widen(self, strands):
                last = self.tokens[-1]
                while len(self.tokens) < strands:
                    self.tokens.append(last)

        def back(n):
            return jnp.minimum(zero & 255, n)

        def row_stats(t, n):
            xx = x_v[rows_at(t * T + n * 32, 32), :].astype(F32)
            mean = jnp.mean(xx, axis=-1, keepdims=True)
            d = xx - mean
            scale = jax.lax.rsqrt(jnp.mean(d * d, axis=-1, keepdims=True) + EPS)
            stat_v[0, rows_at(n * 32, 32), :] = jnp.broadcast_to(mean, (32, 128))
            stat_v[1, rows_at(n * 32, 32), :] = jnp.broadcast_to(scale, (32, 128))

        def normalized(t, offset, lanes):
            wide = lambda k: jnp.concatenate([stat_v[k, pl.ds(offset, 16), :]] * (LW // 128), axis=1)
            xx = x_v[rows_at(t * T + offset, 16), lanes].astype(F32)
            return ((xx - wide(0)) * wide(1)).reshape(2, 8, LW) * mod_v[1, :, lanes]

        def norm1_unit(t, slot, n, scaled=normalized):
            group, part = divmod(n, HD // LW)
            blocks = []
            for col in (part * LW, HD + part * LW):
                for offset in (group * 16, HT + group * 16):
                    lanes = pl.ds(col, LW)
                    hh = scaled(t, offset, lanes) + mod_v[0, :, lanes]
                    blocks.append(hh.reshape(16, LW))
            for j, term in enumerate(_rhs_terms(*blocks)):
                ht_v[slot, j, pl.ds(group * 8, 8), pl.ds(part * LW, LW)] = _pack(term)

        def apart(k):
            return (zero >> k) & 1 if k and split else 0

        def strassen(product, tiles, cycles, extra):
            products = []
            for j in range(7):
                products.append([product(j, k) for k in range(tiles)])
                latest["m"] = products[j][-1][-16:]
                side.spent(cycles)
                extra()
            return products

        def scores(i, slot, extra, consume, cost):
            tiles = HT // 128
            for r in range(0, HD, RC):
                products = strassen(
                    lambda j, k: _dot(_unpack(wt_v[7 * i + j + apart(k), pl.ds(r // 2, RC // 2), :]),
                                      _unpack(ht_v[slot, j, pl.ds(k * 64, 64), :]), NT),
                    tiles, RC * HT // 128, extra)

                def unit(half, o, products=products, r=r):
                    for part in range(2):
                        phi = jnp.concatenate(
                            [_features(_quadrant(2 * half + part, lambda j: products[j][k][o:o + 64]))
                             for k in range(tiles)], axis=1)
                        consume((half * HD + r + o) // 64, pl.ds(part * HT, HT), phi.astype(BF16))

                for half in range(2):
                    for o in range(0, RC, 64):
                        side.defer(cost, functools.partial(unit, half, o))

        def key_features(pair, lanes, phi):
            phik_v[pair, :, lanes] = phi

        def query_features(t, pair, lanes, phi):
            phiq_v[t, pair, :, lanes] = phi

        def values(slot, extra):
            tiles = VC // 128
            for r in range(0, HD, VC):
                products = strassen(
                    lambda j, k: _dot(_unpack(ht_v[slot, j + apart(k)]),
                                      _unpack(wt_v[14 + j, :, pl.ds(r + k * 128, 128)])),
                    tiles, VC * HT // 128, extra)

                def unit(half, part, k, products=products, r=r):
                    v = _quadrant(2 * half + part, lambda j: products[j][k])
                    v = v.T.astype(BF16).reshape(2, 64, HT)
                    vt_v[pl.ds((half * HD + r) // 64 + k * 2, 2), pl.ds(0, 64), pl.ds(part * HT, HT)] = v

                for half in range(2):
                    for part in range(2):
                        for k in range(tiles):
                            side.defer(vcost // tiles, functools.partial(unit, half, part, k))

        def accumulate_kv(j):
            kv = _dot(vt_v[j], phik_v[j], NT)
            kv_v[j] += kv
            latest["m"] = kv[-16:]
            side.spent(T // 8)

        def finish_kv(j):
            row = jax.lax.broadcasted_iota(I32, (80, 128), 0)
            row_head = jnp.where(row < 64, row >> 5, (row >> 3) & 1)
            col_head = jax.lax.broadcasted_iota(I32, (80, 128), 1) & 1
            kvb_v[j] = _pack(jnp.where(row_head == col_head, kv_v[j], 0.0))

        def first_pass(t, plan, order):
            slot = t & 1
            count = [0]

            def extra():
                count[0] += 1
                for task in plan.pop(count[0], ()):
                    task()

            for task in plan.pop(0, ()):
                task()
            for part in order:
                if part == "k":
                    scores(1, slot, extra, key_features, kcost * RC // 256)
                elif part == "q":
                    scores(0, slot, extra, functools.partial(query_features, t), kcost * RC // 256)
                else:
                    values(slot, extra)
            assert not plan
            if order[-1] == "v":
                side.drain()
            for r in range(0, HD, VC):
                for half in range(2):
                    for o in range(0, VC, 64):
                        accumulate_kv((half * HD + r + o) // 64)
            side.drain()

        def plan_norms(plan, t, slot, begin, first, last):
            plan[begin] += [functools.partial(row_stats, t, n) for n in range(T // 32)]
            units = HT // 16 * (HD // LW)
            slots = list(range(first, last + 1))
            for n in range(units):
                plan[slots[len(slots) * n // units]].append(functools.partial(norm1_unit, t, slot, n))

        def attend(t, part, slot, i):
            lanes = pl.ds(part * HT, HT)
            outs = {}
            tasks = []
            for half in range(2):
                for k in range(2):
                    p = half * (NPAIR // 2) + 2 * i + k
                    num = _dot(_unpack(kvb_v[p]), phiq_v[t, p, :, lanes])

                    def unit(num=num, key=(half, k)):
                        outs[key] = [_apply(jnp.multiply, num[h * DH:(h + 1) * DH],
                                            _recip(num[64 + 8 * h:72 + 8 * h] + 1e-6)) for h in range(2)]

                    tasks.append(unit)

            def terms_unit():
                lo, hi = (jnp.concatenate(outs[half, 0] + outs[half, 1], axis=0).T for half in range(2))
                for q, term in enumerate(_lhs_terms(lo[:G], hi[:G], lo[G:], hi[G:])):
                    ot_v[slot, q, :, pl.ds(i * 128, 128)] = _pack(term)
                close2 and written.append(lambda: ot_v[slot, 6 - back(6), pl.ds(G // 2 - 8, 8), pl.ds(i * 128, 128)])

            return tasks + [terms_unit]

        def norm2(xn):
            n = xn.shape[0]
            return _layernorm(xn).reshape(n // 8, 8, D) * mod_v[4] + mod_v[3]

        def output_weights():
            w = wr_v[...].astype(F32)
            w = jnp.concatenate([jnp.broadcast_to(w[j:j + 1], (8, 128)) for j in range(D // 128)], axis=1)
            for i in range(2, 6):
                mod_v[i] = raw(i) + 1.0 if i == 4 else raw(i)
            mod_v[6] = mod_v[4] * w
            mod_v[7] = mod_v[4] * mod_v[5]
            mod_v[8] = mod_v[3] * mod_v[5]
            mod_v[9] = jnp.broadcast_to(jnp.sum(mod_v[3] * w, axis=1, keepdims=True), (8, D))

        def finish_rows(base, y, chain):
            lane = jax.lax.broadcasted_iota(I32, (8, 128), 1)
            acc = r_v[base >> 10]
            for o in range(0, y.shape[0], 8):
                rows = rows_at(base + o, 8)
                xn = x_v[rows, :].astype(F32) + mod_v[2] * chain.enter(y[o:o + 8])
                xn_v[rows, :] = xn
                mean = jnp.mean(xn, axis=-1, keepdims=True)
                d = xn - mean
                scale = jax.lax.rsqrt(jnp.mean(d * d, axis=-1, keepdims=True) + EPS)
                score = jnp.sum(d * mod_v[6], axis=-1, keepdims=True) * scale + mod_v[9, :, :1]
                out = (d * scale) * mod_v[7] + ((d + mean) + mod_v[8])
                out_v[rows, :] = out.astype(BF16)
                acc = jnp.where(lane == ((base + o) & 1023) >> 3, score, acc)
                chain.leave(*[out[:, l:l + 128] for l in range(128, D, 256)])
            r_v[base >> 10] = acc
            lanes = lambda: pl.ds(pl.multiple_of((7 - back(7)) * 128, 128), 128)
            if close2:
                written.append(lambda: pltpu.bitcast(acc, U32))

        written = []
        chains = []
        tokens = collections.deque()

        def mix(slot, extra, lo=0, n=G):
            def product(j, k):
                if k == 0:
                    token = None
                    while written:
                        item = written.pop()()
                        token = item if token is None else token | item
                    tokens.append(token)
                    if len(tokens) > cdelay:
                        token = tokens.popleft()
                        if token is not None:
                            wot_v[7 - back(7), pl.ds(0, 8), pl.ds(0, 128)] = token
                return _dot(_unpack(ot_v[slot, j + apart(k), pl.ds(lo // 2, n // 2), :]),
                            _unpack(wot_v[j, :, pl.ds(k * 128, 128)]))

            return strassen(product, HD // 128, 4 * n, extra)

        def mixed_rows(product, n):
            def rows_of(o):
                part, o = divmod(o, n)
                return jnp.concatenate(
                    [_quadrant(2 * part + half, lambda j: product(j, o)) for half in range(2)], axis=1)
            return rows_of

        def from_values(products):
            return lambda j, o: jnp.concatenate([tile[o:o + EC] for tile in products[j]], axis=1)

        def top2():
            shape = (S // 1024, 8, 128)
            idx = (jax.lax.broadcasted_iota(I32, shape, 0) * 1024 + jax.lax.broadcasted_iota(I32, shape, 2) * 8
                   + jax.lax.broadcasted_iota(I32, shape, 1)).astype(F32)
            m = r_v[...]
            reduce = lambda op, v: op(op(op(v, axis=0), axis=0, keepdims=True), axis=1, keepdims=True)
            picks = []
            for _ in range(2):
                top = reduce(jnp.max, m)
                first = reduce(jnp.min, jnp.where(m == top, idx, float(S - 1)))
                picks.append((jnp.max(first.astype(I32)), top))
                m = jnp.where(idx == first, -jnp.inf, m)
            return picks

        def experts():
            (i1, m1), (i2, m2) = top2()
            bases = [pl.multiple_of(jnp.clip(i >> 4, 0, S // 16 - 1) * 16, 16) for i in (i1, i2)]
            sub = jax.lax.broadcasted_iota(I32, (16, D), 0)
            groups = []
            sel = jnp.zeros((16, D), F32)
            for n, (i, base) in enumerate(zip((i1, i2), bases)):
                xn = xn_v[pl.ds(base, 16), :]
                h2 = norm2(xn).reshape(16, D)
                groups.append((xn, h2))
                row = jnp.sum(jnp.where(sub == i - base, h2, 0.0), axis=0, keepdims=True)
                sel = jnp.where(sub == n, row, sel)
            sel = sel.astype(BF16)
            y = None
            acts = collections.deque()

            def down():
                nonlocal y
                f, g, u = acts.popleft()
                act = (g * jax.nn.sigmoid(g) * u).astype(BF16)
                part = _dot(act, wd_v[pl.ds(f, FC), :])
                y = part if y is None else y + part

            for f in range(0, FF, FC):
                acts.append((f, _dot(sel, wg_v[:, pl.ds(f, FC)]), _dot(sel, wu_v[:, pl.ds(f, FC)])))
                if len(acts) > 1:
                    down()
            down()
            y1, y2 = y[0:1] * jax.nn.sigmoid(m1), y[1:2] * jax.nn.sigmoid(m2)
            for n, (base, (xn, h2)) in enumerate(zip(bases, groups)):
                upd = jnp.where(sub == i1 - base, y1, 0.0) + jnp.where(sub == i2 - base, y2, 0.0)
                full = xn.reshape(2, 8, D) + mod_v[5] * (h2 + upd).reshape(2, 8, D)
                fix_v[n] = full.reshape(16, D).astype(BF16)
            return bases

        kv_v[...] = jnp.zeros(kv_v.shape, F32)
        vt_v[:, pl.ds(64, 16), :] = jnp.ones((NPAIR, 16, T), BF16)
        y_v[...] = jnp.zeros(y_v.shape, F32)
        r_v[...] = jnp.full(r_v.shape, -jnp.inf, F32)
        cc = c_v[...].astype(F32)
        act_v[...] = _pack(jnp.broadcast_to(cc * jax.nn.sigmoid(cc), (16, D)))
        wait("wphi")
        block_diag_phi()
        with scope("w_x0"):
            x_copy(0).wait()
        for n in range(T // 32):
            row_stats(0, n)
        for n in range(D // MC):
            wait(("mod", 1, n))
            modulation(D + n * MC, MC)
        mod_v[1] = raw(1) + 1.0
        for offset in range(0, T, 16):
            for col in range(0, D, LW):
                lanes = pl.ds(col, LW)
                xn_v[pl.ds(offset, 16), lanes] = normalized(0, offset, lanes).reshape(16, LW)
        for n in range(D // MC):
            wait(("mod", 0, n))
            modulation(n * MC, MC)
        mod_v[0] = raw(0)
        wait(("wk", 0), ("wk", 4))
        prep_scores(1, 0)
        for n in range(HT // 16 * (HD // LW)):
            norm1_unit(0, 0, n, lambda t, offset, lanes: xn_v[pl.ds(offset, 16), lanes].reshape(2, 8, LW))
        wait(("wk", 1), ("wk", 5))
        prep_scores(1, 1)

        plan = collections.defaultdict(list)
        plan[3] += [lambda: wait(("wk", 2), ("wk", 6), ("wk", 3), ("wk", 7)),
                    lambda: prep_scores(1, 2), lambda: prep_scores(1, 3)]
        plan[7].append(lambda: wait(("w", 0)))
        for g in range(4):
            plan[8 + g * (nk - 9) // 4].append(functools.partial(prep_scores, 0, g))
        plan[nk] += [lambda: wait(("w", 2)), lambda: x_copy(1).wait()]
        for n in range(HD // 32):
            plan[nk + 1 + n * (nk - 2) // (HD // 32)].append(functools.partial(prep_values, n))
        plan_norms(plan, 1, 1, nk, nk + 4, 2 * nk + nv)
        if marks:
            def mark(n):
                with jax.named_scope(f"mark{n}"):
                    fix_v[0, :, pl.ds(0, 128)] = jnp.zeros((16, 128), BF16)
            for n in marks:
                plan[n].append(functools.partial(mark, n))
        with scope("tile0"):
            first_pass(0, plan, 'kqv')

        def first_step(t, carry):
            @pl.when(t + 1 < NTILE)
            def _():
                x_copy(t + 1).wait()

            for n in range(NTILE - 1):
                pl.when(t == n + 1)(functools.partial(wait, ("mod", n)))

            @pl.when(t == NTILE - 2)
            def _():
                start("wg", "wu", "wd")

            plan = collections.defaultdict(list)
            plan_norms(plan, jnp.minimum(t + 1, NTILE - 1), 1 - (t & 1), 0, lfirst, llast)
            per_step = pl.cdiv(HD // 32, NTILE - 1)
            for n in range(per_step):
                plan[pfirst + n * (plast - pfirst) // per_step].append(functools.partial(
                    lambda n: prep_output(jnp.minimum((t - 1) * per_step + n, HD // 32 - 1)), n))
            tiles = MT
            for n in range(2 * tiles):
                tile = jnp.minimum((t - 1) * tiles + n // 2, 4 * D // 128 - 1)
                plan[mfirst + n * (mlast - mfirst) // (2 * tiles)].append(
                    functools.partial(modulation, 2 * D + tile * 128, 128, n % 2))
            first_pass(t, plan, order)
            return carry

        wait("wo")
        if only in (0, 1):
            with scope("pass1"):
                jax.lax.fori_loop(1, NTILE, first_step, 0)
        if only == 1:
            for j in range(NPAIR):
                finish_kv(j)
            out_v[pl.ds(0, 64), pl.ds(0, 512)] = phiq_v[zero, zero, pl.ds(0, 64), :]
            out_v[pl.ds(64, 80), pl.ds(0, 128)] = _unpack(kvb_v[zero])
            out_v[pl.ds(160, 64), pl.ds(0, 512)] = _unpack(wot_v[zero, pl.ds(0, 32), :])
            out_copy(0).start()
            out_copy(0).wait()
            return

        wait("wr")
        for j in range(NPAIR):
            finish_kv(j)
        tasks = [task for i in range(4) for task in attend(0, 0, 0, i)]
        for task in tasks:
            task()
        output_weights()

        def mix_step(slot, following, base, rows_of, lo=0, n=G, spread=spread):
            state = {"step": 0, "unit": 0}

            def finish(count):
                for _ in range(count):
                    row = state["unit"] * EC
                    finish_rows(base + row, rows_of(row), chains[0])
                    state["unit"] += 1

            def extra():
                state["step"] += 1
                if state["step"] < len(spread):
                    finish(spread[state["step"]] * 16 // EC)

            if following:
                tasks = [task for i in range(4) for task in attend(*following, i)]
                for task in tasks:
                    task()
            finish(spread[0] * 16 // EC)
            return mix(slot, extra, lo, n)

        stored = mixed_rows(lambda j, o: y_v[j, pl.ds(o, EC), :], G)

        def second_step(t, carry):
            latest.clear()
            written.clear()
            tokens.clear()
            chains[:] = [Chain(ne)]
            slot = 2 * (t & 1)
            products = mix_step(slot, (t, 1, slot + 1), jnp.maximum(t * T - 2 * G, 0), stored)
            products = mix_step(slot + 1, (jnp.minimum(t + 1, NTILE - 1), 0, 2 - slot), t * T,
                                mixed_rows(from_values(products), G))
            for j in range(7):
                for k, tile in enumerate(products[j]):
                    y_v[j, :, pl.ds(k * 128, 128)] = tile

            @pl.when(t == 0)
            def _():
                out_copy(0).start()

            @pl.when(t > 0)
            def _():
                out_copy(t).start()

            return carry

        with scope("pass2"):
            jax.lax.fori_loop(0, NTILE, second_step, 0)
        wait("wg", "wu", "wd")
        with scope("last"):
            chain = Chain(2 * G // 8)
            for o in range(0, 2 * G, EC):
                finish_rows(S - 2 * G + o, stored(o), chain)
        out_copy(NTILE).start()
        with scope("experts"):
            b1, b2 = experts()
        with scope("w_out"):
            for n in range(NTILE + 1):
                out_copy(n).wait()
        fix = [pltpu.make_async_copy(fix_v.at[n], out_hbm.at[pl.ds(b, 16)], osems.at[n])
               for n, b in enumerate((b1, b2))]
        fix[0].start()

        @pl.when(b1 != b2)
        def _():
            fix[1].start()
            fix[1].wait()

        fix[0].wait()

    nsem = NTILE + 3 + 2 * D // MC + NTILE - 1 + 2 + 8 + 4
    scratch = [
        pltpu.VMEM((S, D), BF16), pltpu.VMEM((D, 3 * D), BF16), pltpu.VMEM((D, DH), BF16),
        pltpu.VMEM((D, D), BF16), pltpu.VMEM((8, 128), BF16),
        pltpu.VMEM((D, FF), BF16), pltpu.VMEM((D, FF), BF16), pltpu.VMEM((FF, D), BF16),
        pltpu.VMEM((1, D), BF16), pltpu.VMEM((D, 6 * D), BF16),
        pltpu.VMEM((8, D), U32),
        pltpu.VMEM((8, 6 * D), F32),
        pltpu.VMEM((10, 8, D), F32),
        pltpu.VMEM((2, T, 128), F32),
        pltpu.VMEM((D // 128, 64, 128), U32),
        pltpu.VMEM((21, HD // 2, HD), U32),
        pltpu.VMEM((8, HD // 2, HD), U32),
        pltpu.VMEM((2, 8, HT // 2, HD), U32),
        pltpu.VMEM((NTILE, NPAIR, 128, T), BF16),
        pltpu.VMEM((NPAIR, 128, T), BF16),
        pltpu.VMEM((NPAIR, 80, T), BF16),
        pltpu.VMEM((NPAIR, 80, 128), F32),
        pltpu.VMEM((NPAIR, 40, 128), U32),
        pltpu.VMEM((4, 8, G // 2, HD), U32),
        pltpu.VMEM((7, G, HD), F32),
        pltpu.VMEM((S, D), F32),
        pltpu.VMEM((S, D), BF16),
        pltpu.VMEM((S // 1024, 8, 128), F32),
        pltpu.VMEM((2, 16, D), BF16),
        pltpu.SemaphoreType.DMA((nsem,)),
        pltpu.SemaphoreType.DMA((NTILE + 1,)),
    ]

    def fn(A_x, A_wqkv, A_w_phi, A_wo, B_x, B_w_r, B_w_gate, B_w_up, B_w_down, c, w_mod):
        del B_x
        out = pl.pallas_call(
            kernel,
            out_shape=jax.ShapeDtypeStruct((S, D), A_x.dtype),
            in_specs=[pl.BlockSpec(memory_space=pl.ANY)] * 10,
            out_specs=pl.BlockSpec(memory_space=pl.ANY),
            scratch_shapes=scratch,
            compiler_params=pltpu.CompilerParams(vmem_limit_bytes=vlimit * 2**20, flags=flags),
        )(A_x.reshape(S, D), A_wqkv, A_w_phi.reshape(D, DH), A_wo, B_w_r.reshape(8, 128),
          B_w_gate, B_w_up, B_w_down, c, w_mod)
        return out.reshape(A_x.shape)

    return fn


@jax.jit
def pallas_adaLN_cond__linear_kernel_hedgehog__moe_arch_mod__prompt_kernel(
    A_x, A_wqkv, A_w_phi, A_wo, B_x, B_w_r, B_w_gate, B_w_up, B_w_down, c, w_mod
):
    return make()(A_x, A_wqkv, A_w_phi, A_wo, B_x, B_w_r, B_w_gate, B_w_up, B_w_down, c, w_mod)
```

```python
import collections
import contextlib
import functools

import jax
import jax.numpy as jnp
import numpy as np
import jax.experimental.pallas as pl
import jax.experimental.pallas.tpu as pltpu

F32, BF16, I32, U32 = jnp.float32, jnp.bfloat16, jnp.int32, jnp.uint32
S, D, H, DH, FF = 2048, 1024, 32, 32, 3584
HD = D // 2
NPAIR = H // 2
EPS = 1e-5
LOG2E = float(np.log2(np.e))
NN = (((1,), (0,)), ((), ()))
NT = (((1,), (1,)), ((), ()))


def _dot(a, b, dn=NN):
    return jax.lax.dot_general(a, b, dn, preferred_element_type=F32)


def _pack(x):
    n = x.shape[0] // 2
    if x.shape[1] > 128:
        return pltpu.bitcast(x.astype(BF16), U32)
    w = pltpu.bitcast(jnp.concatenate([x[:n], x[n:]], axis=1).astype(BF16), U32)
    return jnp.concatenate([w[:, :128], w[:, 128:]], axis=0)


def _unpack(w):
    return pltpu.bitcast(w, BF16)


def _recip(x):
    r = pl.reciprocal(x, approx=True)
    return r * (2.0 - x * r)


def _lhs_terms(a11, a12, a21, a22):
    return (a11 + a22, a21 + a22, a11, a22, a11 + a12, a21 - a11, a12 - a22)


def _rhs_terms(b11, b12, b21, b22):
    return (b11 + b22, b11, b12 - b22, b21 - b11, b22, b11 + b12, b21 + b22)


_QUADRANTS = (((0, 1), (3, 1), (4, -1), (6, 1)), ((2, 1), (4, 1)), ((1, 1), (3, 1)),
              ((0, 1), (1, -1), (2, 1), (5, 1)))


def _quadrant(q, product):
    total = None
    for j, sign in _QUADRANTS[q]:
        m = product(j)
        total = m if total is None else (total + m if sign > 0 else total - m)
    return total


def _layernorm(x):
    d = x - jnp.mean(x, axis=-1, keepdims=True)
    v = jnp.mean(d * d, axis=-1, keepdims=True)
    return d * jax.lax.rsqrt(v + EPS)


def _per_head(op, p):
    parts = [p[r:r + 8] for r in range(0, p.shape[0], 8)]
    while len(parts) > 1:
        parts = [op(a, b) for a, b in zip(parts[::2], parts[1::2])]
    out = op(parts[0], pltpu.roll(parts[0], 4, 0))
    return op(out, pltpu.roll(out, 2, 0))


def _apply(op, p, stat):
    n = p.shape[0] // 8
    return op(p.reshape(n, 8, p.shape[1]), stat).reshape(p.shape)


def _features(p):
    e_pos = jnp.exp2(_apply(jnp.subtract, p, _per_head(jnp.maximum, p)))
    e_neg = jnp.exp2(_apply(lambda a, low: low - a, p, _per_head(jnp.minimum, p)))
    pos = _apply(jnp.multiply, e_pos, _recip(_per_head(jnp.add, e_pos)))
    neg = _apply(jnp.multiply, e_neg, _recip(_per_head(jnp.add, e_neg)))
    return jnp.concatenate([pos, neg], axis=0)


def _interleaved_source(row):
    return (row & ~63) + ((row & 1) << 5) + ((row & 63) >> 1)


class _Interleaver:
    def __init__(self, ratio):
        self.queue = collections.deque()
        self.ratio = ratio
        self.credit = 0.0

    def defer(self, cost, fn):
        self.queue.append((cost, fn))

    def spent(self, cycles):
        self.credit += cycles * self.ratio
        while self.queue and self.credit >= self.queue[0][0]:
            cost, fn = self.queue.popleft()
            self.credit -= cost
            fn()
        if not self.queue:
            self.credit = 0.0

    def drain(self):
        while self.queue:
            self.queue.popleft()[1]()
        self.credit = 0.0


def make(RC=256, VC=256, LW=512, lfirst=29, FC=256, EC=32, ratio=0.55, vlimit=120, flags=None, S=S,
         prof=False, only=0, cdelay=3, spread=(2, 2, 2, 2, 2, 4, 2), last_rows=128, marks=(),
         vcost=256, split=False, kcost=150, lnv=True, ne=5, close2=False, mfirst=1, mlast=42, order='kqv', llast=41, pfirst=1, plast=6, nl=32, flag=2, RC0=128, sa_at=23, q_at=(10, 11, 12, 13), x1_at=14, l0=8):
    scope = lambda n: jax.named_scope(n) if prof is True or (prof and n in prof) else contextlib.nullcontext()
    T = 512
    HT = T // 2
    NTILE = S // T
    G = 128
    MT = pl.cdiv(4 * D // 128, NTILE - 1)
    nk, nv = 7 * HD // RC, 7 * HD // VC

    def kernel(x_hbm, wqkv_hbm, wphi_hbm, wo_hbm, wr_hbm, wg_hbm, wu_hbm, wd_hbm, c_hbm, wmod_hbm,
               out_hbm,
               x_v, wqkv_v, wphi_v, wo_v, wr_v, wg_v, wu_v, wd_v, c_v, wmod_v,
               act_v, raw_v, mod_v, stat_v, bias_v, bd_v, wot_v, ht_v, h0_v, phiq_v, phik_v, vt_v, kv_v, kvb_v, oa_v, ob_v,
               y_v, xn_v, out_v, r_v, fix_v, sems, osems, *terms_v):
        wq_v, wk_v, wv_v = terms_v[:4], terms_v[4:8], terms_v[8:]

        side = _Interleaver(ratio)
        copies = {}

        def add_copy(name, src, dst):
            copies[name] = pltpu.make_async_copy(src, dst, sems.at[NTILE + len(copies)])

        add_copy("c", c_hbm, c_v)
        add_copy("wphi", wphi_hbm, wphi_v)
        add_copy("wr", wr_hbm, wr_v)
        def add_columns(name, hbm, vmem, lo, n):
            add_copy(name, hbm.at[:, pl.ds(lo, n)], vmem.at[:, pl.ds(lo, n)])

        for n in range(2):
            piece = (pl.ds(n * HD, HD), pl.ds(D, D))
            add_copy(("scale", n), wmod_hbm.at[piece], wmod_v.at[piece])
        add_columns("shift", wmod_hbm, wmod_v, 0, D)
        for n in range(NTILE - 1):
            add_columns(("mod", n), wmod_hbm, wmod_v, 2 * D + n * MT * 128, min(MT * 128, 4 * D - n * MT * 128))
        add_columns("wq", wqkv_hbm, wqkv_v, 0, D)
        for half in range(2):
            for n in range(2):
                add_columns(("wk", n, half), wqkv_hbm, wqkv_v, D + half * HD + n * 256, 256)
            for n, (lo, size) in enumerate(((0, 128), (128, 128), (256, 256))):
                add_columns(("wv", n, half), wqkv_hbm, wqkv_v, 2 * D + half * HD + lo, size)
        both = lambda *name: ((*name, 0), (*name, 1))
        add_copy("wo", wo_hbm, wo_v.at[pl.ds(0, D)])
        add_copy("wg", wg_hbm, wg_v)
        add_copy("wu", wu_hbm, wu_v)
        add_copy("wd", wd_hbm, wd_v)

        def start(*names):
            for n in names:
                copies[n].start()

        def wait(*names):
            with scope("w_" + "_".join(str(n) for n in names)[:20].replace("'", "").replace(" ", "")):
                for n in names:
                    copies[n].wait()

        def rows_at(base, size):
            return pl.ds(base if isinstance(base, int) else pl.multiple_of(base, 8), size)

        def x_copy(t):
            return pltpu.make_async_copy(x_hbm.at[rows_at(t * T, T)], x_v.at[rows_at(t * T, T)], sems.at[t])

        def out_copy(n):
            if isinstance(n, int):
                lo, hi = max(n * T - 2 * G, 0), min((n + 1) * T - 2 * G, S)
                rows = pl.ds(lo, hi - lo)
            else:
                rows = rows_at(n * T - 2 * G, T)
            return pltpu.make_async_copy(out_v.at[rows], out_hbm.at[rows], osems.at[n])

        def modulation(lo, n, half=None):
            rows = pl.ds(0, D) if half is None else pl.ds(half * HD, HD)
            lanes = pl.ds(lo if isinstance(lo, int) else pl.multiple_of(lo, 128), n)
            m = _dot(_unpack(act_v[:, rows]), wmod_v[rows, lanes])[:8]
            raw_v[:, lanes] = m if not half else raw_v[:, lanes] + m

        raw = lambda i: raw_v[:, pl.ds(i * D, D)]

        def block_diag_phi():
            row = _interleaved_source(jax.lax.broadcasted_iota(I32, (128, DH), 0))
            col = jax.lax.broadcasted_iota(I32, (128, DH), 1)
            sel = jnp.where((row & (DH - 1)) == col, 1.0, 0.0).astype(BF16)
            r2 = _interleaved_source(jax.lax.broadcasted_iota(I32, (128, 128), 0)) >> 5
            c2 = jax.lax.broadcasted_iota(I32, (128, 128), 1) >> 5
            for g in range(D // 128):
                tiled = _dot(sel, wphi_v[pl.ds(g * 128, 128), :], NT)
                bd_v[g] = _pack(jnp.where(r2 == c2, tiled, 0.0))

        def prep_scores(i, g):
            parts = []
            for gg in (g, g + HD // 128):
                for half in range(2):
                    w = wqkv_v[pl.ds(half * HD, HD), pl.ds(i * D + gg * 128, 128)]
                    parts.append(_dot(_unpack(bd_v[gg]), w, NT) * LOG2E)
            for j, term in enumerate(_lhs_terms(*parts)):
                (wq_v, wk_v)[i][g][j] = _pack(term)

        def prep_values(g):
            chain = Chain(1)
            for r in range(0, HD, 64):
                blocks = [wqkv_v[pl.ds(row + r, 64), pl.ds(2 * D + col + g * 128, 128)].astype(F32)
                          for col in (0, HD) for row in (0, HD)]
                blocks[3] = chain.enter(blocks[3])
                for j, term in enumerate(_lhs_terms(*blocks)):
                    words = _pack(term)
                    wv_v[g][j, pl.ds(r // 2, 32), :] = words
                chain.leave(words[:8])

        def prep_output(n):
            hold(wo_v)
            lo = wo_v[rows_at(n * 32, 32), :].astype(F32)
            hi = wo_v[rows_at(HD + n * 32, 32), :].astype(F32)
            for j, term in enumerate(_rhs_terms(lo[:, :HD], lo[:, HD:], hi[:, :HD], hi[:, HD:])):
                wot_v[j, rows_at(n * 16, 16), :] = _pack(term)

        start("c")
        x_copy(0).start()
        start(*both("scale"), *both("wv", 0), *both("wv", 1), *both("wv", 2), "shift", "wphi")
        start(*both("wk", 0), *both("wk", 1), "wq")
        x_copy(1).start()
        start("wo")
        for t in range(1, NTILE):
            start(("mod", t - 1))
            if t + 1 < NTILE:
                x_copy(t + 1).start()
        start("wr")
        wait("c")
        bits = pltpu.bitcast(jnp.broadcast_to(c_v[:, :128].astype(F32), (8, 128)), I32)
        zero = jnp.minimum(jnp.max(bits & 0xFF), 0)
        latest = {}

        class Chain:
            def __init__(self, strands):
                self.tokens = collections.deque([None] * strands)

            def enter(self, value):
                token = self.tokens.popleft()
                if token is None:
                    return value
                head = pltpu.bitcast(pltpu.bitcast(value[:8, :128], I32) | token, F32)
                if value.shape[1] > 128:
                    head = jnp.concatenate([head, value[:8, 128:]], axis=1)
                return jnp.concatenate([head, value[8:]], axis=0) if value.shape[0] > 8 else head

            def leave(self, *values):
                token = None
                for value in values:
                    value = pltpu.bitcast(value, I32)
                    token = value if token is None else token | value
                self.tokens.append(token & zero)

            def widen(self, strands):
                last = self.tokens[-1]
                while len(self.tokens) < strands:
                    self.tokens.append(last)

        def hold(ref):
            spare = ref.shape[0] - 16
            back = jnp.clip(zero, 0, spare // 16) * 16
            ref[rows_at(spare - back, 16), pl.ds(0, 128)] = latest["m"].astype(BF16)

        def row_stats(t, n):
            xx = x_v[rows_at(t * T + n * 32, 32), :].astype(F32)
            mean = jnp.mean(xx, axis=-1, keepdims=True)
            d = xx - mean
            scale = jax.lax.rsqrt(jnp.mean(d * d, axis=-1, keepdims=True) + EPS)
            stat_v[0, rows_at(n * 32, 32), :] = jnp.broadcast_to(mean, (32, 128))
            stat_v[1, rows_at(n * 32, 32), :] = jnp.broadcast_to(scale, (32, 128))

        def normalized(t, offset, lanes):
            wide = lambda k: jnp.concatenate([stat_v[k, pl.ds(offset, 16), :]] * (LW // 128), axis=1)
            return (x_v[rows_at(t * T + offset, 16), lanes].astype(F32) - wide(0)) * wide(1)

        def norm1_unit(rows, n, shift=True):
            group, part = divmod(n, HD // LW)
            blocks = []
            for col in (part * LW, HD + part * LW):
                for offset in (group * 16, HT + group * 16):
                    lanes = pl.ds(col, LW)
                    hh = rows(offset, lanes).reshape(2, 8, LW) * mod_v[1, :, lanes]
                    blocks.append((hh + mod_v[0, :, lanes] if shift else hh).reshape(16, LW))
            words = [_pack(term) for term in _rhs_terms(*blocks)]

            def store(target):
                for j, w in enumerate(words):
                    target[j, pl.ds(group * 8, 8), pl.ds(part * LW, LW)] = w

            return store

        def apart(k):
            return (zero >> k) & 1 if k and split else 0

        def strassen(product, tiles, cycles, extra):
            products = []
            for j in range(7):
                products.append([product(j, k) for k in range(tiles)])
                latest["m"] = products[j][-1][-16:]
                side.spent(cycles)
                extra()
            return products

        def scores(i, extra, consume, RC):
            cost = kcost * RC // 256
            tiles = HT // 128
            for r in range(0, HD, RC):
                products = strassen(
                    lambda j, k: _dot(
                        _unpack(jnp.concatenate(
                            [(wq_v, wk_v)[i][g][j + apart(k)] for g in range(r // 128, (r + RC) // 128)], axis=0)),
                        _unpack(ht_v[j, pl.ds(k * 64, 64), :]), NT),
                    tiles, RC * HT // 128, extra)

                def unit(half, o, products=products, r=r):
                    for part in range(2):
                        phi = jnp.concatenate(
                            [_features(_quadrant(2 * half + part, lambda j: products[j][k][o:o + 64]))
                             for k in range(tiles)], axis=1)
                        consume((half * HD + r + o) // 64, pl.ds(part * HT, HT), phi.astype(BF16))

                for half in range(2):
                    for o in range(0, RC, 64):
                        side.defer(cost, functools.partial(unit, half, o))

        def key_features(pair, lanes, phi):
            phik_v[pair, :, lanes] = phi

        def query_features(t, pair, lanes, phi):
            phiq_v[t, pair, :, lanes] = phi

        def store_values(col, part, v):
            v = v.T.astype(BF16).reshape(2, 64, HT)
            vt_v[pl.ds(col // 64, 2), pl.ds(0, 64), pl.ds(part * HT, HT)] = v

        def values(source, extra, consume, VC):
            tiles = VC // 128
            for r in range(0, HD, VC):
                products = strassen(
                    lambda j, k: _dot(_unpack(source[j + apart(k)]), _unpack(wv_v[r // 128 + k][j])),
                    tiles, VC * HT // 128, extra)

                def unit(half, part, k, products=products, r=r):
                    consume(half * HD + r + k * 128, part, _quadrant(2 * half + part, lambda j: products[j][k]))

                for half in range(2):
                    for part in range(2):
                        for k in range(tiles):
                            side.defer(vcost // 2, functools.partial(unit, half, part, k))

        def accumulate_kv(j, first):
            kv = _dot(vt_v[j], phik_v[j], NT)
            kv_v[j] = kv if first else kv_v[j] + kv
            latest["m"] = kv[-16:]
            side.spent(T // 8)

        def finish_kv(j):
            row = jax.lax.broadcasted_iota(I32, (80, 128), 0)
            row_head = jnp.where(row < 64, row >> 5, (row >> 3) & 1)
            col_head = jax.lax.broadcasted_iota(I32, (80, 128), 1) & 1
            kvb_v[j] = _pack(jnp.where(row_head == col_head, kv_v[j], 0.0))

        def follow(plan):
            count = [0]

            def extra():
                count[0] += 1
                for task in plan.pop(count[0], ()):
                    task()

            for task in plan.pop(0, ()):
                task()
            return extra

        def first_pass(t, plan, order, rc):
            extra = follow(plan)
            for part in order:
                if part == "k":
                    scores(1, extra, key_features, rc[0])
                elif part == "q":
                    scores(0, extra, functools.partial(query_features, t), rc[1])
                else:
                    values(ht_v, extra, store_values, VC)
            assert not plan
            if order[-1] == "v":
                side.drain()
            for r in range(0, HD, VC):
                for half in range(2):
                    for o in range(0, VC, 64):
                        accumulate_kv((half * HD + r + o) // 64, isinstance(t, int) and t == 0)
            side.drain()

        def plan_norms(plan, t, begin, first, last, end):
            plan[begin] += [functools.partial(row_stats, t, n) for n in range(T // 32)]
            units = HT // 16 * (HD // LW)
            stores = []

            def unit(n):
                hold(x_v)
                stores.append(norm1_unit(functools.partial(normalized, t), n))

            for n in range(units):
                plan[first + (last - first) * n // units].append(functools.partial(unit, n))
            plan[end].append(lambda: [store(ht_v) for store in stores])

        def attend(t, part, target, i):
            lanes = pl.ds(part * HT, HT)
            outs = {}
            tasks = []
            for half in range(2):
                for k in range(2):
                    p = half * (NPAIR // 2) + 2 * i + k
                    num = _dot(_unpack(kvb_v[p]), phiq_v[t, p, :, lanes])

                    def unit(num=num, key=(half, k)):
                        outs[key] = [_apply(jnp.multiply, num[h * DH:(h + 1) * DH],
                                            _recip(num[64 + 8 * h:72 + 8 * h] + 1e-6)) for h in range(2)]

                    tasks.append(unit)

            def terms_unit():
                lo, hi = (jnp.concatenate(outs[half, 0] + outs[half, 1], axis=0).T for half in range(2))
                for q, term in enumerate(_lhs_terms(lo[:G], hi[:G], lo[G:], hi[G:])):
                    target[q, :, pl.ds(i * 128, 128)] = _pack(term)

            return tasks + [terms_unit]

        def output_weights():
            w = wr_v[...].astype(F32)
            w = jnp.concatenate([jnp.broadcast_to(w[j:j + 1], (8, 128)) for j in range(D // 128)], axis=1)
            for i in range(2, 6):
                mod_v[i] = raw(i) + 1.0 if i == 4 else raw(i)
            mod_v[6] = mod_v[4] * w
            mod_v[7] = mod_v[4] * mod_v[5]
            mod_v[8] = mod_v[3] * mod_v[5]
            mod_v[9] = jnp.broadcast_to(jnp.sum(mod_v[3] * w, axis=1, keepdims=True), (8, D))

        def finish_rows(base, y, chain):
            lane = jax.lax.broadcasted_iota(I32, (8, 128), 1)
            acc = r_v[base >> 10]
            for o in range(0, y.shape[0], 8):
                rows = rows_at(base + o, 8)
                xn = x_v[rows, :].astype(F32) + mod_v[2] * chain.enter(y[o:o + 8])
                mean = jnp.mean(xn, axis=-1, keepdims=True)
                d = xn - mean
                scale = jax.lax.rsqrt(jnp.mean(d * d, axis=-1, keepdims=True) + EPS)
                score = jnp.sum(d * mod_v[6], axis=-1, keepdims=True) * scale + mod_v[9, :, :1]
                normed = d * scale
                xn_v[rows, :] = normed
                out = normed * mod_v[7] + ((d + mean) + mod_v[8])
                out_v[rows, :] = out.astype(BF16)
                acc = jnp.where(lane == ((base + o) & 1023) >> 3, score, acc)
                chain.leave(*[out[:, l:l + 128] for l in range(128, D, 256)])
            r_v[base >> 10] = acc

        chains = []
        tokens = collections.deque()

        def mix(source, extra):
            return strassen(
                lambda j, k: _dot(_unpack(source[j + apart(k)]), _unpack(wot_v[j, :, pl.ds(k * 128, 128)])),
                HD // 128, 4 * G, extra)

        def mixed_rows(product, n):
            def rows_of(o):
                part, o = divmod(o, n)
                return jnp.concatenate(
                    [_quadrant(2 * part + half, lambda j: product(j, o)) for half in range(2)], axis=1)
            return rows_of

        def from_values(products):
            return lambda j, o: jnp.concatenate([tile[o:o + EC] for tile in products[j]], axis=1)

        def top2():
            shape = (S // 1024, 8, 128)
            idx = (jax.lax.broadcasted_iota(I32, shape, 0) * 1024 + jax.lax.broadcasted_iota(I32, shape, 2) * 8
                   + jax.lax.broadcasted_iota(I32, shape, 1)).astype(F32)
            m = r_v[...]
            reduce = lambda op, v: op(op(op(v, axis=0), axis=0, keepdims=True), axis=1, keepdims=True)
            picks = []
            for _ in range(2):
                top = reduce(jnp.max, m)
                first = reduce(jnp.min, jnp.where(m == top, idx, float(S - 1)))
                picks.append((jnp.max(first.astype(I32)), top))
                m = jnp.where(idx == first, -jnp.inf, m)
            return picks

        def experts():
            (i1, m1), (i2, m2) = top2()
            picks = [jnp.clip(i, 0, S - 1) for i in (i1, i2)]
            bases = [pl.multiple_of((i >> 4) * 16, 16) for i in picks]
            sub = jax.lax.broadcasted_iota(I32, (16, D), 0)
            first, second = (jnp.broadcast_to(xn_v[pl.ds(i, 1), :], (16, D)) for i in picks)
            sel = jnp.where(sub == 0, first, second).reshape(2, 8, D) * mod_v[4] + mod_v[3]
            sel = sel.reshape(16, D).astype(BF16)
            y = None
            acts = collections.deque()

            def down():
                nonlocal y
                f, g, u = acts.popleft()
                act = (g * jax.nn.sigmoid(g) * u).astype(BF16)
                part = _dot(act, wd_v[pl.ds(f, FC), :])
                y = part if y is None else y + part

            for f in range(0, FF, FC):
                acts.append((f, _dot(sel, wg_v[:, pl.ds(f, FC)]), _dot(sel, wu_v[:, pl.ds(f, FC)])))
                if len(acts) > flag:
                    down()
            while acts:
                down()
            y1, y2 = y[0:1] * jax.nn.sigmoid(m1), y[1:2] * jax.nn.sigmoid(m2)
            for n, base in enumerate(bases):
                upd = jnp.where(sub == picks[0] - base, y1, 0.0) + jnp.where(sub == picks[1] - base, y2, 0.0)
                full = out_v[pl.ds(base, 16), :].astype(F32).reshape(2, 8, D) + mod_v[5] * upd.reshape(2, 8, D)
                fix_v[n] = full.reshape(16, D).astype(BF16)
            return bases

        cc = c_v[...].astype(F32)
        act_v[...] = _pack(jnp.broadcast_to(cc * jax.nn.sigmoid(cc), (16, D)))
        with scope("w_x0"):
            x_copy(0).wait()
        for n in range(T // 32):
            row_stats(0, n)
        for offset in range(0, T, 16):
            for col in range(0, D, LW):
                xn_v[pl.ds(offset, 16), pl.ds(col, LW)] = normalized(0, offset, pl.ds(col, LW))
        for n in range(2):
            wait(("scale", n))
            modulation(D, D, n)
        mod_v[1] = raw(1) + 1.0
        units = HT // 16 * (HD // LW)
        saved = lambda offset, lanes: xn_v[pl.ds(offset, 16), lanes]
        for n in range(units):
            norm1_unit(saved, n, shift=False)(h0_v)

        def hold_values(col, part, v):
            xn_v[pl.ds(T + part * HT, HT), pl.ds(col, 128)] = v

        def shift_and_bias():
            wait("shift")
            modulation(0, D)
            mod_v[0] = raw(0)

        def release_values(col, part):
            v = xn_v[pl.ds(T + part * HT, HT), pl.ds(col, 128)]
            store_values(col, part, _apply(jnp.add, v, bias_v[:, pl.ds(col, 128)]))

        wait(*both("wv", 0))
        prep_values(0)
        plan = collections.defaultdict(list)
        plan[3] += [lambda: wait(*both("wv", 1)), lambda: prep_values(1)]
        plan[7] += [lambda: wait(*both("wv", 2))]
        plan[8] += [lambda: prep_values(2)]
        plan[15] += [lambda: prep_values(3)]
        plan[sa_at].append(shift_and_bias)
        with scope("values0"):
            values(h0_v, follow(plan), hold_values, 128)
            side.drain()
        assert not plan
        wait("wphi", *both("wk", 0))
        block_diag_phi()
        prep_scores(1, 0)
        prep_scores(1, 1)
        shift = jnp.concatenate([raw(0)] * 2, axis=0).astype(BF16)
        bias_v[...] = _dot(shift, wqkv_v[:, pl.ds(2 * D, D)])[:8]
        for n in range(units):
            norm1_unit(saved, n)(ht_v)

        plan = collections.defaultdict(list)
        def initialize():
            vt_v[:, pl.ds(64, 16), :] = jnp.ones((NPAIR, 16, T), BF16)
            y_v[...] = jnp.zeros(y_v.shape, F32)
            r_v[...] = jnp.full(r_v.shape, -jnp.inf, F32)

        plan[0].append(initialize)
        plan[3] += [lambda: wait(*both("wk", 1)), lambda: prep_scores(1, 2), lambda: prep_scores(1, 3)]
        for n in range(16):
            plan[1 + n * 8 // 16].append(functools.partial(release_values, n // 2 * 128, n % 2))
        plan[q_at[0]].append(lambda: wait("wq"))
        for g in range(4):
            plan[q_at[g]].append(functools.partial(prep_scores, 0, g))
        plan[x1_at].append(lambda: x_copy(1).wait())
        plan_norms(plan, 1, x1_at, x1_at + 2, 14 + 7 * HD // RC0 - l0, 14 + 7 * HD // RC0)
        if marks:
            def mark(n):
                with jax.named_scope(f"mark{n}"):
                    fix_v[0, :, pl.ds(0, 128)] = jnp.zeros((16, 128), BF16)
            for n in marks:
                plan[n].append(functools.partial(mark, n))
        with scope("tile0"):
            first_pass(0, plan, 'kq', (256, RC0))

        def first_step(t, carry):
            @pl.when(t + 1 < NTILE)
            def _():
                x_copy(t + 1).wait()

            for n in range(NTILE - 1):
                pl.when(t == n + 1)(functools.partial(wait, ("mod", n)))

            @pl.when(t == NTILE - 2)
            def _():
                start("wg", "wu", "wd")

            plan = collections.defaultdict(list)
            plan_norms(plan, jnp.clip(t + 1, 0, NTILE - 1), 0, lfirst, llast, 2 * nk + nv)
            per_step = pl.cdiv(HD // 32, NTILE - 1)
            for n in range(per_step):
                plan[pfirst + n * (plast - pfirst) // per_step].append(functools.partial(
                    lambda n: prep_output(jnp.clip((t - 1) * per_step + n, 0, HD // 32 - 1)), n))
            tiles = MT
            for n in range(2 * tiles):
                tile = jnp.clip((t - 1) * tiles + n // 2, 0, 4 * D // 128 - 1)
                plan[mfirst + n * (mlast - mfirst) // (2 * tiles)].append(
                    functools.partial(modulation, 2 * D + tile * 128, 128, n % 2))
            first_pass(t, plan, order, (RC, RC))
            return carry

        wait("wo")
        if only in (0, 1):
            with scope("pass1"):
                jax.lax.fori_loop(1, NTILE, first_step, 0)
        if only == 1:
            for j in range(NPAIR):
                finish_kv(j)
            out_v[pl.ds(0, 64), pl.ds(0, 512)] = phiq_v[zero, zero, pl.ds(0, 64), :]
            out_v[pl.ds(64, 80), pl.ds(0, 128)] = _unpack(kvb_v[zero])
            out_v[pl.ds(160, 64), pl.ds(0, 512)] = _unpack(wot_v[zero, pl.ds(0, 32), :])
            out_copy(0).start()
            out_copy(0).wait()
            return

        wait("wr")
        for j in range(NPAIR):
            finish_kv(j)
        tasks = [task for i in range(4) for task in attend(0, 0, oa_v, i)]
        for task in tasks:
            task()
        output_weights()

        def mix_step(source, following, base, rows_of):
            state = {"step": 0, "unit": 0}

            def finish(count):
                for _ in range(count):
                    row = state["unit"] * EC
                    finish_rows(base + row, rows_of(row), chains[0])
                    state["unit"] += 1

            def extra():
                state["step"] += 1
                if state["step"] < len(spread):
                    finish(spread[state["step"]] * 16 // EC)

            if following:
                tasks = [task for i in range(4) for task in attend(*following, i)]
                for task in tasks:
                    task()
            finish(spread[0] * 16 // EC)
            return mix(source, extra)

        stored = mixed_rows(lambda j, o: y_v[j, pl.ds(o, EC), :], G)

        def second_step(t, carry):
            latest.clear()
            chains[:] = [Chain(ne)]
            products = mix_step(oa_v, (t, 1, ob_v), jnp.clip(t * T - 2 * G, 0, S - 2 * G), stored)
            products = mix_step(ob_v, (jnp.clip(t + 1, 0, NTILE - 1), 0, oa_v), jnp.clip(t, 0, NTILE - 1) * T,
                                mixed_rows(from_values(products), G))
            for j in range(7):
                for k, tile in enumerate(products[j]):
                    y_v[j, :, pl.ds(k * 128, 128)] = tile

            @pl.when(t == 0)
            def _():
                out_copy(0).start()

            @pl.when(t > 0)
            def _():
                out_copy(t).start()

            return carry

        with scope("pass2"):
            jax.lax.fori_loop(0, NTILE, second_step, 0)
        wait("wg", "wu", "wd")
        with scope("last"):
            chain = Chain(nl)
            for o in range(0, 2 * G, EC):
                finish_rows(S - 2 * G + o, stored(o), chain)
        out_copy(NTILE).start()
        with scope("experts"):
            b1, b2 = experts()
        with scope("w_out"):
            for n in range(NTILE + 1):
                out_copy(n).wait()
        fix = [pltpu.make_async_copy(fix_v.at[n], out_hbm.at[pl.ds(b, 16)], osems.at[n])
               for n, b in enumerate((b1, b2))]
        fix[0].start()

        @pl.when(b1 != b2)
        def _():
            fix[1].start()
            fix[1].wait()

        fix[0].wait()

    nsem = NTILE + 3 + 3 + NTILE - 1 + 1 + 10 + 4
    scratch = [
        pltpu.VMEM((S + 16, D), BF16), pltpu.VMEM((D, 3 * D), BF16), pltpu.VMEM((D, DH), BF16),
        pltpu.VMEM((D + 16, D), BF16), pltpu.VMEM((8, 128), BF16),
        pltpu.VMEM((D, FF), BF16), pltpu.VMEM((D, FF), BF16), pltpu.VMEM((FF, D), BF16),
        pltpu.VMEM((1, D), BF16), pltpu.VMEM((D, 6 * D), BF16),
        pltpu.VMEM((8, D), U32),
        pltpu.VMEM((8, 6 * D), F32),
        pltpu.VMEM((10, 8, D), F32),
        pltpu.VMEM((2, T, 128), F32),
        pltpu.VMEM((8, D), F32),
        pltpu.VMEM((D // 128, 64, 128), U32),
        pltpu.VMEM((7, HD // 2, HD), U32),
        pltpu.VMEM((8, HT // 2, HD), U32),
        pltpu.VMEM((7, HT // 2, HD), U32),
        pltpu.VMEM((NTILE, NPAIR, 128, T), BF16),
        pltpu.VMEM((NPAIR, 128, T), BF16),
        pltpu.VMEM((NPAIR, 80, T), BF16),
        pltpu.VMEM((NPAIR, 80, 128), F32),
        pltpu.VMEM((NPAIR, 40, 128), U32),
        pltpu.VMEM((8, G // 2, HD), U32),
        pltpu.VMEM((8, G // 2, HD), U32),
        pltpu.VMEM((7, G, HD), F32),
        pltpu.VMEM((S, D), F32),
        pltpu.VMEM((S, D), BF16),
        pltpu.VMEM((S // 1024, 8, 128), F32),
        pltpu.VMEM((2, 16, D), BF16),
        pltpu.SemaphoreType.DMA((nsem,)),
        pltpu.SemaphoreType.DMA((NTILE + 1,)),
    ] + [pltpu.VMEM((8, 64, HD), U32)] * 8 + [pltpu.VMEM((7, HD // 2, 128), U32)] * 4

    def fn(A_x, A_wqkv, A_w_phi, A_wo, B_x, B_w_r, B_w_gate, B_w_up, B_w_down, c, w_mod):
        del B_x
        out = pl.pallas_call(
            kernel,
            out_shape=jax.ShapeDtypeStruct((S, D), A_x.dtype),
            in_specs=[pl.BlockSpec(memory_space=pl.ANY)] * 10,
            out_specs=pl.BlockSpec(memory_space=pl.ANY),
            scratch_shapes=scratch,
            compiler_params=pltpu.CompilerParams(vmem_limit_bytes=vlimit * 2**20, flags=flags),
        )(A_x.reshape(S, D), A_wqkv, A_w_phi.reshape(D, DH), A_wo, B_w_r.reshape(8, 128),
          B_w_gate, B_w_up, B_w_down, c, w_mod)
        return out.reshape(A_x.shape)

    return fn


@jax.jit
def pallas_adaLN_cond__linear_kernel_hedgehog__moe_arch_mod__prompt_kernel(
    A_x, A_wqkv, A_w_phi, A_wo, B_x, B_w_r, B_w_gate, B_w_up, B_w_down, c, w_mod
):
    return make()(A_x, A_wqkv, A_w_phi, A_wo, B_x, B_w_r, B_w_gate, B_w_up, B_w_down, c, w_mod)
```

```python
import collections
import contextlib
import functools

import jax
import jax.numpy as jnp
import numpy as np
import jax.experimental.pallas as pl
import jax.experimental.pallas.tpu as pltpu

F32, BF16, I32, U32 = jnp.float32, jnp.bfloat16, jnp.int32, jnp.uint32
S, D, H, DH, FF = 2048, 1024, 32, 32, 3584
HD = D // 2
NPAIR = H // 2
EPS = 1e-5
LOG2E = float(np.log2(np.e))
NN = (((1,), (0,)), ((), ()))
NT = (((1,), (1,)), ((), ()))


def _dot(a, b, dn=NN):
    return jax.lax.dot_general(a, b, dn, preferred_element_type=F32)


def _pack(x):
    n = x.shape[0] // 2
    if x.shape[1] > 128:
        return pltpu.bitcast(x.astype(BF16), U32)
    w = pltpu.bitcast(jnp.concatenate([x[:n], x[n:]], axis=1).astype(BF16), U32)
    return jnp.concatenate([w[:, :128], w[:, 128:]], axis=0)


def _unpack(w):
    return pltpu.bitcast(w, BF16)


def _recip(x):
    r = pl.reciprocal(x, approx=True)
    return r * (2.0 - x * r)


def _lhs_terms(a11, a12, a21, a22):
    return (a11 + a22, a21 + a22, a11, a22, a11 + a12, a21 - a11, a12 - a22)


def _rhs_terms(b11, b12, b21, b22):
    return (b11 + b22, b11, b12 - b22, b21 - b11, b22, b11 + b12, b21 + b22)


_QUADRANTS = (((0, 1), (3, 1), (4, -1), (6, 1)), ((2, 1), (4, 1)), ((1, 1), (3, 1)),
              ((0, 1), (1, -1), (2, 1), (5, 1)))


def _quadrant(q, product):
    total = None
    for j, sign in _QUADRANTS[q]:
        m = product(j)
        total = m if total is None else (total + m if sign > 0 else total - m)
    return total


def _layernorm(x):
    d = x - jnp.mean(x, axis=-1, keepdims=True)
    v = jnp.mean(d * d, axis=-1, keepdims=True)
    return d * jax.lax.rsqrt(v + EPS)


def _per_head(op, p):
    parts = [p[r:r + 8] for r in range(0, p.shape[0], 8)]
    while len(parts) > 1:
        parts = [op(a, b) for a, b in zip(parts[::2], parts[1::2])]
    out = op(parts[0], pltpu.roll(parts[0], 4, 0))
    return op(out, pltpu.roll(out, 2, 0))


def _apply(op, p, stat):
    n = p.shape[0] // 8
    return op(p.reshape(n, 8, p.shape[1]), stat).reshape(p.shape)


def _features(p):
    e_pos = jnp.exp2(_apply(jnp.subtract, p, _per_head(jnp.maximum, p)))
    e_neg = jnp.exp2(_apply(lambda a, low: low - a, p, _per_head(jnp.minimum, p)))
    pos = _apply(jnp.multiply, e_pos, _recip(_per_head(jnp.add, e_pos)))
    neg = _apply(jnp.multiply, e_neg, _recip(_per_head(jnp.add, e_neg)))
    return jnp.concatenate([pos, neg], axis=0)


def _interleaved_source(row):
    return (row & ~63) + ((row & 1) << 5) + ((row & 63) >> 1)


class _Interleaver:
    def __init__(self, ratio):
        self.queue = collections.deque()
        self.ratio = ratio
        self.credit = 0.0

    def defer(self, cost, fn):
        self.queue.append((cost, fn))

    def spent(self, cycles):
        self.credit += cycles * self.ratio
        while self.queue and self.credit >= self.queue[0][0]:
            cost, fn = self.queue.popleft()
            self.credit -= cost
            fn()
        if not self.queue:
            self.credit = 0.0

    def drain(self):
        while self.queue:
            self.queue.popleft()[1]()
        self.credit = 0.0


def make(RC=256, VC=256, LW=512, FC=256, EC=32, ratio=0.55, vlimit=120, flags=None, S=S,
         prof=False, only=0, marks=(), vcost=256, kcost=150, mfirst=26, mlast=42, order='kqv',
         lfirst=29, llast=41, pfirst=1, plast=28, flag=2, RC0=128, sa_at=23, q_at=(10, 11, 12, 13), x1_at=16, l0=6,
         every=1, phase=1, ne=3, nl=32):
    scope = lambda n: jax.named_scope(n) if prof is True or (prof and n in prof) else contextlib.nullcontext()
    T = 512
    HT = T // 2
    NTILE = S // T
    G = 128
    NSUB = S // (2 * G)
    MW = 4 * D // NTILE
    nk, nv = 7 * HD // RC, 7 * HD // VC

    def kernel(x_hbm, wqkv_hbm, wphi_hbm, wo_hbm, wr_hbm, wg_hbm, wu_hbm, wd_hbm, c_hbm, wmod_hbm,
               out_hbm,
               x_v, wqkv_v, wphi_v, wo_v, wr_v, wg_v, wu_v, wd_v, c_v, wmod_v,
               act_v, raw_v, mod_v, stat_v, bias_v, bd_v, wot_v, ht_v, h0_v, phiq_v, phik_v, vt_v, kv_v, kvb_v, oa_v, ob_v,
               xn_v, out_v, fix_v, sems, osems, *terms_v):
        wq_v, wk_v, wv_v = terms_v[:4], terms_v[4:8], terms_v[8:]

        side = _Interleaver(ratio)
        copies = {}

        def add_copy(name, src, dst):
            copies[name] = pltpu.make_async_copy(src, dst, sems.at[NTILE + len(copies)])

        add_copy("c", c_hbm, c_v)
        add_copy("wphi", wphi_hbm, wphi_v)
        add_copy("wr", wr_hbm, wr_v)
        def add_columns(name, hbm, vmem, lo, n):
            add_copy(name, hbm.at[:, pl.ds(lo, n)], vmem.at[:, pl.ds(lo, n)])

        for n in range(2):
            piece = (pl.ds(n * HD, HD), pl.ds(D, D))
            add_copy(("scale", n), wmod_hbm.at[piece], wmod_v.at[piece])
        add_columns("shift", wmod_hbm, wmod_v, 0, D)
        for t in range(NTILE):
            add_columns(("mod", t), wmod_hbm, wmod_v, 2 * D + t * MW, MW)
        add_columns("wq", wqkv_hbm, wqkv_v, 0, D)
        add_columns("wk", wqkv_hbm, wqkv_v, D, D)
        for half in range(2):
            for n, (lo, size) in enumerate(((0, 128), (128, 128), (256, 256))):
                add_columns(("wv", n, half), wqkv_hbm, wqkv_v, 2 * D + half * HD + lo, size)
        both = lambda *name: ((*name, 0), (*name, 1))
        add_copy("wo", wo_hbm, wo_v.at[pl.ds(0, D)])
        add_copy("wg", wg_hbm, wg_v)
        add_copy("wu", wu_hbm, wu_v)
        add_copy("wd", wd_hbm, wd_v)

        def start(*names):
            for n in names:
                copies[n].start()

        def wait(*names):
            with scope("w_" + "_".join(str(n) for n in names)[:20].replace("'", "").replace(" ", "")):
                for n in names:
                    copies[n].wait()

        def rows_at(base, size):
            return pl.ds(base if isinstance(base, int) else pl.multiple_of(base, 8), size)

        def x_copy(t):
            return pltpu.make_async_copy(x_hbm.at[rows_at(t * T, T)], x_v.at[rows_at(t * T, T)], sems.at[t])

        def out_copy(n):
            rows = pl.ds(n * 2 * G, 2 * G)
            return pltpu.make_async_copy(out_v.at[rows], out_hbm.at[rows], osems.at[n])

        def modulation(lo, n, half=None):
            rows = pl.ds(0, D) if half is None else pl.ds(half * HD, HD)
            lanes = pl.ds(lo if isinstance(lo, int) else pl.multiple_of(lo, 128), n)
            m = _dot(_unpack(act_v[:, rows]), wmod_v[rows, lanes])[:8]
            raw_v[:, lanes] = m if not half else raw_v[:, lanes] + m

        raw = lambda i: raw_v[:, pl.ds(i * D, D)]

        def block_diag_phi():
            row = _interleaved_source(jax.lax.broadcasted_iota(I32, (128, DH), 0))
            col = jax.lax.broadcasted_iota(I32, (128, DH), 1)
            sel = jnp.where((row & (DH - 1)) == col, 1.0, 0.0).astype(BF16)
            r2 = _interleaved_source(jax.lax.broadcasted_iota(I32, (128, 128), 0)) >> 5
            c2 = jax.lax.broadcasted_iota(I32, (128, 128), 1) >> 5
            for g in range(D // 128):
                tiled = _dot(sel, wphi_v[pl.ds(g * 128, 128), :], NT)
                bd_v[g] = _pack(jnp.where(r2 == c2, tiled, 0.0))

        def prep_scores(i, g):
            parts = []
            for gg in (g, g + HD // 128):
                for half in range(2):
                    w = wqkv_v[pl.ds(half * HD, HD), pl.ds(i * D + gg * 128, 128)]
                    parts.append(_dot(_unpack(bd_v[gg]), w, NT) * LOG2E)
            for j, term in enumerate(_lhs_terms(*parts)):
                (wq_v, wk_v)[i][g][j] = _pack(term)

        def prep_values(g):
            chain = Chain(1)
            for r in range(0, HD, 64):
                blocks = [wqkv_v[pl.ds(row + r, 64), pl.ds(2 * D + col + g * 128, 128)].astype(F32)
                          for col in (0, HD) for row in (0, HD)]
                blocks[3] = chain.enter(blocks[3])
                for j, term in enumerate(_lhs_terms(*blocks)):
                    words = _pack(term)
                    wv_v[g][j, pl.ds(r // 2, 32), :] = words
                chain.leave(words[:8])

        def prep_output(n):
            hold(wo_v)
            lo = wo_v[rows_at(n * 16, 16), :].astype(F32)
            hi = wo_v[rows_at(HD + n * 16, 16), :].astype(F32)
            for j, term in enumerate(_rhs_terms(lo[:, :HD], lo[:, HD:], hi[:, :HD], hi[:, HD:])):
                wot_v[j, rows_at(n * 8, 8), :] = _pack(term)

        start("c")
        x_copy(0).start()
        start(*both("scale"), *both("wv", 0), *both("wv", 1), *both("wv", 2), "shift", "wphi", "wk", "wq")
        x_copy(1).start()
        start(("mod", 0), "wo")
        for t in range(1, NTILE):
            start(("mod", t))
            if t + 1 < NTILE:
                x_copy(t + 1).start()
        start("wr")
        wait("c")
        bits = pltpu.bitcast(jnp.broadcast_to(c_v[:, :128].astype(F32), (8, 128)), I32)
        zero = jnp.minimum(jnp.max(bits & 0xFF), 0)
        latest = {}

        class Chain:
            def __init__(self, strands):
                self.tokens = collections.deque([None] * strands)

            def enter(self, value):
                token = self.tokens.popleft()
                if token is None:
                    return value
                head = pltpu.bitcast(pltpu.bitcast(value[:8, :128], I32) | token, F32)
                if value.shape[1] > 128:
                    head = jnp.concatenate([head, value[:8, 128:]], axis=1)
                return jnp.concatenate([head, value[8:]], axis=0) if value.shape[0] > 8 else head

            def leave(self, *values):
                token = None
                for value in values:
                    value = pltpu.bitcast(value, I32)
                    token = value if token is None else token | value
                self.tokens.append(token & zero)

            def widen(self, strands):
                last = self.tokens[-1]
                while len(self.tokens) < strands:
                    self.tokens.append(last)

        def hold(ref):
            spare = ref.shape[0] - 16
            back = jnp.clip(zero, 0, spare // 16) * 16
            ref[rows_at(spare - back, 16), pl.ds(0, 128)] = latest["m"].astype(BF16)

        def row_stats(t, n):
            xx = x_v[rows_at(t * T + n * 32, 32), :].astype(F32)
            mean = jnp.mean(xx, axis=-1, keepdims=True)
            d = xx - mean
            scale = jax.lax.rsqrt(jnp.mean(d * d, axis=-1, keepdims=True) + EPS)
            stat_v[0, rows_at(n * 32, 32), :] = jnp.broadcast_to(mean, (32, 128))
            stat_v[1, rows_at(n * 32, 32), :] = jnp.broadcast_to(scale, (32, 128))

        def normalized(t, offset, lanes):
            wide = lambda k: jnp.concatenate([stat_v[k, pl.ds(offset, 16), :]] * (LW // 128), axis=1)
            return (x_v[rows_at(t * T + offset, 16), lanes].astype(F32) - wide(0)) * wide(1)

        def norm1_unit(rows, n, shift=True):
            group, part = divmod(n, HD // LW)
            blocks = []
            for col in (part * LW, HD + part * LW):
                for offset in (group * 16, HT + group * 16):
                    lanes = pl.ds(col, LW)
                    hh = rows(offset, lanes).reshape(2, 8, LW) * mod_v[1, :, lanes]
                    blocks.append((hh + mod_v[0, :, lanes] if shift else hh).reshape(16, LW))
            words = [_pack(term) for term in _rhs_terms(*blocks)]

            def store(target):
                for j, w in enumerate(words):
                    target[j, pl.ds(group * 8, 8), pl.ds(part * LW, LW)] = w

            return store

        def strassen(product, tiles, cycles, extra):
            products = []
            for j in range(7):
                products.append([product(j, k) for k in range(tiles)])
                latest["m"] = products[j][-1][-16:]
                side.spent(cycles)
                extra()
            return products

        def scores(i, extra, consume, RC):
            cost = kcost * RC // 256
            tiles = HT // 128
            for r in range(0, HD, RC):
                products = strassen(
                    lambda j, k: _dot(
                        _unpack(jnp.concatenate(
                            [(wq_v, wk_v)[i][g][j] for g in range(r // 128, (r + RC) // 128)], axis=0)),
                        _unpack(ht_v[j, pl.ds(k * 64, 64), :]), NT),
                    tiles, RC * HT // 128, extra)

                def unit(half, o, products=products, r=r):
                    for part in range(2):
                        phi = jnp.concatenate(
                            [_features(_quadrant(2 * half + part, lambda j: products[j][k][o:o + 64]))
                             for k in range(tiles)], axis=1)
                        consume((half * HD + r + o) // 64, pl.ds(part * HT, HT), phi.astype(BF16))

                for half in range(2):
                    for o in range(0, RC, 64):
                        side.defer(cost, functools.partial(unit, half, o))

        def key_features(pair, lanes, phi):
            phik_v[pair, :, lanes] = phi

        def query_features(t, pair, lanes, phi):
            phiq_v[t, pair, :, lanes] = phi

        def store_values(col, part, v):
            v = v.T.astype(BF16).reshape(2, 64, HT)
            vt_v[pl.ds(col // 64, 2), pl.ds(0, 64), pl.ds(part * HT, HT)] = v

        def values(source, extra, consume, VC):
            tiles = VC // 128
            for r in range(0, HD, VC):
                products = strassen(
                    lambda j, k: _dot(_unpack(source[j]), _unpack(wv_v[r // 128 + k][j])),
                    tiles, VC * HT // 128, extra)

                def unit(half, part, k, products=products, r=r):
                    consume(half * HD + r + k * 128, part, _quadrant(2 * half + part, lambda j: products[j][k]))

                for half in range(2):
                    for part in range(2):
                        for k in range(tiles):
                            side.defer(vcost // 2, functools.partial(unit, half, part, k))

        def accumulate_kv(j, first):
            kv = _dot(vt_v[j], phik_v[j], NT)
            kv_v[j] = kv if first else kv_v[j] + kv
            latest["m"] = kv[-16:]
            side.spent(T // 8)

        def finish_kv(j):
            row = jax.lax.broadcasted_iota(I32, (80, 128), 0)
            row_head = jnp.where(row < 64, row >> 5, (row >> 3) & 1)
            col_head = jax.lax.broadcasted_iota(I32, (80, 128), 1) & 1
            kvb_v[j] = _pack(jnp.where(row_head == col_head, kv_v[j], 0.0))

        def follow(plan):
            count = [0]

            def extra():
                count[0] += 1
                for task in plan.pop(count[0], ()):
                    task()

            for task in plan.pop(0, ()):
                task()
            return extra

        def first_pass(t, plan, order, rc):
            extra = follow(plan)
            for part in order:
                if part == "k":
                    scores(1, extra, key_features, rc[0])
                elif part == "q":
                    scores(0, extra, functools.partial(query_features, t), rc[1])
                else:
                    values(ht_v, extra, store_values, VC)
            assert not plan
            if order[-1] == "v":
                side.drain()
            for r in range(0, HD, VC):
                for half in range(2):
                    for o in range(0, VC, 64):
                        accumulate_kv((half * HD + r + o) // 64, isinstance(t, int) and t == 0)
            side.drain()

        def plan_norms(plan, t, begin, first, last, end):
            plan[begin] += [functools.partial(row_stats, t, n) for n in range(T // 32)]
            units = HT // 16 * (HD // LW)
            stores = []

            def unit(n):
                hold(x_v)
                stores.append(norm1_unit(functools.partial(normalized, t), n))

            for n in range(units):
                plan[first + (last - first) * n // units].append(functools.partial(unit, n))
            plan[end].append(lambda: [store(ht_v) for store in stores])

        def plan_modulation(plan, t, first, last):
            steps = 2 * MW // 128
            for n in range(steps):
                plan[first + (last - first) * n // steps].append(
                    functools.partial(modulation, 2 * D + t * MW + n // 2 * 128, 128, n % 2))

        def attend(t, part, target, i):
            lanes = pl.ds(part * HT, HT)
            outs = {}
            tasks = []
            for half in range(2):
                for k in range(2):
                    p = half * (NPAIR // 2) + 2 * i + k
                    num = _dot(_unpack(kvb_v[p]), phiq_v[t, p, :, lanes])

                    def unit(num=num, key=(half, k)):
                        outs[key] = [_apply(jnp.multiply, num[h * DH:(h + 1) * DH],
                                            _recip(num[64 + 8 * h:72 + 8 * h] + 1e-6)) for h in range(2)]

                    tasks.append(unit)

            def terms_unit():
                lo, hi = (jnp.concatenate(outs[half, 0] + outs[half, 1], axis=0).T for half in range(2))
                for q, term in enumerate(_lhs_terms(lo[:G], hi[:G], lo[G:], hi[G:])):
                    target[q, :, pl.ds(i * 128, 128)] = _pack(term)

            return tasks + [terms_unit]

        def output_weights():
            w = wr_v[...].astype(F32)
            w = jnp.concatenate([jnp.broadcast_to(w[j:j + 1], (8, 128)) for j in range(D // 128)], axis=1)
            for i in range(2, 6):
                mod_v[i] = raw(i) + 1.0 if i == 4 else raw(i)
            mod_v[6] = mod_v[4] * w
            mod_v[7] = mod_v[4] * mod_v[5]
            mod_v[8] = mod_v[3] * mod_v[5]
            mod_v[9] = jnp.broadcast_to(jnp.sum(mod_v[3] * w, axis=1, keepdims=True), (8, D))

        ranks = {}

        def finish_rows(base, y, chain):
            lane = jax.lax.broadcasted_iota(I32, (8, 128), 1)
            acc = ranks.get(base >> 10, jnp.full((8, 128), -jnp.inf, F32))
            for o in range(0, y.shape[0], 8):
                rows = rows_at(base + o, 8)
                xn = x_v[rows, :].astype(F32) + mod_v[2] * chain.enter(y[o:o + 8])
                mean = jnp.mean(xn, axis=-1, keepdims=True)
                d = xn - mean
                scale = jax.lax.rsqrt(jnp.mean(d * d, axis=-1, keepdims=True) + EPS)
                score = jnp.sum(d * mod_v[6], axis=-1, keepdims=True) * scale + mod_v[9, :, :1]
                normed = d * scale
                xn_v[rows, :] = normed
                out = normed * mod_v[7] + ((d + mean) + mod_v[8])
                out_v[rows, :] = out.astype(BF16)
                acc = jnp.where(lane == ((base + o) & 1023) >> 3, score, acc)
                chain.leave(*[out[:, l:l + 128] for l in range(128, D, 256)])
            ranks[base >> 10] = acc

        tokens = collections.deque()

        def mix(source, extra):
            return strassen(
                lambda j, k: _dot(_unpack(source[j]), _unpack(wot_v[j, :, pl.ds(k * 128, 128)])),
                HD // 128, 4 * G, extra)

        def mixed_rows(product, n):
            def rows_of(o):
                part, o = divmod(o, n)
                return jnp.concatenate(
                    [_quadrant(2 * part + half, lambda j: product(j, o)) for half in range(2)], axis=1)
            return rows_of

        def from_values(products):
            return lambda j, o: jnp.concatenate([tile[o:o + EC] for tile in products[j]], axis=1)

        def top2():
            shape = (S // 1024, 8, 128)
            idx = (jax.lax.broadcasted_iota(I32, shape, 0) * 1024 + jax.lax.broadcasted_iota(I32, shape, 2) * 8
                   + jax.lax.broadcasted_iota(I32, shape, 1)).astype(F32)
            m = jnp.stack([ranks[b] for b in range(S // 1024)])
            reduce = lambda op, v: op(op(op(v, axis=0), axis=0, keepdims=True), axis=1, keepdims=True)
            picks = []
            for _ in range(2):
                top = reduce(jnp.max, m)
                first = reduce(jnp.min, jnp.where(m == top, idx, float(S - 1)))
                picks.append((jnp.max(first.astype(I32)), top))
                m = jnp.where(idx == first, -jnp.inf, m)
            return picks

        def experts():
            (i1, m1), (i2, m2) = top2()
            picks = [jnp.clip(i, 0, S - 1) for i in (i1, i2)]
            bases = [pl.multiple_of((i >> 4) * 16, 16) for i in picks]
            sub = jax.lax.broadcasted_iota(I32, (16, D), 0)
            first, second = (jnp.broadcast_to(xn_v[pl.ds(i, 1), :], (16, D)) for i in picks)
            sel = jnp.where(sub == 0, first, second).reshape(2, 8, D) * mod_v[4] + mod_v[3]
            sel = sel.reshape(16, D).astype(BF16)
            y = None
            acts = collections.deque()

            def down():
                nonlocal y
                f, g, u = acts.popleft()
                act = (g * jax.nn.sigmoid(g) * u).astype(BF16)
                part = _dot(act, wd_v[pl.ds(f, FC), :])
                y = part if y is None else y + part

            for f in range(0, FF, FC):
                acts.append((f, _dot(sel, wg_v[:, pl.ds(f, FC)]), _dot(sel, wu_v[:, pl.ds(f, FC)])))
                if len(acts) > flag:
                    down()
            while acts:
                down()
            y1, y2 = y[0:1] * jax.nn.sigmoid(m1), y[1:2] * jax.nn.sigmoid(m2)
            for n, base in enumerate(bases):
                upd = jnp.where(sub == picks[0] - base, y1, 0.0) + jnp.where(sub == picks[1] - base, y2, 0.0)
                full = out_v[pl.ds(base, 16), :].astype(F32).reshape(2, 8, D) + mod_v[5] * upd.reshape(2, 8, D)
                fix_v[n] = full.reshape(16, D).astype(BF16)
            return bases

        cc = c_v[...].astype(F32)
        act_v[...] = _pack(jnp.broadcast_to(cc * jax.nn.sigmoid(cc), (16, D)))
        with scope("w_x0"):
            x_copy(0).wait()
        for n in range(T // 32):
            row_stats(0, n)
        for offset in range(0, T, 16):
            for col in range(0, D, LW):
                xn_v[pl.ds(offset, 16), pl.ds(col, LW)] = normalized(0, offset, pl.ds(col, LW))
        for n in range(2):
            wait(("scale", n))
            modulation(D, D, n)
        mod_v[1] = raw(1) + 1.0
        units = HT // 16 * (HD // LW)
        saved = lambda offset, lanes: xn_v[pl.ds(offset, 16), lanes]
        for n in range(units):
            norm1_unit(saved, n, shift=False)(h0_v)

        def hold_values(col, part, v):
            xn_v[pl.ds(T + part * HT, HT), pl.ds(col, 128)] = v

        def shift_and_bias():
            wait("shift")
            modulation(0, D)
            mod_v[0] = raw(0)

        def release_values(col, part):
            v = xn_v[pl.ds(T + part * HT, HT), pl.ds(col, 128)]
            store_values(col, part, _apply(jnp.add, v, bias_v[:, pl.ds(col, 128)]))

        wait(*both("wv", 0))
        prep_values(0)
        plan = collections.defaultdict(list)
        plan[3] += [lambda: wait(*both("wv", 1)), lambda: prep_values(1)]
        plan[7] += [lambda: wait(*both("wv", 2))]
        plan[8] += [lambda: prep_values(2)]
        plan[15] += [lambda: prep_values(3)]
        plan[sa_at].append(shift_and_bias)
        with scope("values0"):
            values(h0_v, follow(plan), hold_values, 128)
            side.drain()
        assert not plan
        wait("wphi", "wk")
        block_diag_phi()
        for g in range(4):
            prep_scores(1, g)
        shift = jnp.concatenate([raw(0)] * 2, axis=0).astype(BF16)
        bias_v[...] = _dot(shift, wqkv_v[:, pl.ds(2 * D, D)])[:8]
        for n in range(units):
            norm1_unit(saved, n)(ht_v)

        plan = collections.defaultdict(list)
        def initialize():
            vt_v[:, pl.ds(64, 16), :] = jnp.ones((NPAIR, 16, T), BF16)

        plan[0].append(initialize)
        for n in range(16):
            plan[1 + n * 8 // 16].append(functools.partial(release_values, n // 2 * 128, n % 2))
        plan[q_at[0]] += [lambda: wait("wq", ("mod", 0)), lambda: x_copy(1).wait()]
        for g in range(4):
            plan[q_at[g]].append(functools.partial(prep_scores, 0, g))
        plan_norms(plan, 1 + (zero & 1), q_at[0], x1_at, 14 + 7 * HD // RC0 - l0, 14 + 7 * HD // RC0)
        plan_modulation(plan, zero & 1, x1_at + 1, 14 + 7 * HD // RC0 - l0 + 1)
        if marks:
            def mark(n):
                with jax.named_scope(f"mark{n}"):
                    fix_v[0, :, pl.ds(0, 128)] = jnp.zeros((16, 128), BF16)
            for n in marks:
                plan[n].append(functools.partial(mark, n))
        with scope("tile0"):
            first_pass(0, plan, 'kq', (256, RC0))

        def first_step(t, carry):
            @pl.when(t + 1 < NTILE)
            def _():
                x_copy(t + 1).wait()

            for n in range(1, NTILE):
                pl.when(t == n)(functools.partial(wait, ("mod", n)))

            @pl.when(t == 1)
            def _():
                start("wg", "wu", "wd")

            plan = collections.defaultdict(list)
            plan_norms(plan, jnp.clip(t + 1, 0, NTILE - 1), 0, lfirst, llast, 2 * nk + nv)
            per_step = pl.cdiv(HD // 16, NTILE - 1)
            for n in range(per_step):
                plan[pfirst + n * (plast - pfirst) // per_step].append(functools.partial(
                    lambda n: prep_output(jnp.clip((t - 1) * per_step + n, 0, HD // 16 - 1)), n))
            plan_modulation(plan, jnp.clip(t, 0, NTILE - 1), mfirst, mlast)
            first_pass(t, plan, order, (RC, RC))
            return carry

        wait("wo")
        if only in (0, 1):
            with scope("pass1"):
                jax.lax.fori_loop(1, NTILE, first_step, 0)
        if only == 1:
            for j in range(NPAIR):
                finish_kv(j)
            out_v[pl.ds(0, 64), pl.ds(0, 512)] = phiq_v[zero, zero, pl.ds(0, 64), :]
            out_v[pl.ds(64, 80), pl.ds(0, 128)] = _unpack(kvb_v[zero])
            out_v[pl.ds(160, 64), pl.ds(0, 512)] = _unpack(wot_v[zero, pl.ds(0, 32), :])
            out_copy(0).start()
            out_copy(0).wait()
            return

        wait("wr", "wg", "wu", "wd")
        for j in range(NPAIR):
            finish_kv(j)
        tasks = [task for i in range(4) for task in attend(0, 0, oa_v, i)]
        for task in tasks:
            task()
        output_weights()

        rows_of = None
        sent = []
        chain = Chain(ne)
        with scope("pass2"):
            for n in range(NSUB):
                source, target = ((oa_v, ob_v), (ob_v, oa_v))[n % 2]
                if n + 1 < NSUB:
                    tasks = [task for i in range(4) for task in attend((n + 1) // 2, (n + 1) % 2, target, i)]
                    for task in tasks:
                        task()
                for row in range(0, 2 * G, EC) if rows_of else ():
                    finish_rows((n - 1) * 2 * G + row, rows_of(row), chain)
                rows_of = mixed_rows(from_values(mix(source, lambda: None)), G)
                if n > 0:
                    out_copy(n - 1).start()
                    sent.append(n - 1)
                if n % every == phase % every and len(sent) > 1:
                    while len(sent) > 1:
                        out_copy(sent.pop(0)).wait()
                    chain = Chain(ne)
        with scope("last"):
            chain = Chain(nl)
            for row in range(0, 2 * G, EC):
                finish_rows(S - 2 * G + row, rows_of(row), chain)
        out_copy(NSUB - 1).start()
        sent.append(NSUB - 1)
        with scope("experts"):
            b1, b2 = experts()
        with scope("w_out"):
            for n in sent:
                out_copy(n).wait()
        fix = [pltpu.make_async_copy(fix_v.at[n], out_hbm.at[pl.ds(b, 16)], osems.at[n])
               for n, b in enumerate((b1, b2))]
        fix[0].start()

        @pl.when(b1 != b2)
        def _():
            fix[1].start()
            fix[1].wait()

        fix[0].wait()

    nsem = NTILE + 3 + 3 + NTILE + 1 + 7 + 4
    scratch = [
        pltpu.VMEM((S + 16, D), BF16), pltpu.VMEM((D, 3 * D), BF16), pltpu.VMEM((D, DH), BF16),
        pltpu.VMEM((D + 16, D), BF16), pltpu.VMEM((8, 128), BF16),
        pltpu.VMEM((D, FF), BF16), pltpu.VMEM((D, FF), BF16), pltpu.VMEM((FF, D), BF16),
        pltpu.VMEM((1, D), BF16), pltpu.VMEM((D, 6 * D), BF16),
        pltpu.VMEM((8, D), U32),
        pltpu.VMEM((8, 6 * D), F32),
        pltpu.VMEM((10, 8, D), F32),
        pltpu.VMEM((2, T, 128), F32),
        pltpu.VMEM((8, D), F32),
        pltpu.VMEM((D // 128, 64, 128), U32),
        pltpu.VMEM((7, HD // 2, HD), U32),
        pltpu.VMEM((7, HT // 2, HD), U32),
        pltpu.VMEM((7, HT // 2, HD), U32),
        pltpu.VMEM((NTILE, NPAIR, 128, T), BF16),
        pltpu.VMEM((NPAIR, 128, T), BF16),
        pltpu.VMEM((NPAIR, 80, T), BF16),
        pltpu.VMEM((NPAIR, 80, 128), F32),
        pltpu.VMEM((NPAIR, 40, 128), U32),
        pltpu.VMEM((7, G // 2, HD), U32),
        pltpu.VMEM((7, G // 2, HD), U32),
        pltpu.VMEM((S, D), F32),
        pltpu.VMEM((S, D), BF16),
        pltpu.VMEM((2, 16, D), BF16),
        pltpu.SemaphoreType.DMA((nsem,)),
        pltpu.SemaphoreType.DMA((NSUB,)),
    ] + [pltpu.VMEM((7, 64, HD), U32)] * 8 + [pltpu.VMEM((7, HD // 2, 128), U32)] * 4

    def fn(A_x, A_wqkv, A_w_phi, A_wo, B_x, B_w_r, B_w_gate, B_w_up, B_w_down, c, w_mod):
        del B_x
        out = pl.pallas_call(
            kernel,
            out_shape=jax.ShapeDtypeStruct((S, D), A_x.dtype),
            in_specs=[pl.BlockSpec(memory_space=pl.ANY)] * 10,
            out_specs=pl.BlockSpec(memory_space=pl.ANY),
            scratch_shapes=scratch,
            compiler_params=pltpu.CompilerParams(vmem_limit_bytes=vlimit * 2**20, flags=flags),
        )(A_x.reshape(S, D), A_wqkv, A_w_phi.reshape(D, DH), A_wo, B_w_r.reshape(8, 128),
          B_w_gate, B_w_up, B_w_down, c, w_mod)
        return out.reshape(A_x.shape)

    return fn


@jax.jit
def pallas_adaLN_cond__linear_kernel_hedgehog__moe_arch_mod__prompt_kernel(
    A_x, A_wqkv, A_w_phi, A_wo, B_x, B_w_r, B_w_gate, B_w_up, B_w_down, c, w_mod
):
    return make(RC0=256, l0=2, x1_at=13)(A_x, A_wqkv, A_w_phi, A_wo, B_x, B_w_r, B_w_gate, B_w_up, B_w_down, c, w_mod)
```

```python
import collections
import contextlib
import functools

import jax
import jax.numpy as jnp
import numpy as np
import jax.experimental.pallas as pl
import jax.experimental.pallas.tpu as pltpu

F32, BF16, I32, U32 = jnp.float32, jnp.bfloat16, jnp.int32, jnp.uint32
S, D, H, DH, FF = 2048, 1024, 32, 32, 3584
HD = D // 2
NPAIR = H // 2
EPS = 1e-5
LOG2E = float(np.log2(np.e))
NN = (((1,), (0,)), ((), ()))
NT = (((1,), (1,)), ((), ()))


def _dot(a, b, dn=NN):
    return jax.lax.dot_general(a, b, dn, preferred_element_type=F32)


def _pack(x):
    n = x.shape[0] // 2
    if x.shape[1] > 128:
        return pltpu.bitcast(x.astype(BF16), U32)
    w = pltpu.bitcast(jnp.concatenate([x[:n], x[n:]], axis=1).astype(BF16), U32)
    return jnp.concatenate([w[:, :128], w[:, 128:]], axis=0)


def _unpack(w):
    return pltpu.bitcast(w, BF16)


def _recip(x):
    r = pl.reciprocal(x, approx=True)
    return r * (2.0 - x * r)


def _lhs_terms(a11, a12, a21, a22):
    return (a11 + a22, a21 + a22, a11, a22, a11 + a12, a21 - a11, a12 - a22)


def _rhs_terms(b11, b12, b21, b22):
    return (b11 + b22, b11, b12 - b22, b21 - b11, b22, b11 + b12, b21 + b22)


_QUADRANTS = (((0, 1), (3, 1), (4, -1), (6, 1)), ((2, 1), (4, 1)), ((1, 1), (3, 1)),
              ((0, 1), (1, -1), (2, 1), (5, 1)))


def _quadrant(q, product):
    total = None
    for j, sign in _QUADRANTS[q]:
        m = product(j)
        total = m if total is None else (total + m if sign > 0 else total - m)
    return total


def _layernorm(x):
    d = x - jnp.mean(x, axis=-1, keepdims=True)
    v = jnp.mean(d * d, axis=-1, keepdims=True)
    return d * jax.lax.rsqrt(v + EPS)


def _per_head(op, p):
    parts = [p[r:r + 8] for r in range(0, p.shape[0], 8)]
    while len(parts) > 1:
        parts = [op(a, b) for a, b in zip(parts[::2], parts[1::2])]
    out = op(parts[0], pltpu.roll(parts[0], 4, 0))
    return op(out, pltpu.roll(out, 2, 0))


def _apply(op, p, stat):
    n = p.shape[0] // 8
    return op(p.reshape(n, 8, p.shape[1]), stat).reshape(p.shape)


def _features(p):
    e_pos = jnp.exp2(_apply(jnp.subtract, p, _per_head(jnp.maximum, p)))
    e_neg = jnp.exp2(_apply(lambda a, low: low - a, p, _per_head(jnp.minimum, p)))
    pos = _apply(jnp.multiply, e_pos, _recip(_per_head(jnp.add, e_pos)))
    neg = _apply(jnp.multiply, e_neg, _recip(_per_head(jnp.add, e_neg)))
    return jnp.concatenate([pos, neg], axis=0)


def _interleaved_source(row):
    return (row & ~63) + ((row & 1) << 5) + ((row & 63) >> 1)


class _Interleaver:
    def __init__(self, ratio):
        self.queue = collections.deque()
        self.ratio = ratio
        self.credit = 0.0

    def defer(self, cost, fn):
        self.queue.append((cost, fn))

    def spent(self, cycles):
        self.credit += cycles * self.ratio
        while self.queue and self.credit >= self.queue[0][0]:
            cost, fn = self.queue.popleft()
            self.credit -= cost
            fn()
        if not self.queue:
            self.credit = 0.0

    def drain(self):
        while self.queue:
            self.queue.popleft()[1]()
        self.credit = 0.0


def make(RC=256, VC=256, LW=512, FC=256, EC=32, ratio=0.55, vlimit=120, flags=None, S=S,
         prof=False, only=0, marks=(), vcost=256, kcost=150, mfirst=26, mlast=42, order='kqv',
         lfirst=29, llast=41, pfirst=1, plast=28, flag=2, RC0=128, sa_at=23, q_at=(10, 11, 12, 13), slots0=tuple((s + 7 * c, d) for c in range(4) for s, d in ((18, 1), (18, 3), (19, 2), (19, 4))), k_at=3,
         every=1, phase=1, ne=3, nl=32):
    scope = lambda n: jax.named_scope(n) if prof is True or (prof and n in prof) else contextlib.nullcontext()
    T = 512
    HT = T // 2
    NTILE = S // T
    G = 128
    NSUB = S // (2 * G)
    MW = 4 * D // NTILE
    nk, nv = 7 * HD // RC, 7 * HD // VC

    def kernel(x_hbm, wqkv_hbm, wphi_hbm, wo_hbm, wr_hbm, wg_hbm, wu_hbm, wd_hbm, c_hbm, wmod_hbm,
               out_hbm,
               x_v, wqkv_v, wphi_v, wo_v, wr_v, wg_v, wu_v, wd_v, c_v, wmod_v,
               act_v, raw_v, mod_v, stat_v, bias_v, bd_v, wot_v, ht_v, h0_v, phiq_v, phik_v, vt_v, kv_v, kvb_v, oa_v, ob_v,
               xn_v, out_v, fix_v, sems, osems, *terms_v):
        wq_v, wk_v, wv_v = terms_v[:4], terms_v[4:8], terms_v[8:]

        side = _Interleaver(ratio)
        copies = {}

        def add_copy(name, src, dst):
            copies[name] = pltpu.make_async_copy(src, dst, sems.at[NTILE + len(copies)])

        add_copy("c", c_hbm, c_v)
        add_copy("wphi", wphi_hbm, wphi_v)
        add_copy("wr", wr_hbm, wr_v)
        def add_columns(name, hbm, vmem, lo, n):
            add_copy(name, hbm.at[:, pl.ds(lo, n)], vmem.at[:, pl.ds(lo, n)])

        for n in range(2):
            piece = (pl.ds(n * HD, HD), pl.ds(D, D))
            add_copy(("scale", n), wmod_hbm.at[piece], wmod_v.at[piece])
        add_columns("shift", wmod_hbm, wmod_v, 0, D)
        for t in range(NTILE):
            add_columns(("mod", t), wmod_hbm, wmod_v, 2 * D + t * MW, MW)
        add_columns("wq", wqkv_hbm, wqkv_v, 0, D)
        for half in range(2):
            for n in range(2):
                add_columns(("wk", n, half), wqkv_hbm, wqkv_v, D + half * HD + n * 256, 256)
            for n, (lo, size) in enumerate(((0, 128), (128, 128), (256, 256))):
                add_columns(("wv", n, half), wqkv_hbm, wqkv_v, 2 * D + half * HD + lo, size)
        both = lambda *name: ((*name, 0), (*name, 1))
        add_copy("wo", wo_hbm, wo_v.at[pl.ds(0, D)])
        add_copy("wg", wg_hbm, wg_v)
        add_copy("wu", wu_hbm, wu_v)
        add_copy("wd", wd_hbm, wd_v)

        def start(*names):
            for n in names:
                copies[n].start()

        def wait(*names):
            with scope("w_" + "_".join(str(n) for n in names)[:20].replace("'", "").replace(" ", "")):
                for n in names:
                    copies[n].wait()

        def rows_at(base, size):
            return pl.ds(base if isinstance(base, int) else pl.multiple_of(base, 8), size)

        def x_copy(t):
            return pltpu.make_async_copy(x_hbm.at[rows_at(t * T, T)], x_v.at[rows_at(t * T, T)], sems.at[t])

        def out_copy(n):
            rows = pl.ds(n * 2 * G, 2 * G)
            return pltpu.make_async_copy(out_v.at[rows], out_hbm.at[rows], osems.at[n])

        def modulation(lo, n, half=None):
            rows = pl.ds(0, D) if half is None else pl.ds(half * HD, HD)
            lanes = pl.ds(lo if isinstance(lo, int) else pl.multiple_of(lo, 128), n)
            m = _dot(_unpack(act_v[:, rows]), wmod_v[rows, lanes])[:8]
            raw_v[:, lanes] = m if not half else raw_v[:, lanes] + m

        raw = lambda i: raw_v[:, pl.ds(i * D, D)]

        def block_diag_phi():
            row = _interleaved_source(jax.lax.broadcasted_iota(I32, (128, DH), 0))
            col = jax.lax.broadcasted_iota(I32, (128, DH), 1)
            sel = jnp.where((row & (DH - 1)) == col, 1.0, 0.0).astype(BF16)
            r2 = _interleaved_source(jax.lax.broadcasted_iota(I32, (128, 128), 0)) >> 5
            c2 = jax.lax.broadcasted_iota(I32, (128, 128), 1) >> 5
            for g in range(D // 128):
                tiled = _dot(sel, wphi_v[pl.ds(g * 128, 128), :], NT)
                bd_v[g] = _pack(jnp.where(r2 == c2, tiled, 0.0))

        def prep_scores(i, g):
            parts = []
            for gg in (g, g + HD // 128):
                for half in range(2):
                    w = wqkv_v[pl.ds(half * HD, HD), pl.ds(i * D + gg * 128, 128)]
                    parts.append(_dot(_unpack(bd_v[gg]), w, NT) * LOG2E)
            for j, term in enumerate(_lhs_terms(*parts)):
                (wq_v, wk_v)[i][g][j] = _pack(term)

        def prep_values(g):
            chain = Chain(1)
            for r in range(0, HD, 64):
                blocks = [wqkv_v[pl.ds(row + r, 64), pl.ds(2 * D + col + g * 128, 128)].astype(F32)
                          for col in (0, HD) for row in (0, HD)]
                blocks[3] = chain.enter(blocks[3])
                for j, term in enumerate(_lhs_terms(*blocks)):
                    words = _pack(term)
                    wv_v[g][j, pl.ds(r // 2, 32), :] = words
                chain.leave(words[:8])

        def prep_output(n):
            hold(wo_v)
            lo = wo_v[rows_at(n * 16, 16), :].astype(F32)
            hi = wo_v[rows_at(HD + n * 16, 16), :].astype(F32)
            for j, term in enumerate(_rhs_terms(lo[:, :HD], lo[:, HD:], hi[:, :HD], hi[:, HD:])):
                wot_v[j, rows_at(n * 8, 8), :] = _pack(term)

        start("c")
        x_copy(0).start()
        start(*both("scale"), *both("wv", 0), *both("wv", 1), *both("wv", 2), "shift", "wphi")
        start(*both("wk", 0), *both("wk", 1), "wq")
        x_copy(1).start()
        start("wo")
        for t in range(1, NTILE):
            start(("mod", t))
            if t + 1 < NTILE:
                x_copy(t + 1).start()
        start(("mod", 0))
        start("wr")
        wait("c")
        bits = pltpu.bitcast(jnp.broadcast_to(c_v[:, :128].astype(F32), (8, 128)), I32)
        zero = jnp.minimum(jnp.max(bits & 0xFF), 0)
        latest = {}

        class Chain:
            def __init__(self, strands):
                self.tokens = collections.deque([None] * strands)

            def enter(self, value):
                token = self.tokens.popleft()
                if token is None:
                    return value
                head = pltpu.bitcast(pltpu.bitcast(value[:8, :128], I32) | token, F32)
                if value.shape[1] > 128:
                    head = jnp.concatenate([head, value[:8, 128:]], axis=1)
                return jnp.concatenate([head, value[8:]], axis=0) if value.shape[0] > 8 else head

            def leave(self, *values):
                token = None
                for value in values:
                    value = pltpu.bitcast(value, I32)
                    token = value if token is None else token | value
                self.tokens.append(token & zero)

            def widen(self, strands):
                last = self.tokens[-1]
                while len(self.tokens) < strands:
                    self.tokens.append(last)

        clock = [0]
        due = collections.defaultdict(list)

        def finish_within(delay, *values):
            token = None
            for value in values:
                value = pltpu.bitcast(value, U32)
                for r in range(0, value.shape[0], 8):
                    for l in range(0, value.shape[1], 128):
                        part = value[r:r + 8, l:l + 128]
                        token = part if token is None else token | part
            due[clock[0] + delay].append(token & zero.astype(U32))

        def gated(ref, j):
            clock[0] += 1
            tokens = [token for when in sorted(due) if when < clock[0] for token in due.pop(when)]
            if tokens:
                corner = (j, pl.ds(0, 8), pl.ds(0, 128))
                ref[corner] = functools.reduce(jnp.bitwise_or, tokens, ref[corner])
            return ref[j]

        def hold(ref):
            spare = ref.shape[0] - 16
            back = jnp.clip(zero, 0, spare // 16) * 16
            ref[rows_at(spare - back, 16), pl.ds(0, 128)] = latest["m"].astype(BF16)

        def row_stats(t, n):
            xx = x_v[rows_at(t * T + n * 32, 32), :].astype(F32)
            mean = jnp.mean(xx, axis=-1, keepdims=True)
            d = xx - mean
            scale = jax.lax.rsqrt(jnp.mean(d * d, axis=-1, keepdims=True) + EPS)
            stat_v[0, rows_at(n * 32, 32), :] = jnp.broadcast_to(mean, (32, 128))
            stat_v[1, rows_at(n * 32, 32), :] = jnp.broadcast_to(scale, (32, 128))

        def normalized(t, offset, lanes):
            wide = lambda k: jnp.concatenate([stat_v[k, pl.ds(offset, 16), :]] * (LW // 128), axis=1)
            return (x_v[rows_at(t * T + offset, 16), lanes].astype(F32) - wide(0)) * wide(1)

        def norm1_unit(rows, n, shift=True, delay=0):
            group, part = divmod(n, HD // LW)
            blocks = []
            for col in (part * LW, HD + part * LW):
                for offset in (group * 16, HT + group * 16):
                    lanes = pl.ds(col, LW)
                    hh = rows(offset, lanes).reshape(2, 8, LW) * mod_v[1, :, lanes]
                    blocks.append((hh + mod_v[0, :, lanes] if shift else hh).reshape(16, LW))
            words = [_pack(term) for term in _rhs_terms(*blocks)]
            if delay:
                finish_within(delay, *words)

            def store(target):
                for j, w in enumerate(words):
                    target[j, pl.ds(group * 8, 8), pl.ds(part * LW, LW)] = w

            return store

        def strassen(product, tiles, cycles, extra):
            products = []
            for j in range(7):
                products.append([product(j, k) for k in range(tiles)])
                latest["m"] = products[j][-1][-16:]
                side.spent(cycles)
                extra()
            return products

        def scores(i, extra, consume, RC):
            cost = kcost * RC // 256
            tiles = HT // 128
            for r in range(0, HD, RC):
                products = strassen(
                    lambda j, k: _dot(
                        _unpack(jnp.concatenate(
                            [(wq_v, wk_v)[i][g][j] for g in range(r // 128, (r + RC) // 128)], axis=0)),
                        _unpack(gated(ht_v, j)[k * 64:(k + 1) * 64]), NT),
                    tiles, RC * HT // 128, extra)

                def unit(half, o, products=products, r=r):
                    for part in range(2):
                        phi = jnp.concatenate(
                            [_features(_quadrant(2 * half + part, lambda j: products[j][k][o:o + 64]))
                             for k in range(tiles)], axis=1)
                        consume((half * HD + r + o) // 64, pl.ds(part * HT, HT), phi.astype(BF16))

                for half in range(2):
                    for o in range(0, RC, 64):
                        side.defer(cost, functools.partial(unit, half, o))

        def key_features(pair, lanes, phi):
            phik_v[pair, :, lanes] = phi

        def query_features(t, pair, lanes, phi):
            phiq_v[t, pair, :, lanes] = phi

        def store_values(col, part, v):
            v = v.T.astype(BF16).reshape(2, 64, HT)
            vt_v[pl.ds(col // 64, 2), pl.ds(0, 64), pl.ds(part * HT, HT)] = v

        def values(source, extra, consume, VC):
            tiles = VC // 128
            for r in range(0, HD, VC):
                products = strassen(
                    lambda j, k: _dot(_unpack(source[j]), _unpack(wv_v[r // 128 + k][j])),
                    tiles, VC * HT // 128, extra)

                def unit(half, part, k, products=products, r=r):
                    consume(half * HD + r + k * 128, part, _quadrant(2 * half + part, lambda j: products[j][k]))

                for half in range(2):
                    for part in range(2):
                        for k in range(tiles):
                            side.defer(vcost // 2, functools.partial(unit, half, part, k))

        def accumulate_kv(j, first):
            kv = _dot(vt_v[j], phik_v[j], NT)
            kv_v[j] = kv if first else kv_v[j] + kv
            latest["m"] = kv[-16:]
            side.spent(T // 8)

        def finish_kv(j):
            row = jax.lax.broadcasted_iota(I32, (80, 128), 0)
            row_head = jnp.where(row < 64, row >> 5, (row >> 3) & 1)
            col_head = jax.lax.broadcasted_iota(I32, (80, 128), 1) & 1
            kvb_v[j] = _pack(jnp.where(row_head == col_head, kv_v[j], 0.0))

        def follow(plan):
            count = [0]

            def extra():
                count[0] += 1
                for task in plan.pop(count[0], ()):
                    task()

            for task in plan.pop(0, ()):
                task()
            return extra

        def first_pass(t, plan, order, rc):
            due.clear()
            extra = follow(plan)
            for part in order:
                if part == "k":
                    scores(1, extra, key_features, rc[0])
                elif part == "q":
                    scores(0, extra, functools.partial(query_features, t), rc[1])
                else:
                    values(ht_v, extra, store_values, VC)
            assert not plan
            if order[-1] == "v":
                side.drain()
            for r in range(0, HD, VC):
                for half in range(2):
                    for o in range(0, VC, 64):
                        accumulate_kv((half * HD + r + o) // 64, isinstance(t, int) and t == 0)
            side.drain()

        def plan_norms(plan, t, begin, first, last, end):
            plan[begin] += [functools.partial(row_stats, t, n) for n in range(T // 32)]
            units = HT // 16 * (HD // LW)
            stores = []

            def unit(n):
                hold(x_v)
                stores.append(norm1_unit(functools.partial(normalized, t), n))

            for n in range(units):
                plan[first + (last - first) * n // units].append(functools.partial(unit, n))
            plan[end].append(lambda: [store(ht_v) for store in stores])

        def plan_modulation(plan, t, first, last):
            steps = 2 * MW // 128
            for n in range(steps):
                plan[first + (last - first) * n // steps].append(
                    functools.partial(modulation, 2 * D + t * MW + n // 2 * 128, 128, n % 2))

        def attend(t, part, target, i):
            lanes = pl.ds(part * HT, HT)
            outs = {}
            tasks = []
            for half in range(2):
                for k in range(2):
                    p = half * (NPAIR // 2) + 2 * i + k
                    num = _dot(_unpack(kvb_v[p]), phiq_v[t, p, :, lanes])

                    def unit(num=num, key=(half, k)):
                        outs[key] = [_apply(jnp.multiply, num[h * DH:(h + 1) * DH],
                                            _recip(num[64 + 8 * h:72 + 8 * h] + 1e-6)) for h in range(2)]

                    tasks.append(unit)

            def terms_unit():
                lo, hi = (jnp.concatenate(outs[half, 0] + outs[half, 1], axis=0).T for half in range(2))
                for q, term in enumerate(_lhs_terms(lo[:G], hi[:G], lo[G:], hi[G:])):
                    target[q, :, pl.ds(i * 128, 128)] = _pack(term)

            return tasks + [terms_unit]

        def output_weights():
            w = wr_v[...].astype(F32)
            w = jnp.concatenate([jnp.broadcast_to(w[j:j + 1], (8, 128)) for j in range(D // 128)], axis=1)
            for i in range(2, 6):
                mod_v[i] = raw(i) + 1.0 if i == 4 else raw(i)
            mod_v[6] = mod_v[4] * w
            mod_v[7] = mod_v[4] * mod_v[5]
            mod_v[8] = mod_v[3] * mod_v[5]
            mod_v[9] = jnp.broadcast_to(jnp.sum(mod_v[3] * w, axis=1, keepdims=True), (8, D))

        ranks = {}

        def finish_rows(base, y, chain):
            lane = jax.lax.broadcasted_iota(I32, (8, 128), 1)
            acc = ranks.get(base >> 10, jnp.full((8, 128), -jnp.inf, F32))
            for o in range(0, y.shape[0], 8):
                rows = rows_at(base + o, 8)
                xn = x_v[rows, :].astype(F32) + mod_v[2] * chain.enter(y[o:o + 8])
                mean = jnp.mean(xn, axis=-1, keepdims=True)
                d = xn - mean
                scale = jax.lax.rsqrt(jnp.mean(d * d, axis=-1, keepdims=True) + EPS)
                score = jnp.sum(d * mod_v[6], axis=-1, keepdims=True) * scale + mod_v[9, :, :1]
                normed = d * scale
                xn_v[rows, :] = normed
                out = normed * mod_v[7] + ((d + mean) + mod_v[8])
                out_v[rows, :] = out.astype(BF16)
                acc = jnp.where(lane == ((base + o) & 1023) >> 3, score, acc)
                chain.leave(*[out[:, l:l + 128] for l in range(128, D, 256)])
            ranks[base >> 10] = acc

        tokens = collections.deque()

        def mix(source, extra):
            return strassen(
                lambda j, k: _dot(_unpack(source[j]), _unpack(wot_v[j, :, pl.ds(k * 128, 128)])),
                HD // 128, 4 * G, extra)

        def mixed_rows(product, n):
            def rows_of(o):
                part, o = divmod(o, n)
                return jnp.concatenate(
                    [_quadrant(2 * part + half, lambda j: product(j, o)) for half in range(2)], axis=1)
            return rows_of

        def from_values(products):
            return lambda j, o: jnp.concatenate([tile[o:o + EC] for tile in products[j]], axis=1)

        def top2():
            shape = (S // 1024, 8, 128)
            idx = (jax.lax.broadcasted_iota(I32, shape, 0) * 1024 + jax.lax.broadcasted_iota(I32, shape, 2) * 8
                   + jax.lax.broadcasted_iota(I32, shape, 1)).astype(F32)
            m = jnp.stack([ranks[b] for b in range(S // 1024)])
            reduce = lambda op, v: op(op(op(v, axis=0), axis=0, keepdims=True), axis=1, keepdims=True)
            picks = []
            for _ in range(2):
                top = reduce(jnp.max, m)
                first = reduce(jnp.min, jnp.where(m == top, idx, float(S - 1)))
                picks.append((jnp.max(first.astype(I32)), top))
                m = jnp.where(idx == first, -jnp.inf, m)
            return picks

        def experts():
            (i1, m1), (i2, m2) = top2()
            picks = [jnp.clip(i, 0, S - 1) for i in (i1, i2)]
            bases = [pl.multiple_of((i >> 4) * 16, 16) for i in picks]
            sub = jax.lax.broadcasted_iota(I32, (16, D), 0)
            first, second = (jnp.broadcast_to(xn_v[pl.ds(i, 1), :], (16, D)) for i in picks)
            sel = jnp.where(sub == 0, first, second).reshape(2, 8, D) * mod_v[4] + mod_v[3]
            sel = sel.reshape(16, D).astype(BF16)
            y = None
            acts = collections.deque()

            def down():
                nonlocal y
                f, g, u = acts.popleft()
                act = (g * jax.nn.sigmoid(g) * u).astype(BF16)
                part = _dot(act, wd_v[pl.ds(f, FC), :])
                y = part if y is None else y + part

            for f in range(0, FF, FC):
                acts.append((f, _dot(sel, wg_v[:, pl.ds(f, FC)]), _dot(sel, wu_v[:, pl.ds(f, FC)])))
                if len(acts) > flag:
                    down()
            while acts:
                down()
            y1, y2 = y[0:1] * jax.nn.sigmoid(m1), y[1:2] * jax.nn.sigmoid(m2)
            for n, base in enumerate(bases):
                upd = jnp.where(sub == picks[0] - base, y1, 0.0) + jnp.where(sub == picks[1] - base, y2, 0.0)
                full = out_v[pl.ds(base, 16), :].astype(F32).reshape(2, 8, D) + mod_v[5] * upd.reshape(2, 8, D)
                fix_v[n] = full.reshape(16, D).astype(BF16)
            return bases

        cc = c_v[...].astype(F32)
        act_v[...] = _pack(jnp.broadcast_to(cc * jax.nn.sigmoid(cc), (16, D)))
        with scope("w_x0"):
            x_copy(0).wait()
        for n in range(T // 32):
            row_stats(0, n)
        for offset in range(0, T, 16):
            for col in range(0, D, LW):
                xn_v[pl.ds(offset, 16), pl.ds(col, LW)] = normalized(0, offset, pl.ds(col, LW))
        for n in range(2):
            wait(("scale", n))
            modulation(D, D, n)
        mod_v[1] = raw(1) + 1.0
        units = HT // 16 * (HD // LW)
        saved = lambda offset, lanes: xn_v[pl.ds(offset, 16), lanes]
        for n in range(units):
            norm1_unit(saved, n, shift=False)(h0_v)

        def hold_values(col, part, v):
            xn_v[pl.ds(T + part * HT, HT), pl.ds(col, 128)] = v

        def shift_and_bias():
            wait("shift")
            modulation(0, D)
            mod_v[0] = raw(0)

        def release_values(col, part):
            v = xn_v[pl.ds(T + part * HT, HT), pl.ds(col, 128)]
            store_values(col, part, _apply(jnp.add, v, bias_v[:, pl.ds(col, 128)]))

        wait(*both("wv", 0))
        prep_values(0)
        plan = collections.defaultdict(list)
        plan[3] += [lambda: wait(*both("wv", 1)), lambda: prep_values(1)]
        plan[7] += [lambda: wait(*both("wv", 2))]
        plan[8] += [lambda: prep_values(2)]
        plan[15] += [lambda: prep_values(3)]
        plan[sa_at].append(shift_and_bias)
        with scope("values0"):
            values(h0_v, follow(plan), hold_values, 128)
            side.drain()
        assert not plan
        wait("wphi", *both("wk", 0))
        block_diag_phi()
        prep_scores(1, 0)
        prep_scores(1, 1)
        shift = jnp.concatenate([raw(0)] * 2, axis=0).astype(BF16)
        bias_v[...] = _dot(shift, wqkv_v[:, pl.ds(2 * D, D)])[:8]
        for n in range(units):
            norm1_unit(saved, n)(ht_v)

        plan = collections.defaultdict(list)
        def initialize():
            vt_v[:, pl.ds(64, 16), :] = jnp.ones((NPAIR, 16, T), BF16)

        plan[0].append(initialize)
        plan[k_at] += [lambda: wait(*both("wk", 1)), lambda: prep_scores(1, 2), lambda: prep_scores(1, 3)]
        for n in range(16):
            plan[1 + n * 8 // 16].append(functools.partial(release_values, n // 2 * 128, n % 2))
        plan[q_at[0]] += [lambda: wait("wq"), lambda: x_copy(1).wait()]
        for g in range(4):
            plan[q_at[g]].append(functools.partial(prep_scores, 0, g))
        stores = []

        def second_norm(n, delay):
            for block in (n // 2, T // 64 + n // 2) if n % 2 == 0 else ():
                row_stats(1, block)
            stores.append(norm1_unit(functools.partial(normalized, 1), n, delay=delay))

        for n, (slot, delay) in enumerate(slots0):
            plan[slot].append(functools.partial(second_norm, n, delay))
        plan[14 + 7 * HD // RC0].append(lambda: [store(ht_v) for store in stores])
        if marks:
            def mark(n):
                with jax.named_scope(f"mark{n}"):
                    fix_v[0, :, pl.ds(0, 128)] = jnp.zeros((16, 128), BF16)
            for n in marks:
                plan[n].append(functools.partial(mark, n))
        with scope("tile0"):
            first_pass(0, plan, 'kq', (256, RC0))

        def first_step(t, carry):
            @pl.when(t + 1 < NTILE)
            def _():
                x_copy(t + 1).wait()

            for n in range(1, NTILE):
                pl.when(t == n)(functools.partial(wait, ("mod", n)))

            @pl.when(t == 1)
            def _():
                start("wg", "wu", "wd")

            plan = collections.defaultdict(list)
            plan_norms(plan, jnp.clip(t + 1, 0, NTILE - 1), 0, lfirst, llast, 2 * nk + nv)
            per_step = pl.cdiv(HD // 16, NTILE - 1)
            for n in range(per_step):
                plan[pfirst + n * (plast - pfirst) // per_step].append(functools.partial(
                    lambda n: prep_output(jnp.clip((t - 1) * per_step + n, 0, HD // 16 - 1)), n))
            plan_modulation(plan, jnp.clip(t, 0, NTILE - 1), mfirst, mlast)
            first_pass(t, plan, order, (RC, RC))
            return carry

        wait("wo")
        if only in (0, 1):
            with scope("pass1"):
                jax.lax.fori_loop(1, NTILE, first_step, 0)
        if only == 1:
            for j in range(NPAIR):
                finish_kv(j)
            out_v[pl.ds(0, 64), pl.ds(0, 512)] = phiq_v[zero, zero, pl.ds(0, 64), :]
            out_v[pl.ds(64, 80), pl.ds(0, 128)] = _unpack(kvb_v[zero])
            out_v[pl.ds(160, 64), pl.ds(0, 512)] = _unpack(wot_v[zero, pl.ds(0, 32), :])
            out_copy(0).start()
            out_copy(0).wait()
            return

        wait(("mod", 0), "wr", "wg", "wu", "wd")
        modulation(2 * D, MW // 2)
        for j in range(NPAIR):
            finish_kv(j)
        tasks = [task for i in range(4) for task in attend(0, 0, oa_v, i)]
        modulation(2 * D + MW // 2, MW // 2)
        for task in tasks:
            task()
        output_weights()

        rows_of = None
        sent = []
        chain = Chain(ne)
        with scope("pass2"):
            for n in range(NSUB):
                source, target = ((oa_v, ob_v), (ob_v, oa_v))[n % 2]
                if n + 1 < NSUB:
                    tasks = [task for i in range(4) for task in attend((n + 1) // 2, (n + 1) % 2, target, i)]
                    for task in tasks:
                        task()
                for row in range(0, 2 * G, EC) if rows_of else ():
                    finish_rows((n - 1) * 2 * G + row, rows_of(row), chain)
                rows_of = mixed_rows(from_values(mix(source, lambda: None)), G)
                if n > 0:
                    out_copy(n - 1).start()
                    sent.append(n - 1)
                if n % every == phase % every and len(sent) > 1:
                    while len(sent) > 1:
                        out_copy(sent.pop(0)).wait()
                    chain = Chain(ne)
        with scope("last"):
            chain = Chain(nl)
            for row in range(0, 2 * G, EC):
                finish_rows(S - 2 * G + row, rows_of(row), chain)
        out_copy(NSUB - 1).start()
        sent.append(NSUB - 1)
        with scope("experts"):
            b1, b2 = experts()
        with scope("w_out"):
            for n in sent:
                out_copy(n).wait()
        fix = [pltpu.make_async_copy(fix_v.at[n], out_hbm.at[pl.ds(b, 16)], osems.at[n])
               for n, b in enumerate((b1, b2))]
        fix[0].start()

        @pl.when(b1 != b2)
        def _():
            fix[1].start()
            fix[1].wait()

        fix[0].wait()

    nsem = NTILE + 3 + 3 + NTILE + 1 + 10 + 4
    scratch = [
        pltpu.VMEM((S + 16, D), BF16), pltpu.VMEM((D, 3 * D), BF16), pltpu.VMEM((D, DH), BF16),
        pltpu.VMEM((D + 16, D), BF16), pltpu.VMEM((8, 128), BF16),
        pltpu.VMEM((D, FF), BF16), pltpu.VMEM((D, FF), BF16), pltpu.VMEM((FF, D), BF16),
        pltpu.VMEM((1, D), BF16), pltpu.VMEM((D, 6 * D), BF16),
        pltpu.VMEM((8, D), U32),
        pltpu.VMEM((8, 6 * D), F32),
        pltpu.VMEM((10, 8, D), F32),
        pltpu.VMEM((2, T, 128), F32),
        pltpu.VMEM((8, D), F32),
        pltpu.VMEM((D // 128, 64, 128), U32),
        pltpu.VMEM((7, HD // 2, HD), U32),
        pltpu.VMEM((7, HT // 2, HD), U32),
        pltpu.VMEM((7, HT // 2, HD), U32),
        pltpu.VMEM((NTILE, NPAIR, 128, T), BF16),
        pltpu.VMEM((NPAIR, 128, T), BF16),
        pltpu.VMEM((NPAIR, 80, T), BF16),
        pltpu.VMEM((NPAIR, 80, 128), F32),
        pltpu.VMEM((NPAIR, 40, 128), U32),
        pltpu.VMEM((7, G // 2, HD), U32),
        pltpu.VMEM((7, G // 2, HD), U32),
        pltpu.VMEM((S, D), F32),
        pltpu.VMEM((S, D), BF16),
        pltpu.VMEM((2, 16, D), BF16),
        pltpu.SemaphoreType.DMA((nsem,)),
        pltpu.SemaphoreType.DMA((NSUB,)),
    ] + [pltpu.VMEM((7, 64, HD), U32)] * 8 + [pltpu.VMEM((7, HD // 2, 128), U32)] * 4

    def fn(A_x, A_wqkv, A_w_phi, A_wo, B_x, B_w_r, B_w_gate, B_w_up, B_w_down, c, w_mod):
        del B_x
        out = pl.pallas_call(
            kernel,
            out_shape=jax.ShapeDtypeStruct((S, D), A_x.dtype),
            in_specs=[pl.BlockSpec(memory_space=pl.ANY)] * 10,
            out_specs=pl.BlockSpec(memory_space=pl.ANY),
            scratch_shapes=scratch,
            compiler_params=pltpu.CompilerParams(vmem_limit_bytes=vlimit * 2**20, flags=flags),
        )(A_x.reshape(S, D), A_wqkv, A_w_phi.reshape(D, DH), A_wo, B_w_r.reshape(8, 128),
          B_w_gate, B_w_up, B_w_down, c, w_mod)
        return out.reshape(A_x.shape)

    return fn


@jax.jit
def pallas_adaLN_cond__linear_kernel_hedgehog__moe_arch_mod__prompt_kernel(
    A_x, A_wqkv, A_w_phi, A_wo, B_x, B_w_r, B_w_gate, B_w_up, B_w_down, c, w_mod
):
    return make(k_at=5)(A_x, A_wqkv, A_w_phi, A_wo, B_x, B_w_r, B_w_gate, B_w_up, B_w_down, c, w_mod)
```

```python
import collections
import contextlib
import functools

import jax
import jax.numpy as jnp
import numpy as np
import jax.experimental.pallas as pl
import jax.experimental.pallas.tpu as pltpu

F32, BF16, I32, U32 = jnp.float32, jnp.bfloat16, jnp.int32, jnp.uint32
S, D, H, DH, FF = 2048, 1024, 32, 32, 3584
HD = D // 2
NPAIR = H // 2
EPS = 1e-5
LOG2E = float(np.log2(np.e))
NN = (((1,), (0,)), ((), ()))
NT = (((1,), (1,)), ((), ()))


def _dot(a, b, dn=NN):
    return jax.lax.dot_general(a, b, dn, preferred_element_type=F32)


def _pack(x):
    n = x.shape[0] // 2
    if x.shape[1] > 128:
        return pltpu.bitcast(x.astype(BF16), U32)
    w = pltpu.bitcast(jnp.concatenate([x[:n], x[n:]], axis=1).astype(BF16), U32)
    return jnp.concatenate([w[:, :128], w[:, 128:]], axis=0)


def _unpack(w):
    return pltpu.bitcast(w, BF16)


def _recip(x):
    r = pl.reciprocal(x, approx=True)
    return r * (2.0 - x * r)


def _lhs_terms(a11, a12, a21, a22):
    return (a11 + a22, a21 + a22, a11, a22, a11 + a12, a21 - a11, a12 - a22)


def _rhs_terms(b11, b12, b21, b22):
    return (b11 + b22, b11, b12 - b22, b21 - b11, b22, b11 + b12, b21 + b22)


_QUADRANTS = (((0, 1), (3, 1), (4, -1), (6, 1)), ((2, 1), (4, 1)), ((1, 1), (3, 1)),
              ((0, 1), (1, -1), (2, 1), (5, 1)))


def _quadrant(q, product):
    total = None
    for j, sign in _QUADRANTS[q]:
        m = product(j)
        total = m if total is None else (total + m if sign > 0 else total - m)
    return total


def _layernorm(x):
    d = x - jnp.mean(x, axis=-1, keepdims=True)
    v = jnp.mean(d * d, axis=-1, keepdims=True)
    return d * jax.lax.rsqrt(v + EPS)


def _per_head(op, p):
    parts = [p[r:r + 8] for r in range(0, p.shape[0], 8)]
    while len(parts) > 1:
        parts = [op(a, b) for a, b in zip(parts[::2], parts[1::2])]
    out = op(parts[0], pltpu.roll(parts[0], 4, 0))
    return op(out, pltpu.roll(out, 2, 0))


def _apply(op, p, stat):
    n = p.shape[0] // 8
    return op(p.reshape(n, 8, p.shape[1]), stat).reshape(p.shape)


def _features(p):
    e_pos = jnp.exp2(_apply(jnp.subtract, p, _per_head(jnp.maximum, p)))
    e_neg = jnp.exp2(_apply(lambda a, low: low - a, p, _per_head(jnp.minimum, p)))
    pos = _apply(jnp.multiply, e_pos, _recip(_per_head(jnp.add, e_pos)))
    neg = _apply(jnp.multiply, e_neg, _recip(_per_head(jnp.add, e_neg)))
    return jnp.concatenate([pos, neg], axis=0)


def _interleaved_source(row):
    return (row & ~63) + ((row & 1) << 5) + ((row & 63) >> 1)


class _Interleaver:
    def __init__(self, ratio):
        self.queue = collections.deque()
        self.ratio = ratio
        self.credit = 0.0

    def defer(self, cost, fn):
        self.queue.append((cost, fn))

    def spent(self, cycles):
        self.credit += cycles * self.ratio
        while self.queue and self.credit >= self.queue[0][0]:
            cost, fn = self.queue.popleft()
            self.credit -= cost
            fn()
        if not self.queue:
            self.credit = 0.0

    def drain(self):
        while self.queue:
            self.queue.popleft()[1]()
        self.credit = 0.0


def make(RC=256, VC=256, LW=512, FC=256, EC=32, ratio=0.55, vlimit=120, flags=None, S=S,
         prof=False, only=0, marks=(), vcost=256, kcost=150, mfirst=26, mlast=42, order='kqv',
         lfirst=29, llast=41, pfirst=1, plast=28, flag=2, RC0=128, sa_at=23, q_at=(10, 11, 12, 13), slots0=tuple((s + 7 * c, d) for c in range(4) for s, d in ((18, 1), (18, 3), (19, 2), (19, 4))), k_at=5,
         ne=3, nl=32, edelay=40, barriers=(), tail=32, ne_tail=5):
    scope = lambda n: jax.named_scope(n) if prof is True or (prof and n in prof) else contextlib.nullcontext()
    T = 512
    HT = T // 2
    NTILE = S // T
    G = 128
    NSUB = S // (2 * G)
    MW = 4 * D // NTILE
    nk, nv = 7 * HD // RC, 7 * HD // VC

    def kernel(x_hbm, wqkv_hbm, wphi_hbm, wo_hbm, wr_hbm, wg_hbm, wu_hbm, wd_hbm, c_hbm, wmod_hbm,
               out_hbm,
               x_v, wqkv_v, wphi_v, wo_v, wr_v, wg_v, wu_v, wd_v, c_v, wmod_v,
               act_v, raw_v, mod_v, stat_v, bias_v, bd_v, wot_v, ht_v, h0_v, phiq_v, phik_v, vt_v, kv_v, kvb_v, oa_v, ob_v,
               xn_v, out_v, fix_v, sems, osems, *terms_v):
        wq_v, wk_v, wv_v = terms_v[:4], terms_v[4:8], terms_v[8:]

        side = _Interleaver(ratio)
        copies = {}

        def add_copy(name, src, dst):
            copies[name] = pltpu.make_async_copy(src, dst, sems.at[NTILE + len(copies)])

        add_copy("c", c_hbm, c_v)
        add_copy("wphi", wphi_hbm, wphi_v)
        add_copy("wr", wr_hbm, wr_v)
        def add_columns(name, hbm, vmem, lo, n):
            add_copy(name, hbm.at[:, pl.ds(lo, n)], vmem.at[:, pl.ds(lo, n)])

        for n in range(2):
            piece = (pl.ds(n * HD, HD), pl.ds(D, D))
            add_copy(("scale", n), wmod_hbm.at[piece], wmod_v.at[piece])
        add_columns("shift", wmod_hbm, wmod_v, 0, D)
        for t in range(NTILE):
            add_columns(("mod", t), wmod_hbm, wmod_v, 2 * D + t * MW, MW)
        add_columns("wq", wqkv_hbm, wqkv_v, 0, D)
        for half in range(2):
            for n in range(2):
                add_columns(("wk", n, half), wqkv_hbm, wqkv_v, D + half * HD + n * 256, 256)
            for n, (lo, size) in enumerate(((0, 128), (128, 128), (256, 256))):
                add_columns(("wv", n, half), wqkv_hbm, wqkv_v, 2 * D + half * HD + lo, size)
        both = lambda *name: ((*name, 0), (*name, 1))
        add_copy("wo", wo_hbm, wo_v.at[pl.ds(0, D)])
        add_copy("wg", wg_hbm, wg_v)
        add_copy("wu", wu_hbm, wu_v)
        add_copy("wd", wd_hbm, wd_v)

        def start(*names):
            for n in names:
                copies[n].start()

        def wait(*names):
            with scope("w_" + "_".join(str(n) for n in names)[:20].replace("'", "").replace(" ", "")):
                for n in names:
                    copies[n].wait()

        def rows_at(base, size):
            return pl.ds(base if isinstance(base, int) else pl.multiple_of(base, 8), size)

        def x_copy(t):
            return pltpu.make_async_copy(x_hbm.at[rows_at(t * T, T)], x_v.at[rows_at(t * T, T)], sems.at[t])

        def out_copy(n):
            rows = pl.ds(n * 2 * G, 2 * G)
            return pltpu.make_async_copy(out_v.at[rows], out_hbm.at[rows], osems.at[n])

        def modulation(lo, n, half=None):
            rows = pl.ds(0, D) if half is None else pl.ds(half * HD, HD)
            lanes = pl.ds(lo if isinstance(lo, int) else pl.multiple_of(lo, 128), n)
            m = _dot(_unpack(act_v[:, rows]), wmod_v[rows, lanes])[:8]
            raw_v[:, lanes] = m if not half else raw_v[:, lanes] + m

        raw = lambda i: raw_v[:, pl.ds(i * D, D)]

        def block_diag_phi():
            row = _interleaved_source(jax.lax.broadcasted_iota(I32, (128, DH), 0))
            col = jax.lax.broadcasted_iota(I32, (128, DH), 1)
            sel = jnp.where((row & (DH - 1)) == col, 1.0, 0.0).astype(BF16)
            r2 = _interleaved_source(jax.lax.broadcasted_iota(I32, (128, 128), 0)) >> 5
            c2 = jax.lax.broadcasted_iota(I32, (128, 128), 1) >> 5
            for g in range(D // 128):
                tiled = _dot(sel, wphi_v[pl.ds(g * 128, 128), :], NT)
                bd_v[g] = _pack(jnp.where(r2 == c2, tiled, 0.0))

        def prep_scores(i, g):
            parts = []
            for gg in (g, g + HD // 128):
                for half in range(2):
                    w = wqkv_v[pl.ds(half * HD, HD), pl.ds(i * D + gg * 128, 128)]
                    parts.append(_dot(_unpack(bd_v[gg]), w, NT) * LOG2E)
            for j, term in enumerate(_lhs_terms(*parts)):
                (wq_v, wk_v)[i][g][j] = _pack(term)

        def prep_values(g):
            chain = Chain(1)
            for r in range(0, HD, 64):
                blocks = [wqkv_v[pl.ds(row + r, 64), pl.ds(2 * D + col + g * 128, 128)].astype(F32)
                          for col in (0, HD) for row in (0, HD)]
                blocks[3] = chain.enter(blocks[3])
                for j, term in enumerate(_lhs_terms(*blocks)):
                    words = _pack(term)
                    wv_v[g][j, pl.ds(r // 2, 32), :] = words
                chain.leave(words[:8])

        def prep_output(n):
            hold(wo_v)
            lo = wo_v[rows_at(n * 16, 16), :].astype(F32)
            hi = wo_v[rows_at(HD + n * 16, 16), :].astype(F32)
            for j, term in enumerate(_rhs_terms(lo[:, :HD], lo[:, HD:], hi[:, :HD], hi[:, HD:])):
                wot_v[j, rows_at(n * 8, 8), :] = _pack(term)

        start("c")
        x_copy(0).start()
        start(*both("scale"), *both("wv", 0), *both("wv", 1), *both("wv", 2), "shift", "wphi")
        start(*both("wk", 0), *both("wk", 1), "wq")
        x_copy(1).start()
        start("wo")
        for t in range(1, NTILE):
            start(("mod", t))
            if t + 1 < NTILE:
                x_copy(t + 1).start()
        start(("mod", 0))
        start("wr")
        wait("c")
        bits = pltpu.bitcast(jnp.broadcast_to(c_v[:, :128].astype(F32), (8, 128)), I32)
        zero = jnp.minimum(jnp.max(bits & 0xFF), 0)
        latest = {}

        class Chain:
            def __init__(self, strands):
                self.tokens = collections.deque([None] * strands)

            def enter(self, value):
                token = self.tokens.popleft()
                if token is None:
                    return value
                head = pltpu.bitcast(pltpu.bitcast(value[:8, :128], I32) | token, F32)
                if value.shape[1] > 128:
                    head = jnp.concatenate([head, value[:8, 128:]], axis=1)
                return jnp.concatenate([head, value[8:]], axis=0) if value.shape[0] > 8 else head

            def leave(self, *values):
                token = None
                for value in values:
                    value = pltpu.bitcast(value, I32)
                    token = value if token is None else token | value
                self.tokens.append(token & zero)

            def widen(self, strands):
                last = self.tokens[-1]
                while len(self.tokens) < strands:
                    self.tokens.append(last)

        clock = [0]
        due = collections.defaultdict(list)

        def finish_within(delay, *values):
            token = None
            for value in values:
                value = pltpu.bitcast(value, U32)
                for r in range(0, value.shape[0], 8):
                    for l in range(0, value.shape[1], 128):
                        part = value[r:r + 8, l:l + 128]
                        token = part if token is None else token | part
            due[clock[0] + delay].append(token & zero.astype(U32))

        def gated(ref, j, row=0):
            clock[0] += 1
            tokens = [token for when in sorted(due) if when < clock[0] for token in due.pop(when)]
            if tokens:
                corner = (j, pl.ds(row, 8), pl.ds(0, 128))
                ref[corner] = functools.reduce(jnp.bitwise_or, tokens, ref[corner])
            return ref[j]

        def hold(ref):
            spare = ref.shape[0] - 16
            back = jnp.clip(zero, 0, spare // 16) * 16
            ref[rows_at(spare - back, 16), pl.ds(0, 128)] = latest["m"].astype(BF16)

        def row_stats(t, n):
            xx = x_v[rows_at(t * T + n * 32, 32), :].astype(F32)
            mean = jnp.mean(xx, axis=-1, keepdims=True)
            d = xx - mean
            scale = jax.lax.rsqrt(jnp.mean(d * d, axis=-1, keepdims=True) + EPS)
            stat_v[0, rows_at(n * 32, 32), :] = jnp.broadcast_to(mean, (32, 128))
            stat_v[1, rows_at(n * 32, 32), :] = jnp.broadcast_to(scale, (32, 128))

        def normalized(t, offset, lanes):
            wide = lambda k: jnp.concatenate([stat_v[k, pl.ds(offset, 16), :]] * (LW // 128), axis=1)
            return (x_v[rows_at(t * T + offset, 16), lanes].astype(F32) - wide(0)) * wide(1)

        def norm1_unit(rows, n, shift=True, delay=0):
            group, part = divmod(n, HD // LW)
            blocks = []
            for col in (part * LW, HD + part * LW):
                for offset in (group * 16, HT + group * 16):
                    lanes = pl.ds(col, LW)
                    hh = rows(offset, lanes).reshape(2, 8, LW) * mod_v[1, :, lanes]
                    blocks.append((hh + mod_v[0, :, lanes] if shift else hh).reshape(16, LW))
            words = [_pack(term) for term in _rhs_terms(*blocks)]
            if delay:
                finish_within(delay, *words)

            def store(target):
                for j, w in enumerate(words):
                    target[j, pl.ds(group * 8, 8), pl.ds(part * LW, LW)] = w

            return store

        def strassen(product, tiles, cycles, extra):
            products = []
            for j in range(7):
                products.append([product(j, k) for k in range(tiles)])
                latest["m"] = products[j][-1][-16:]
                side.spent(cycles)
                extra()
            return products

        def scores(i, extra, consume, RC):
            cost = kcost * RC // 256
            tiles = HT // 128
            for r in range(0, HD, RC):
                products = strassen(
                    lambda j, k: _dot(
                        _unpack(jnp.concatenate(
                            [(wq_v, wk_v)[i][g][j] for g in range(r // 128, (r + RC) // 128)], axis=0)),
                        _unpack(gated(ht_v, j, k * 64)[k * 64:(k + 1) * 64]), NT),
                    tiles, RC * HT // 128, extra)

                def unit(half, o, products=products, r=r):
                    for part in range(2):
                        phi = jnp.concatenate(
                            [_features(_quadrant(2 * half + part, lambda j: products[j][k][o:o + 64]))
                             for k in range(tiles)], axis=1)
                        consume((half * HD + r + o) // 64, pl.ds(part * HT, HT), phi.astype(BF16))

                for half in range(2):
                    for o in range(0, RC, 64):
                        side.defer(cost, functools.partial(unit, half, o))

        def key_features(pair, lanes, phi):
            phik_v[pair, :, lanes] = phi

        def query_features(t, pair, lanes, phi):
            phiq_v[t, pair, :, lanes] = phi

        def store_values(col, part, v):
            v = v.T.astype(BF16).reshape(2, 64, HT)
            vt_v[pl.ds(col // 64, 2), pl.ds(0, 64), pl.ds(part * HT, HT)] = v

        def values(source, extra, consume, VC):
            tiles = VC // 128
            for r in range(0, HD, VC):
                products = strassen(
                    lambda j, k: _dot(_unpack(source[j]), _unpack(wv_v[r // 128 + k][j])),
                    tiles, VC * HT // 128, extra)

                def unit(half, part, k, products=products, r=r):
                    consume(half * HD + r + k * 128, part, _quadrant(2 * half + part, lambda j: products[j][k]))

                for half in range(2):
                    for part in range(2):
                        for k in range(tiles):
                            side.defer(vcost // 2, functools.partial(unit, half, part, k))

        def accumulate_kv(j, first):
            kv = _dot(vt_v[j], phik_v[j], NT)
            kv_v[j] = kv if first else kv_v[j] + kv
            latest["m"] = kv[-16:]
            side.spent(T // 8)

        def finish_kv(j):
            row = jax.lax.broadcasted_iota(I32, (80, 128), 0)
            row_head = jnp.where(row < 64, row >> 5, (row >> 3) & 1)
            col_head = jax.lax.broadcasted_iota(I32, (80, 128), 1) & 1
            kvb_v[j] = _pack(jnp.where(row_head == col_head, kv_v[j], 0.0))

        def follow(plan):
            count = [0]

            def extra():
                count[0] += 1
                for task in plan.pop(count[0], ()):
                    task()

            for task in plan.pop(0, ()):
                task()
            return extra

        def first_pass(t, plan, order, rc):
            due.clear()
            extra = follow(plan)
            for part in order:
                if part == "k":
                    scores(1, extra, key_features, rc[0])
                elif part == "q":
                    scores(0, extra, functools.partial(query_features, t), rc[1])
                else:
                    values(ht_v, extra, store_values, VC)
            assert not plan
            if order[-1] == "v":
                side.drain()
            for r in range(0, HD, VC):
                for half in range(2):
                    for o in range(0, VC, 64):
                        accumulate_kv((half * HD + r + o) // 64, isinstance(t, int) and t == 0)
            side.drain()

        def plan_norms(plan, t, begin, first, last, end):
            plan[begin] += [functools.partial(row_stats, t, n) for n in range(T // 32)]
            units = HT // 16 * (HD // LW)
            stores = []

            def unit(n):
                hold(x_v)
                stores.append(norm1_unit(functools.partial(normalized, t), n))

            for n in range(units):
                plan[first + (last - first) * n // units].append(functools.partial(unit, n))
            plan[end].append(lambda: [store(ht_v) for store in stores])

        def plan_modulation(plan, t, first, last):
            steps = 2 * MW // 128
            for n in range(steps):
                plan[first + (last - first) * n // steps].append(
                    functools.partial(modulation, 2 * D + t * MW + n // 2 * 128, 128, n % 2))

        def attend(t, part, target, i):
            lanes = pl.ds(part * HT, HT)
            outs = {}
            tasks = []
            for half in range(2):
                for k in range(2):
                    p = half * (NPAIR // 2) + 2 * i + k
                    num = _dot(_unpack(kvb_v[p]), phiq_v[t, p, :, lanes])

                    def unit(num=num, key=(half, k)):
                        outs[key] = [_apply(jnp.multiply, num[h * DH:(h + 1) * DH],
                                            _recip(num[64 + 8 * h:72 + 8 * h] + 1e-6)) for h in range(2)]

                    tasks.append(unit)

            def terms_unit():
                lo, hi = (jnp.concatenate(outs[half, 0] + outs[half, 1], axis=0).T for half in range(2))
                for q, term in enumerate(_lhs_terms(lo[:G], hi[:G], lo[G:], hi[G:])):
                    target[q, :, pl.ds(i * 128, 128)] = _pack(term)

            return tasks + [terms_unit]

        def output_weights():
            w = wr_v[...].astype(F32)
            w = jnp.concatenate([jnp.broadcast_to(w[j:j + 1], (8, 128)) for j in range(D // 128)], axis=1)
            for i in range(2, 6):
                mod_v[i] = raw(i) + 1.0 if i == 4 else raw(i)
            mod_v[6] = mod_v[4] * w
            mod_v[7] = mod_v[4] * mod_v[5]
            mod_v[8] = mod_v[3] * mod_v[5]
            mod_v[9] = jnp.broadcast_to(jnp.sum(mod_v[3] * w, axis=1, keepdims=True), (8, D))

        ranks = {}

        def finish_rows(base, y, chain):
            lane = jax.lax.broadcasted_iota(I32, (8, 128), 1)
            acc = ranks.get(base >> 10, jnp.full((8, 128), -jnp.inf, F32))
            for o in range(0, y.shape[0], 8):
                rows = rows_at(base + o, 8)
                xn = x_v[rows, :].astype(F32) + mod_v[2] * chain.enter(y[o:o + 8])
                mean = jnp.mean(xn, axis=-1, keepdims=True)
                d = xn - mean
                scale = jax.lax.rsqrt(jnp.mean(d * d, axis=-1, keepdims=True) + EPS)
                score = jnp.sum(d * mod_v[6], axis=-1, keepdims=True) * scale + mod_v[9, :, :1]
                normed = d * scale
                xn_v[rows, :] = normed
                out = normed * mod_v[7] + ((d + mean) + mod_v[8])
                out_v[rows, :] = out.astype(BF16)
                acc = jnp.where(lane == ((base + o) & 1023) >> 3, score, acc)
                chain.leave(*[out[:, l:l + 128] for l in range(128, D, 256)])
            ranks[base >> 10] = acc

        tokens = collections.deque()

        def mix(source, lo=0, n=G):
            return strassen(
                lambda j, k: _dot(_unpack(gated(source, j, lo // 2)[lo // 2:(lo + n) // 2]),
                                  _unpack(wot_v[j, :, pl.ds(k * 128, 128)])),
                HD // 128, 4 * n, lambda: None)

        def mixed_rows(product, n):
            def rows_of(o):
                part, o = divmod(o, n)
                return jnp.concatenate(
                    [_quadrant(2 * part + half, lambda j: product(j, o)) for half in range(2)], axis=1)
            return rows_of

        def from_values(products):
            return lambda j, o: jnp.concatenate([tile[o:o + EC] for tile in products[j]], axis=1)

        def top2():
            shape = (S // 1024, 8, 128)
            idx = (jax.lax.broadcasted_iota(I32, shape, 0) * 1024 + jax.lax.broadcasted_iota(I32, shape, 2) * 8
                   + jax.lax.broadcasted_iota(I32, shape, 1)).astype(F32)
            m = jnp.stack([ranks[b] for b in range(S // 1024)])
            reduce = lambda op, v: op(op(op(v, axis=0), axis=0, keepdims=True), axis=1, keepdims=True)
            picks = []
            for _ in range(2):
                top = reduce(jnp.max, m)
                first = reduce(jnp.min, jnp.where(m == top, idx, float(S - 1)))
                picks.append((jnp.max(first.astype(I32)), top))
                m = jnp.where(idx == first, -jnp.inf, m)
            return picks

        def experts():
            (i1, m1), (i2, m2) = top2()
            picks = [jnp.clip(i, 0, S - 1) for i in (i1, i2)]
            bases = [pl.multiple_of((i >> 4) * 16, 16) for i in picks]
            sub = jax.lax.broadcasted_iota(I32, (16, D), 0)
            first, second = (jnp.broadcast_to(xn_v[pl.ds(i, 1), :], (16, D)) for i in picks)
            sel = jnp.where(sub == 0, first, second).reshape(2, 8, D) * mod_v[4] + mod_v[3]
            sel = sel.reshape(16, D).astype(BF16)
            y = None
            acts = collections.deque()

            def down():
                nonlocal y
                f, g, u = acts.popleft()
                act = (g * jax.nn.sigmoid(g) * u).astype(BF16)
                part = _dot(act, wd_v[pl.ds(f, FC), :])
                y = part if y is None else y + part

            for f in range(0, FF, FC):
                acts.append((f, _dot(sel, wg_v[:, pl.ds(f, FC)]), _dot(sel, wu_v[:, pl.ds(f, FC)])))
                if len(acts) > flag:
                    down()
            while acts:
                down()
            y1, y2 = y[0:1] * jax.nn.sigmoid(m1), y[1:2] * jax.nn.sigmoid(m2)
            for n, base in enumerate(bases):
                upd = jnp.where(sub == picks[0] - base, y1, 0.0) + jnp.where(sub == picks[1] - base, y2, 0.0)
                full = out_v[pl.ds(base, 16), :].astype(F32).reshape(2, 8, D) + mod_v[5] * upd.reshape(2, 8, D)
                fix_v[n] = full.reshape(16, D).astype(BF16)
            return bases

        cc = c_v[...].astype(F32)
        act_v[...] = _pack(jnp.broadcast_to(cc * jax.nn.sigmoid(cc), (16, D)))
        with scope("w_x0"):
            x_copy(0).wait()
        for n in range(T // 32):
            row_stats(0, n)
        for offset in range(0, T, 16):
            for col in range(0, D, LW):
                xn_v[pl.ds(offset, 16), pl.ds(col, LW)] = normalized(0, offset, pl.ds(col, LW))
        for n in range(2):
            wait(("scale", n))
            modulation(D, D, n)
        mod_v[1] = raw(1) + 1.0
        units = HT // 16 * (HD // LW)
        saved = lambda offset, lanes: xn_v[pl.ds(offset, 16), lanes]
        for n in range(units):
            norm1_unit(saved, n, shift=False)(h0_v)

        def hold_values(col, part, v):
            xn_v[pl.ds(T + part * HT, HT), pl.ds(col, 128)] = v

        def shift_and_bias():
            wait("shift")
            modulation(0, D)
            mod_v[0] = raw(0)

        def release_values(col, part):
            v = xn_v[pl.ds(T + part * HT, HT), pl.ds(col, 128)]
            store_values(col, part, _apply(jnp.add, v, bias_v[:, pl.ds(col, 128)]))

        wait(*both("wv", 0))
        prep_values(0)
        plan = collections.defaultdict(list)
        plan[3] += [lambda: wait(*both("wv", 1)), lambda: prep_values(1)]
        plan[7] += [lambda: wait(*both("wv", 2))]
        plan[8] += [lambda: prep_values(2)]
        plan[15] += [lambda: prep_values(3)]
        plan[sa_at].append(shift_and_bias)
        with scope("values0"):
            values(h0_v, follow(plan), hold_values, 128)
            side.drain()
        assert not plan
        wait("wphi", *both("wk", 0))
        block_diag_phi()
        prep_scores(1, 0)
        prep_scores(1, 1)
        shift = jnp.concatenate([raw(0)] * 2, axis=0).astype(BF16)
        bias_v[...] = _dot(shift, wqkv_v[:, pl.ds(2 * D, D)])[:8]
        for n in range(units):
            norm1_unit(saved, n)(ht_v)

        plan = collections.defaultdict(list)
        def initialize():
            vt_v[:, pl.ds(64, 16), :] = jnp.ones((NPAIR, 16, T), BF16)

        plan[0].append(initialize)
        plan[k_at] += [lambda: wait(*both("wk", 1)), lambda: prep_scores(1, 2), lambda: prep_scores(1, 3)]
        for n in range(16):
            plan[1 + n * 8 // 16].append(functools.partial(release_values, n // 2 * 128, n % 2))
        plan[q_at[0]] += [lambda: wait("wq"), lambda: x_copy(1).wait()]
        for g in range(4):
            plan[q_at[g]].append(functools.partial(prep_scores, 0, g))
        stores = []

        def second_norm(n, delay):
            for block in (n // 2, T // 64 + n // 2) if n % 2 == 0 else ():
                row_stats(1, block)
            stores.append(norm1_unit(functools.partial(normalized, 1), n, delay=delay))

        for n, (slot, delay) in enumerate(slots0):
            plan[slot].append(functools.partial(second_norm, n, delay))
        plan[14 + 7 * HD // RC0].append(lambda: [store(ht_v) for store in stores])
        if marks:
            def mark(n):
                with jax.named_scope(f"mark{n}"):
                    fix_v[0, :, pl.ds(0, 128)] = jnp.zeros((16, 128), BF16)
            for n in marks:
                plan[n].append(functools.partial(mark, n))
        with scope("tile0"):
            first_pass(0, plan, 'kq', (256, RC0))

        def first_step(t, carry):
            @pl.when(t + 1 < NTILE)
            def _():
                x_copy(t + 1).wait()

            for n in range(1, NTILE):
                pl.when(t == n)(functools.partial(wait, ("mod", n)))

            @pl.when(t == 1)
            def _():
                start("wg", "wu", "wd")

            plan = collections.defaultdict(list)
            plan_norms(plan, jnp.clip(t + 1, 0, NTILE - 1), 0, lfirst, llast, 2 * nk + nv)
            per_step = pl.cdiv(HD // 16, NTILE - 1)
            for n in range(per_step):
                plan[pfirst + n * (plast - pfirst) // per_step].append(functools.partial(
                    lambda n: prep_output(jnp.clip((t - 1) * per_step + n, 0, HD // 16 - 1)), n))
            plan_modulation(plan, jnp.clip(t, 0, NTILE - 1), mfirst, mlast)
            first_pass(t, plan, order, (RC, RC))
            return carry

        wait("wo")
        if only in (0, 1):
            with scope("pass1"):
                jax.lax.fori_loop(1, NTILE, first_step, 0)
        if only == 1:
            for j in range(NPAIR):
                finish_kv(j)
            out_v[pl.ds(0, 64), pl.ds(0, 512)] = phiq_v[zero, zero, pl.ds(0, 64), :]
            out_v[pl.ds(64, 80), pl.ds(0, 128)] = _unpack(kvb_v[zero])
            out_v[pl.ds(160, 64), pl.ds(0, 512)] = _unpack(wot_v[zero, pl.ds(0, 32), :])
            out_copy(0).start()
            out_copy(0).wait()
            return

        wait(("mod", 0), "wr", "wg", "wu", "wd")
        modulation(2 * D, MW // 2)
        for j in range(NPAIR):
            finish_kv(j)
        tasks = [task for i in range(4) for task in attend(0, 0, oa_v, i)]
        modulation(2 * D + MW // 2, MW // 2)
        for task in tasks:
            task()
        output_weights()

        def finish(base, rows_of, rows, strands, delay):
            chain = Chain(strands)
            for o in range(0, rows, EC):
                row, y = rows_of(o)
                finish_rows(base + row, y, chain)
            if delay:
                finish_within(delay, *chain.tokens)

        def mixed(source, lo, n):
            rows_of = mixed_rows(from_values(mix(source, lo, n)), n)
            return lambda o: (lo + o // n * G + o % n, rows_of(o))

        rows_of = None
        sent = []
        due.clear()
        with scope("pass2"):
            for n in range(NSUB):
                source, target = ((oa_v, ob_v), (ob_v, oa_v))[n % 2]
                if n + 1 < NSUB:
                    tasks = [task for i in range(4) for task in attend((n + 1) // 2, (n + 1) % 2, target, i)]
                    for task in tasks:
                        task()
                if n + 1 < NSUB or not tail:
                    if rows_of:
                        finish((n - 1) * 2 * G, rows_of, 2 * G, ne, edelay)
                    rows_of = mixed(source, 0, G)
                    left = 2 * G
                else:
                    finish((n - 1) * 2 * G, rows_of, 2 * G, ne_tail, edelay)
                    rows_of = mixed(source, 0, G - tail)
                    finish(n * 2 * G, rows_of, 2 * (G - tail), ne_tail, edelay)
                    rows_of = mixed(source, G - tail, tail)
                    left = 2 * tail
                if n > 1:
                    out_copy(n - 2).start()
                    sent.append(n - 2)
                if n in barriers:
                    while len(sent) > 1:
                        out_copy(sent.pop(0)).wait()
        with scope("last"):
            finish(S - 2 * G, rows_of, left, nl, 0)
        out_copy(NSUB - 2).start()
        sent.append(NSUB - 2)
        out_copy(NSUB - 1).start()
        sent.append(NSUB - 1)
        with scope("experts"):
            b1, b2 = experts()
        with scope("w_out"):
            for n in sent:
                out_copy(n).wait()
        fix = [pltpu.make_async_copy(fix_v.at[n], out_hbm.at[pl.ds(b, 16)], osems.at[n])
               for n, b in enumerate((b1, b2))]
        fix[0].start()

        @pl.when(b1 != b2)
        def _():
            fix[1].start()
            fix[1].wait()

        fix[0].wait()

    nsem = NTILE + 3 + 3 + NTILE + 1 + 10 + 4
    scratch = [
        pltpu.VMEM((S + 16, D), BF16), pltpu.VMEM((D, 3 * D), BF16), pltpu.VMEM((D, DH), BF16),
        pltpu.VMEM((D + 16, D), BF16), pltpu.VMEM((8, 128), BF16),
        pltpu.VMEM((D, FF), BF16), pltpu.VMEM((D, FF), BF16), pltpu.VMEM((FF, D), BF16),
        pltpu.VMEM((1, D), BF16), pltpu.VMEM((D, 6 * D), BF16),
        pltpu.VMEM((8, D), U32),
        pltpu.VMEM((8, 6 * D), F32),
        pltpu.VMEM((10, 8, D), F32),
        pltpu.VMEM((2, T, 128), F32),
        pltpu.VMEM((8, D), F32),
        pltpu.VMEM((D // 128, 64, 128), U32),
        pltpu.VMEM((7, HD // 2, HD), U32),
        pltpu.VMEM((7, HT // 2, HD), U32),
        pltpu.VMEM((7, HT // 2, HD), U32),
        pltpu.VMEM((NTILE, NPAIR, 128, T), BF16),
        pltpu.VMEM((NPAIR, 128, T), BF16),
        pltpu.VMEM((NPAIR, 80, T), BF16),
        pltpu.VMEM((NPAIR, 80, 128), F32),
        pltpu.VMEM((NPAIR, 40, 128), U32),
        pltpu.VMEM((7, G // 2, HD), U32),
        pltpu.VMEM((7, G // 2, HD), U32),
        pltpu.VMEM((S, D), F32),
        pltpu.VMEM((S, D), BF16),
        pltpu.VMEM((2, 16, D), BF16),
        pltpu.SemaphoreType.DMA((nsem,)),
        pltpu.SemaphoreType.DMA((NSUB,)),
    ] + [pltpu.VMEM((7, 64, HD), U32)] * 8 + [pltpu.VMEM((7, HD // 2, 128), U32)] * 4

    def fn(A_x, A_wqkv, A_w_phi, A_wo, B_x, B_w_r, B_w_gate, B_w_up, B_w_down, c, w_mod):
        del B_x
        out = pl.pallas_call(
            kernel,
            out_shape=jax.ShapeDtypeStruct((S, D), A_x.dtype),
            in_specs=[pl.BlockSpec(memory_space=pl.ANY)] * 10,
            out_specs=pl.BlockSpec(memory_space=pl.ANY),
            scratch_shapes=scratch,
            compiler_params=pltpu.CompilerParams(vmem_limit_bytes=vlimit * 2**20, flags=flags),
        )(A_x.reshape(S, D), A_wqkv, A_w_phi.reshape(D, DH), A_wo, B_w_r.reshape(8, 128),
          B_w_gate, B_w_up, B_w_down, c, w_mod)
        return out.reshape(A_x.shape)

    return fn


@jax.jit
def pallas_adaLN_cond__linear_kernel_hedgehog__moe_arch_mod__prompt_kernel(
    A_x, A_wqkv, A_w_phi, A_wo, B_x, B_w_r, B_w_gate, B_w_up, B_w_down, c, w_mod
):
    return make()(A_x, A_wqkv, A_w_phi, A_wo, B_x, B_w_r, B_w_gate, B_w_up, B_w_down, c, w_mod)
```

```python
import collections
import contextlib
import functools

import jax
import jax.numpy as jnp
import numpy as np
import jax.experimental.pallas as pl
import jax.experimental.pallas.tpu as pltpu

F32, BF16, I32, U32 = jnp.float32, jnp.bfloat16, jnp.int32, jnp.uint32
S, D, H, DH, FF = 2048, 1024, 32, 32, 3584
HD = D // 2
NPAIR = H // 2
EPS = 1e-5
LOG2E = float(np.log2(np.e))
NN = (((1,), (0,)), ((), ()))
NT = (((1,), (1,)), ((), ()))


def _dot(a, b, dn=NN):
    return jax.lax.dot_general(a, b, dn, preferred_element_type=F32)


def _pack(x):
    n = x.shape[0] // 2
    if x.shape[1] > 128:
        return pltpu.bitcast(x.astype(BF16), U32)
    w = pltpu.bitcast(jnp.concatenate([x[:n], x[n:]], axis=1).astype(BF16), U32)
    return jnp.concatenate([w[:, :128], w[:, 128:]], axis=0)


def _unpack(w):
    return pltpu.bitcast(w, BF16)


def _recip(x):
    r = pl.reciprocal(x, approx=True)
    return r * (2.0 - x * r)


def _lhs_terms(a11, a12, a21, a22):
    return (a11 + a22, a21 + a22, a11, a22, a11 + a12, a21 - a11, a12 - a22)


def _rhs_terms(b11, b12, b21, b22):
    return (b11 + b22, b11, b12 - b22, b21 - b11, b22, b11 + b12, b21 + b22)


_QUADRANTS = (((0, 1), (3, 1), (4, -1), (6, 1)), ((2, 1), (4, 1)), ((1, 1), (3, 1)),
              ((0, 1), (1, -1), (2, 1), (5, 1)))


def _quadrant(q, product):
    total = None
    for j, sign in _QUADRANTS[q]:
        m = product(j)
        total = m if total is None else (total + m if sign > 0 else total - m)
    return total


def _layernorm(x):
    d = x - jnp.mean(x, axis=-1, keepdims=True)
    v = jnp.mean(d * d, axis=-1, keepdims=True)
    return d * jax.lax.rsqrt(v + EPS)


def _per_head(op, p):
    parts = [p[r:r + 8] for r in range(0, p.shape[0], 8)]
    while len(parts) > 1:
        parts = [op(a, b) for a, b in zip(parts[::2], parts[1::2])]
    out = op(parts[0], pltpu.roll(parts[0], 4, 0))
    return op(out, pltpu.roll(out, 2, 0))


def _apply(op, p, stat):
    n = p.shape[0] // 8
    return op(p.reshape(n, 8, p.shape[1]), stat).reshape(p.shape)


def _features(p):
    e_pos = jnp.exp2(_apply(jnp.subtract, p, _per_head(jnp.maximum, p)))
    e_neg = jnp.exp2(_apply(lambda a, low: low - a, p, _per_head(jnp.minimum, p)))
    pos = _apply(jnp.multiply, e_pos, _recip(_per_head(jnp.add, e_pos)))
    neg = _apply(jnp.multiply, e_neg, _recip(_per_head(jnp.add, e_neg)))
    return jnp.concatenate([pos, neg], axis=0)


def _interleaved_source(row):
    return (row & ~63) + ((row & 1) << 5) + ((row & 63) >> 1)


class _Interleaver:
    def __init__(self, ratio):
        self.queue = collections.deque()
        self.ratio = ratio
        self.credit = 0.0

    def defer(self, cost, fn):
        self.queue.append((cost, fn))

    def spent(self, cycles):
        self.credit += cycles * self.ratio
        while self.queue and self.credit >= self.queue[0][0]:
            cost, fn = self.queue.popleft()
            self.credit -= cost
            fn()
        if not self.queue:
            self.credit = 0.0

    def drain(self):
        while self.queue:
            self.queue.popleft()[1]()
        self.credit = 0.0


def make(RC=256, VC=256, LW=512, FC=256, EC=32, ratio=0.55, vlimit=120, flags=None, S=S,
         prof=False, only=0, marks=(), vcost=256, kcost=150, mfirst=1, mlast=42,
         flag=2, RC0=128, a_at=1, m0=2, m1=26, sa_at=23, k_at=5,
         slots0=tuple((s, d) for s in range(6, 12) for d in (4, 5)),
         slots1=tuple((s, d) for s in range(33, 41) for d in (2, 3)),
         wo_split=(0, 0, 16, 32), pslots=((1,), (1, 2, 3, 4, 10, 11, 17, 18, 24, 25, 31, 32), (1, 2, 3, 4, 10, 17, 24, 31, 33, 34, 35, 36, 37, 38, 39, 40)), pdelay=2,
         ne=3, nl=32, edelay=40, barriers=(), tail=32, ne_tail=5, att_at=None, ffn=1):
    scope = lambda n: jax.named_scope(n) if prof is True or (prof and n in prof) else contextlib.nullcontext()
    T = 512
    HT = T // 2
    NTILE = S // T
    G = 128
    NSUB = S // (2 * G)
    MW = 4 * D // NTILE
    nk, nv = 7 * HD // RC, 7 * HD // VC

    def kernel(x_hbm, wqkv_hbm, wphi_hbm, wo_hbm, wr_hbm, wg_hbm, wu_hbm, wd_hbm, c_hbm, wmod_hbm,
               out_hbm,
               x_v, wqkv_v, wphi_v, wo_v, wr_v, wg_v, wu_v, wd_v, c_v, wmod_v,
               act_v, raw_v, mod_v, stat_v, bias_v, bd_v, wot_v, ht_v, h0_v, phiq_v, phik_v, vt_v, kv_v, kvb_v, oa_v, ob_v,
               xn_v, out_v, fix_v, sems, osems, *terms_v):
        wq_v, wk_v, wv_v = terms_v[:4], terms_v[4:8], terms_v[8:]

        side = _Interleaver(ratio)
        copies = {}

        def add_copy(name, src, dst):
            copies[name] = pltpu.make_async_copy(src, dst, sems.at[NTILE + len(copies)])

        add_copy("c", c_hbm, c_v)
        add_copy("wphi", wphi_hbm, wphi_v)
        add_copy("wr", wr_hbm, wr_v)
        def add_columns(name, hbm, vmem, lo, n):
            add_copy(name, hbm.at[:, pl.ds(lo, n)], vmem.at[:, pl.ds(lo, n)])

        for n in range(2):
            piece = (pl.ds(n * HD, HD), pl.ds(D, D))
            add_copy(("scale", n), wmod_hbm.at[piece], wmod_v.at[piece])
        add_columns("shift", wmod_hbm, wmod_v, 0, D)
        for t in range(NTILE):
            add_columns(("mod", t), wmod_hbm, wmod_v, 2 * D + t * MW, MW)
        add_columns("wq", wqkv_hbm, wqkv_v, 0, D)
        for half in range(2):
            for n in range(2):
                add_columns(("wk", n, half), wqkv_hbm, wqkv_v, D + half * HD + n * 256, 256)
            for n, (lo, size) in enumerate(((0, 128), (128, 128), (256, 256))):
                add_columns(("wv", n, half), wqkv_hbm, wqkv_v, 2 * D + half * HD + lo, size)
        both = lambda *name: ((*name, 0), (*name, 1))
        add_copy("wo", wo_hbm, wo_v.at[pl.ds(0, D)])
        add_copy("wg", wg_hbm, wg_v)
        add_copy("wu", wu_hbm, wu_v)
        add_copy("wd", wd_hbm, wd_v)

        def start(*names, priority=0):
            for n in names:
                copies[n].start(priority=priority)

        def wait(*names):
            with scope("w_" + "_".join(str(n) for n in names)[:20].replace("'", "").replace(" ", "")):
                for n in names:
                    copies[n].wait()

        def rows_at(base, size):
            return pl.ds(base if isinstance(base, int) else pl.multiple_of(base, 8), size)

        def x_copy(t):
            return pltpu.make_async_copy(x_hbm.at[rows_at(t * T, T)], x_v.at[rows_at(t * T, T)], sems.at[t])

        def out_copy(n):
            rows = pl.ds(n * 2 * G, 2 * G)
            return pltpu.make_async_copy(out_v.at[rows], out_hbm.at[rows], osems.at[n])

        def modulation(lo, n, half=None):
            rows = pl.ds(0, D) if half is None else pl.ds(half * HD, HD)
            lanes = pl.ds(lo if isinstance(lo, int) else pl.multiple_of(lo, 128), n)
            m = _dot(_unpack(act_v[:, rows]), wmod_v[rows, lanes])[:8]
            raw_v[:, lanes] = m if not half else raw_v[:, lanes] + m

        raw = lambda i: raw_v[:, pl.ds(i * D, D)]

        def block_diag_phi():
            row = _interleaved_source(jax.lax.broadcasted_iota(I32, (128, DH), 0))
            col = jax.lax.broadcasted_iota(I32, (128, DH), 1)
            sel = jnp.where((row & (DH - 1)) == col, 1.0, 0.0).astype(BF16)
            r2 = _interleaved_source(jax.lax.broadcasted_iota(I32, (128, 128), 0)) >> 5
            c2 = jax.lax.broadcasted_iota(I32, (128, 128), 1) >> 5
            for g in range(D // 128):
                tiled = _dot(sel, wphi_v[pl.ds(g * 128, 128), :], NT)
                bd_v[g] = _pack(jnp.where(r2 == c2, tiled, 0.0))

        def prep_scores(i, g):
            parts = []
            for gg in (g, g + HD // 128):
                for half in range(2):
                    w = wqkv_v[pl.ds(half * HD, HD), pl.ds(i * D + gg * 128, 128)]
                    parts.append(_dot(_unpack(bd_v[gg]), w, NT) * LOG2E)
            for j, term in enumerate(_lhs_terms(*parts)):
                (wq_v, wk_v)[i][g][j] = _pack(term)

        def prep_values(g):
            chain = Chain(1)
            for r in range(0, HD, 64):
                blocks = [wqkv_v[pl.ds(row + r, 64), pl.ds(2 * D + col + g * 128, 128)].astype(F32)
                          for col in (0, HD) for row in (0, HD)]
                blocks[3] = chain.enter(blocks[3])
                for j, term in enumerate(_lhs_terms(*blocks)):
                    words = _pack(term)
                    wv_v[g][j, pl.ds(r // 2, 32), :] = words
                chain.leave(words[:8])

        def prep_output(n):
            lo = wo_v[rows_at(n * 16, 16), :].astype(F32)
            hi = wo_v[rows_at(HD + n * 16, 16), :].astype(F32)
            words = [_pack(term) for term in _rhs_terms(lo[:, :HD], lo[:, HD:], hi[:, :HD], hi[:, HD:])]
            for j, w in enumerate(words):
                wot_v[j, rows_at(n * 8, 8), :] = w
            finish_within(pdelay, *words)

        start("c")
        x_copy(0).start()
        start(*both("scale"), *both("wv", 0), *both("wv", 1), *both("wv", 2), "shift", "wphi")
        start(*both("wk", 0), *both("wk", 1))
        x_copy(1).start()
        start("wq")
        for t in range(1, NTILE):
            if t + 1 < NTILE:
                x_copy(t + 1).start()
            start(("mod", t))
            if t == 1:
                start("wo")
        start(("mod", 0))
        start("wr")
        wait("c")
        bits = pltpu.bitcast(jnp.broadcast_to(c_v[:, :128].astype(F32), (8, 128)), I32)
        zero = jnp.minimum(jnp.max(bits & 0xFF), 0)
        latest = {}

        class Chain:
            def __init__(self, strands):
                self.tokens = collections.deque([None] * strands)

            def enter(self, value):
                token = self.tokens.popleft()
                if token is None:
                    return value
                head = pltpu.bitcast(pltpu.bitcast(value[:8, :128], I32) | token, F32)
                if value.shape[1] > 128:
                    head = jnp.concatenate([head, value[:8, 128:]], axis=1)
                return jnp.concatenate([head, value[8:]], axis=0) if value.shape[0] > 8 else head

            def leave(self, *values):
                token = None
                for value in values:
                    value = pltpu.bitcast(value, I32)
                    token = value if token is None else token | value
                self.tokens.append(token & zero)

            def widen(self, strands):
                last = self.tokens[-1]
                while len(self.tokens) < strands:
                    self.tokens.append(last)

        clock = [0]
        due = collections.defaultdict(list)

        def finish_within(delay, *values):
            token = None
            for value in values:
                value = pltpu.bitcast(value, U32)
                for r in range(0, value.shape[0], 8):
                    for l in range(0, value.shape[1], 128):
                        part = value[r:r + 8, l:l + 128]
                        token = part if token is None else token | part
            due[clock[0] + delay].append(token & zero.astype(U32))

        def gated(ref, j, row=0):
            clock[0] += 1
            tokens = [token for when in sorted(due) if when < clock[0] for token in due.pop(when)]
            if tokens:
                corner = (j, pl.ds(row, 8), pl.ds(0, 128))
                ref[corner] = functools.reduce(jnp.bitwise_or, tokens, ref[corner])
            return ref[j]

        def row_stats(t, n):
            xx = x_v[rows_at(t * T + n * 32, 32), :].astype(F32)
            mean = jnp.mean(xx, axis=-1, keepdims=True)
            d = xx - mean
            scale = jax.lax.rsqrt(jnp.mean(d * d, axis=-1, keepdims=True) + EPS)
            stat_v[0, rows_at(n * 32, 32), :] = jnp.broadcast_to(mean, (32, 128))
            stat_v[1, rows_at(n * 32, 32), :] = jnp.broadcast_to(scale, (32, 128))

        def normalized(t, offset, lanes):
            wide = lambda k: jnp.concatenate([stat_v[k, pl.ds(offset, 16), :]] * (LW // 128), axis=1)
            return (x_v[rows_at(t * T + offset, 16), lanes].astype(F32) - wide(0)) * wide(1)

        def norm1_unit(rows, n, shift=True, delay=0):
            group, part = divmod(n, HD // LW)
            blocks = []
            for col in (part * LW, HD + part * LW):
                for offset in (group * 16, HT + group * 16):
                    lanes = pl.ds(col, LW)
                    hh = rows(offset, lanes).reshape(2, 8, LW) * mod_v[1, :, lanes]
                    blocks.append((hh + mod_v[0, :, lanes] if shift else hh).reshape(16, LW))
            words = [_pack(term) for term in _rhs_terms(*blocks)]
            if delay:
                finish_within(delay, *words)

            def store(target):
                for j, w in enumerate(words):
                    target[j, pl.ds(group * 8, 8), pl.ds(part * LW, LW)] = w

            return store

        def strassen(product, tiles, cycles, extra):
            products = []
            for j in range(7):
                products.append([product(j, k) for k in range(tiles)])
                latest["m"] = products[j][-1][-16:]
                side.spent(cycles)
                extra()
            return products

        def scores(i, source, extra, consume, RC):
            cost = kcost * RC // 256
            tiles = HT // 128
            for r in range(0, HD, RC):
                products = strassen(
                    lambda j, k: _dot(
                        _unpack(jnp.concatenate(
                            [(wq_v, wk_v)[i][g][j] for g in range(r // 128, (r + RC) // 128)], axis=0)),
                        _unpack(gated(source, j, k * 64)[k * 64:(k + 1) * 64]), NT),
                    tiles, RC * HT // 128, extra)

                def unit(half, o, products=products, r=r):
                    for part in range(2):
                        phi = jnp.concatenate(
                            [_features(_quadrant(2 * half + part, lambda j: products[j][k][o:o + 64]))
                             for k in range(tiles)], axis=1)
                        consume((half * HD + r + o) // 64, pl.ds(part * HT, HT), phi.astype(BF16))

                for half in range(2):
                    for o in range(0, RC, 64):
                        side.defer(cost, functools.partial(unit, half, o))

        def key_features(pair, lanes, phi):
            phik_v[pair, :, lanes] = phi

        def query_features(t, pair, lanes, phi):
            phiq_v[t, pair, :, lanes] = phi

        def store_values(col, part, v):
            v = v.T.astype(BF16).reshape(2, 64, HT)
            vt_v[pl.ds(col // 64, 2), pl.ds(0, 64), pl.ds(part * HT, HT)] = v

        def values(source, extra, consume, VC):
            tiles = VC // 128
            for r in range(0, HD, VC):
                products = strassen(
                    lambda j, k: _dot(_unpack(source[j]), _unpack(gated(wv_v[r // 128 + k], j))),
                    tiles, VC * HT // 128, extra)

                def unit(half, part, k, products=products, r=r):
                    consume(half * HD + r + k * 128, part, _quadrant(2 * half + part, lambda j: products[j][k]))

                for half in range(2):
                    for part in range(2):
                        for k in range(tiles):
                            side.defer(vcost // 2, functools.partial(unit, half, part, k))

        def accumulate_kv(j, first):
            kv = _dot(vt_v[j], phik_v[j], NT)
            kv_v[j] = kv if first else kv_v[j] + kv
            latest["m"] = kv[-16:]
            side.spent(T // 8)

        def finish_kv(j):
            row = jax.lax.broadcasted_iota(I32, (80, 128), 0)
            row_head = jnp.where(row < 64, row >> 5, (row >> 3) & 1)
            col_head = jax.lax.broadcasted_iota(I32, (80, 128), 1) & 1
            kvb_v[j] = _pack(jnp.where(row_head == col_head, kv_v[j], 0.0))

        def follow(plan):
            count = [0]

            def extra():
                count[0] += 1
                for task in plan.pop(count[0], ()):
                    task()

            for task in plan.pop(0, ()):
                task()
            return extra

        def all_kv(first):
            for r in range(0, HD, VC):
                for half in range(2):
                    for o in range(0, VC, 64):
                        accumulate_kv((half * HD + r + o) // 64, first)
            side.drain()

        def next_norm(t, n, delay):
            for block in (n // 2, T // 64 + n // 2) if n % 2 == 0 else ():
                row_stats(t, block)
            return norm1_unit(functools.partial(normalized, t), n, delay=delay)

        def plan_modulation(plan, t, first, last):
            steps = 2 * MW // 128
            for n in range(steps):
                plan[first + (last - first) * n // steps].append(
                    functools.partial(modulation, 2 * D + t * MW + n // 2 * 128, 128, n % 2))

        def attend(t, part, target, i):
            lanes = pl.ds(part * HT, HT)
            outs = {}
            tasks = []
            for half in range(2):
                for k in range(2):
                    p = half * (NPAIR // 2) + 2 * i + k
                    num = _dot(_unpack(kvb_v[p]), phiq_v[t, p, :, lanes])

                    def unit(num=num, key=(half, k)):
                        outs[key] = [_apply(jnp.multiply, num[h * DH:(h + 1) * DH],
                                            _recip(num[64 + 8 * h:72 + 8 * h] + 1e-6)) for h in range(2)]

                    tasks.append(unit)

            def terms_unit():
                lo, hi = (jnp.concatenate(outs[half, 0] + outs[half, 1], axis=0).T for half in range(2))
                for q, term in enumerate(_lhs_terms(lo[:G], hi[:G], lo[G:], hi[G:])):
                    target[q, :, pl.ds(i * 128, 128)] = _pack(term)

            return tasks + [terms_unit]

        def output_weights():
            w = wr_v[...].astype(F32)
            w = jnp.concatenate([jnp.broadcast_to(w[j:j + 1], (8, 128)) for j in range(D // 128)], axis=1)
            for i in range(2, 6):
                mod_v[i] = raw(i) + 1.0 if i == 4 else raw(i)
            mod_v[6] = mod_v[4] * w
            mod_v[7] = mod_v[4] * mod_v[5]
            mod_v[8] = mod_v[3] * mod_v[5]
            mod_v[9] = jnp.broadcast_to(jnp.sum(mod_v[3] * w, axis=1, keepdims=True), (8, D))

        ranks = {}

        def finish_rows(base, y, chain):
            lane = jax.lax.broadcasted_iota(I32, (8, 128), 1)
            acc = ranks.get(base >> 10, jnp.full((8, 128), -jnp.inf, F32))
            for o in range(0, y.shape[0], 8):
                rows = rows_at(base + o, 8)
                xn = x_v[rows, :].astype(F32) + mod_v[2] * chain.enter(y[o:o + 8])
                mean = jnp.mean(xn, axis=-1, keepdims=True)
                d = xn - mean
                scale = jax.lax.rsqrt(jnp.mean(d * d, axis=-1, keepdims=True) + EPS)
                score = jnp.sum(d * mod_v[6], axis=-1, keepdims=True) * scale + mod_v[9, :, :1]
                normed = d * scale
                xn_v[rows, :] = normed
                out = normed * mod_v[7] + ((d + mean) + mod_v[8])
                out_v[rows, :] = out.astype(BF16)
                acc = jnp.where(lane == ((base + o) & 1023) >> 3, score, acc)
                chain.leave(*[out[:, l:l + 128] for l in range(128, D, 256)])
            ranks[base >> 10] = acc

        tokens = collections.deque()

        def mix(source, lo, n, extra):
            return strassen(
                lambda j, k: _dot(_unpack(gated(source, j, lo // 2)[lo // 2:(lo + n) // 2]),
                                  _unpack(wot_v[j, :, pl.ds(k * 128, 128)])),
                HD // 128, 4 * n, extra)

        def mixed_rows(product, n):
            def rows_of(o):
                part, o = divmod(o, n)
                return jnp.concatenate(
                    [_quadrant(2 * part + half, lambda j: product(j, o)) for half in range(2)], axis=1)
            return rows_of

        def from_values(products):
            return lambda j, o: jnp.concatenate([tile[o:o + EC] for tile in products[j]], axis=1)

        def top2():
            shape = (S // 1024, 8, 128)
            idx = (jax.lax.broadcasted_iota(I32, shape, 0) * 1024 + jax.lax.broadcasted_iota(I32, shape, 2) * 8
                   + jax.lax.broadcasted_iota(I32, shape, 1)).astype(F32)
            m = jnp.stack([ranks[b] for b in range(S // 1024)])
            reduce = lambda op, v: op(op(op(v, axis=0), axis=0, keepdims=True), axis=1, keepdims=True)
            picks = []
            for _ in range(2):
                top = reduce(jnp.max, m)
                first = reduce(jnp.min, jnp.where(m == top, idx, float(S - 1)))
                picks.append((jnp.max(first.astype(I32)), top))
                m = jnp.where(idx == first, -jnp.inf, m)
            return picks

        def experts():
            (i1, m1), (i2, m2) = top2()
            picks = [jnp.clip(i, 0, S - 1) for i in (i1, i2)]
            bases = [pl.multiple_of((i >> 4) * 16, 16) for i in picks]
            sub = jax.lax.broadcasted_iota(I32, (16, D), 0)
            first, second = (jnp.broadcast_to(xn_v[pl.ds(i, 1), :], (16, D)) for i in picks)
            sel = jnp.where(sub == 0, first, second).reshape(2, 8, D) * mod_v[4] + mod_v[3]
            sel = sel.reshape(16, D).astype(BF16)
            y = None
            acts = collections.deque()

            def down():
                nonlocal y
                f, g, u = acts.popleft()
                act = (g * jax.nn.sigmoid(g) * u).astype(BF16)
                part = _dot(act, wd_v[pl.ds(f, FC), :])
                y = part if y is None else y + part

            for f in range(0, FF, FC):
                acts.append((f, _dot(sel, wg_v[:, pl.ds(f, FC)]), _dot(sel, wu_v[:, pl.ds(f, FC)])))
                if len(acts) > flag:
                    down()
            while acts:
                down()
            y1, y2 = y[0:1] * jax.nn.sigmoid(m1), y[1:2] * jax.nn.sigmoid(m2)
            for n, base in enumerate(bases):
                upd = jnp.where(sub == picks[0] - base, y1, 0.0) + jnp.where(sub == picks[1] - base, y2, 0.0)
                full = out_v[pl.ds(base, 16), :].astype(F32).reshape(2, 8, D) + mod_v[5] * upd.reshape(2, 8, D)
                fix_v[n] = full.reshape(16, D).astype(BF16)
            return bases

        cc = c_v[...].astype(F32)
        act_v[...] = _pack(jnp.broadcast_to(cc * jax.nn.sigmoid(cc), (16, D)))
        with scope("w_x0"):
            x_copy(0).wait()
        for n in range(T // 32):
            row_stats(0, n)
        for offset in range(0, T, 16):
            for col in range(0, D, LW):
                xn_v[pl.ds(offset, 16), pl.ds(col, LW)] = normalized(0, offset, pl.ds(col, LW))
        for n in range(2):
            wait(("scale", n))
            modulation(D, D, n)
        mod_v[1] = raw(1) + 1.0
        units = HT // 16 * (HD // LW)
        saved = lambda offset, lanes: xn_v[pl.ds(offset, 16), lanes]
        for n in range(units):
            norm1_unit(saved, n, shift=False)(h0_v)

        def hold_values(col, part, v):
            xn_v[pl.ds(T + part * HT, HT), pl.ds(col, 128)] = v

        def shift_and_bias():
            wait("shift")
            modulation(0, D)
            mod_v[0] = raw(0)

        def release_values(col, part):
            v = xn_v[pl.ds(T + part * HT, HT), pl.ds(col, 128)]
            store_values(col, part, _apply(jnp.add, v, bias_v[:, pl.ds(col, 128)]))

        wait(*both("wv", 0))
        prep_values(0)
        plan = collections.defaultdict(list)
        plan[3] += [lambda: wait(*both("wv", 1)), lambda: prep_values(1)]
        plan[7] += [lambda: wait(*both("wv", 2))]
        plan[8] += [lambda: prep_values(2)]
        plan[15] += [lambda: prep_values(3)]
        plan[sa_at].append(shift_and_bias)
        with scope("values0"):
            values(h0_v, follow(plan), hold_values, 128)
            side.drain()
        assert not plan
        wait("wphi", *both("wk", 0))
        block_diag_phi()
        prep_scores(1, 0)
        prep_scores(1, 1)
        shift = jnp.concatenate([raw(0)] * 2, axis=0).astype(BF16)
        bias_v[...] = _dot(shift, wqkv_v[:, pl.ds(2 * D, D)])[:8]
        for n in range(units):
            norm1_unit(saved, n)(h0_v)

        plan = collections.defaultdict(list)
        def initialize():
            vt_v[:, pl.ds(64, 16), :] = jnp.ones((NPAIR, 16, T), BF16)

        plan[0].append(initialize)
        plan[k_at] += [lambda: wait(*both("wk", 1)), lambda: prep_scores(1, 2), lambda: prep_scores(1, 3)]
        for n in range(16):
            plan[1 + n * 8 // 16].append(functools.partial(release_values, n // 2 * 128, n % 2))
        plan[k_at].insert(0, lambda: x_copy(1).wait())

        second_norm = lambda n, delay: next_norm(1, n, delay)(ht_v)
        for n, (slot, delay) in enumerate(slots0):
            plan[slot].append(functools.partial(second_norm, n, delay))
        with scope("tile0"):
            scores(1, h0_v, follow(plan), key_features, RC)
            assert not plan
            wait("wq")
            for g in range(4):
                prep_scores(0, g)
                side.spent(512)
            side.drain()
            for n in range(len(slots0), units):
                second_norm(n, 0)
            all_kv(True)

        def first_step(t):
            wait(("mod", t))
            if t + 1 < NTILE:
                x_copy(t + 1).wait()
            if t == 2:
                wait("wo")
            if ffn == 0 and t == 1:
                start("wg", "wu", "wd", priority=1)
            if ffn == 1:
                start(("wg", "wu", "wd")[t - 1])
            if ffn == 2:
                start(("wg", "wu", "wd")[t - 1], priority=1)
            plan = collections.defaultdict(list)
            stores = []
            if t + 1 < NTILE:
                for n, (slot, delay) in enumerate(slots1):
                    plan[slot].append(functools.partial(
                        lambda n, delay: stores.append(next_norm(t + 1, n, delay)), n, delay))
                plan[2 * nk + nv].append(lambda: [store(ht_v) for store in stores])
            lo, hi = wo_split[t - 1], wo_split[t]
            for n in range(lo, hi):
                plan[pslots[t - 1][len(pslots[t - 1]) * (n - lo) // (hi - lo)]].append(functools.partial(prep_output, n))
            plan_modulation(plan, t, mfirst, mlast)
            due.clear()
            extra = follow(plan)
            scores(1, ht_v, extra, key_features, RC)
            scores(0, ht_v, extra, functools.partial(query_features, t), RC)
            values(ht_v, extra, store_values, VC)
            assert not plan
            side.drain()
            all_kv(False)

        with scope("pass1"):
            for t in range(1, NTILE):
                first_step(t)
        if only == 1:
            for j in range(NPAIR):
                finish_kv(j)
            out_v[pl.ds(0, 64), pl.ds(0, 512)] = phiq_v[zero, zero, pl.ds(0, 64), :]
            out_v[pl.ds(64, 80), pl.ds(0, 128)] = _unpack(kvb_v[zero])
            out_v[pl.ds(160, 64), pl.ds(0, 512)] = _unpack(wot_v[zero, pl.ds(0, 32), :])
            out_copy(0).start()
            out_copy(0).wait()
            return

        wait(("mod", 0), "wr", "wg", "wu", "wd")
        order = [(n + 2) % NSUB for n in range(NSUB)]
        plan = collections.defaultdict(list)
        plan[0] += [functools.partial(finish_kv, j) for j in range(NPAIR)]

        def first_attention():
            tasks = [task for i in range(4) for task in attend(order[0] // 2, order[0] % 2, oa_v, i)]
            for task in tasks:
                task()

        plan[a_at].append(first_attention)
        plan_modulation(plan, 0, m0, m1)
        plan[m1].append(output_weights)
        due.clear()
        scores(0, h0_v, follow(plan), functools.partial(query_features, 0), RC0)

        def finish(base, rows_of, rows, strands, delay):
            chain = Chain(strands)
            for o in range(0, rows, EC):
                row, y = rows_of(o)
                finish_rows(base + row, y, chain)
            if delay:
                finish_within(delay, *chain.tokens)

        def mixed(source, lo, n, plan):
            rows_of = mixed_rows(from_values(mix(source, lo, n, follow(plan))), n)
            return lambda o: (lo + o // n * G + o % n, rows_of(o))

        rows_of = None
        sent = []
        due.clear()
        with scope("pass2"):
            for n in range(NSUB):
                source, target = ((oa_v, ob_v), (ob_v, oa_v))[n % 2]
                plan = collections.defaultdict(list)

                def attention(i):
                    for task in attend(order[n + 1] // 2, order[n + 1] % 2, target, i):
                        task()

                split = tail and n + 1 == NSUB
                if n + 1 < NSUB and att_at is None:
                    tasks = [task for i in range(4) for task in attend(order[n + 1] // 2, order[n + 1] % 2, target, i)]
                    for task in tasks:
                        task()
                elif n + 1 < NSUB:
                    for i in range(4):
                        plan[att_at[i]].append(functools.partial(attention, i))
                if rows_of:
                    at = att_at[-1] if att_at and n + 1 < NSUB else 0
                    plan[at].append(functools.partial(
                        finish, order[n - 1] * 2 * G, rows_of, 2 * G, ne_tail if split else ne, edelay - 4 * at))
                if not split:
                    rows_of = mixed(source, 0, G, plan)
                    left = 2 * G
                else:
                    rows_of = mixed(source, 0, G - tail, plan)
                    finish(order[n] * 2 * G, rows_of, 2 * (G - tail), ne_tail, edelay)
                    rows_of = mixed(source, G - tail, tail, plan)
                    left = 2 * tail
                if n > 1:
                    out_copy(order[n - 2]).start()
                    sent.append(order[n - 2])
                if n in barriers:
                    while len(sent) > 1:
                        out_copy(sent.pop(0)).wait()
        with scope("last"):
            finish(order[-1] * 2 * G, rows_of, left, nl, 0)
        out_copy(order[-2]).start()
        sent.append(order[-2])
        out_copy(order[-1]).start()
        sent.append(order[-1])
        with scope("experts"):
            b1, b2 = experts()
        with scope("w_out"):
            for n in sent:
                out_copy(n).wait()
        fix = [pltpu.make_async_copy(fix_v.at[n], out_hbm.at[pl.ds(b, 16)], osems.at[n])
               for n, b in enumerate((b1, b2))]
        fix[0].start()

        @pl.when(b1 != b2)
        def _():
            fix[1].start()
            fix[1].wait()

        fix[0].wait()

    nsem = NTILE + 3 + 3 + NTILE + 1 + 10 + 4
    scratch = [
        pltpu.VMEM((S + 16, D), BF16), pltpu.VMEM((D, 3 * D), BF16), pltpu.VMEM((D, DH), BF16),
        pltpu.VMEM((D + 16, D), BF16), pltpu.VMEM((8, 128), BF16),
        pltpu.VMEM((D, FF), BF16), pltpu.VMEM((D, FF), BF16), pltpu.VMEM((FF, D), BF16),
        pltpu.VMEM((1, D), BF16), pltpu.VMEM((D, 6 * D), BF16),
        pltpu.VMEM((8, D), U32),
        pltpu.VMEM((8, 6 * D), F32),
        pltpu.VMEM((10, 8, D), F32),
        pltpu.VMEM((2, T, 128), F32),
        pltpu.VMEM((8, D), F32),
        pltpu.VMEM((D // 128, 64, 128), U32),
        pltpu.VMEM((7, HD // 2, HD), U32),
        pltpu.VMEM((7, HT // 2, HD), U32),
        pltpu.VMEM((7, HT // 2, HD), U32),
        pltpu.VMEM((NTILE, NPAIR, 128, T), BF16),
        pltpu.VMEM((NPAIR, 128, T), BF16),
        pltpu.VMEM((NPAIR, 80, T), BF16),
        pltpu.VMEM((NPAIR, 80, 128), F32),
        pltpu.VMEM((NPAIR, 40, 128), U32),
        pltpu.VMEM((7, G // 2, HD), U32),
        pltpu.VMEM((7, G // 2, HD), U32),
        pltpu.VMEM((S, D), F32),
        pltpu.VMEM((S, D), BF16),
        pltpu.VMEM((2, 16, D), BF16),
        pltpu.SemaphoreType.DMA((nsem,)),
        pltpu.SemaphoreType.DMA((NSUB,)),
    ] + [pltpu.VMEM((7, 64, HD), U32)] * 8 + [pltpu.VMEM((7, HD // 2, 128), U32)] * 4

    def fn(A_x, A_wqkv, A_w_phi, A_wo, B_x, B_w_r, B_w_gate, B_w_up, B_w_down, c, w_mod):
        del B_x
        out = pl.pallas_call(
            kernel,
            out_shape=jax.ShapeDtypeStruct((S, D), A_x.dtype),
            in_specs=[pl.BlockSpec(memory_space=pl.ANY)] * 10,
            out_specs=pl.BlockSpec(memory_space=pl.ANY),
            scratch_shapes=scratch,
            compiler_params=pltpu.CompilerParams(vmem_limit_bytes=vlimit * 2**20, flags=flags),
        )(A_x.reshape(S, D), A_wqkv, A_w_phi.reshape(D, DH), A_wo, B_w_r.reshape(8, 128),
          B_w_gate, B_w_up, B_w_down, c, w_mod)
        return out.reshape(A_x.shape)

    return fn


@jax.jit
def pallas_adaLN_cond__linear_kernel_hedgehog__moe_arch_mod__prompt_kernel(
    A_x, A_wqkv, A_w_phi, A_wo, B_x, B_w_r, B_w_gate, B_w_up, B_w_down, c, w_mod
):
    return make()(A_x, A_wqkv, A_w_phi, A_wo, B_x, B_w_r, B_w_gate, B_w_up, B_w_down, c, w_mod)
```

```python
import collections
import contextlib
import functools

import jax
import jax.numpy as jnp
import numpy as np
import jax.experimental.pallas as pl
import jax.experimental.pallas.tpu as pltpu

F32, BF16, I32, U32 = jnp.float32, jnp.bfloat16, jnp.int32, jnp.uint32
S, D, H, DH, FF = 2048, 1024, 32, 32, 3584
HD = D // 2
NPAIR = H // 2
EPS = 1e-5
LOG2E = float(np.log2(np.e))
NN = (((1,), (0,)), ((), ()))
NT = (((1,), (1,)), ((), ()))


def _dot(a, b, dn=NN):
    return jax.lax.dot_general(a, b, dn, preferred_element_type=F32)


def _pack(x):
    n = x.shape[0] // 2
    if x.shape[1] > 128:
        return pltpu.bitcast(x.astype(BF16), U32)
    w = pltpu.bitcast(jnp.concatenate([x[:n], x[n:]], axis=1).astype(BF16), U32)
    return jnp.concatenate([w[:, :128], w[:, 128:]], axis=0)


def _unpack(w):
    return pltpu.bitcast(w, BF16)


def _recip(x):
    r = pl.reciprocal(x, approx=True)
    return r * (2.0 - x * r)


def _lhs_terms(a11, a12, a21, a22):
    return (a11 + a22, a21 + a22, a11, a22, a11 + a12, a21 - a11, a12 - a22)


def _rhs_terms(b11, b12, b21, b22):
    return (b11 + b22, b11, b12 - b22, b21 - b11, b22, b11 + b12, b21 + b22)


_QUADRANTS = (((0, 1), (3, 1), (4, -1), (6, 1)), ((2, 1), (4, 1)), ((1, 1), (3, 1)),
              ((0, 1), (1, -1), (2, 1), (5, 1)))


def _quadrant(q, product):
    total = None
    for j, sign in _QUADRANTS[q]:
        m = product(j)
        total = m if total is None else (total + m if sign > 0 else total - m)
    return total


def _layernorm(x):
    d = x - jnp.mean(x, axis=-1, keepdims=True)
    v = jnp.mean(d * d, axis=-1, keepdims=True)
    return d * jax.lax.rsqrt(v + EPS)


def _per_head(op, p):
    parts = [p[r:r + 8] for r in range(0, p.shape[0], 8)]
    while len(parts) > 1:
        parts = [op(a, b) for a, b in zip(parts[::2], parts[1::2])]
    out = op(parts[0], pltpu.roll(parts[0], 4, 0))
    return op(out, pltpu.roll(out, 2, 0))


def _apply(op, p, stat):
    n = p.shape[0] // 8
    return op(p.reshape(n, 8, p.shape[1]), stat).reshape(p.shape)


def _features(p):
    e_pos = jnp.exp2(_apply(jnp.subtract, p, _per_head(jnp.maximum, p)))
    e_neg = jnp.exp2(_apply(lambda a, low: low - a, p, _per_head(jnp.minimum, p)))
    pos = _apply(jnp.multiply, e_pos, _recip(_per_head(jnp.add, e_pos)))
    neg = _apply(jnp.multiply, e_neg, _recip(_per_head(jnp.add, e_neg)))
    return jnp.concatenate([pos, neg], axis=0)


def _interleaved_source(row):
    return (row & ~63) + ((row & 1) << 5) + ((row & 63) >> 1)


class _Interleaver:
    def __init__(self, ratio):
        self.queue = collections.deque()
        self.ratio = ratio
        self.credit = 0.0

    def defer(self, cost, fn):
        self.queue.append((cost, fn))

    def spent(self, cycles):
        self.credit += cycles * self.ratio
        while self.queue and self.credit >= self.queue[0][0]:
            cost, fn = self.queue.popleft()
            self.credit -= cost
            fn()
        if not self.queue:
            self.credit = 0.0

    def drain(self):
        while self.queue:
            self.queue.popleft()[1]()
        self.credit = 0.0


def make(RC=256, VC=256, LW=512, FC=256, EC=32, ratio=0.55, vlimit=120, flags=None, S=S,
         prof=False, only=0, marks=(), vcost=256, kcost=150, mfirst=29, mlast=42,
         flag=2, RC0=128, a_at=0, m0=4, m1=26, sa_at=23, k_at=5,
         slots0=tuple((s, d) for s in range(6, 13) for d in (3, 4))[:13],
         slots1=tuple((s, d) for s in range(33, 41) for d in (2, 3)),
         pslots=((), tuple(range(3, 27))), pdelay=2,
         ne=3, nl=32, edelay=40, barriers=(), tail=64, ne_tail=4, att_at=None, ffn=1, keep=True):
    scope = lambda n: jax.named_scope(n) if prof is True or (prof and n in prof) else contextlib.nullcontext()
    T = 512
    HT = T // 2
    NTILE = S // T
    G = 128
    NSUB = S // (2 * G)
    MW = 4 * D // NTILE
    nk, nv = 7 * HD // RC, 7 * HD // VC

    def kernel(x_hbm, wqkv_hbm, wphi_hbm, wo_hbm, wr_hbm, wg_hbm, wu_hbm, wd_hbm, c_hbm, wmod_hbm,
               out_hbm,
               x_v, wqkv_v, wphi_v, wo_v, wr_v, wg_v, wu_v, wd_v, c_v, wmod_v,
               act_v, raw_v, mod_v, stat_v, bias_v, bd_v, wot_v, ht_v, h0_v, phiq_v, phik_v, vt_v, kv_v, kvb_v, oa_v, ob_v,
               xn_v, out_v, fix_v, sems, osems, *terms_v):
        wq_v, wk_v, wv_v = terms_v[:4], terms_v[4:8], terms_v[8:]

        side = _Interleaver(ratio)
        copies = {}

        def add_copy(name, src, dst):
            copies[name] = pltpu.make_async_copy(src, dst, sems.at[NTILE + len(copies)])

        add_copy("c", c_hbm, c_v)
        add_copy("wphi", wphi_hbm, wphi_v)
        add_copy("wr", wr_hbm, wr_v)
        def add_columns(name, hbm, vmem, lo, n):
            add_copy(name, hbm.at[:, pl.ds(lo, n)], vmem.at[:, pl.ds(lo, n)])

        for n in range(2):
            piece = (pl.ds(n * HD, HD), pl.ds(D, D))
            add_copy(("scale", n), wmod_hbm.at[piece], wmod_v.at[piece])
        add_columns("shift", wmod_hbm, wmod_v, 0, D)
        for t in range(NTILE):
            add_columns(("mod", t), wmod_hbm, wmod_v, 2 * D + t * MW, MW)
        add_columns("wq", wqkv_hbm, wqkv_v, 0, D)
        for half in range(2):
            for n in range(2):
                add_columns(("wk", n, half), wqkv_hbm, wqkv_v, D + half * HD + n * 256, 256)
            for n, (lo, size) in enumerate(((0, 128), (128, 128), (256, 256))):
                add_columns(("wv", n, half), wqkv_hbm, wqkv_v, 2 * D + half * HD + lo, size)
        both = lambda *name: ((*name, 0), (*name, 1))
        add_copy("wo", wo_hbm, wo_v.at[pl.ds(0, D)])
        add_copy("wg", wg_hbm, wg_v)
        add_copy("wu", wu_hbm, wu_v)
        add_copy("wd", wd_hbm, wd_v)

        def start(*names, priority=0):
            for n in names:
                copies[n].start(priority=priority)

        def wait(*names):
            with scope("w_" + "_".join(str(n) for n in names)[:20].replace("'", "").replace(" ", "")):
                for n in names:
                    copies[n].wait()

        def rows_at(base, size):
            return pl.ds(base if isinstance(base, int) else pl.multiple_of(base, 8), size)

        def x_copy(t):
            return pltpu.make_async_copy(x_hbm.at[rows_at(t * T, T)], x_v.at[rows_at(t * T, T)], sems.at[t])

        def out_copy(n):
            rows = pl.ds(n * 2 * G, 2 * G)
            return pltpu.make_async_copy(out_v.at[rows], out_hbm.at[rows], osems.at[n])

        def modulation(lo, n, half=None):
            rows = pl.ds(0, D) if half is None else pl.ds(half * HD, HD)
            lanes = pl.ds(lo if isinstance(lo, int) else pl.multiple_of(lo, 128), n)
            m = _dot(_unpack(act_v[:, rows]), wmod_v[rows, lanes])[:8]
            raw_v[:, lanes] = m if not half else raw_v[:, lanes] + m

        raw = lambda i: raw_v[:, pl.ds(i * D, D)]

        def block_diag_phi():
            row = _interleaved_source(jax.lax.broadcasted_iota(I32, (128, DH), 0))
            col = jax.lax.broadcasted_iota(I32, (128, DH), 1)
            sel = jnp.where((row & (DH - 1)) == col, 1.0, 0.0).astype(BF16)
            r2 = _interleaved_source(jax.lax.broadcasted_iota(I32, (128, 128), 0)) >> 5
            c2 = jax.lax.broadcasted_iota(I32, (128, 128), 1) >> 5
            for g in range(D // 128):
                tiled = _dot(sel, wphi_v[pl.ds(g * 128, 128), :], NT)
                bd_v[g] = _pack(jnp.where(r2 == c2, tiled, 0.0))

        def prep_scores(i, g):
            parts = []
            for gg in (g, g + HD // 128):
                for half in range(2):
                    w = wqkv_v[pl.ds(half * HD, HD), pl.ds(i * D + gg * 128, 128)]
                    parts.append(_dot(_unpack(bd_v[gg]), w, NT) * LOG2E)
            for j, term in enumerate(_lhs_terms(*parts)):
                (wq_v, wk_v)[i][g][j] = _pack(term)

        def prep_values(g):
            chain = Chain(1)
            for r in range(0, HD, 64):
                blocks = [wqkv_v[pl.ds(row + r, 64), pl.ds(2 * D + col + g * 128, 128)].astype(F32)
                          for col in (0, HD) for row in (0, HD)]
                blocks[3] = chain.enter(blocks[3])
                for j, term in enumerate(_lhs_terms(*blocks)):
                    words = _pack(term)
                    wv_v[g][j, pl.ds(r // 2, 32), :] = words
                chain.leave(words[:8])

        def prep_output(n):
            lo = wo_v[rows_at(n * 16, 16), :].astype(F32)
            hi = wo_v[rows_at(HD + n * 16, 16), :].astype(F32)
            words = [_pack(term) for term in _rhs_terms(lo[:, :HD], lo[:, HD:], hi[:, :HD], hi[:, HD:])]
            for j, w in enumerate(words):
                wot_v[j, rows_at(n * 8, 8), :] = w
            finish_within(pdelay, *words)

        start("c")
        x_copy(0).start()
        start(*both("scale"), *both("wv", 0), *both("wv", 1), *both("wv", 2), "shift", "wphi")
        start(*both("wk", 0), *both("wk", 1))
        x_copy(1).start()
        start("wq")
        for t in range(1, NTILE):
            if t + 1 < NTILE:
                x_copy(t + 1).start()
            start(("mod", t))
            if t == NTILE - 1:
                start("wo")
        start(("mod", 0))
        start("wr")
        wait("c")
        bits = pltpu.bitcast(jnp.broadcast_to(c_v[:, :128].astype(F32), (8, 128)), I32)
        zero = jnp.minimum(jnp.max(bits & 0xFF), 0)
        latest = {}

        class Chain:
            def __init__(self, strands):
                self.tokens = collections.deque([None] * strands)

            def enter(self, value):
                token = self.tokens.popleft()
                if token is None:
                    return value
                head = pltpu.bitcast(pltpu.bitcast(value[:8, :128], I32) | token, F32)
                if value.shape[1] > 128:
                    head = jnp.concatenate([head, value[:8, 128:]], axis=1)
                return jnp.concatenate([head, value[8:]], axis=0) if value.shape[0] > 8 else head

            def leave(self, *values):
                token = None
                for value in values:
                    value = pltpu.bitcast(value, I32)
                    token = value if token is None else token | value
                self.tokens.append(token & zero)

            def widen(self, strands):
                last = self.tokens[-1]
                while len(self.tokens) < strands:
                    self.tokens.append(last)

        clock = [0]
        due = collections.defaultdict(list)

        def finish_within(delay, *values):
            token = None
            for value in values:
                value = pltpu.bitcast(value, U32)
                for r in range(0, value.shape[0], 8):
                    for l in range(0, value.shape[1], 128):
                        part = value[r:r + 8, l:l + 128]
                        token = part if token is None else token | part
            due[clock[0] + delay].append(token & zero.astype(U32))

        def gated(ref, j, row=0):
            clock[0] += 1
            tokens = [token for when in sorted(due) if when < clock[0] for token in due.pop(when)]
            if tokens:
                corner = (j, pl.ds(row, 8), pl.ds(0, 128))
                ref[corner] = functools.reduce(jnp.bitwise_or, tokens, ref[corner])
            return ref[j]

        def row_stats(t, n):
            xx = x_v[rows_at(t * T + n * 32, 32), :].astype(F32)
            mean = jnp.mean(xx, axis=-1, keepdims=True)
            d = xx - mean
            scale = jax.lax.rsqrt(jnp.mean(d * d, axis=-1, keepdims=True) + EPS)
            stat_v[0, rows_at(n * 32, 32), :] = jnp.broadcast_to(mean, (32, 128))
            stat_v[1, rows_at(n * 32, 32), :] = jnp.broadcast_to(scale, (32, 128))

        def normalized(t, offset, lanes):
            wide = lambda k: jnp.concatenate([stat_v[k, pl.ds(offset, 16), :]] * (LW // 128), axis=1)
            return (x_v[rows_at(t * T + offset, 16), lanes].astype(F32) - wide(0)) * wide(1)

        def norm1_unit(rows, n, shift=True, delay=0):
            group, part = divmod(n, HD // LW)
            blocks = []
            for col in (part * LW, HD + part * LW):
                for offset in (group * 16, HT + group * 16):
                    lanes = pl.ds(col, LW)
                    hh = rows(offset, lanes).reshape(2, 8, LW) * mod_v[1, :, lanes]
                    blocks.append((hh + mod_v[0, :, lanes] if shift else hh).reshape(16, LW))
            words = [_pack(term) for term in _rhs_terms(*blocks)]
            if delay:
                finish_within(delay, *words)

            def store(target):
                for j, w in enumerate(words):
                    target[j, pl.ds(group * 8, 8), pl.ds(part * LW, LW)] = w

            return store

        def strassen(product, tiles, cycles, extra):
            products = []
            for j in range(7):
                products.append([product(j, k) for k in range(tiles)])
                latest["m"] = products[j][-1][-16:]
                side.spent(cycles)
                extra()
            return products

        def scores(i, source, extra, consume, RC):
            cost = kcost * RC // 256
            tiles = HT // 128
            for r in range(0, HD, RC):
                products = strassen(
                    lambda j, k: _dot(
                        _unpack(jnp.concatenate(
                            [(wq_v, wk_v)[i][g][j] for g in range(r // 128, (r + RC) // 128)], axis=0)),
                        _unpack(gated(source, j, k * 64)[k * 64:(k + 1) * 64]), NT),
                    tiles, RC * HT // 128, extra)

                def unit(half, o, products=products, r=r):
                    for part in range(2):
                        phi = jnp.concatenate(
                            [_features(_quadrant(2 * half + part, lambda j: products[j][k][o:o + 64]))
                             for k in range(tiles)], axis=1)
                        consume((half * HD + r + o) // 64, pl.ds(part * HT, HT), phi.astype(BF16))

                for half in range(2):
                    for o in range(0, RC, 64):
                        side.defer(cost, functools.partial(unit, half, o))

        def key_features(pair, lanes, phi):
            phik_v[pair, :, lanes] = phi

        def query_features(t, pair, lanes, phi):
            phiq_v[t, pair, :, lanes] = phi

        def store_values(col, part, v):
            v = v.T.astype(BF16).reshape(2, 64, HT)
            vt_v[pl.ds(col // 64, 2), pl.ds(0, 64), pl.ds(part * HT, HT)] = v

        def values(source, extra, consume, VC):
            tiles = VC // 128
            for r in range(0, HD, VC):
                products = strassen(
                    lambda j, k: _dot(_unpack(source[j]), _unpack(gated(wv_v[r // 128 + k], j))),
                    tiles, VC * HT // 128, extra)

                def unit(half, part, k, products=products, r=r):
                    consume(half * HD + r + k * 128, part, _quadrant(2 * half + part, lambda j: products[j][k]))

                for half in range(2):
                    for part in range(2):
                        for k in range(tiles):
                            side.defer(vcost // 2, functools.partial(unit, half, part, k))

        def accumulate_kv(j, first):
            kv = _dot(vt_v[j], phik_v[j], NT)
            kv_v[j] = kv if first else kv_v[j] + kv
            latest["m"] = kv[-16:]
            side.spent(T // 8)

        def finish_kv(j):
            row = jax.lax.broadcasted_iota(I32, (80, 128), 0)
            row_head = jnp.where(row < 64, row >> 5, (row >> 3) & 1)
            col_head = jax.lax.broadcasted_iota(I32, (80, 128), 1) & 1
            kvb_v[j] = _pack(jnp.where(row_head == col_head, kv_v[j], 0.0))

        def follow(plan):
            count = [0]

            def extra():
                count[0] += 1
                for task in plan.pop(count[0], ()):
                    task()

            for task in plan.pop(0, ()):
                task()
            return extra

        def all_kv(first):
            for r in range(0, HD, VC):
                for half in range(2):
                    for o in range(0, VC, 64):
                        accumulate_kv((half * HD + r + o) // 64, first)
            side.drain()

        def next_norm(t, n, delay):
            for block in (n // 2, T // 64 + n // 2) if n % 2 == 0 else ():
                row_stats(t, block)
            return norm1_unit(functools.partial(normalized, t), n, delay=delay)

        def plan_modulation(plan, t, first, last):
            steps = 2 * MW // 128
            for n in range(steps):
                plan[first + (last - first) * n // steps].append(
                    functools.partial(modulation, 2 * D + t * MW + n // 2 * 128, 128, n % 2))

        def attend(t, part, target, i):
            lanes = pl.ds(part * HT, HT)
            outs = {}
            tasks = []
            for half in range(2):
                for k in range(2):
                    p = half * (NPAIR // 2) + 2 * i + k
                    num = _dot(_unpack(kvb_v[p]), phiq_v[t, p, :, lanes])

                    def unit(num=num, key=(half, k)):
                        outs[key] = [_apply(jnp.multiply, num[h * DH:(h + 1) * DH],
                                            _recip(num[64 + 8 * h:72 + 8 * h] + 1e-6)) for h in range(2)]

                    tasks.append(unit)

            def terms_unit():
                lo, hi = (jnp.concatenate(outs[half, 0] + outs[half, 1], axis=0).T for half in range(2))
                for q, term in enumerate(_lhs_terms(lo[:G], hi[:G], lo[G:], hi[G:])):
                    target[q, :, pl.ds(i * 128, 128)] = _pack(term)

            return tasks + [terms_unit]

        def output_weights():
            w = wr_v[...].astype(F32)
            w = jnp.concatenate([jnp.broadcast_to(w[j:j + 1], (8, 128)) for j in range(D // 128)], axis=1)
            for i in range(2, 6):
                mod_v[i] = raw(i) + 1.0 if i == 4 else raw(i)
            mod_v[6] = mod_v[4] * w
            mod_v[7] = mod_v[4] * mod_v[5]
            mod_v[8] = mod_v[3] * mod_v[5]
            mod_v[9] = jnp.broadcast_to(jnp.sum(mod_v[3] * w, axis=1, keepdims=True), (8, D))

        ranks = {}

        def finish_rows(base, y, chain):
            lane = jax.lax.broadcasted_iota(I32, (8, 128), 1)
            acc = ranks.get(base >> 10, jnp.full((8, 128), -jnp.inf, F32))
            for o in range(0, y.shape[0], 8):
                rows = rows_at(base + o, 8)
                xn = x_v[rows, :].astype(F32) + mod_v[2] * chain.enter(y[o:o + 8])
                mean = jnp.mean(xn, axis=-1, keepdims=True)
                d = xn - mean
                scale = jax.lax.rsqrt(jnp.mean(d * d, axis=-1, keepdims=True) + EPS)
                score = jnp.sum(d * mod_v[6], axis=-1, keepdims=True) * scale + mod_v[9, :, :1]
                normed = d * scale
                xn_v[rows, :] = normed
                out = normed * mod_v[7] + ((d + mean) + mod_v[8])
                out_v[rows, :] = out.astype(BF16)
                acc = jnp.where(lane == ((base + o) & 1023) >> 3, score, acc)
                chain.leave(*[out[:, l:l + 128] for l in range(128, D, 256)])
            ranks[base >> 10] = acc

        tokens = collections.deque()

        def mix(source, lo, n, extra):
            return strassen(
                lambda j, k: _dot(_unpack(gated(source, j, lo // 2)[lo // 2:(lo + n) // 2]),
                                  _unpack(wot_v[j, :, pl.ds(k * 128, 128)])),
                HD // 128, 4 * n, extra)

        def mixed_rows(product, n):
            def rows_of(o):
                part, o = divmod(o, n)
                return jnp.concatenate(
                    [_quadrant(2 * part + half, lambda j: product(j, o)) for half in range(2)], axis=1)
            return rows_of

        def from_values(products):
            return lambda j, o: jnp.concatenate([tile[o:o + EC] for tile in products[j]], axis=1)

        def top2():
            shape = (S // 1024, 8, 128)
            idx = (jax.lax.broadcasted_iota(I32, shape, 0) * 1024 + jax.lax.broadcasted_iota(I32, shape, 2) * 8
                   + jax.lax.broadcasted_iota(I32, shape, 1)).astype(F32)
            m = jnp.stack([ranks[b] for b in range(S // 1024)])
            reduce = lambda op, v: op(op(op(v, axis=0), axis=0, keepdims=True), axis=1, keepdims=True)
            picks = []
            for _ in range(2):
                top = reduce(jnp.max, m)
                first = reduce(jnp.min, jnp.where(m == top, idx, float(S - 1)))
                picks.append((jnp.max(first.astype(I32)), top))
                m = jnp.where(idx == first, -jnp.inf, m)
            return picks

        def experts():
            (i1, m1), (i2, m2) = top2()
            picks = [jnp.clip(i, 0, S - 1) for i in (i1, i2)]
            bases = [pl.multiple_of((i >> 4) * 16, 16) for i in picks]
            sub = jax.lax.broadcasted_iota(I32, (16, D), 0)
            first, second = (jnp.broadcast_to(xn_v[pl.ds(i, 1), :], (16, D)) for i in picks)
            sel = jnp.where(sub == 0, first, second).reshape(2, 8, D) * mod_v[4] + mod_v[3]
            sel = sel.reshape(16, D).astype(BF16)
            y = None
            acts = collections.deque()

            def down():
                nonlocal y
                f, g, u = acts.popleft()
                act = (g * jax.nn.sigmoid(g) * u).astype(BF16)
                part = _dot(act, wd_v[pl.ds(f, FC), :])
                y = part if y is None else y + part

            for f in range(0, FF, FC):
                acts.append((f, _dot(sel, wg_v[:, pl.ds(f, FC)]), _dot(sel, wu_v[:, pl.ds(f, FC)])))
                if len(acts) > flag:
                    down()
            while acts:
                down()
            y1, y2 = y[0:1] * jax.nn.sigmoid(m1), y[1:2] * jax.nn.sigmoid(m2)
            for n, base in enumerate(bases):
                upd = jnp.where(sub == picks[0] - base, y1, 0.0) + jnp.where(sub == picks[1] - base, y2, 0.0)
                full = out_v[pl.ds(base, 16), :].astype(F32).reshape(2, 8, D) + mod_v[5] * upd.reshape(2, 8, D)
                fix_v[n] = full.reshape(16, D).astype(BF16)
            return bases

        cc = c_v[...].astype(F32)
        act_v[...] = _pack(jnp.broadcast_to(cc * jax.nn.sigmoid(cc), (16, D)))
        with scope("w_x0"):
            x_copy(0).wait()
        for n in range(T // 32):
            row_stats(0, n)
        for offset in range(0, T, 16) if keep else ():
            for col in range(0, D, LW):
                xn_v[pl.ds(offset, 16), pl.ds(col, LW)] = normalized(0, offset, pl.ds(col, LW))
        for n in range(2):
            wait(("scale", n))
            modulation(D, D, n)
        mod_v[1] = raw(1) + 1.0
        units = HT // 16 * (HD // LW)
        saved = (lambda offset, lanes: xn_v[pl.ds(offset, 16), lanes]) if keep else functools.partial(normalized, 0)
        for n in range(units):
            norm1_unit(saved, n, shift=False)(h0_v)

        def hold_values(col, part, v):
            xn_v[pl.ds(T + part * HT, HT), pl.ds(col, 128)] = v

        def shift_and_bias():
            wait("shift")
            modulation(0, D)
            mod_v[0] = raw(0)

        def release_values(col, part):
            v = xn_v[pl.ds(T + part * HT, HT), pl.ds(col, 128)]
            store_values(col, part, _apply(jnp.add, v, bias_v[:, pl.ds(col, 128)]))

        wait(*both("wv", 0))
        prep_values(0)
        plan = collections.defaultdict(list)
        plan[3] += [lambda: wait(*both("wv", 1)), lambda: prep_values(1)]
        plan[7] += [lambda: wait(*both("wv", 2))]
        plan[8] += [lambda: prep_values(2)]
        plan[15] += [lambda: prep_values(3)]
        plan[sa_at].append(shift_and_bias)
        with scope("values0"):
            values(h0_v, follow(plan), hold_values, 128)
            side.drain()
        assert not plan
        wait("wphi", *both("wk", 0))
        block_diag_phi()
        prep_scores(1, 0)
        prep_scores(1, 1)
        shift = jnp.concatenate([raw(0)] * 2, axis=0).astype(BF16)
        bias_v[...] = _dot(shift, wqkv_v[:, pl.ds(2 * D, D)])[:8]
        for n in range(units):
            norm1_unit(saved, n)(h0_v)

        plan = collections.defaultdict(list)
        def initialize():
            vt_v[:, pl.ds(64, 16), :] = jnp.ones((NPAIR, 16, T), BF16)

        plan[0].append(initialize)
        plan[k_at] += [lambda: wait(*both("wk", 1)), lambda: prep_scores(1, 2), lambda: prep_scores(1, 3)]
        for n in range(16):
            plan[1 + n * 8 // 16].append(functools.partial(release_values, n // 2 * 128, n % 2))
        plan[k_at].insert(0, lambda: x_copy(1).wait())

        second_norm = lambda n, delay: next_norm(1, n, delay)(ht_v)
        for n, (slot, delay) in enumerate(slots0):
            plan[slot].append(functools.partial(second_norm, n, delay))
        with scope("tile0"):
            scores(1, h0_v, follow(plan), key_features, RC)
            assert not plan
            wait("wq")
            for g in range(4):
                prep_scores(0, g)
                side.spent(512)
            side.drain()
            for n in range(len(slots0), units):
                second_norm(n, 0)
            all_kv(True)

        def first_step(t):
            wait(("mod", t))
            if t + 1 < NTILE:
                x_copy(t + 1).wait()

            if ffn == 0 and t == 1:
                start("wg", "wu", "wd", priority=1)
            if ffn == 1:
                start(("wg", "wu", "wd")[t - 1])
            if ffn == 2:
                start(("wg", "wu", "wd")[t - 1], priority=1)
            plan = collections.defaultdict(list)
            stores = []
            if t + 1 < NTILE:
                for n, (slot, delay) in enumerate(slots1):
                    plan[slot].append(functools.partial(
                        lambda n, delay: stores.append(next_norm(t + 1, n, delay)), n, delay))
                plan[2 * nk + nv].append(lambda: [store(ht_v) for store in stores])
            if t == NTILE - 1:
                for n, slot in enumerate(pslots[0]):
                    plan[slot].append(functools.partial(prep_output, n))
            plan_modulation(plan, t, mfirst, mlast)
            due.clear()
            extra = follow(plan)
            scores(1, ht_v, extra, key_features, RC)
            scores(0, ht_v, extra, functools.partial(query_features, t), RC)
            values(ht_v, extra, store_values, VC)
            assert not plan
            side.drain()
            all_kv(False)

        with scope("pass1"):
            for t in range(1, NTILE):
                first_step(t)
        if only == 1:
            for j in range(NPAIR):
                finish_kv(j)
            out_v[pl.ds(0, 64), pl.ds(0, 512)] = phiq_v[zero, zero, pl.ds(0, 64), :]
            out_v[pl.ds(64, 80), pl.ds(0, 128)] = _unpack(kvb_v[zero])
            out_v[pl.ds(160, 64), pl.ds(0, 512)] = _unpack(wot_v[zero, pl.ds(0, 32), :])
            out_copy(0).start()
            out_copy(0).wait()
            return

        wait(("mod", 0), "wo", "wr", "wg", "wu", "wd")
        order = [(n + 2) % NSUB for n in range(NSUB)]
        plan = collections.defaultdict(list)
        plan[0] += [functools.partial(finish_kv, j) for j in range(NPAIR)]

        def first_attention():
            tasks = [task for i in range(4) for task in attend(order[0] // 2, order[0] % 2, oa_v, i)]
            for task in tasks:
                task()

        plan[a_at].append(first_attention)
        plan_modulation(plan, 0, m0, m1)
        left = range(len(pslots[0]), HD // 16)
        for i, n in enumerate(left):
            plan[pslots[1][len(pslots[1]) * i // len(left)]].append(functools.partial(prep_output, n))
        plan[m1].append(output_weights)
        due.clear()
        scores(0, h0_v, follow(plan), functools.partial(query_features, 0), RC0)

        def finish(base, rows_of, rows, strands, delay):
            chain = Chain(strands)
            for o in range(0, rows, EC):
                row, y = rows_of(o)
                finish_rows(base + row, y, chain)
            if delay:
                finish_within(delay, *chain.tokens)

        def mixed(source, lo, n, plan):
            rows_of = mixed_rows(from_values(mix(source, lo, n, follow(plan))), n)
            return lambda o: (lo + o // n * G + o % n, rows_of(o))

        rows_of = None
        sent = []
        due.clear()
        with scope("pass2"):
            for n in range(NSUB):
                source, target = ((oa_v, ob_v), (ob_v, oa_v))[n % 2]
                plan = collections.defaultdict(list)

                def attention(i):
                    for task in attend(order[n + 1] // 2, order[n + 1] % 2, target, i):
                        task()

                split = tail and n + 1 == NSUB
                if n + 1 < NSUB and att_at is None:
                    tasks = [task for i in range(4) for task in attend(order[n + 1] // 2, order[n + 1] % 2, target, i)]
                    for task in tasks:
                        task()
                elif n + 1 < NSUB:
                    for i in range(4):
                        plan[att_at[i]].append(functools.partial(attention, i))
                if rows_of:
                    at = att_at[-1] if att_at and n + 1 < NSUB else 0
                    plan[at].append(functools.partial(
                        finish, order[n - 1] * 2 * G, rows_of, 2 * G, ne_tail if split else ne, edelay - 4 * at))
                if not split:
                    rows_of = mixed(source, 0, G, plan)
                    left = 2 * G
                else:
                    rows_of = mixed(source, 0, G - tail, plan)
                    finish(order[n] * 2 * G, rows_of, 2 * (G - tail), ne_tail, edelay)
                    rows_of = mixed(source, G - tail, tail, plan)
                    left = 2 * tail
                if n > 1:
                    out_copy(order[n - 2]).start()
                    sent.append(order[n - 2])
                if n in barriers:
                    while len(sent) > 1:
                        out_copy(sent.pop(0)).wait()
        with scope("last"):
            finish(order[-1] * 2 * G, rows_of, left, nl, 0)
        out_copy(order[-2]).start()
        sent.append(order[-2])
        out_copy(order[-1]).start()
        sent.append(order[-1])
        with scope("experts"):
            b1, b2 = experts()
        with scope("w_out"):
            for n in sent:
                out_copy(n).wait()
        fix = [pltpu.make_async_copy(fix_v.at[n], out_hbm.at[pl.ds(b, 16)], osems.at[n])
               for n, b in enumerate((b1, b2))]
        fix[0].start()

        @pl.when(b1 != b2)
        def _():
            fix[1].start()
            fix[1].wait()

        fix[0].wait()

    nsem = NTILE + 3 + 3 + NTILE + 1 + 10 + 4
    scratch = [
        pltpu.VMEM((S + 16, D), BF16), pltpu.VMEM((D, 3 * D), BF16), pltpu.VMEM((D, DH), BF16),
        pltpu.VMEM((D + 16, D), BF16), pltpu.VMEM((8, 128), BF16),
        pltpu.VMEM((D, FF), BF16), pltpu.VMEM((D, FF), BF16), pltpu.VMEM((FF, D), BF16),
        pltpu.VMEM((1, D), BF16), pltpu.VMEM((D, 6 * D), BF16),
        pltpu.VMEM((8, D), U32),
        pltpu.VMEM((8, 6 * D), F32),
        pltpu.VMEM((10, 8, D), F32),
        pltpu.VMEM((2, T, 128), F32),
        pltpu.VMEM((8, D), F32),
        pltpu.VMEM((D // 128, 64, 128), U32),
        pltpu.VMEM((7, HD // 2, HD), U32),
        pltpu.VMEM((7, HT // 2, HD), U32),
        pltpu.VMEM((7, HT // 2, HD), U32),
        pltpu.VMEM((NTILE, NPAIR, 128, T), BF16),
        pltpu.VMEM((NPAIR, 128, T), BF16),
        pltpu.VMEM((NPAIR, 80, T), BF16),
        pltpu.VMEM((NPAIR, 80, 128), F32),
        pltpu.VMEM((NPAIR, 40, 128), U32),
        pltpu.VMEM((7, G // 2, HD), U32),
        pltpu.VMEM((7, G // 2, HD), U32),
        pltpu.VMEM((S, D), F32),
        pltpu.VMEM((S, D), BF16),
        pltpu.VMEM((2, 16, D), BF16),
        pltpu.SemaphoreType.DMA((nsem,)),
        pltpu.SemaphoreType.DMA((NSUB,)),
    ] + [pltpu.VMEM((7, 64, HD), U32)] * 8 + [pltpu.VMEM((7, HD // 2, 128), U32)] * 4

    def fn(A_x, A_wqkv, A_w_phi, A_wo, B_x, B_w_r, B_w_gate, B_w_up, B_w_down, c, w_mod):
        del B_x
        out = pl.pallas_call(
            kernel,
            out_shape=jax.ShapeDtypeStruct((S, D), A_x.dtype),
            in_specs=[pl.BlockSpec(memory_space=pl.ANY)] * 10,
            out_specs=pl.BlockSpec(memory_space=pl.ANY),
            scratch_shapes=scratch,
            compiler_params=pltpu.CompilerParams(vmem_limit_bytes=vlimit * 2**20, flags=flags),
        )(A_x.reshape(S, D), A_wqkv, A_w_phi.reshape(D, DH), A_wo, B_w_r.reshape(8, 128),
          B_w_gate, B_w_up, B_w_down, c, w_mod)
        return out.reshape(A_x.shape)

    return fn


@jax.jit
def pallas_adaLN_cond__linear_kernel_hedgehog__moe_arch_mod__prompt_kernel(
    A_x, A_wqkv, A_w_phi, A_wo, B_x, B_w_r, B_w_gate, B_w_up, B_w_down, c, w_mod
):
    return make()(A_x, A_wqkv, A_w_phi, A_wo, B_x, B_w_r, B_w_gate, B_w_up, B_w_down, c, w_mod)
```

```python
import collections
import functools

import jax
import jax.numpy as jnp
import numpy as np
import jax.experimental.pallas as pl
import jax.experimental.pallas.tpu as pltpu

F32, BF16, I32, U32 = jnp.float32, jnp.bfloat16, jnp.int32, jnp.uint32
S, D, HEADS, DH, FF = 2048, 1024, 32, 32, 3584
EPS = 1e-5
LOG2E = float(np.log2(np.e))

HD = D // 2
NPAIR = HEADS // 2
T = 512
HT = T // 2
NTILE = S // T
G = 128
NSTEP = S // (2 * G)
MOD_COLS = 4 * D // NTILE
NORM_UNITS = HT // 16
FF_CHUNK = 256

NN = (((1,), (0,)), ((), ()))
NT = (((1,), (1,)), ((), ()))


def _dot(a, b, dims=NN):
    return jax.lax.dot_general(a, b, dims, preferred_element_type=F32)


def _pack(x):
    n = x.shape[0] // 2
    if x.shape[1] > 128:
        return pltpu.bitcast(x.astype(BF16), U32)
    w = pltpu.bitcast(jnp.concatenate([x[:n], x[n:]], axis=1).astype(BF16), U32)
    return jnp.concatenate([w[:, :128], w[:, 128:]], axis=0)


def _unpack(w):
    return pltpu.bitcast(w, BF16)


def _recip(x):
    r = pl.reciprocal(x, approx=True)
    return r * (2.0 - x * r)


def _lhs_terms(a11, a12, a21, a22):
    return (a11 + a22, a21 + a22, a11, a22, a11 + a12, a21 - a11, a12 - a22)


def _rhs_terms(b11, b12, b21, b22):
    return (b11 + b22, b11, b12 - b22, b21 - b11, b22, b11 + b12, b21 + b22)


_QUADRANTS = (((0, 1), (3, 1), (4, -1), (6, 1)), ((2, 1), (4, 1)), ((1, 1), (3, 1)),
              ((0, 1), (1, -1), (2, 1), (5, 1)))


def _quadrant(q, product):
    total = None
    for j, sign in _QUADRANTS[q]:
        m = product(j)
        total = m if total is None else (total + m if sign > 0 else total - m)
    return total


def _per_head(op, p):
    parts = [p[r:r + 8] for r in range(0, p.shape[0], 8)]
    while len(parts) > 1:
        parts = [op(a, b) for a, b in zip(parts[::2], parts[1::2])]
    out = op(parts[0], pltpu.roll(parts[0], 4, 0))
    return op(out, pltpu.roll(out, 2, 0))


def _apply(op, p, rows8):
    return op(p.reshape(p.shape[0] // 8, 8, p.shape[1]), rows8).reshape(p.shape)


def _features(p):
    e_pos = jnp.exp2(_apply(jnp.subtract, p, _per_head(jnp.maximum, p)))
    e_neg = jnp.exp2(_apply(lambda a, low: low - a, p, _per_head(jnp.minimum, p)))
    pos = _apply(jnp.multiply, e_pos, _recip(_per_head(jnp.add, e_pos)))
    neg = _apply(jnp.multiply, e_neg, _recip(_per_head(jnp.add, e_neg)))
    return jnp.concatenate([pos, neg], axis=0)


def _interleaved_source(row):
    return (row & ~63) + ((row & 1) << 5) + ((row & 63) >> 1)


class _Backlog:
    def __init__(self):
        self.queue = collections.deque()
        self.credit = 0.0

    def defer(self, cost, task):
        self.queue.append((cost, task))

    def spent(self, cycles):
        self.credit += 0.55 * cycles
        while self.queue and self.credit >= self.queue[0][0]:
            cost, task = self.queue.popleft()
            self.credit -= cost
            task()
        if not self.queue:
            self.credit = 0.0

    def drain(self):
        while self.queue:
            self.queue.popleft()[1]()
        self.credit = 0.0


def _follow(plan):
    count = 0

    def step():
        nonlocal count
        count += 1
        for task in plan.pop(count, ()):
            task()

    for task in plan.pop(0, ()):
        task()
    return step


def _kernel(x_hbm, wqkv_hbm, wphi_hbm, wo_hbm, wr_hbm, wg_hbm, wu_hbm, wd_hbm, c_hbm, wmod_hbm,
            out_hbm,
            x_v, wqkv_v, wphi_v, wo_v, wr_v, wg_v, wu_v, wd_v, c_v, wmod_v,
            act_v, raw_v, mod_v, stat_v, bias_v, fold_v, wot_v, h_v, h0_v,
            phiq_v, phik_v, vt_v, kv_v, summary_v, oa_v, ob_v, norm_v, out_v, fix_v,
            in_sems, out_sems, *terms_v):
    wq_v, wk_v, wv_v = terms_v[:4], terms_v[4:8], terms_v[8:]
    backlog = _Backlog()
    new_plan = lambda: collections.defaultdict(list)

    copies = {}

    def add_copy(name, src, dst, part=Ellipsis):
        if part is not Ellipsis:
            src, dst = src.at[part], dst.at[part]
        copies[name] = pltpu.make_async_copy(src, dst, in_sems.at[len(copies)])

    columns = lambda lo, n: (pl.ds(0, D), pl.ds(lo, n))
    for name, src, dst in (("c", c_hbm, c_v), ("wphi", wphi_hbm, wphi_v), ("wr", wr_hbm, wr_v),
                           ("wo", wo_hbm, wo_v), ("wg", wg_hbm, wg_v), ("wu", wu_hbm, wu_v),
                           ("wd", wd_hbm, wd_v)):
        add_copy(name, src, dst)
    add_copy("wq", wqkv_hbm, wqkv_v, columns(0, D))
    for t in range(NTILE):
        add_copy(("x", t), x_hbm, x_v, pl.ds(t * T, T))
        add_copy(("mod", t), wmod_hbm, wmod_v, columns(2 * D + t * MOD_COLS, MOD_COLS))
    for half in range(2):
        add_copy(("shift", half), wmod_hbm, wmod_v, (pl.ds(half * HD, HD), pl.ds(0, D)))
        add_copy(("scale", half), wmod_hbm, wmod_v, (pl.ds(half * HD, HD), pl.ds(D, D)))
        for n in range(2):
            add_copy(("wk", n, half), wqkv_hbm, wqkv_v, columns(D + half * HD + n * 256, 256))
        for n, (lo, size) in enumerate(((0, 128), (128, 128), (256, 256))):
            add_copy(("wv", n, half), wqkv_hbm, wqkv_v, columns(2 * D + half * HD + lo, size))
    both = lambda *name: ((*name, 0), (*name, 1))

    def start(*names):
        for name in names:
            copies[name].start()

    def wait(*names):
        for name in names:
            copies[name].wait()

    def out_copy(step):
        rows = pl.ds(step * 2 * G, 2 * G)
        return pltpu.make_async_copy(out_v.at[rows], out_hbm.at[rows], out_sems.at[step])

    start("c", ("x", 0), *both("scale"), *both("wv", 0), *both("wv", 1), *both("wv", 2), "wphi",
          *both("wk", 0), *both("shift"), *both("wk", 1), ("x", 1), "wq",
          ("x", 2), ("mod", 1), ("x", 3), ("mod", 2), ("mod", 3), "wo", ("mod", 0), "wr")
    wait("c")

    bits = pltpu.bitcast(jnp.broadcast_to(c_v[:, :128].astype(F32), (8, 128)), I32)
    zero = jnp.minimum(jnp.max(bits & 0xFF), 0)

    class Chain:
        def __init__(self, strands):
            self.tokens = collections.deque([None] * strands)

        def enter(self, rows8):
            token = self.tokens.popleft()
            if token is None:
                return rows8
            head = pltpu.bitcast(pltpu.bitcast(rows8[:, :128], I32) | token, F32)
            return jnp.concatenate([head, rows8[:, 128:]], axis=1)

        def leave(self, *values):
            words = [pltpu.bitcast(value, I32) for value in values]
            self.tokens.append(functools.reduce(jnp.bitwise_or, words) & zero)

    clock = 0
    due = collections.defaultdict(list)

    def finish_within(delay, *values):
        parts = [pltpu.bitcast(value, U32)[r:r + 8, l:l + 128] for value in values
                 for r in range(0, value.shape[0], 8) for l in range(0, value.shape[1], 128)]
        due[clock + delay].append(functools.reduce(jnp.bitwise_or, parts) & zero.astype(U32))

    def gated(ref, j, row=0):
        nonlocal clock
        clock += 1
        tokens = [token for when in sorted(due) if when < clock for token in due.pop(when)]
        if tokens:
            corner = (j, pl.ds(row, 8), pl.ds(0, 128))
            ref[corner] = functools.reduce(jnp.bitwise_or, tokens, ref[corner])
        return ref[j]

    def modulation(lo, n, half):
        rows, lanes = pl.ds(half * HD, HD), pl.ds(lo, n)
        m = _dot(_unpack(act_v[:, rows]), wmod_v[rows, lanes])[:8]
        raw_v[:, lanes] = raw_v[:, lanes] + m if half else m

    raw = lambda i: raw_v[:, pl.ds(i * D, D)]

    def plan_modulation(plan, t, first, last):
        steps = 2 * MOD_COLS // 128
        for n in range(steps):
            plan[first + (last - first) * n // steps].append(
                functools.partial(modulation, 2 * D + t * MOD_COLS + n // 2 * 128, 128, n % 2))

    def output_weights():
        w = wr_v[...].astype(F32)
        w = jnp.concatenate([jnp.broadcast_to(w[j:j + 1], (8, 128)) for j in range(D // 128)], axis=1)
        for i in range(2, 6):
            mod_v[i] = raw(i) + 1.0 if i == 4 else raw(i)
        mod_v[6] = mod_v[4] * w
        mod_v[7] = mod_v[4] * mod_v[5]
        mod_v[8] = mod_v[3] * mod_v[5]
        mod_v[9] = jnp.broadcast_to(jnp.sum(mod_v[3] * w, axis=1, keepdims=True), (8, D))

    def feature_maps():
        row = _interleaved_source(jax.lax.broadcasted_iota(I32, (128, DH), 0))
        col = jax.lax.broadcasted_iota(I32, (128, DH), 1)
        select = jnp.where((row & (DH - 1)) == col, 1.0, 0.0).astype(BF16)
        row_head = _interleaved_source(jax.lax.broadcasted_iota(I32, (128, 128), 0)) >> 5
        col_head = jax.lax.broadcasted_iota(I32, (128, 128), 1) >> 5
        for g in range(D // 128):
            tiled = _dot(select, wphi_v[pl.ds(g * 128, 128), :], NT)
            fold_v[g] = _pack(jnp.where(row_head == col_head, tiled, 0.0))

    def prep_scores(i, g):
        blocks = []
        for group in (g, g + HD // 128):
            for half in range(2):
                w = wqkv_v[pl.ds(half * HD, HD), pl.ds(i * D + group * 128, 128)]
                blocks.append(_dot(_unpack(fold_v[group]), w, NT) * LOG2E)
        for j, term in enumerate(_lhs_terms(*blocks)):
            (wq_v, wk_v)[i][g][j] = _pack(term)

    def prep_values(g):
        chain = Chain(1)
        for r in range(0, HD, 64):
            blocks = [wqkv_v[pl.ds(row + r, 64), pl.ds(2 * D + col + g * 128, 128)].astype(F32)
                      for col in (0, HD) for row in (0, HD)]
            token = chain.tokens.popleft()
            if token is not None:
                head = pltpu.bitcast(pltpu.bitcast(blocks[3][:8], I32) | token, F32)
                blocks[3] = jnp.concatenate([head, blocks[3][8:]], axis=0)
            for j, term in enumerate(_lhs_terms(*blocks)):
                words = _pack(term)
                wv_v[g][j, pl.ds(r // 2, 32), :] = words
            chain.leave(words[:8])

    def prep_output(n):
        lo = wo_v[pl.ds(n * 16, 16), :].astype(F32)
        hi = wo_v[pl.ds(HD + n * 16, 16), :].astype(F32)
        words = [_pack(term) for term in _rhs_terms(lo[:, :HD], lo[:, HD:], hi[:, :HD], hi[:, HD:])]
        for j, w in enumerate(words):
            wot_v[j, pl.ds(n * 8, 8), :] = w
        finish_within(2, *words)

    def row_stats(t, n):
        xx = x_v[pl.ds(t * T + n * 32, 32), :].astype(F32)
        mean = jnp.mean(xx, axis=-1, keepdims=True)
        d = xx - mean
        scale = jax.lax.rsqrt(jnp.mean(d * d, axis=-1, keepdims=True) + EPS)
        stat_v[0, pl.ds(n * 32, 32), :] = jnp.broadcast_to(mean, (32, 128))
        stat_v[1, pl.ds(n * 32, 32), :] = jnp.broadcast_to(scale, (32, 128))

    def normalized(t, offset, lanes):
        wide = lambda k: jnp.concatenate([stat_v[k, pl.ds(offset, 16), :]] * (HD // 128), axis=1)
        return (x_v[pl.ds(t * T + offset, 16), lanes].astype(F32) - wide(0)) * wide(1)

    def norm_terms(rows, n, shift=True, delay=0):
        blocks = []
        for lanes in (pl.ds(0, HD), pl.ds(HD, HD)):
            for offset in (n * 16, HT + n * 16):
                hh = rows(offset, lanes).reshape(2, 8, HD) * mod_v[1, :, lanes]
                blocks.append((hh + mod_v[0, :, lanes] if shift else hh).reshape(16, HD))
        words = [_pack(term) for term in _rhs_terms(*blocks)]
        if delay:
            finish_within(delay, *words)

        def store(target):
            for j, w in enumerate(words):
                target[j, pl.ds(n * 8, 8), :] = w

        return store

    def tile_norm(t, n, delay):
        if n % 2 == 0:
            row_stats(t, n // 2)
            row_stats(t, HT // 32 + n // 2)
        return norm_terms(functools.partial(normalized, t), n, delay=delay)

    def products(product, tiles, cycles, hook):
        result = []
        for j in range(7):
            result.append([product(j, k) for k in range(tiles)])
            backlog.spent(cycles)
            hook()
        return result

    def features(weights, source, hook, target, rows):
        for r in range(0, HD, rows):
            m = products(
                lambda j, k: _dot(
                    _unpack(jnp.concatenate([weights[g][j] for g in range(r // 128, (r + rows) // 128)], axis=0)),
                    _unpack(gated(source, j, k * 64)[k * 64:(k + 1) * 64]), NT),
                HT // 128, rows * HT // 128, hook)

            def unit(half, o, m=m, r=r):
                for part in range(2):
                    phi = jnp.concatenate(
                        [_features(_quadrant(2 * half + part, lambda j: m[j][k][o:o + 64]))
                         for k in range(HT // 128)], axis=1)
                    target((half * HD + r + o) // 64, pl.ds(part * HT, HT), phi.astype(BF16))

            for half in range(2):
                for o in range(0, rows, 64):
                    backlog.defer(150 * rows // 256, functools.partial(unit, half, o))

    def store_keys(pair, lanes, phi):
        phik_v[pair, :, lanes] = phi

    def store_queries(t, pair, lanes, phi):
        phiq_v[t, pair, :, lanes] = phi

    def store_values(col, part, v):
        v = v.T.astype(BF16).reshape(2, 64, HT)
        vt_v[pl.ds(col // 64, 2), pl.ds(0, 64), pl.ds(part * HT, HT)] = v

    def values(source, hook, target, cols):
        for r in range(0, HD, cols):
            m = products(
                lambda j, k: _dot(_unpack(source[j]), _unpack(gated(wv_v[r // 128 + k], j))),
                cols // 128, cols * HT // 128, hook)

            def unit(half, part, k, m=m, r=r):
                target(half * HD + r + k * 128, part, _quadrant(2 * half + part, lambda j: m[j][k]))

            for half in range(2):
                for part in range(2):
                    for k in range(cols // 128):
                        backlog.defer(128, functools.partial(unit, half, part, k))

    def accumulate_summary(first):
        backlog.drain()
        for r in range(0, HD, 256):
            for half in range(2):
                for o in range(0, 256, 64):
                    pair = (half * HD + r + o) // 64
                    kv = _dot(vt_v[pair], phik_v[pair], NT)
                    kv_v[pair] = kv if first else kv_v[pair] + kv

    def finish_summary(pair):
        row = jax.lax.broadcasted_iota(I32, (80, 128), 0)
        row_head = jnp.where(row < 64, row >> 5, (row >> 3) & 1)
        col_head = jax.lax.broadcasted_iota(I32, (80, 128), 1) & 1
        summary_v[pair] = _pack(jnp.where(row_head == col_head, kv_v[pair], 0.0))

    def attend(step, target):
        t, lanes = step // 2, pl.ds(step % 2 * 2 * G, 2 * G)
        pairs = [[[half * NPAIR // 2 + 2 * i + k for k in range(2)] for half in range(2)] for i in range(4)]
        nums = {p: _dot(_unpack(summary_v[p]), phiq_v[t, p, :, lanes])
                for group in pairs for side in group for p in side}
        for i, group in enumerate(pairs):
            heads = [[_apply(jnp.multiply, nums[p][h * DH:(h + 1) * DH],
                             _recip(nums[p][64 + 8 * h:72 + 8 * h] + 1e-6))
                      for p in side for h in range(2)] for side in group]
            lo, hi = (jnp.concatenate(side, axis=0).T for side in heads)
            for j, term in enumerate(_lhs_terms(lo[:G], hi[:G], lo[G:], hi[G:])):
                target[j, :, pl.ds(i * 128, 128)] = _pack(term)

    def project_output(source, lo, n, hook):
        m = products(
            lambda j, k: _dot(_unpack(gated(source, j, lo // 2)[lo // 2:(lo + n) // 2]),
                              _unpack(wot_v[j, :, pl.ds(k * 128, 128)])),
            HD // 128, 4 * n, hook)

        def rows(o):
            part, o = divmod(o, n)
            piece = lambda j: jnp.concatenate([tile[o:o + 32] for tile in m[j]], axis=1)
            return lo + part * G + o, jnp.concatenate(
                [_quadrant(2 * part + half, piece) for half in range(2)], axis=1)

        return rows

    scores = {}

    def finish(step, rows, count, strands, delay):
        chain = Chain(strands)
        lane = jax.lax.broadcasted_iota(I32, (8, 128), 1)
        for start_row in range(0, count, 32):
            row, y = rows(start_row)
            for o in range(0, 32, 8):
                base = step * 2 * G + row + o
                xn = x_v[pl.ds(base, 8), :].astype(F32) + mod_v[2] * chain.enter(y[o:o + 8])
                mean = jnp.mean(xn, axis=-1, keepdims=True)
                d = xn - mean
                scale = jax.lax.rsqrt(jnp.mean(d * d, axis=-1, keepdims=True) + EPS)
                score = jnp.sum(d * mod_v[6], axis=-1, keepdims=True) * scale + mod_v[9, :, :1]
                normed = d * scale
                norm_v[pl.ds(base, 8), :] = normed
                out = normed * mod_v[7] + ((d + mean) + mod_v[8])
                out_v[pl.ds(base, 8), :] = out.astype(BF16)
                held = scores.get(base // 1024, jnp.full((8, 128), -jnp.inf, F32))
                scores[base // 1024] = jnp.where(lane == base % 1024 // 8, score, held)
                chain.leave(*[out[:, l:l + 128] for l in range(128, D, 256)])
        if delay:
            finish_within(delay, *chain.tokens)

    def top_two():
        shape = (S // 1024, 8, 128)
        index = (jax.lax.broadcasted_iota(I32, shape, 0) * 1024 + jax.lax.broadcasted_iota(I32, shape, 2) * 8
                 + jax.lax.broadcasted_iota(I32, shape, 1)).astype(F32)
        left = jnp.stack([scores[b] for b in range(S // 1024)])
        reduce = lambda op, v: op(op(op(v, axis=0), axis=0, keepdims=True), axis=1, keepdims=True)
        picks = []
        for _ in range(2):
            top = reduce(jnp.max, left)
            first = reduce(jnp.min, jnp.where(left == top, index, float(S - 1)))
            picks.append((jnp.clip(jnp.max(first.astype(I32)), 0, S - 1), top))
            left = jnp.where(index == first, -jnp.inf, left)
        return picks

    def routed_update():
        (row1, score1), (row2, score2) = top_two()
        sub = jax.lax.broadcasted_iota(I32, (16, D), 0)
        first, second = (jnp.broadcast_to(norm_v[pl.ds(row, 1), :], (16, D)) for row in (row1, row2))
        selected = jnp.where(sub == 0, first, second).reshape(2, 8, D) * mod_v[4] + mod_v[3]
        selected = selected.reshape(16, D).astype(BF16)
        pending = collections.deque()
        parts = []

        def down():
            f, g, u = pending.popleft()
            act = (g * jax.nn.sigmoid(g) * u).astype(BF16)
            part = _dot(act, wd_v[pl.ds(f, FF_CHUNK), :])
            parts.append(parts.pop() + part if parts else part)

        for f in range(0, FF, FF_CHUNK):
            pending.append((f, _dot(selected, wg_v[:, pl.ds(f, FF_CHUNK)]),
                            _dot(selected, wu_v[:, pl.ds(f, FF_CHUNK)])))
            if len(pending) > 2:
                down()
        while pending:
            down()
        y1, y2 = parts[0][0:1] * jax.nn.sigmoid(score1), parts[0][1:2] * jax.nn.sigmoid(score2)
        bases = [pl.multiple_of((row >> 4) * 16, 16) for row in (row1, row2)]
        for n, base in enumerate(bases):
            update = jnp.where(sub == row1 - base, y1, 0.0) + jnp.where(sub == row2 - base, y2, 0.0)
            rows = out_v[pl.ds(base, 16), :].astype(F32).reshape(2, 8, D) + mod_v[5] * update.reshape(2, 8, D)
            fix_v[n] = rows.reshape(16, D).astype(BF16)
        return bases

    cc = c_v[...].astype(F32)
    act_v[...] = _pack(jnp.broadcast_to(cc * jax.nn.sigmoid(cc), (16, D)))
    wait(("x", 0))
    for n in range(T // 32):
        row_stats(0, n)
    for offset in range(0, T, 16):
        for lanes in (pl.ds(0, HD), pl.ds(HD, HD)):
            norm_v[pl.ds(offset, 16), lanes] = normalized(0, offset, lanes)
    for half in range(2):
        wait(("scale", half))
        modulation(D, D, half)
    mod_v[1] = raw(1) + 1.0
    first_rows = lambda offset, lanes: norm_v[pl.ds(offset, 16), lanes]
    for n in range(NORM_UNITS):
        norm_terms(first_rows, n, shift=False)(h0_v)

    def hold_values(col, part, v):
        norm_v[pl.ds(T + part * HT, HT), pl.ds(col, 128)] = v

    def release_values(col, part):
        v = norm_v[pl.ds(T + part * HT, HT), pl.ds(col, 128)]
        store_values(col, part, _apply(jnp.add, v, bias_v[:, pl.ds(col, 128)]))

    wait(*both("wv", 0))
    prep_values(0)
    plan = new_plan()
    plan[3] += [lambda: wait(*both("wv", 1)), lambda: prep_values(1)]
    plan[7] += [lambda: wait(*both("wv", 2))]
    plan[8] += [lambda: prep_values(2)]
    plan[15] += [lambda: prep_values(3)]
    plan[24] += [lambda: wait("wphi", *both("wk", 0)), feature_maps, lambda: prep_scores(1, 0)]
    plan[24] += [lambda: prep_scores(1, 1)]
    values(h0_v, _follow(plan), hold_values, 128)
    backlog.drain()

    for half in range(2):
        wait(("shift", half))
        modulation(0, D, half)
    mod_v[0] = raw(0)
    shift = jnp.concatenate([raw(0)] * 2, axis=0).astype(BF16)
    bias_v[...] = _dot(shift, wqkv_v[:, pl.ds(2 * D, D)])[:8]
    for n in range(NORM_UNITS):
        norm_terms(first_rows, n)(h0_v)

    def ones_rows():
        vt_v[:, pl.ds(64, 16), :] = jnp.ones((NPAIR, 16, T), BF16)

    plan = new_plan()
    plan[0].append(ones_rows)
    plan[3] += [lambda: wait(("x", 1), *both("wk", 1)), lambda: prep_scores(1, 2), lambda: prep_scores(1, 3)]
    for n in range(16):
        plan[1 + n // 2].append(functools.partial(release_values, n // 2 * 128, n % 2))
    early = 13
    for n in range(early):
        plan[6 + n // 2].append(functools.partial(lambda n: tile_norm(1, n, 3 + n % 2)(h_v), n))
    features(wk_v, h0_v, _follow(plan), store_keys, 256)
    wait("wq")
    for g in range(4):
        prep_scores(0, g)
        backlog.spent(512)
    backlog.drain()
    for n in range(early, NORM_UNITS):
        tile_norm(1, n, 0)(h_v)
    accumulate_summary(first=True)

    for t in range(1, NTILE):
        wait(("mod", t))
        plan = new_plan()
        if t + 1 < NTILE:
            wait(("x", t + 1))
            stores = []
            for n in range(NORM_UNITS):
                plan[33 + n // 2].append(
                    functools.partial(lambda n: stores.append(tile_norm(t + 1, n, 2 + n % 2)), n))
            plan[42].append(lambda: [store(h_v) for store in stores])
        start(("wg", "wu", "wd")[t - 1])
        plan_modulation(plan, t, 29, 42)
        due.clear()
        hook = _follow(plan)
        features(wk_v, h_v, hook, store_keys, 256)
        features(wq_v, h_v, hook, functools.partial(store_queries, t), 256)
        values(h_v, hook, store_values, 256)
        accumulate_summary(first=False)

    order = [(n + T // (2 * G)) % NSTEP for n in range(NSTEP)]
    wait(("mod", 0), "wo", "wr", "wg", "wu", "wd")
    plan = new_plan()
    plan[0] += [functools.partial(finish_summary, pair) for pair in range(NPAIR)]
    plan[0].append(lambda: attend(order[0], oa_v))
    plan_modulation(plan, 0, 4, 26)
    for n in range(HD // 16):
        plan[3 + 24 * n // (HD // 16)].append(functools.partial(prep_output, n))
    plan[26].append(output_weights)
    due.clear()
    features(wq_v, h0_v, _follow(plan), functools.partial(store_queries, 0), 128)

    due.clear()
    rows = None
    for n in range(NSTEP):
        source, target = ((oa_v, ob_v), (ob_v, oa_v))[n % 2]
        if n + 1 < NSTEP:
            attend(order[n + 1], target)
            if rows:
                finish(order[n - 1], rows, 2 * G, 3, 40)
            rows = project_output(source, 0, G, lambda: None)
        else:
            finish(order[n - 1], rows, 2 * G, 4, 40)
            rows = project_output(source, 0, G // 2, lambda: None)
            finish(order[n], rows, G, 4, 40)
            rows = project_output(source, G // 2, G // 2, lambda: None)
        if n > 1:
            out_copy(order[n - 2]).start()
    finish(order[-1], rows, G, G // 8, 0)
    out_copy(order[-2]).start()
    out_copy(order[-1]).start()

    base1, base2 = routed_update()
    for step in order:
        out_copy(step).wait()
    fix = [pltpu.make_async_copy(fix_v.at[n], out_hbm.at[pl.ds(base, 16)], out_sems.at[n])
           for n, base in enumerate((base1, base2))]
    fix[0].start()

    @pl.when(base1 != base2)
    def _():
        fix[1].start()
        fix[1].wait()

    fix[0].wait()


def _scratch():
    vmem = pltpu.VMEM
    return [
        vmem((S, D), BF16), vmem((D, 3 * D), BF16), vmem((D, DH), BF16), vmem((D, D), BF16),
        vmem((8, 128), BF16), vmem((D, FF), BF16), vmem((D, FF), BF16), vmem((FF, D), BF16),
        vmem((1, D), BF16), vmem((D, 6 * D), BF16),
        vmem((8, D), U32), vmem((8, 6 * D), F32), vmem((10, 8, D), F32), vmem((2, T, 128), F32),
        vmem((8, D), F32), vmem((D // 128, 64, 128), U32), vmem((7, HD // 2, HD), U32),
        vmem((7, HT // 2, HD), U32), vmem((7, HT // 2, HD), U32),
        vmem((NTILE, NPAIR, 128, T), BF16), vmem((NPAIR, 128, T), BF16), vmem((NPAIR, 80, T), BF16),
        vmem((NPAIR, 80, 128), F32), vmem((NPAIR, 40, 128), U32),
        vmem((7, G // 2, HD), U32), vmem((7, G // 2, HD), U32),
        vmem((S, D), F32), vmem((S, D), BF16), vmem((2, 16, D), BF16),
        pltpu.SemaphoreType.DMA((8 + 2 * NTILE + 14,)), pltpu.SemaphoreType.DMA((NSTEP,)),
    ] + [vmem((7, 64, HD), U32)] * 8 + [vmem((7, HD // 2, 128), U32)] * 4


@jax.jit
def pallas_adaLN_cond__linear_kernel_hedgehog__moe_arch_mod__prompt_kernel(
    A_x: jax.Array,
    A_wqkv: jax.Array,
    A_w_phi: jax.Array,
    A_wo: jax.Array,
    B_x: jax.Array,
    B_w_r: jax.Array,
    B_w_gate: jax.Array,
    B_w_up: jax.Array,
    B_w_down: jax.Array,
    c: jax.Array,
    w_mod: jax.Array,
):
    del B_x
    out = pl.pallas_call(
        _kernel,
        out_shape=jax.ShapeDtypeStruct((S, D), A_x.dtype),
        in_specs=[pl.BlockSpec(memory_space=pl.ANY)] * 10,
        out_specs=pl.BlockSpec(memory_space=pl.ANY),
        scratch_shapes=_scratch(),
        compiler_params=pltpu.CompilerParams(vmem_limit_bytes=120 * 2**20),
    )(A_x.reshape(S, D), A_wqkv, A_w_phi.reshape(D, DH), A_wo, B_w_r.reshape(8, 128),
      B_w_gate, B_w_up, B_w_down, c, w_mod)
    return out.reshape(A_x.shape)
```

```python
import collections
import functools

import jax
import jax.numpy as jnp
import numpy as np
import jax.experimental.pallas as pl
import jax.experimental.pallas.tpu as pltpu

F32, BF16, I32, U32 = jnp.float32, jnp.bfloat16, jnp.int32, jnp.uint32
S, D, HEADS, DH, FF = 2048, 1024, 32, 32, 3584
EPS = 1e-5
LOG2E = float(np.log2(np.e))

HD = D // 2
NPAIR = HEADS // 2
T = 512
HT = T // 2
NTILE = S // T
G = 128
NSTEP = S // (2 * G)
MOD_COLS = 4 * D // NTILE
NORM_UNITS = HT // 16
FF_CHUNK = 256

NN = (((1,), (0,)), ((), ()))
NT = (((1,), (1,)), ((), ()))


def _dot(a, b, dims=NN):
    return jax.lax.dot_general(a, b, dims, preferred_element_type=F32)


def _pack(x):
    n = x.shape[0] // 2
    if x.shape[1] > 128:
        return pltpu.bitcast(x.astype(BF16), U32)
    w = pltpu.bitcast(jnp.concatenate([x[:n], x[n:]], axis=1).astype(BF16), U32)
    return jnp.concatenate([w[:, :128], w[:, 128:]], axis=0)


def _unpack(w):
    return pltpu.bitcast(w, BF16)


def _recip(x):
    r = pl.reciprocal(x, approx=True)
    return r * (2.0 - x * r)


def _lhs_terms(a11, a12, a21, a22):
    return (a11 + a22, a21 + a22, a11, a22, a11 + a12, a21 - a11, a12 - a22)


def _rhs_terms(b11, b12, b21, b22):
    return (b11 + b22, b11, b12 - b22, b21 - b11, b22, b11 + b12, b21 + b22)


_QUADRANTS = (((0, 1), (3, 1), (4, -1), (6, 1)), ((2, 1), (4, 1)), ((1, 1), (3, 1)),
              ((0, 1), (1, -1), (2, 1), (5, 1)))


def _quadrant(q, product):
    total = None
    for j, sign in _QUADRANTS[q]:
        m = product(j)
        total = m if total is None else (total + m if sign > 0 else total - m)
    return total


def _per_head(op, p):
    parts = [p[r:r + 8] for r in range(0, p.shape[0], 8)]
    while len(parts) > 1:
        parts = [op(a, b) for a, b in zip(parts[::2], parts[1::2])]
    out = op(parts[0], pltpu.roll(parts[0], 4, 0))
    return op(out, pltpu.roll(out, 2, 0))


def _apply(op, p, rows8):
    return op(p.reshape(p.shape[0] // 8, 8, p.shape[1]), rows8).reshape(p.shape)


def _features(p):
    e_pos = jnp.exp2(_apply(jnp.subtract, p, _per_head(jnp.maximum, p)))
    e_neg = jnp.exp2(_apply(lambda a, low: low - a, p, _per_head(jnp.minimum, p)))
    pos = _apply(jnp.multiply, e_pos, _recip(_per_head(jnp.add, e_pos)))
    neg = _apply(jnp.multiply, e_neg, _recip(_per_head(jnp.add, e_neg)))
    return jnp.concatenate([pos, neg], axis=0)


def _interleaved_source(row):
    return (row & ~63) + ((row & 1) << 5) + ((row & 63) >> 1)


class _Backlog:
    def __init__(self):
        self.queue = collections.deque()
        self.credit = 0.0

    def defer(self, cost, task):
        self.queue.append((cost, task))

    def spent(self, cycles):
        self.credit += 0.55 * cycles
        while self.queue and self.credit >= self.queue[0][0]:
            cost, task = self.queue.popleft()
            self.credit -= cost
            task()
        if not self.queue:
            self.credit = 0.0

    def drain(self):
        while self.queue:
            self.queue.popleft()[1]()
        self.credit = 0.0


def _follow(plan):
    count = 0

    def step():
        nonlocal count
        count += 1
        for task in plan.pop(count, ()):
            task()

    for task in plan.pop(0, ()):
        task()
    return step


def _kernel(x_hbm, wqkv_hbm, wphi_hbm, wo_hbm, wr_hbm, wg_hbm, wu_hbm, wd_hbm, c_hbm, wmod_hbm,
            out_hbm,
            x_v, wqkv_v, wphi_v, wo_v, wr_v, wg_v, wu_v, wd_v, c_v, wmod_v,
            act_v, column_v, raw_v, mod_v, stat_v, bias_v, fold_v, wot_v, h_v, h0_v,
            phiq_v, phik_v, vt_v, kv_v, summary_v, oa_v, ob_v, norm_v, out_v, fix_v,
            in_sems, out_sems, *terms_v):
    wq_v, wk_v, wv_v = terms_v[:4], terms_v[4:8], terms_v[8:]
    backlog = _Backlog()
    new_plan = lambda: collections.defaultdict(list)

    copies = {}

    def add_copy(name, src, dst, part=Ellipsis):
        if part is not Ellipsis:
            src, dst = src.at[part], dst.at[part]
        copies[name] = pltpu.make_async_copy(src, dst, in_sems.at[len(copies)])

    columns = lambda lo, n: (pl.ds(0, D), pl.ds(lo, n))
    for name, src, dst in (("c", c_hbm, c_v), ("wphi", wphi_hbm, wphi_v), ("wr", wr_hbm, wr_v),
                           ("wo", wo_hbm, wo_v), ("wg", wg_hbm, wg_v), ("wu", wu_hbm, wu_v),
                           ("wd", wd_hbm, wd_v)):
        add_copy(name, src, dst)
    add_copy("wq", wqkv_hbm, wqkv_v, columns(0, D))
    for t in range(NTILE):
        add_copy(("x", t), x_hbm, x_v, pl.ds(t * T, T))
        add_copy(("mod", t), wmod_hbm, wmod_v, columns(2 * D + t * MOD_COLS, MOD_COLS))
    for half in range(2):
        add_copy(("shift", half), wmod_hbm, wmod_v, (pl.ds(half * HD, HD), pl.ds(0, D)))
        add_copy(("scale", half), wmod_hbm, wmod_v, (pl.ds(half * HD, HD), pl.ds(D, D)))
        for n in range(2):
            add_copy(("wk", n, half), wqkv_hbm, wqkv_v, columns(D + half * HD + n * 256, 256))
        for n, (lo, size) in enumerate(((0, 128), (128, 128), (256, 256))):
            add_copy(("wv", n, half), wqkv_hbm, wqkv_v, columns(2 * D + half * HD + lo, size))
    both = lambda *name: ((*name, 0), (*name, 1))

    def start(*names):
        for name in names:
            copies[name].start()

    def wait(*names):
        for name in names:
            copies[name].wait()

    def out_copy(step):
        rows = pl.ds(step * 2 * G, 2 * G)
        return pltpu.make_async_copy(out_v.at[rows], out_hbm.at[rows], out_sems.at[step])

    start("c", ("x", 0), *both("scale"), *both("wv", 0), *both("wv", 1), *both("wv", 2), "wphi",
          *both("wk", 0), *both("shift"), *both("wk", 1), ("x", 1), "wq",
          ("x", 2), ("mod", 1), ("x", 3), ("mod", 2), ("mod", 3), ("mod", 0), "wo", "wr")
    wait("c")

    bits = pltpu.bitcast(jnp.broadcast_to(c_v[:, :128].astype(F32), (8, 128)), I32)
    zero = jnp.minimum(jnp.max(bits & 0xFF), 0)

    class Chain:
        def __init__(self, strands):
            self.tokens = collections.deque([None] * strands)

        def enter(self, rows8):
            token = self.tokens.popleft()
            if token is None:
                return rows8
            head = pltpu.bitcast(pltpu.bitcast(rows8[:, :128], I32) | token, F32)
            return jnp.concatenate([head, rows8[:, 128:]], axis=1)

        def leave(self, *values):
            words = [pltpu.bitcast(value, I32) for value in values]
            self.tokens.append(functools.reduce(jnp.bitwise_or, words) & zero)

    clock = 0
    due = collections.defaultdict(list)

    def finish_within(delay, *values):
        parts = [pltpu.bitcast(value, U32)[r:r + 8, l:l + 128] for value in values
                 for r in range(0, value.shape[0], 8) for l in range(0, value.shape[1], 128)]
        due[clock + delay].append(functools.reduce(jnp.bitwise_or, parts) & zero.astype(U32))

    def gated(ref, j, row=0):
        nonlocal clock
        clock += 1
        tokens = [token for when in sorted(due) if when < clock for token in due.pop(when)]
        if tokens:
            corner = (j, pl.ds(row, 8), pl.ds(0, 128))
            ref[corner] = functools.reduce(jnp.bitwise_or, tokens, ref[corner])
        return ref[j]

    def modulation(lo, n, half):
        rows, lanes = pl.ds(half * HD, HD), pl.ds(lo, n)
        m = _dot(_unpack(act_v[:, rows]), wmod_v[rows, lanes])[:8]
        raw_v[:, lanes] = raw_v[:, lanes] + m if half else m

    raw = lambda i: raw_v[:, pl.ds(i * D, D)]

    def plan_modulation(plan, t, first, last):
        steps = 2 * MOD_COLS // 128
        for n in range(steps):
            plan[first + (last - first) * n // steps].append(
                functools.partial(modulation, 2 * D + t * MOD_COLS + n // 2 * 128, 128, n % 2))

    def plan_vector_modulation(plan, slots):
        sums = {}

        def column():
            stat_rows = jnp.broadcast_to(_unpack(act_v[...]).astype(F32)[:1], (128, D))
            column_v[...] = stat_rows.T

        def unit(i, k):
            total = sums.get(i)
            for r in range(k, k + 64, 8):
                w = wmod_v[pl.ds(r, 8), pl.ds(i * D, D)].astype(F32)
                term = w * jnp.concatenate([column_v[pl.ds(r, 8), :]] * (D // 128), axis=1)
                total = term if total is None else total + term
            sums[i] = total
            finish_within(2, total)
            if k + 64 == D:
                raw_v[:, pl.ds(i * D, D)] = jnp.broadcast_to(jnp.sum(total, axis=0, keepdims=True), (8, D))

        plan[0].append(column)
        units = [(i, k) for i in range(2, 6) for k in range(0, D, 64)]
        for n, (i, k) in enumerate(units):
            plan[slots[len(slots) * n // len(units)]].append(functools.partial(unit, i, k))

    def output_weights():
        w = wr_v[...].astype(F32)
        w = jnp.concatenate([jnp.broadcast_to(w[j:j + 1], (8, 128)) for j in range(D // 128)], axis=1)
        for i in range(2, 6):
            mod_v[i] = raw(i) + 1.0 if i == 4 else raw(i)
        mod_v[6] = mod_v[4] * w
        mod_v[7] = mod_v[4] * mod_v[5]
        mod_v[8] = mod_v[3] * mod_v[5]
        mod_v[9] = jnp.broadcast_to(jnp.sum(mod_v[3] * w, axis=1, keepdims=True), (8, D))

    def feature_maps():
        row = _interleaved_source(jax.lax.broadcasted_iota(I32, (128, DH), 0))
        col = jax.lax.broadcasted_iota(I32, (128, DH), 1)
        select = jnp.where((row & (DH - 1)) == col, 1.0, 0.0).astype(BF16)
        row_head = _interleaved_source(jax.lax.broadcasted_iota(I32, (128, 128), 0)) >> 5
        col_head = jax.lax.broadcasted_iota(I32, (128, 128), 1) >> 5
        for g in range(D // 128):
            tiled = _dot(select, wphi_v[pl.ds(g * 128, 128), :], NT)
            fold_v[g] = _pack(jnp.where(row_head == col_head, tiled, 0.0))

    def prep_scores(i, g):
        blocks = []
        for group in (g, g + HD // 128):
            for half in range(2):
                w = wqkv_v[pl.ds(half * HD, HD), pl.ds(i * D + group * 128, 128)]
                blocks.append(_dot(_unpack(fold_v[group]), w, NT) * LOG2E)
        for j, term in enumerate(_lhs_terms(*blocks)):
            (wq_v, wk_v)[i][g][j] = _pack(term)

    def prep_values(g):
        chain = Chain(1)
        for r in range(0, HD, 64):
            blocks = [wqkv_v[pl.ds(row + r, 64), pl.ds(2 * D + col + g * 128, 128)].astype(F32)
                      for col in (0, HD) for row in (0, HD)]
            token = chain.tokens.popleft()
            if token is not None:
                head = pltpu.bitcast(pltpu.bitcast(blocks[3][:8], I32) | token, F32)
                blocks[3] = jnp.concatenate([head, blocks[3][8:]], axis=0)
            for j, term in enumerate(_lhs_terms(*blocks)):
                words = _pack(term)
                wv_v[g][j, pl.ds(r // 2, 32), :] = words
            chain.leave(words[:8])

    def prep_output(n):
        lo = wo_v[pl.ds(n * 16, 16), :].astype(F32)
        hi = wo_v[pl.ds(HD + n * 16, 16), :].astype(F32)
        words = [_pack(term) for term in _rhs_terms(lo[:, :HD], lo[:, HD:], hi[:, :HD], hi[:, HD:])]
        for j, w in enumerate(words):
            wot_v[j, pl.ds(n * 8, 8), :] = w
        finish_within(2, *words)

    def row_stats(t, n):
        xx = x_v[pl.ds(t * T + n * 32, 32), :].astype(F32)
        mean = jnp.mean(xx, axis=-1, keepdims=True)
        d = xx - mean
        scale = jax.lax.rsqrt(jnp.mean(d * d, axis=-1, keepdims=True) + EPS)
        stat_v[0, pl.ds(n * 32, 32), :] = jnp.broadcast_to(mean, (32, 128))
        stat_v[1, pl.ds(n * 32, 32), :] = jnp.broadcast_to(scale, (32, 128))

    def normalized(t, offset, lanes):
        wide = lambda k: jnp.concatenate([stat_v[k, pl.ds(offset, 16), :]] * (HD // 128), axis=1)
        return (x_v[pl.ds(t * T + offset, 16), lanes].astype(F32) - wide(0)) * wide(1)

    def norm_terms(rows, n, shift=True, delay=0):
        blocks = []
        for lanes in (pl.ds(0, HD), pl.ds(HD, HD)):
            for offset in (n * 16, HT + n * 16):
                hh = rows(offset, lanes).reshape(2, 8, HD) * mod_v[1, :, lanes]
                blocks.append((hh + mod_v[0, :, lanes] if shift else hh).reshape(16, HD))
        words = [_pack(term) for term in _rhs_terms(*blocks)]
        if delay:
            finish_within(delay, *words)

        def store(target):
            for j, w in enumerate(words):
                target[j, pl.ds(n * 8, 8), :] = w

        return store

    def tile_norm(t, n, delay):
        if n % 2 == 0:
            row_stats(t, n // 2)
            row_stats(t, HT // 32 + n // 2)
        return norm_terms(functools.partial(normalized, t), n, delay=delay)

    def products(product, tiles, cycles, hook):
        result = []
        for j in range(7):
            result.append([product(j, k) for k in range(tiles)])
            backlog.spent(cycles)
            hook()
        return result

    def features(weights, source, hook, target, rows):
        for r in range(0, HD, rows):
            m = products(
                lambda j, k: _dot(
                    _unpack(jnp.concatenate([weights[g][j] for g in range(r // 128, (r + rows) // 128)], axis=0)),
                    _unpack(gated(source, j, k * 64)[k * 64:(k + 1) * 64]), NT),
                HT // 128, rows * HT // 128, hook)

            def unit(half, o, m=m, r=r):
                for part in range(2):
                    phi = jnp.concatenate(
                        [_features(_quadrant(2 * half + part, lambda j: m[j][k][o:o + 64]))
                         for k in range(HT // 128)], axis=1)
                    target((half * HD + r + o) // 64, pl.ds(part * HT, HT), phi.astype(BF16))

            for half in range(2):
                for o in range(0, rows, 64):
                    backlog.defer(150 * rows // 256, functools.partial(unit, half, o))

    def store_keys(pair, lanes, phi):
        phik_v[pair, :, lanes] = phi

    def store_queries(t, pair, lanes, phi):
        phiq_v[t, pair, :, lanes] = phi

    def store_values(col, part, v):
        v = v.T.astype(BF16).reshape(2, 64, HT)
        vt_v[pl.ds(col // 64, 2), pl.ds(0, 64), pl.ds(part * HT, HT)] = v

    def values(source, hook, target, cols):
        for r in range(0, HD, cols):
            m = products(
                lambda j, k: _dot(_unpack(source[j]), _unpack(gated(wv_v[r // 128 + k], j))),
                cols // 128, cols * HT // 128, hook)

            def unit(half, part, k, m=m, r=r):
                target(half * HD + r + k * 128, part, _quadrant(2 * half + part, lambda j: m[j][k]))

            for half in range(2):
                for part in range(2):
                    for k in range(cols // 128):
                        backlog.defer(128, functools.partial(unit, half, part, k))

    def accumulate_summary(first):
        backlog.drain()
        for r in range(0, HD, 256):
            for half in range(2):
                for o in range(0, 256, 64):
                    pair = (half * HD + r + o) // 64
                    kv = _dot(vt_v[pair], phik_v[pair], NT)
                    kv_v[pair] = kv if first else kv_v[pair] + kv

    def finish_summary(pair):
        row = jax.lax.broadcasted_iota(I32, (80, 128), 0)
        row_head = jnp.where(row < 64, row >> 5, (row >> 3) & 1)
        col_head = jax.lax.broadcasted_iota(I32, (80, 128), 1) & 1
        summary_v[pair] = _pack(jnp.where(row_head == col_head, kv_v[pair], 0.0))

    def attend(step, target):
        t, lanes = step // 2, pl.ds(step % 2 * 2 * G, 2 * G)
        pairs = [[[half * NPAIR // 2 + 2 * i + k for k in range(2)] for half in range(2)] for i in range(4)]
        nums = {p: _dot(_unpack(summary_v[p]), phiq_v[t, p, :, lanes])
                for group in pairs for side in group for p in side}
        sides = []
        for i, group in enumerate(pairs):
            heads = [[_apply(jnp.multiply, nums[p][h * DH:(h + 1) * DH],
                             _recip(nums[p][64 + 8 * h:72 + 8 * h] + 1e-6))
                      for p in side for h in range(2)] for side in group]
            sides.append([jnp.concatenate(side, axis=0).T for side in heads])
            if i % 2:
                lo, hi = (jnp.concatenate([sides[i - 1][s], sides[i][s]], axis=1) for s in range(2))
                for j, term in enumerate(_lhs_terms(lo[:G], hi[:G], lo[G:], hi[G:])):
                    target[j, :, pl.ds((i - 1) * 128, 256)] = term.astype(BF16)

    def project_output(source, lo, n, hook):
        m = products(
            lambda j, k: _dot(source[j, pl.ds(lo, n), :],
                              _unpack(gated(wot_v, j)[:, k * 128:(k + 1) * 128])),
            HD // 128, 4 * n, hook)

        def rows(o):
            part, o = divmod(o, n)
            piece = lambda j: jnp.concatenate([tile[o:o + 32] for tile in m[j]], axis=1)
            return lo + part * G + o, jnp.concatenate(
                [_quadrant(2 * part + half, piece) for half in range(2)], axis=1)

        return rows

    scores = {}

    def finish(step, rows, count, strands, delay):
        chain = Chain(strands)
        lane = jax.lax.broadcasted_iota(I32, (8, 128), 1)
        for start_row in range(0, count, 32):
            row, y = rows(start_row)
            for o in range(0, 32, 8):
                base = step * 2 * G + row + o
                xn = x_v[pl.ds(base, 8), :].astype(F32) + mod_v[2] * chain.enter(y[o:o + 8])
                mean = jnp.mean(xn, axis=-1, keepdims=True)
                d = xn - mean
                scale = jax.lax.rsqrt(jnp.mean(d * d, axis=-1, keepdims=True) + EPS)
                score = jnp.sum(d * mod_v[6], axis=-1, keepdims=True) * scale + mod_v[9, :, :1]
                normed = d * scale
                norm_v[pl.ds(base, 8), :] = normed
                out = normed * mod_v[7] + ((d + mean) + mod_v[8])
                out_v[pl.ds(base, 8), :] = out.astype(BF16)
                held = scores.get(base // 1024, jnp.full((8, 128), -jnp.inf, F32))
                scores[base // 1024] = jnp.where(lane == base % 1024 // 8, score, held)
                chain.leave(*[out[:, l:l + 128] for l in range(128, D, 256)])
        if delay:
            finish_within(delay, *chain.tokens)

    def top_two():
        shape = (S // 1024, 8, 128)
        index = (jax.lax.broadcasted_iota(I32, shape, 0) * 1024 + jax.lax.broadcasted_iota(I32, shape, 2) * 8
                 + jax.lax.broadcasted_iota(I32, shape, 1)).astype(F32)
        left = jnp.stack([scores[b] for b in range(S // 1024)])
        reduce = lambda op, v: op(op(op(v, axis=0), axis=0, keepdims=True), axis=1, keepdims=True)
        top = reduce(jnp.max, left)
        first = reduce(jnp.min, jnp.where(left == top, index, float(S)))
        below = reduce(jnp.max, jnp.where(left == top, -jnp.inf, left))
        tied = reduce(jnp.min, jnp.where((left == top) & (index != first), index, float(S)))
        lower = reduce(jnp.min, jnp.where((left == below) & (left != top), index, float(S)))
        second = jnp.where(tied < S, tied, lower)
        row = lambda v: jnp.clip(jnp.max(v.astype(I32)), 0, S - 1)
        return (row(first), top), (row(second), jnp.where(tied < S, top, below))

    def routed_update():
        (row1, score1), (row2, score2) = top_two()
        sub = jax.lax.broadcasted_iota(I32, (16, D), 0)
        first, second = (jnp.broadcast_to(norm_v[pl.ds(row, 1), :], (16, D)) for row in (row1, row2))
        selected = jnp.where(sub == 0, first, second).reshape(2, 8, D) * mod_v[4] + mod_v[3]
        selected = selected.reshape(16, D).astype(BF16)
        pending = collections.deque()
        parts = []

        def down():
            f, g, u = pending.popleft()
            act = (g * jax.nn.sigmoid(g) * u).astype(BF16)
            part = _dot(act, wd_v[pl.ds(f, FF_CHUNK), :])
            parts.append(parts.pop() + part if parts else part)

        for f in range(0, FF, FF_CHUNK):
            pending.append((f, _dot(selected, wg_v[:, pl.ds(f, FF_CHUNK)]),
                            _dot(selected, wu_v[:, pl.ds(f, FF_CHUNK)])))
            if len(pending) > 2:
                down()
        while pending:
            down()
        y1, y2 = parts[0][0:1] * jax.nn.sigmoid(score1), parts[0][1:2] * jax.nn.sigmoid(score2)
        bases = [pl.multiple_of((row >> 4) * 16, 16) for row in (row1, row2)]
        for n, base in enumerate(bases):
            update = jnp.where(sub == row1 - base, y1, 0.0) + jnp.where(sub == row2 - base, y2, 0.0)
            rows = out_v[pl.ds(base, 16), :].astype(F32).reshape(2, 8, D) + mod_v[5] * update.reshape(2, 8, D)
            fix_v[n] = rows.reshape(16, D).astype(BF16)
        return bases

    cc = c_v[...].astype(F32)
    act_v[...] = _pack(jnp.broadcast_to(cc * jax.nn.sigmoid(cc), (16, D)))
    wait(("x", 0))
    for n in range(T // 32):
        row_stats(0, n)
    for offset in range(0, T, 16):
        for lanes in (pl.ds(0, HD), pl.ds(HD, HD)):
            norm_v[pl.ds(offset, 16), lanes] = normalized(0, offset, lanes)
    for half in range(2):
        wait(("scale", half))
        modulation(D, D, half)
    mod_v[1] = raw(1) + 1.0
    first_rows = lambda offset, lanes: norm_v[pl.ds(offset, 16), lanes]
    for n in range(NORM_UNITS):
        norm_terms(first_rows, n, shift=False)(h0_v)

    def hold_values(col, part, v):
        norm_v[pl.ds(T + part * HT, HT), pl.ds(col, 128)] = v

    def release_values(col, part):
        v = norm_v[pl.ds(T + part * HT, HT), pl.ds(col, 128)]
        store_values(col, part, _apply(jnp.add, v, bias_v[:, pl.ds(col, 128)]))

    wait(*both("wv", 0))
    prep_values(0)
    plan = new_plan()
    plan[3] += [lambda: wait(*both("wv", 1)), lambda: prep_values(1)]
    plan[7] += [lambda: wait(*both("wv", 2))]
    plan[8] += [lambda: prep_values(2)]
    plan[15] += [lambda: prep_values(3)]
    plan[24] += [lambda: wait("wphi", *both("wk", 0)), feature_maps, lambda: prep_scores(1, 0)]
    plan[24] += [lambda: prep_scores(1, 1)]
    values(h0_v, _follow(plan), hold_values, 128)
    backlog.drain()

    for half in range(2):
        wait(("shift", half))
        modulation(0, D, half)
    mod_v[0] = raw(0)
    shift = jnp.concatenate([raw(0)] * 2, axis=0).astype(BF16)
    bias_v[...] = _dot(shift, wqkv_v[:, pl.ds(2 * D, D)])[:8]
    for n in range(NORM_UNITS):
        norm_terms(first_rows, n)(h0_v)

    def ones_rows():
        vt_v[:, pl.ds(64, 16), :] = jnp.ones((NPAIR, 16, T), BF16)

    plan = new_plan()
    plan[0].append(ones_rows)
    plan[3] += [lambda: wait(("x", 1), *both("wk", 1)), lambda: prep_scores(1, 2), lambda: prep_scores(1, 3)]
    for n in range(16):
        plan[1 + n // 2].append(functools.partial(release_values, n // 2 * 128, n % 2))
    early = 13
    for n in range(early):
        plan[6 + n // 2].append(functools.partial(lambda n: tile_norm(1, n, 3 + n % 2)(h_v), n))
    features(wk_v, h0_v, _follow(plan), store_keys, 256)
    wait("wq")
    for g in range(4):
        prep_scores(0, g)
        backlog.spent(512)
    backlog.drain()
    for n in range(early, NORM_UNITS):
        tile_norm(1, n, 0)(h_v)
    accumulate_summary(first=True)

    for t in range(1, NTILE):
        if t == NTILE - 1:
            wait(*[("mod", i) for i in range(NTILE)])
        plan = new_plan()
        if t + 1 < NTILE:
            wait(("x", t + 1))
            stores = []
            for n in range(NORM_UNITS):
                plan[32 + (10 * n) // 16].append(
                    functools.partial(lambda n: stores.append(tile_norm(t + 1, n, 2 + n % 2)), n))
            plan[42].append(lambda: [store(h_v) for store in stores])
        start(("wg", "wu", "wd")[t - 1])
        if t == NTILE - 1:
            plan_vector_modulation(plan, (1, 2, 3, 32, 33, 34, 35, 36, 37, 38, 39, 40, 41, 42))
        due.clear()
        hook = _follow(plan)
        features(wk_v, h_v, hook, store_keys, 256)
        features(wq_v, h_v, hook, functools.partial(store_queries, t), 256)
        values(h_v, hook, store_values, 256)
        accumulate_summary(first=False)

    order = [(n + T // (2 * G)) % NSTEP for n in range(NSTEP)]
    wait("wo", "wr", "wg", "wu", "wd")
    plan = new_plan()
    plan[0] += [functools.partial(finish_summary, pair) for pair in range(NPAIR)]
    plan[0].append(lambda: attend(order[0], oa_v))
    for n in range(HD // 16):
        plan[3 + 24 * n // (HD // 16)].append(functools.partial(prep_output, n))
    plan[26].append(output_weights)
    due.clear()
    features(wq_v, h0_v, _follow(plan), functools.partial(store_queries, 0), 128)

    due.clear()
    rows = None
    for n in range(NSTEP):
        source, target = ((oa_v, ob_v), (ob_v, oa_v))[n % 2]
        if n + 1 < NSTEP:
            attend(order[n + 1], target)
            if rows:
                finish(order[n - 1], rows, 2 * G, 3, 44)
            rows = project_output(source, 0, G, lambda: None)
        else:
            finish(order[n - 1], rows, 2 * G, 6, 26)
            rows = project_output(source, 0, G // 2, lambda: None)
            finish(order[n], rows, G, 8, 24)
            rows = project_output(source, G // 2, G // 2, lambda: None)
        if n > 1:
            out_copy(order[n - 2]).start()
    finish(order[-1], rows, G, G // 8, 0)
    out_copy(order[-2]).start()
    out_copy(order[-1]).start()

    base1, base2 = routed_update()
    for step in order:
        out_copy(step).wait()
    fix = [pltpu.make_async_copy(fix_v.at[n], out_hbm.at[pl.ds(base, 16)], out_sems.at[n])
           for n, base in enumerate((base1, base2))]
    fix[0].start()

    @pl.when(base1 != base2)
    def _():
        fix[1].start()
        fix[1].wait()

    fix[0].wait()


def _scratch():
    vmem = pltpu.VMEM
    return [
        vmem((S, D), BF16), vmem((D, 3 * D), BF16), vmem((D, DH), BF16), vmem((D, D), BF16),
        vmem((8, 128), BF16), vmem((D, FF), BF16), vmem((D, FF), BF16), vmem((FF, D), BF16),
        vmem((1, D), BF16), vmem((D, 6 * D), BF16),
        vmem((8, D), U32), vmem((D, 128), F32), vmem((8, 6 * D), F32), vmem((10, 8, D), F32), vmem((2, T, 128), F32),
        vmem((8, D), F32), vmem((D // 128, 64, 128), U32), vmem((7, HD // 2, HD), U32),
        vmem((7, HT // 2, HD), U32), vmem((7, HT // 2, HD), U32),
        vmem((NTILE, NPAIR, 128, T), BF16), vmem((NPAIR, 128, T), BF16), vmem((NPAIR, 80, T), BF16),
        vmem((NPAIR, 80, 128), F32), vmem((NPAIR, 40, 128), U32),
        vmem((7, G, HD), BF16), vmem((7, G, HD), BF16),
        vmem((S, D), F32), vmem((S, D), BF16), vmem((2, 16, D), BF16),
        pltpu.SemaphoreType.DMA((8 + 2 * NTILE + 14,)), pltpu.SemaphoreType.DMA((NSTEP,)),
    ] + [vmem((7, 64, HD), U32)] * 8 + [vmem((7, HD // 2, 128), U32)] * 4


@jax.jit
def pallas_adaLN_cond__linear_kernel_hedgehog__moe_arch_mod__prompt_kernel(
    A_x: jax.Array,
    A_wqkv: jax.Array,
    A_w_phi: jax.Array,
    A_wo: jax.Array,
    B_x: jax.Array,
    B_w_r: jax.Array,
    B_w_gate: jax.Array,
    B_w_up: jax.Array,
    B_w_down: jax.Array,
    c: jax.Array,
    w_mod: jax.Array,
):
    del B_x
    out = pl.pallas_call(
        _kernel,
        out_shape=jax.ShapeDtypeStruct((S, D), A_x.dtype),
        in_specs=[pl.BlockSpec(memory_space=pl.ANY)] * 10,
        out_specs=pl.BlockSpec(memory_space=pl.ANY),
        scratch_shapes=_scratch(),
        compiler_params=pltpu.CompilerParams(vmem_limit_bytes=120 * 2**20),
    )(A_x.reshape(S, D), A_wqkv, A_w_phi.reshape(D, DH), A_wo, B_w_r.reshape(8, 128),
      B_w_gate, B_w_up, B_w_down, c, w_mod)
    return out.reshape(A_x.shape)
```

```python
import collections
import functools

import jax
import jax.numpy as jnp
import numpy as np
import jax.experimental.pallas as pl
import jax.experimental.pallas.tpu as pltpu

F32, BF16, I32, U32 = jnp.float32, jnp.bfloat16, jnp.int32, jnp.uint32
S, D, HEADS, DH, FF = 2048, 1024, 32, 32, 3584
EPS = 1e-5
LOG2E = float(np.log2(np.e))

HD = D // 2
NPAIR = HEADS // 2
T = 512
HT = T // 2
NTILE = S // T
G = 128
NSTEP = S // (2 * G)
MOD_COLS = 4 * D // NTILE
NORM_UNITS = HT // 16
FF_CHUNK = 256

NN = (((1,), (0,)), ((), ()))
NT = (((1,), (1,)), ((), ()))


def _dot(a, b, dims=NN):
    return jax.lax.dot_general(a, b, dims, preferred_element_type=F32)


def _pack(x):
    n = x.shape[0] // 2
    if x.shape[1] > 128:
        return pltpu.bitcast(x.astype(BF16), U32)
    w = pltpu.bitcast(jnp.concatenate([x[:n], x[n:]], axis=1).astype(BF16), U32)
    return jnp.concatenate([w[:, :128], w[:, 128:]], axis=0)


def _unpack(w):
    return pltpu.bitcast(w, BF16)


def _recip(x):
    r = pl.reciprocal(x, approx=True)
    return r * (2.0 - x * r)


def _lhs_terms(a11, a12, a21, a22):
    return (a11 + a22, a21 + a22, a11, a22, a11 + a12, a21 - a11, a12 - a22)


def _rhs_terms(b11, b12, b21, b22):
    return (b11 + b22, b11, b12 - b22, b21 - b11, b22, b11 + b12, b21 + b22)


_QUADRANTS = (((0, 1), (3, 1), (4, -1), (6, 1)), ((2, 1), (4, 1)), ((1, 1), (3, 1)),
              ((0, 1), (1, -1), (2, 1), (5, 1)))


def _quadrant(q, product):
    total = None
    for j, sign in _QUADRANTS[q]:
        m = product(j)
        total = m if total is None else (total + m if sign > 0 else total - m)
    return total


def _per_head(op, p):
    parts = [p[r:r + 8] for r in range(0, p.shape[0], 8)]
    while len(parts) > 1:
        parts = [op(a, b) for a, b in zip(parts[::2], parts[1::2])]
    out = op(parts[0], pltpu.roll(parts[0], 4, 0))
    return op(out, pltpu.roll(out, 2, 0))


def _apply(op, p, rows8):
    return op(p.reshape(p.shape[0] // 8, 8, p.shape[1]), rows8).reshape(p.shape)


def _features(p):
    e_pos = jnp.exp2(_apply(jnp.subtract, p, _per_head(jnp.maximum, p)))
    e_neg = jnp.exp2(_apply(lambda a, low: low - a, p, _per_head(jnp.minimum, p)))
    pos = _apply(jnp.multiply, e_pos, _recip(_per_head(jnp.add, e_pos)))
    neg = _apply(jnp.multiply, e_neg, _recip(_per_head(jnp.add, e_neg)))
    return jnp.concatenate([pos, neg], axis=0)


def _interleaved_source(row):
    return (row & ~63) + ((row & 1) << 5) + ((row & 63) >> 1)


class _Backlog:
    def __init__(self):
        self.queue = collections.deque()
        self.credit = 0.0

    def defer(self, cost, task):
        self.queue.append((cost, task))

    def spent(self, cycles):
        self.credit += 0.55 * cycles
        while self.queue and self.credit >= self.queue[0][0]:
            cost, task = self.queue.popleft()
            self.credit -= cost
            task()
        if not self.queue:
            self.credit = 0.0

    def drain(self):
        while self.queue:
            self.queue.popleft()[1]()
        self.credit = 0.0


def _follow(plan):
    count = 0

    def step():
        nonlocal count
        count += 1
        for task in plan.pop(count, ()):
            task()

    for task in plan.pop(0, ()):
        task()
    return step


def _kernel(x_hbm, wqkv_hbm, wphi_hbm, wo_hbm, wr_hbm, wg_hbm, wu_hbm, wd_hbm, c_hbm, wmod_hbm,
            out_hbm,
            x_v, wqkv_v, wphi_v, wo_v, wr_v, wg_v, wu_v, wd_v, c_v, wmod_v,
            act_v, column_v, raw_v, mod_v, stat_v, bias_v, fold_v, wot_v, h_v, h0_v,
            phiq_v, phik_v, vt_v, kv_v, summary_v, oa_v, ob_v, norm_v, out_v, fix_v,
            in_sems, out_sems, *terms_v):
    wq_v, wk_v, wv_v = terms_v[:4], terms_v[4:8], terms_v[8:]
    backlog = _Backlog()
    new_plan = lambda: collections.defaultdict(list)

    copies = {}

    def add_copy(name, src, dst, part=Ellipsis):
        if part is not Ellipsis:
            src, dst = src.at[part], dst.at[part]
        copies[name] = pltpu.make_async_copy(src, dst, in_sems.at[len(copies)])

    columns = lambda lo, n: (pl.ds(0, D), pl.ds(lo, n))
    for name, src, dst in (("c", c_hbm, c_v), ("wphi", wphi_hbm, wphi_v), ("wr", wr_hbm, wr_v),
                           ("wo", wo_hbm, wo_v), ("wg", wg_hbm, wg_v), ("wu", wu_hbm, wu_v),
                           ("wd", wd_hbm, wd_v)):
        add_copy(name, src, dst)
    add_copy("wq", wqkv_hbm, wqkv_v, columns(0, D))
    for t in range(NTILE):
        add_copy(("x", t), x_hbm, x_v, pl.ds(t * T, T))
        add_copy(("mod", t), wmod_hbm, wmod_v, columns(2 * D + t * MOD_COLS, MOD_COLS))
    for half in range(2):
        add_copy(("shift", half), wmod_hbm, wmod_v, (pl.ds(half * HD, HD), pl.ds(0, D)))
        add_copy(("scale", half), wmod_hbm, wmod_v, (pl.ds(half * HD, HD), pl.ds(D, D)))
        for n in range(2):
            add_copy(("wk", n, half), wqkv_hbm, wqkv_v, columns(D + half * HD + n * 256, 256))
        for n, (lo, size) in enumerate(((0, 128), (128, 128), (256, 256))):
            add_copy(("wv", n, half), wqkv_hbm, wqkv_v, columns(2 * D + half * HD + lo, size))
    both = lambda *name: ((*name, 0), (*name, 1))

    def start(*names):
        for name in names:
            copies[name].start()

    def wait(*names):
        for name in names:
            copies[name].wait()

    def out_copy(step):
        rows = pl.ds(step * 2 * G, 2 * G)
        return pltpu.make_async_copy(out_v.at[rows], out_hbm.at[rows], out_sems.at[step])

    start("c", ("x", 0), *both("scale"), *both("wv", 0), *both("wv", 1), *both("wv", 2),
          *both("shift"), "wphi", *both("wk", 0), *both("wk", 1), ("x", 1), "wq",
          ("x", 2), ("mod", 1), ("x", 3), ("mod", 2), ("mod", 3), ("mod", 0), "wo", "wr")
    wait("c")

    bits = pltpu.bitcast(jnp.broadcast_to(c_v[:, :128].astype(F32), (8, 128)), I32)
    zero = jnp.minimum(jnp.max(bits & 0xFF), 0)

    class Chain:
        def __init__(self, strands):
            self.tokens = collections.deque([None] * strands)

        def enter(self, rows8):
            token = self.tokens.popleft()
            if token is None:
                return rows8
            head = pltpu.bitcast(pltpu.bitcast(rows8[:, :128], I32) | token, F32)
            return jnp.concatenate([head, rows8[:, 128:]], axis=1)

        def leave(self, *values):
            words = [pltpu.bitcast(value, I32) for value in values]
            self.tokens.append(functools.reduce(jnp.bitwise_or, words) & zero)

    clock = 0
    due = collections.defaultdict(list)

    def finish_within(delay, *values):
        parts = [pltpu.bitcast(value, U32)[r:r + 8, l:l + 128] for value in values
                 for r in range(0, value.shape[0], 8) for l in range(0, value.shape[1], 128)]
        due[clock + delay].append(functools.reduce(jnp.bitwise_or, parts) & zero.astype(U32))

    def gated(ref, j, row=0):
        nonlocal clock
        clock += 1
        tokens = [token for when in sorted(due) if when < clock for token in due.pop(when)]
        if tokens:
            corner = (j, pl.ds(row, 8), pl.ds(0, 128))
            ref[corner] = functools.reduce(jnp.bitwise_or, tokens, ref[corner])
        return ref[j]

    def modulation(lo, n, half):
        rows, lanes = pl.ds(half * HD, HD), pl.ds(lo, n)
        m = _dot(_unpack(act_v[:, rows]), wmod_v[rows, lanes])[:8]
        raw_v[:, lanes] = raw_v[:, lanes] + m if half else m

    raw = lambda i: raw_v[:, pl.ds(i * D, D)]

    def store_column(rows):
        column_v[...] = jnp.broadcast_to(rows[:1], (128, D)).T

    def plan_vector_modulation(plan, slots):
        sums = {}

        def unit(i, k):
            total = sums.get(i)
            for r in range(k, k + 64, 8):
                w = wmod_v[pl.ds(r, 8), pl.ds(i * D, D)].astype(F32)
                term = w * jnp.concatenate([column_v[pl.ds(r, 8), :]] * (D // 128), axis=1)
                total = term if total is None else total + term
            sums[i] = total
            finish_within(2, total)
            if k + 64 == D:
                raw_v[:, pl.ds(i * D, D)] = jnp.broadcast_to(jnp.sum(total, axis=0, keepdims=True), (8, D))

        plan[0].append(lambda: store_column(_unpack(act_v[...]).astype(F32)))
        units = [(i, k) for i in range(2, 6) for k in range(0, D, 64)]
        for n, (i, k) in enumerate(units):
            plan[slots[len(slots) * n // len(units)]].append(functools.partial(unit, i, k))

    def output_weights():
        w = wr_v[...].astype(F32)
        w = jnp.concatenate([jnp.broadcast_to(w[j:j + 1], (8, 128)) for j in range(D // 128)], axis=1)
        for i in range(2, 6):
            mod_v[i] = raw(i) + 1.0 if i == 4 else raw(i)
        mod_v[6] = mod_v[4] * w
        mod_v[7] = mod_v[4] * mod_v[5]
        mod_v[8] = mod_v[3] * mod_v[5]
        mod_v[9] = jnp.broadcast_to(jnp.sum(mod_v[3] * w, axis=1, keepdims=True), (8, D))

    def feature_maps():
        row = _interleaved_source(jax.lax.broadcasted_iota(I32, (128, DH), 0))
        col = jax.lax.broadcasted_iota(I32, (128, DH), 1)
        select = jnp.where((row & (DH - 1)) == col, 1.0, 0.0).astype(BF16)
        row_head = _interleaved_source(jax.lax.broadcasted_iota(I32, (128, 128), 0)) >> 5
        col_head = jax.lax.broadcasted_iota(I32, (128, 128), 1) >> 5
        for g in range(D // 128):
            tiled = _dot(select, wphi_v[pl.ds(g * 128, 128), :], NT)
            fold_v[g] = _pack(jnp.where(row_head == col_head, tiled, 0.0))

    def prep_scores(i, g):
        blocks = []
        for group in (g, g + HD // 128):
            for half in range(2):
                w = wqkv_v[pl.ds(half * HD, HD), pl.ds(i * D + group * 128, 128)]
                blocks.append(_dot(_unpack(fold_v[group]), w, NT) * LOG2E)
        for j, term in enumerate(_lhs_terms(*blocks)):
            (wq_v, wk_v)[i][g][j] = _pack(term)

    def prep_values(g):
        chain = Chain(1)
        for r in range(0, HD, 64):
            blocks = [wqkv_v[pl.ds(row + r, 64), pl.ds(2 * D + col + g * 128, 128)].astype(F32)
                      for col in (0, HD) for row in (0, HD)]
            token = chain.tokens.popleft()
            if token is not None:
                head = pltpu.bitcast(pltpu.bitcast(blocks[3][:8], I32) | token, F32)
                blocks[3] = jnp.concatenate([head, blocks[3][8:]], axis=0)
            for j, term in enumerate(_lhs_terms(*blocks)):
                words = _pack(term)
                wv_v[g][j, pl.ds(r // 2, 32), :] = words
            chain.leave(words[:8])

    def prep_output(n):
        lo = wo_v[pl.ds(n * 16, 16), :].astype(F32)
        hi = wo_v[pl.ds(HD + n * 16, 16), :].astype(F32)
        words = [_pack(term) for term in _rhs_terms(lo[:, :HD], lo[:, HD:], hi[:, :HD], hi[:, HD:])]
        for j, w in enumerate(words):
            wot_v[j, pl.ds(n * 8, 8), :] = w
        finish_within(2, *words)

    def row_stats(t, n):
        xx = x_v[pl.ds(t * T + n * 32, 32), :].astype(F32)
        mean = jnp.mean(xx, axis=-1, keepdims=True)
        d = xx - mean
        scale = jax.lax.rsqrt(jnp.mean(d * d, axis=-1, keepdims=True) + EPS)
        stat_v[0, pl.ds(n * 32, 32), :] = jnp.broadcast_to(mean, (32, 128))
        stat_v[1, pl.ds(n * 32, 32), :] = jnp.broadcast_to(scale, (32, 128))

    def normalized(t, offset, lanes):
        wide = lambda k: jnp.concatenate([stat_v[k, pl.ds(offset, 16), :]] * (HD // 128), axis=1)
        return (x_v[pl.ds(t * T + offset, 16), lanes].astype(F32) - wide(0)) * wide(1)

    def norm_terms(rows, n, shift=True, delay=0):
        blocks = []
        for lanes in (pl.ds(0, HD), pl.ds(HD, HD)):
            for offset in (n * 16, HT + n * 16):
                hh = rows(offset, lanes).reshape(2, 8, HD) * mod_v[1, :, lanes]
                blocks.append((hh + mod_v[0, :, lanes] if shift else hh).reshape(16, HD))
        words = [_pack(term) for term in _rhs_terms(*blocks)]
        if delay:
            finish_within(delay, *words)

        def store(target):
            for j, w in enumerate(words):
                target[j, pl.ds(n * 8, 8), :] = w

        return store

    def tile_norm(t, n, delay):
        if n % 2 == 0:
            row_stats(t, n // 2)
            row_stats(t, HT // 32 + n // 2)
        return norm_terms(functools.partial(normalized, t), n, delay=delay)

    def products(product, tiles, cycles, hook):
        result = []
        for j in range(7):
            result.append([product(j, k) for k in range(tiles)])
            backlog.spent(cycles)
            hook()
        return result

    def features(weights, source, hook, target, rows):
        for r in range(0, HD, rows):
            m = products(
                lambda j, k: _dot(
                    _unpack(jnp.concatenate([weights[g][j] for g in range(r // 128, (r + rows) // 128)], axis=0)),
                    _unpack(gated(source, j, k * 64)[k * 64:(k + 1) * 64]), NT),
                HT // 128, rows * HT // 128, hook)

            def unit(half, o, m=m, r=r):
                for part in range(2):
                    phi = jnp.concatenate(
                        [_features(_quadrant(2 * half + part, lambda j: m[j][k][o:o + 64]))
                         for k in range(HT // 128)], axis=1)
                    target((half * HD + r + o) // 64, pl.ds(part * HT, HT), phi.astype(BF16))

            for half in range(2):
                for o in range(0, rows, 64):
                    backlog.defer(150 * rows // 256, functools.partial(unit, half, o))

    def store_keys(pair, lanes, phi):
        phik_v[pair, :, lanes] = phi

    def store_queries(t, pair, lanes, phi):
        phiq_v[t, pair, :, lanes] = phi

    def store_values(col, part, v):
        v = v.T.astype(BF16).reshape(2, 64, HT)
        vt_v[pl.ds(col // 64, 2), pl.ds(0, 64), pl.ds(part * HT, HT)] = v

    def values(source, hook, target, cols):
        for r in range(0, HD, cols):
            m = products(
                lambda j, k: _dot(_unpack(source[j]), _unpack(gated(wv_v[r // 128 + k], j))),
                cols // 128, cols * HT // 128, hook)

            def unit(half, part, k, m=m, r=r):
                target(half * HD + r + k * 128, part, _quadrant(2 * half + part, lambda j: m[j][k]))

            for half in range(2):
                for part in range(2):
                    for k in range(cols // 128):
                        backlog.defer(128, functools.partial(unit, half, part, k))

    def accumulate_summary(first):
        backlog.drain()
        for r in range(0, HD, 256):
            for half in range(2):
                for o in range(0, 256, 64):
                    pair = (half * HD + r + o) // 64
                    kv = _dot(vt_v[pair], phik_v[pair], NT)
                    if first:
                        bias = _apply(jnp.multiply, column_v[pl.ds(pair * 64, 64), :], kv[64:72])
                        kv_v[pair] = jnp.concatenate([kv[:64] + bias, kv[64:]], axis=0)
                    else:
                        kv_v[pair] = kv_v[pair] + kv

    def finish_summary(pair):
        row = jax.lax.broadcasted_iota(I32, (80, 128), 0)
        row_head = jnp.where(row < 64, row >> 5, (row >> 3) & 1)
        col_head = jax.lax.broadcasted_iota(I32, (80, 128), 1) & 1
        summary_v[pair] = _pack(jnp.where(row_head == col_head, kv_v[pair], 0.0))

    def attend(step, target):
        t, lanes = step // 2, pl.ds(step % 2 * 2 * G, 2 * G)
        pairs = [[[half * NPAIR // 2 + 2 * i + k for k in range(2)] for half in range(2)] for i in range(4)]
        nums = {p: _dot(_unpack(summary_v[p]), phiq_v[t, p, :, lanes])
                for group in pairs for side in group for p in side}
        sides = []
        for i, group in enumerate(pairs):
            heads = [[_apply(jnp.multiply, nums[p][h * DH:(h + 1) * DH],
                             _recip(nums[p][64 + 8 * h:72 + 8 * h] + 1e-6))
                      for p in side for h in range(2)] for side in group]
            sides.append([jnp.concatenate(side, axis=0).T for side in heads])
            if i % 2:
                lo, hi = (jnp.concatenate([sides[i - 1][s], sides[i][s]], axis=1) for s in range(2))
                for j, term in enumerate(_lhs_terms(lo[:G], hi[:G], lo[G:], hi[G:])):
                    target[j, :, pl.ds((i - 1) * 128, 256)] = term.astype(BF16)

    def project_output(source, lo, n, hook):
        m = products(
            lambda j, k: _dot(source[j, pl.ds(lo, n), :],
                              _unpack(gated(wot_v, j)[:, k * 128:(k + 1) * 128])),
            HD // 128, 4 * n, hook)

        def rows(o):
            part, o = divmod(o, n)
            piece = lambda j: jnp.concatenate([tile[o:o + 32] for tile in m[j]], axis=1)
            return lo + part * G + o, jnp.concatenate(
                [_quadrant(2 * part + half, piece) for half in range(2)], axis=1)

        return rows

    scores = {}

    def finish(step, rows, count, strands, delay):
        chain = Chain(strands)
        lane = jax.lax.broadcasted_iota(I32, (8, 128), 1)
        for start_row in range(0, count, 32):
            row, y = rows(start_row)
            for o in range(0, 32, 8):
                base = step * 2 * G + row + o
                xn = x_v[pl.ds(base, 8), :].astype(F32) + mod_v[2] * chain.enter(y[o:o + 8])
                mean = jnp.mean(xn, axis=-1, keepdims=True)
                d = xn - mean
                scale = jax.lax.rsqrt(jnp.mean(d * d, axis=-1, keepdims=True) + EPS)
                score = jnp.sum(d * mod_v[6], axis=-1, keepdims=True) * scale + mod_v[9, :, :1]
                normed = d * scale
                norm_v[pl.ds(base, 8), :] = normed
                out = normed * mod_v[7] + ((d + mean) + mod_v[8])
                out_v[pl.ds(base, 8), :] = out.astype(BF16)
                held = scores.get(base // 1024, jnp.full((8, 128), -jnp.inf, F32))
                scores[base // 1024] = jnp.where(lane == base % 1024 // 8, score, held)
                chain.leave(*[out[:, l:l + 128] for l in range(128, D, 256)])
        if delay:
            finish_within(delay, *chain.tokens)

    def top_two():
        shape = (S // 1024, 8, 128)
        index = (jax.lax.broadcasted_iota(I32, shape, 0) * 1024 + jax.lax.broadcasted_iota(I32, shape, 2) * 8
                 + jax.lax.broadcasted_iota(I32, shape, 1)).astype(F32)
        left = jnp.stack([scores[b] for b in range(S // 1024)])
        reduce = lambda op, v: op(op(op(v, axis=0), axis=0, keepdims=True), axis=1, keepdims=True)
        top = reduce(jnp.max, left)
        first = reduce(jnp.min, jnp.where(left == top, index, float(S)))
        below = reduce(jnp.max, jnp.where(left == top, -jnp.inf, left))
        tied = reduce(jnp.min, jnp.where((left == top) & (index != first), index, float(S)))
        lower = reduce(jnp.min, jnp.where((left == below) & (left != top), index, float(S)))
        second = jnp.where(tied < S, tied, lower)
        row = lambda v: jnp.clip(jnp.max(v.astype(I32)), 0, S - 1)
        return (row(first), top), (row(second), jnp.where(tied < S, top, below))

    def routed_update():
        (row1, score1), (row2, score2) = top_two()
        sub = jax.lax.broadcasted_iota(I32, (16, D), 0)
        first, second = (jnp.broadcast_to(norm_v[pl.ds(row, 1), :], (16, D)) for row in (row1, row2))
        selected = jnp.where(sub == 0, first, second).reshape(2, 8, D) * mod_v[4] + mod_v[3]
        selected = selected.reshape(16, D).astype(BF16)
        pending = collections.deque()
        parts = []

        def down():
            f, g, u = pending.popleft()
            act = (g * jax.nn.sigmoid(g) * u).astype(BF16)
            part = _dot(act, wd_v[pl.ds(f, FF_CHUNK), :])
            parts.append(parts.pop() + part if parts else part)

        for f in range(0, FF, FF_CHUNK):
            pending.append((f, _dot(selected, wg_v[:, pl.ds(f, FF_CHUNK)]),
                            _dot(selected, wu_v[:, pl.ds(f, FF_CHUNK)])))
            if len(pending) > 2:
                down()
        while pending:
            down()
        y1, y2 = parts[0][0:1] * jax.nn.sigmoid(score1), parts[0][1:2] * jax.nn.sigmoid(score2)
        bases = [pl.multiple_of((row >> 4) * 16, 16) for row in (row1, row2)]
        for n, base in enumerate(bases):
            update = jnp.where(sub == row1 - base, y1, 0.0) + jnp.where(sub == row2 - base, y2, 0.0)
            rows = out_v[pl.ds(base, 16), :].astype(F32).reshape(2, 8, D) + mod_v[5] * update.reshape(2, 8, D)
            fix_v[n] = rows.reshape(16, D).astype(BF16)
        return bases

    cc = c_v[...].astype(F32)
    act_v[...] = _pack(jnp.broadcast_to(cc * jax.nn.sigmoid(cc), (16, D)))
    wait(("x", 0))
    for n in range(T // 32):
        row_stats(0, n)
    for offset in range(0, T, 16):
        for lanes in (pl.ds(0, HD), pl.ds(HD, HD)):
            norm_v[pl.ds(offset, 16), lanes] = normalized(0, offset, lanes)
    for half in range(2):
        wait(("scale", half))
        modulation(D, D, half)
    mod_v[1] = raw(1) + 1.0
    first_rows = lambda offset, lanes: norm_v[pl.ds(offset, 16), lanes]
    for n in range(NORM_UNITS):
        norm_terms(first_rows, n, shift=False)(h_v)

    wait(*both("wv", 0))
    prep_values(0)
    plan = new_plan()
    plan[3] += [lambda: wait(*both("wv", 1)), lambda: prep_values(1)]
    plan[7] += [lambda: wait(*both("wv", 2))]
    plan[8] += [lambda: prep_values(2)]
    plan[15] += [lambda: prep_values(3)]
    plan[28] += [lambda: wait("wphi", *both("wk", 0)), feature_maps, lambda: prep_scores(1, 0)]
    plan[28] += [lambda: prep_scores(1, 1)]

    def shift_vector():
        wait(*both("shift"))
        for half in range(2):
            modulation(0, D, half)
        mod_v[0] = raw(0)

    def shift_bias():
        shift = jnp.concatenate([raw(0)] * 2, axis=0).astype(BF16)
        bias_v[...] = _dot(shift, wqkv_v[:, pl.ds(2 * D, D)])[:8]

    plan[21].append(shift_vector)
    plan[21].append(shift_bias)
    for n in range(NORM_UNITS):
        plan[22 + (28 - 22) * n // NORM_UNITS].append(
            functools.partial(lambda n: norm_terms(first_rows, n, delay=1)(h0_v), n))
    values(h_v, _follow(plan), store_values, 128)
    backlog.drain()

    def ones_rows():
        vt_v[:, pl.ds(64, 16), :] = jnp.ones((NPAIR, 16, T), BF16)

    plan = new_plan()
    plan[0].append(ones_rows)
    plan[3] += [lambda: wait(("x", 1), *both("wk", 1)), lambda: prep_scores(1, 2), lambda: prep_scores(1, 3)]
    plan[1].append(lambda: store_column(bias_v[...]))
    early = 13
    for n in range(early):
        plan[6 + n // 2].append(functools.partial(lambda n: tile_norm(1, n, 3 + n % 2)(h_v), n))
    features(wk_v, h0_v, _follow(plan), store_keys, 256)
    wait("wq")
    for g in range(4):
        prep_scores(0, g)
        backlog.spent(512)
    backlog.drain()
    for n in range(early, NORM_UNITS):
        tile_norm(1, n, 0)(h_v)
    accumulate_summary(first=True)

    for t in range(1, NTILE):
        if t == NTILE - 1:
            wait(*[("mod", i) for i in range(NTILE)])
        plan = new_plan()
        if t + 1 < NTILE:
            wait(("x", t + 1))
            stores = []
            for n in range(NORM_UNITS):
                plan[32 + (10 * n) // 16].append(
                    functools.partial(lambda n: stores.append(tile_norm(t + 1, n, 2 + n % 2)), n))
            plan[42].append(lambda: [store(h_v) for store in stores])
        start(("wg", "wu", "wd")[t - 1])
        if t == NTILE - 1:
            plan_vector_modulation(plan, (1, 2, 3, 32, 33, 34, 35, 36, 37, 38, 39, 40, 41, 42))
        due.clear()
        hook = _follow(plan)
        features(wk_v, h_v, hook, store_keys, 256)
        features(wq_v, h_v, hook, functools.partial(store_queries, t), 256)
        values(h_v, hook, store_values, 256)
        accumulate_summary(first=False)

    order = [(n + T // (2 * G)) % NSTEP for n in range(NSTEP)]
    wait("wo", "wr", "wg", "wu", "wd")
    plan = new_plan()
    plan[0] += [functools.partial(finish_summary, pair) for pair in range(NPAIR)]
    plan[0].append(lambda: attend(order[0], oa_v))
    for n in range(HD // 16):
        plan[3 + 24 * n // (HD // 16)].append(functools.partial(prep_output, n))
    plan[26].append(output_weights)
    due.clear()
    features(wq_v, h0_v, _follow(plan), functools.partial(store_queries, 0), 128)

    due.clear()
    rows = None
    for n in range(NSTEP):
        source, target = ((oa_v, ob_v), (ob_v, oa_v))[n % 2]
        if n + 1 < NSTEP:
            attend(order[n + 1], target)
            if rows:
                finish(order[n - 1], rows, 2 * G, 3, 44)
            rows = project_output(source, 0, G, lambda: None)
        else:
            finish(order[n - 1], rows, 2 * G, 6, 26)
            rows = project_output(source, 0, G // 2, lambda: None)
            finish(order[n], rows, G, 8, 24)
            rows = project_output(source, G // 2, G // 2, lambda: None)
        if n > 1:
            out_copy(order[n - 2]).start()
    finish(order[-1], rows, G, G // 8, 0)
    out_copy(order[-2]).start()
    out_copy(order[-1]).start()

    base1, base2 = routed_update()
    for step in order:
        out_copy(step).wait()
    fix = [pltpu.make_async_copy(fix_v.at[n], out_hbm.at[pl.ds(base, 16)], out_sems.at[n])
           for n, base in enumerate((base1, base2))]
    fix[0].start()

    @pl.when(base1 != base2)
    def _():
        fix[1].start()
        fix[1].wait()

    fix[0].wait()


def _scratch():
    vmem = pltpu.VMEM
    return [
        vmem((S, D), BF16), vmem((D, 3 * D), BF16), vmem((D, DH), BF16), vmem((D, D), BF16),
        vmem((8, 128), BF16), vmem((D, FF), BF16), vmem((D, FF), BF16), vmem((FF, D), BF16),
        vmem((1, D), BF16), vmem((D, 6 * D), BF16),
        vmem((8, D), U32), vmem((D, 128), F32), vmem((8, 6 * D), F32), vmem((10, 8, D), F32), vmem((2, T, 128), F32),
        vmem((8, D), F32), vmem((D // 128, 64, 128), U32), vmem((7, HD // 2, HD), U32),
        vmem((7, HT // 2, HD), U32), vmem((7, HT // 2, HD), U32),
        vmem((NTILE, NPAIR, 128, T), BF16), vmem((NPAIR, 128, T), BF16), vmem((NPAIR, 80, T), BF16),
        vmem((NPAIR, 80, 128), F32), vmem((NPAIR, 40, 128), U32),
        vmem((7, G, HD), BF16), vmem((7, G, HD), BF16),
        vmem((S, D), F32), vmem((S, D), BF16), vmem((2, 16, D), BF16),
        pltpu.SemaphoreType.DMA((8 + 2 * NTILE + 14,)), pltpu.SemaphoreType.DMA((NSTEP,)),
    ] + [vmem((7, 64, HD), U32)] * 8 + [vmem((7, HD // 2, 128), U32)] * 4


@jax.jit
def pallas_adaLN_cond__linear_kernel_hedgehog__moe_arch_mod__prompt_kernel(
    A_x: jax.Array,
    A_wqkv: jax.Array,
    A_w_phi: jax.Array,
    A_wo: jax.Array,
    B_x: jax.Array,
    B_w_r: jax.Array,
    B_w_gate: jax.Array,
    B_w_up: jax.Array,
    B_w_down: jax.Array,
    c: jax.Array,
    w_mod: jax.Array,
):
    del B_x
    out = pl.pallas_call(
        _kernel,
        out_shape=jax.ShapeDtypeStruct((S, D), A_x.dtype),
        in_specs=[pl.BlockSpec(memory_space=pl.ANY)] * 10,
        out_specs=pl.BlockSpec(memory_space=pl.ANY),
        scratch_shapes=_scratch(),
        compiler_params=pltpu.CompilerParams(vmem_limit_bytes=120 * 2**20),
    )(A_x.reshape(S, D), A_wqkv, A_w_phi.reshape(D, DH), A_wo, B_w_r.reshape(8, 128),
      B_w_gate, B_w_up, B_w_down, c, w_mod)
    return out.reshape(A_x.shape)
```

```python
import collections
import functools

import jax
import jax.numpy as jnp
import numpy as np
import jax.experimental.pallas as pl
import jax.experimental.pallas.tpu as pltpu

F32, BF16, I32, U32 = jnp.float32, jnp.bfloat16, jnp.int32, jnp.uint32
S, D, HEADS, DH, FF = 2048, 1024, 32, 32, 3584
EPS = 1e-5
LOG2E = float(np.log2(np.e))

HD = D // 2
NPAIR = HEADS // 2
T = 512
HT = T // 2
NTILE = S // T
G = 128
NSTEP = S // (2 * G)
MOD_COLS = 4 * D // NTILE
NORM_UNITS = HT // 16
FF_CHUNK = 256

NN = (((1,), (0,)), ((), ()))
NT = (((1,), (1,)), ((), ()))


def _dot(a, b, dims=NN):
    return jax.lax.dot_general(a, b, dims, preferred_element_type=F32)


def _pack(x):
    n = x.shape[0] // 2
    if x.shape[1] > 128:
        return pltpu.bitcast(x.astype(BF16), U32)
    w = pltpu.bitcast(jnp.concatenate([x[:n], x[n:]], axis=1).astype(BF16), U32)
    return jnp.concatenate([w[:, :128], w[:, 128:]], axis=0)


def _unpack(w):
    return pltpu.bitcast(w, BF16)


def _recip(x):
    r = pl.reciprocal(x, approx=True)
    return r * (2.0 - x * r)


def _lhs_terms(a11, a12, a21, a22):
    return (a11 + a22, a21 + a22, a11, a22, a11 + a12, a21 - a11, a12 - a22)


def _rhs_terms(b11, b12, b21, b22):
    return (b11 + b22, b11, b12 - b22, b21 - b11, b22, b11 + b12, b21 + b22)


_QUADRANTS = (((0, 1), (3, 1), (4, -1), (6, 1)), ((2, 1), (4, 1)), ((1, 1), (3, 1)),
              ((0, 1), (1, -1), (2, 1), (5, 1)))


def _quadrant(q, product):
    total = None
    for j, sign in _QUADRANTS[q]:
        m = product(j)
        total = m if total is None else (total + m if sign > 0 else total - m)
    return total


def _per_head(op, p):
    parts = [p[r:r + 8] for r in range(0, p.shape[0], 8)]
    while len(parts) > 1:
        parts = [op(a, b) for a, b in zip(parts[::2], parts[1::2])]
    out = op(parts[0], pltpu.roll(parts[0], 4, 0))
    return op(out, pltpu.roll(out, 2, 0))


def _apply(op, p, rows8):
    return op(p.reshape(p.shape[0] // 8, 8, p.shape[1]), rows8).reshape(p.shape)


def _features(p):
    e_pos = jnp.exp2(_apply(jnp.subtract, p, _per_head(jnp.maximum, p)))
    e_neg = jnp.exp2(_apply(lambda a, low: low - a, p, _per_head(jnp.minimum, p)))
    pos = _apply(jnp.multiply, e_pos, _recip(_per_head(jnp.add, e_pos)))
    neg = _apply(jnp.multiply, e_neg, _recip(_per_head(jnp.add, e_neg)))
    return jnp.concatenate([pos, neg], axis=0)


def _interleaved_source(row):
    return (row & ~63) + ((row & 1) << 5) + ((row & 63) >> 1)


class _Backlog:
    def __init__(self):
        self.queue = collections.deque()
        self.credit = 0.0

    def defer(self, cost, task):
        self.queue.append((cost, task))

    def spent(self, cycles):
        self.credit += 0.55 * cycles
        while self.queue and self.credit >= self.queue[0][0]:
            cost, task = self.queue.popleft()
            self.credit -= cost
            task()
        if not self.queue:
            self.credit = 0.0

    def drain(self):
        while self.queue:
            self.queue.popleft()[1]()
        self.credit = 0.0


def _follow(plan):
    count = 0

    def step():
        nonlocal count
        count += 1
        for task in plan.pop(count, ()):
            task()

    for task in plan.pop(0, ()):
        task()
    return step


def _kernel(x_hbm, wqkv_hbm, wphi_hbm, wo_hbm, wr_hbm, wg_hbm, wu_hbm, wd_hbm, c_hbm, wmod_hbm,
            out_hbm,
            x_v, wqkv_v, wphi_v, wo_v, wr_v, wg_v, wu_v, wd_v, c_v, wmod_v,
            act_v, column_v, raw_v, mod_v, stat_v, bias_v, fold_v, wot_v, h_v, h0_v,
            phiq_v, phik_v, vt_v, kv_v, summary_v, oa_v, ob_v, norm_v, out_v, fix_v,
            in_sems, out_sems, *terms_v):
    wq_v, wk_v, wv_v = terms_v[:4], terms_v[4:8], terms_v[8:]
    backlog = _Backlog()
    new_plan = lambda: collections.defaultdict(list)

    copies = {}

    def add_copy(name, src, dst, part=Ellipsis):
        if part is not Ellipsis:
            src, dst = src.at[part], dst.at[part]
        copies[name] = pltpu.make_async_copy(src, dst, in_sems.at[len(copies)])

    columns = lambda lo, n: (pl.ds(0, D), pl.ds(lo, n))
    for name, src, dst in (("c", c_hbm, c_v), ("wphi", wphi_hbm, wphi_v), ("wr", wr_hbm, wr_v),
                           ("wo", wo_hbm, wo_v), ("wg", wg_hbm, wg_v), ("wu", wu_hbm, wu_v),
                           ("wd", wd_hbm, wd_v)):
        add_copy(name, src, dst)
    add_copy("wq", wqkv_hbm, wqkv_v, columns(0, D))
    for t in range(NTILE):
        add_copy(("x", t), x_hbm, x_v, pl.ds(t * T, T))
        add_copy(("mod", t), wmod_hbm, wmod_v, columns(2 * D + t * MOD_COLS, MOD_COLS))
    for half in range(2):
        add_copy(("shift", half), wmod_hbm, wmod_v, (pl.ds(half * HD, HD), pl.ds(0, D)))
        add_copy(("scale", half), wmod_hbm, wmod_v, (pl.ds(half * HD, HD), pl.ds(D, D)))
        for n in range(2):
            add_copy(("wk", n, half), wqkv_hbm, wqkv_v, columns(D + half * HD + n * 256, 256))
        for n, (lo, size) in enumerate(((0, 128), (128, 128), (256, 256))):
            add_copy(("wv", n, half), wqkv_hbm, wqkv_v, columns(2 * D + half * HD + lo, size))
    both = lambda *name: ((*name, 0), (*name, 1))

    def start(*names):
        for name in names:
            copies[name].start()

    def wait(*names):
        for name in names:
            copies[name].wait()

    def out_copy(step):
        rows = pl.ds(step * 2 * G, 2 * G)
        return pltpu.make_async_copy(out_v.at[rows], out_hbm.at[rows], out_sems.at[step])

    start("c", ("x", 0), *both("scale"), *both("wv", 0), *both("wv", 1), *both("wv", 2),
          *both("shift"), "wphi", *both("wk", 0), *both("wk", 1), ("x", 1), "wq",
          ("x", 2), ("mod", 1), ("x", 3), ("mod", 2), ("mod", 3), ("mod", 0), "wo", "wr")
    wait("c")

    bits = pltpu.bitcast(jnp.broadcast_to(c_v[:, :128].astype(F32), (8, 128)), I32)
    zero = jnp.minimum(jnp.max(bits & 0xFF), 0)

    class Chain:
        def __init__(self, strands):
            self.tokens = collections.deque([None] * strands)

        def enter(self, rows8):
            token = self.tokens.popleft()
            if token is None:
                return rows8
            head = pltpu.bitcast(pltpu.bitcast(rows8[:, :128], I32) | token, F32)
            return jnp.concatenate([head, rows8[:, 128:]], axis=1)

        def leave(self, *values):
            words = [pltpu.bitcast(value, I32) for value in values]
            self.tokens.append(functools.reduce(jnp.bitwise_or, words) & zero)

    clock = 0
    due = collections.defaultdict(list)

    def finish_within(delay, *values):
        parts = [pltpu.bitcast(value, U32)[r:r + 8, l:l + 128] for value in values
                 for r in range(0, value.shape[0], 8) for l in range(0, value.shape[1], 128)]
        due[clock + delay].append(functools.reduce(jnp.bitwise_or, parts) & zero.astype(U32))

    def gated(ref, j, row=0):
        nonlocal clock
        clock += 1
        tokens = [token for when in sorted(due) if when < clock for token in due.pop(when)]
        if tokens:
            corner = (j, pl.ds(row, 8), pl.ds(0, 128))
            ref[corner] = functools.reduce(jnp.bitwise_or, tokens, ref[corner])
        return ref[j]

    def modulation(lo, n, half):
        rows, lanes = pl.ds(half * HD, HD), pl.ds(lo, n)
        m = _dot(_unpack(act_v[:, rows]), wmod_v[rows, lanes])[:8]
        raw_v[:, lanes] = raw_v[:, lanes] + m if half else m

    raw = lambda i: raw_v[:, pl.ds(i * D, D)]

    def store_column(rows):
        column_v[...] = jnp.broadcast_to(rows[:1], (128, D)).T

    def plan_vector_modulation(plan, slots):
        sums = {}

        def unit(i, k):
            total = sums.get(i)
            for r in range(k, k + 64, 8):
                w = wmod_v[pl.ds(r, 8), pl.ds(i * D, D)].astype(F32)
                term = w * jnp.concatenate([column_v[pl.ds(r, 8), :]] * (D // 128), axis=1)
                total = term if total is None else total + term
            sums[i] = total
            finish_within(2, total)
            if k + 64 == D:
                raw_v[:, pl.ds(i * D, D)] = jnp.broadcast_to(jnp.sum(total, axis=0, keepdims=True), (8, D))

        plan[0].append(lambda: store_column(_unpack(act_v[...]).astype(F32)))
        units = [(i, k) for i in range(2, 6) for k in range(0, D, 64)]
        for n, (i, k) in enumerate(units):
            plan[slots[len(slots) * n // len(units)]].append(functools.partial(unit, i, k))

    def output_weights():
        w = wr_v[...].astype(F32)
        w = jnp.concatenate([jnp.broadcast_to(w[j:j + 1], (8, 128)) for j in range(D // 128)], axis=1)
        for i in range(2, 6):
            mod_v[i] = raw(i) + 1.0 if i == 4 else raw(i)
        mod_v[6] = mod_v[4] * w
        mod_v[7] = mod_v[4] * mod_v[5]
        mod_v[8] = mod_v[3] * mod_v[5]
        mod_v[9] = jnp.broadcast_to(jnp.sum(mod_v[3] * w, axis=1, keepdims=True), (8, D))

    def feature_maps():
        row = _interleaved_source(jax.lax.broadcasted_iota(I32, (128, DH), 0))
        col = jax.lax.broadcasted_iota(I32, (128, DH), 1)
        select = jnp.where((row & (DH - 1)) == col, 1.0, 0.0).astype(BF16)
        row_head = _interleaved_source(jax.lax.broadcasted_iota(I32, (128, 128), 0)) >> 5
        col_head = jax.lax.broadcasted_iota(I32, (128, 128), 1) >> 5
        for g in range(D // 128):
            tiled = _dot(select, wphi_v[pl.ds(g * 128, 128), :], NT)
            fold_v[g] = _pack(jnp.where(row_head == col_head, tiled, 0.0))

    def prep_scores(i, g):
        blocks = []
        for group in (g, g + HD // 128):
            for half in range(2):
                w = wqkv_v[pl.ds(half * HD, HD), pl.ds(i * D + group * 128, 128)]
                blocks.append(_dot(_unpack(fold_v[group]), w, NT) * LOG2E)
        for j, term in enumerate(_lhs_terms(*blocks)):
            (wq_v, wk_v)[i][g][j] = _pack(term)

    def prep_values(g):
        chain = Chain(1)
        for r in range(0, HD, 64):
            blocks = [wqkv_v[pl.ds(row + r, 64), pl.ds(2 * D + col + g * 128, 128)].astype(F32)
                      for col in (0, HD) for row in (0, HD)]
            token = chain.tokens.popleft()
            if token is not None:
                head = pltpu.bitcast(pltpu.bitcast(blocks[3][:8], I32) | token, F32)
                blocks[3] = jnp.concatenate([head, blocks[3][8:]], axis=0)
            for j, term in enumerate(_lhs_terms(*blocks)):
                words = _pack(term)
                wv_v[g][j, pl.ds(r // 2, 32), :] = words
            chain.leave(words[:8])

    def prep_output(n):
        lo = wo_v[pl.ds(n * 16, 16), :].astype(F32)
        hi = wo_v[pl.ds(HD + n * 16, 16), :].astype(F32)
        words = [_pack(term) for term in _rhs_terms(lo[:, :HD], lo[:, HD:], hi[:, :HD], hi[:, HD:])]
        for j, w in enumerate(words):
            wot_v[j, pl.ds(n * 8, 8), :] = w
        finish_within(3, *words)

    def row_stats(t, n):
        xx = x_v[pl.ds(t * T + n * 32, 32), :].astype(F32)
        mean = jnp.mean(xx, axis=-1, keepdims=True)
        d = xx - mean
        scale = jax.lax.rsqrt(jnp.mean(d * d, axis=-1, keepdims=True) + EPS)
        stat_v[0, pl.ds(n * 32, 32), :] = jnp.broadcast_to(mean, (32, 128))
        stat_v[1, pl.ds(n * 32, 32), :] = jnp.broadcast_to(scale, (32, 128))

    def normalized(t, offset, lanes):
        wide = lambda k: jnp.concatenate([stat_v[k, pl.ds(offset, 16), :]] * (HD // 128), axis=1)
        return (x_v[pl.ds(t * T + offset, 16), lanes].astype(F32) - wide(0)) * wide(1)

    def norm_terms(rows, n, shift=True, delay=0):
        blocks = []
        for lanes in (pl.ds(0, HD), pl.ds(HD, HD)):
            for offset in (n * 16, HT + n * 16):
                hh = rows(offset, lanes).reshape(2, 8, HD) * mod_v[1, :, lanes]
                blocks.append((hh + mod_v[0, :, lanes] if shift else hh).reshape(16, HD))
        words = [_pack(term) for term in _rhs_terms(*blocks)]
        if delay:
            finish_within(delay, *words)

        def store(target):
            for j, w in enumerate(words):
                target[j, pl.ds(n * 8, 8), :] = w

        return store

    def tile_norm(t, n, delay):
        if n % 2 == 0:
            row_stats(t, n // 2)
            row_stats(t, HT // 32 + n // 2)
        return norm_terms(functools.partial(normalized, t), n, delay=delay)

    def products(product, tiles, cycles, hook):
        result = []
        for j in range(7):
            result.append([product(j, k) for k in range(tiles)])
            backlog.spent(cycles)
            hook()
        return result

    def features(weights, source, hook, target, rows):
        for r in range(0, HD, rows):
            m = products(
                lambda j, k: _dot(
                    _unpack(jnp.concatenate([weights[g][j] for g in range(r // 128, (r + rows) // 128)], axis=0)),
                    _unpack(gated(source, j, k * 64)[k * 64:(k + 1) * 64]), NT),
                HT // 128, rows * HT // 128, hook)

            def unit(half, o, m=m, r=r):
                for part in range(2):
                    phi = jnp.concatenate(
                        [_features(_quadrant(2 * half + part, lambda j: m[j][k][o:o + 64]))
                         for k in range(HT // 128)], axis=1)
                    target((half * HD + r + o) // 64, pl.ds(part * HT, HT), phi.astype(BF16))

            for half in range(2):
                for o in range(0, rows, 64):
                    backlog.defer(150 * rows // 256, functools.partial(unit, half, o))

    def store_keys(pair, lanes, phi):
        phik_v[pair, :, lanes] = phi

    def store_queries(t, pair, lanes, phi):
        phiq_v[t, pair, :, lanes] = phi

    def store_values(col, part, v):
        v = v.T.astype(BF16).reshape(2, 64, HT)
        vt_v[pl.ds(col // 64, 2), pl.ds(0, 64), pl.ds(part * HT, HT)] = v

    def values(source, hook, target, cols):
        for r in range(0, HD, cols):
            m = products(
                lambda j, k: _dot(_unpack(source[j]), _unpack(gated(wv_v[r // 128 + k], j))),
                cols // 128, cols * HT // 128, hook)

            def unit(half, part, k, m=m, r=r):
                target(half * HD + r + k * 128, part, _quadrant(2 * half + part, lambda j: m[j][k]))

            for half in range(2):
                for part in range(2):
                    for k in range(cols // 128):
                        backlog.defer(128, functools.partial(unit, half, part, k))

    def accumulate_summary(first):
        backlog.drain()
        for r in range(0, HD, 256):
            for half in range(2):
                for o in range(0, 256, 64):
                    pair = (half * HD + r + o) // 64
                    kv = _dot(vt_v[pair], phik_v[pair], NT)
                    if first:
                        bias = _apply(jnp.multiply, column_v[pl.ds(pair * 64, 64), :], kv[64:72])
                        kv_v[pair] = jnp.concatenate([kv[:64] + bias, kv[64:]], axis=0)
                    else:
                        kv_v[pair] = kv_v[pair] + kv

    def finish_summary(pair):
        row = jax.lax.broadcasted_iota(I32, (80, 128), 0)
        row_head = jnp.where(row < 64, row >> 5, (row >> 3) & 1)
        col_head = jax.lax.broadcasted_iota(I32, (80, 128), 1) & 1
        summary_v[pair] = _pack(jnp.where(row_head == col_head, kv_v[pair], 0.0))

    def attend(step, target):
        t, lanes = step // 2, pl.ds(step % 2 * 2 * G, 2 * G)
        pairs = [[[half * NPAIR // 2 + 2 * i + k for k in range(2)] for half in range(2)] for i in range(4)]
        nums = {p: _dot(_unpack(summary_v[p]), phiq_v[t, p, :, lanes])
                for group in pairs for side in group for p in side}
        sides = []
        for i, group in enumerate(pairs):
            heads = [[_apply(jnp.multiply, nums[p][h * DH:(h + 1) * DH],
                             _recip(nums[p][64 + 8 * h:72 + 8 * h] + 1e-6))
                      for p in side for h in range(2)] for side in group]
            sides.append([jnp.concatenate(side, axis=0).T for side in heads])
            if i % 2:
                lo, hi = (jnp.concatenate([sides[i - 1][s], sides[i][s]], axis=1) for s in range(2))
                for j, term in enumerate(_lhs_terms(lo[:G], hi[:G], lo[G:], hi[G:])):
                    target[j, :, pl.ds((i - 1) * 128, 256)] = term.astype(BF16)

    def project_output(source, lo, n, hook):
        m = products(
            lambda j, k: _dot(source[j, pl.ds(lo, n), :],
                              _unpack(gated(wot_v, j)[:, k * 128:(k + 1) * 128])),
            HD // 128, 4 * n, hook)

        def rows(o):
            part, o = divmod(o, n)
            piece = lambda j: jnp.concatenate([tile[o:o + 32] for tile in m[j]], axis=1)
            return lo + part * G + o, jnp.concatenate(
                [_quadrant(2 * part + half, piece) for half in range(2)], axis=1)

        return rows

    scores = {}

    def finish(step, rows, count, strands, delay):
        chain = Chain(strands)
        lane = jax.lax.broadcasted_iota(I32, (8, 128), 1)
        for start_row in range(0, count, 32):
            row, y = rows(start_row)
            for o in range(0, 32, 8):
                base = step * 2 * G + row + o
                xn = x_v[pl.ds(base, 8), :].astype(F32) + mod_v[2] * chain.enter(y[o:o + 8])
                mean = jnp.mean(xn, axis=-1, keepdims=True)
                d = xn - mean
                scale = jax.lax.rsqrt(jnp.mean(d * d, axis=-1, keepdims=True) + EPS)
                score = jnp.sum(d * mod_v[6], axis=-1, keepdims=True) * scale + mod_v[9, :, :1]
                normed = d * scale
                norm_v[pl.ds(base, 8), :] = normed
                out = normed * mod_v[7] + ((d + mean) + mod_v[8])
                out_v[pl.ds(base, 8), :] = out.astype(BF16)
                held = scores.get(base // 1024, jnp.full((8, 128), -jnp.inf, F32))
                scores[base // 1024] = jnp.where(lane == base % 1024 // 8, score, held)
                chain.leave(*[out[:, l:l + 128] for l in range(128, D, 256)])
        if delay:
            finish_within(delay, *chain.tokens)

    def top_two():
        shape = (S // 1024, 8, 128)
        index = (jax.lax.broadcasted_iota(I32, shape, 0) * 1024 + jax.lax.broadcasted_iota(I32, shape, 2) * 8
                 + jax.lax.broadcasted_iota(I32, shape, 1)).astype(F32)
        left = jnp.stack([scores[b] for b in range(S // 1024)])
        reduce = lambda op, v: op(op(op(v, axis=0), axis=0, keepdims=True), axis=1, keepdims=True)
        top = reduce(jnp.max, left)
        first = reduce(jnp.min, jnp.where(left == top, index, float(S)))
        below = reduce(jnp.max, jnp.where(left == top, -jnp.inf, left))
        tied = reduce(jnp.min, jnp.where((left == top) & (index != first), index, float(S)))
        lower = reduce(jnp.min, jnp.where((left == below) & (left != top), index, float(S)))
        second = jnp.where(tied < S, tied, lower)
        row = lambda v: jnp.clip(jnp.max(v.astype(I32)), 0, S - 1)
        return (row(first), top), (row(second), jnp.where(tied < S, top, below))

    def routed_update():
        (row1, score1), (row2, score2) = top_two()
        sub = jax.lax.broadcasted_iota(I32, (16, D), 0)
        first, second = (jnp.broadcast_to(norm_v[pl.ds(row, 1), :], (16, D)) for row in (row1, row2))
        selected = jnp.where(sub == 0, first, second).reshape(2, 8, D) * mod_v[4] + mod_v[3]
        selected = selected.reshape(16, D).astype(BF16)
        pending = collections.deque()
        parts = []

        def down():
            f, g, u = pending.popleft()
            act = (g * jax.nn.sigmoid(g) * u).astype(BF16)
            part = _dot(act, wd_v[pl.ds(f, FF_CHUNK), :])
            parts.append(parts.pop() + part if parts else part)

        for f in range(0, FF, FF_CHUNK):
            pending.append((f, _dot(selected, wg_v[:, pl.ds(f, FF_CHUNK)]),
                            _dot(selected, wu_v[:, pl.ds(f, FF_CHUNK)])))
            if len(pending) > 2:
                down()
        while pending:
            down()
        y1, y2 = parts[0][0:1] * jax.nn.sigmoid(score1), parts[0][1:2] * jax.nn.sigmoid(score2)
        bases = [pl.multiple_of((row >> 4) * 16, 16) for row in (row1, row2)]
        for n, base in enumerate(bases):
            update = jnp.where(sub == row1 - base, y1, 0.0) + jnp.where(sub == row2 - base, y2, 0.0)
            rows = out_v[pl.ds(base, 16), :].astype(F32).reshape(2, 8, D) + mod_v[5] * update.reshape(2, 8, D)
            fix_v[n] = rows.reshape(16, D).astype(BF16)
        return bases

    cc = c_v[...].astype(F32)
    act_v[...] = _pack(jnp.broadcast_to(cc * jax.nn.sigmoid(cc), (16, D)))
    wait(("x", 0))
    for n in range(T // 32):
        row_stats(0, n)
    for offset in range(0, T, 16):
        for lanes in (pl.ds(0, HD), pl.ds(HD, HD)):
            norm_v[pl.ds(offset, 16), lanes] = normalized(0, offset, lanes)
    for half in range(2):
        wait(("scale", half))
        modulation(D, D, half)
    mod_v[1] = raw(1) + 1.0
    first_rows = lambda offset, lanes: norm_v[pl.ds(offset, 16), lanes]
    for n in range(NORM_UNITS):
        norm_terms(first_rows, n, shift=False)(h_v)

    wait(*both("wv", 0))
    prep_values(0)
    plan = new_plan()
    plan[3] += [lambda: wait(*both("wv", 1)), lambda: prep_values(1)]
    plan[7] += [lambda: wait(*both("wv", 2))]
    plan[8] += [lambda: prep_values(2)]
    plan[15] += [lambda: prep_values(3)]
    plan[28] += [lambda: wait("wphi", *both("wk", 0)), feature_maps,
                 lambda: prep_scores(1, 0), lambda: prep_scores(1, 1)]

    def shift_vector():
        wait(*both("shift"))
        for half in range(2):
            modulation(0, D, half)
        mod_v[0] = raw(0)

    def shift_bias():
        shift = jnp.concatenate([raw(0)] * 2, axis=0).astype(BF16)
        bias_v[...] = _dot(shift, wqkv_v[:, pl.ds(2 * D, D)])[:8]

    plan[21].append(shift_vector)
    plan[21].append(shift_bias)
    for n in range(NORM_UNITS):
        plan[22 + 6 * n // NORM_UNITS].append(
            functools.partial(lambda n: norm_terms(first_rows, n, delay=1)(h0_v), n))
    values(h_v, _follow(plan), store_values, 128)
    backlog.drain()

    def ones_rows():
        vt_v[:, pl.ds(64, 16), :] = jnp.ones((NPAIR, 16, T), BF16)

    plan = new_plan()
    plan[0].append(ones_rows)
    plan[3] += [lambda: wait(("x", 1), *both("wk", 1)), lambda: prep_scores(1, 2), lambda: prep_scores(1, 3)]
    plan[1].append(lambda: store_column(bias_v[...]))
    early = 13
    for n in range(early):
        plan[6 + n // 2].append(functools.partial(lambda n: tile_norm(1, n, 3 + n % 2)(h_v), n))
    features(wk_v, h0_v, _follow(plan), store_keys, 256)
    wait("wq")
    for g in range(4):
        prep_scores(0, g)
        backlog.spent(512)
    backlog.drain()
    for n in range(early, NORM_UNITS):
        tile_norm(1, n, 0)(h_v)
    accumulate_summary(first=True)

    for t in range(1, NTILE):
        if t == NTILE - 1:
            wait(*[("mod", i) for i in range(NTILE)])
        plan = new_plan()
        if t + 1 < NTILE:
            wait(("x", t + 1))
        if t == NTILE - 2:
            wait("wo")
        if t + 1 < NTILE:
            stores = []
            for n in range(NORM_UNITS):
                plan[32 + (10 * n) // 16].append(
                    functools.partial(lambda n: stores.append(tile_norm(t + 1, n, 2 + n % 2)), n))
            plan[42].append(lambda: [store(h_v) for store in stores])
        start(("wg", "wu", "wd")[t - 1])
        if t >= NTILE - 2:
            slots = range(4 if t == NTILE - 1 else 1, 32, 2)
            for n in range(16):
                plan[slots[len(slots) * n // 16]].append(functools.partial(prep_output, t % 2 * 16 + n))
        if t == NTILE - 1:
            plan_vector_modulation(plan, (1, 2, 3, 32, 33, 34, 35, 36, 37, 38, 39, 40, 41, 42))
        due.clear()
        hook = _follow(plan)
        features(wk_v, h_v, hook, store_keys, 256)
        features(wq_v, h_v, hook, functools.partial(store_queries, t), 256)
        values(h_v, hook, store_values, 256)
        accumulate_summary(first=False)

    order = [(n + T // (2 * G)) % NSTEP for n in range(NSTEP)]
    wait("wr", "wg", "wu", "wd")
    plan = new_plan()
    plan[0] += [functools.partial(finish_summary, pair) for pair in range(NPAIR)]
    plan[10].append(output_weights)
    due.clear()
    features(wq_v, h0_v, _follow(plan), functools.partial(store_queries, 0), 128)
    attend(order[0], oa_v)

    due.clear()
    rows = None
    for n in range(NSTEP):
        source, target = ((oa_v, ob_v), (ob_v, oa_v))[n % 2]
        if n + 1 < NSTEP:
            attend(order[n + 1], target)
            if rows:
                finish(order[n - 1], rows, 2 * G, 3, 44)
            rows = project_output(source, 0, G, lambda: None)
        else:
            finish(order[n - 1], rows, 2 * G, 6, 26)
            rows = project_output(source, 0, G // 2, lambda: None)
            finish(order[n], rows, G, 8, 24)
            rows = project_output(source, G // 2, G // 2, lambda: None)
        if n > 1:
            out_copy(order[n - 2]).start()
    finish(order[-1], rows, G, G // 8, 0)
    out_copy(order[-2]).start()
    out_copy(order[-1]).start()

    base1, base2 = routed_update()
    for step in order:
        out_copy(step).wait()
    fix = [pltpu.make_async_copy(fix_v.at[n], out_hbm.at[pl.ds(base, 16)], out_sems.at[n])
           for n, base in enumerate((base1, base2))]
    fix[0].start()

    @pl.when(base1 != base2)
    def _():
        fix[1].start()
        fix[1].wait()

    fix[0].wait()


def _scratch():
    vmem = pltpu.VMEM
    return [
        vmem((S, D), BF16), vmem((D, 3 * D), BF16), vmem((D, DH), BF16), vmem((D, D), BF16),
        vmem((8, 128), BF16), vmem((D, FF), BF16), vmem((D, FF), BF16), vmem((FF, D), BF16),
        vmem((1, D), BF16), vmem((D, 6 * D), BF16),
        vmem((8, D), U32), vmem((D, 128), F32), vmem((8, 6 * D), F32), vmem((10, 8, D), F32), vmem((2, T, 128), F32),
        vmem((8, D), F32), vmem((D // 128, 64, 128), U32), vmem((7, HD // 2, HD), U32),
        vmem((7, HT // 2, HD), U32), vmem((7, HT // 2, HD), U32),
        vmem((NTILE, NPAIR, 128, T), BF16), vmem((NPAIR, 128, T), BF16), vmem((NPAIR, 80, T), BF16),
        vmem((NPAIR, 80, 128), F32), vmem((NPAIR, 40, 128), U32),
        vmem((7, G, HD), BF16), vmem((7, G, HD), BF16),
        vmem((S, D), F32), vmem((S, D), BF16), vmem((2, 16, D), BF16),
        pltpu.SemaphoreType.DMA((8 + 2 * NTILE + 14,)), pltpu.SemaphoreType.DMA((NSTEP,)),
    ] + [vmem((7, 64, HD), U32)] * 8 + [vmem((7, HD // 2, 128), U32)] * 4


@jax.jit
def pallas_adaLN_cond__linear_kernel_hedgehog__moe_arch_mod__prompt_kernel(
    A_x: jax.Array,
    A_wqkv: jax.Array,
    A_w_phi: jax.Array,
    A_wo: jax.Array,
    B_x: jax.Array,
    B_w_r: jax.Array,
    B_w_gate: jax.Array,
    B_w_up: jax.Array,
    B_w_down: jax.Array,
    c: jax.Array,
    w_mod: jax.Array,
):
    del B_x
    out = pl.pallas_call(
        _kernel,
        out_shape=jax.ShapeDtypeStruct((S, D), A_x.dtype),
        in_specs=[pl.BlockSpec(memory_space=pl.ANY)] * 10,
        out_specs=pl.BlockSpec(memory_space=pl.ANY),
        scratch_shapes=_scratch(),
        compiler_params=pltpu.CompilerParams(vmem_limit_bytes=120 * 2**20),
    )(A_x.reshape(S, D), A_wqkv, A_w_phi.reshape(D, DH), A_wo, B_w_r.reshape(8, 128),
      B_w_gate, B_w_up, B_w_down, c, w_mod)
    return out.reshape(A_x.shape)
```

```python
import collections
import functools

import jax
import jax.numpy as jnp
import numpy as np
import jax.experimental.pallas as pl
import jax.experimental.pallas.tpu as pltpu

F32, BF16, I32, U32 = jnp.float32, jnp.bfloat16, jnp.int32, jnp.uint32
S, D, HEADS, DH, FF = 2048, 1024, 32, 32, 3584
EPS = 1e-5
LOG2E = float(np.log2(np.e))

HD = D // 2
NPAIR = HEADS // 2
T = 512
HT = T // 2
NTILE = S // T
G = 128
NSTEP = S // (2 * G)
MOD_COLS = 4 * D // NTILE
NORM_UNITS = HT // 16
FF_CHUNK = 256

NN = (((1,), (0,)), ((), ()))
NT = (((1,), (1,)), ((), ()))


def _dot(a, b, dims=NN):
    return jax.lax.dot_general(a, b, dims, preferred_element_type=F32)


def _pack(x):
    n = x.shape[0] // 2
    if x.shape[1] > 128:
        return pltpu.bitcast(x.astype(BF16), U32)
    w = pltpu.bitcast(jnp.concatenate([x[:n], x[n:]], axis=1).astype(BF16), U32)
    return jnp.concatenate([w[:, :128], w[:, 128:]], axis=0)


def _unpack(w):
    return pltpu.bitcast(w, BF16)


def _recip(x):
    r = pl.reciprocal(x, approx=True)
    return r * (2.0 - x * r)


def _lhs_terms(a11, a12, a21, a22):
    return (a11 + a22, a21 + a22, a11, a22, a11 + a12, a21 - a11, a12 - a22)


def _rhs_terms(b11, b12, b21, b22):
    return (b11 + b22, b11, b12 - b22, b21 - b11, b22, b11 + b12, b21 + b22)


_QUADRANTS = (((0, 1), (3, 1), (4, -1), (6, 1)), ((2, 1), (4, 1)), ((1, 1), (3, 1)),
              ((0, 1), (1, -1), (2, 1), (5, 1)))


def _quadrant(q, product):
    total = None
    for j, sign in _QUADRANTS[q]:
        m = product(j)
        total = m if total is None else (total + m if sign > 0 else total - m)
    return total


def _per_head(op, p):
    parts = [p[r:r + 8] for r in range(0, p.shape[0], 8)]
    while len(parts) > 1:
        parts = [op(a, b) for a, b in zip(parts[::2], parts[1::2])]
    out = op(parts[0], pltpu.roll(parts[0], 4, 0))
    return op(out, pltpu.roll(out, 2, 0))


def _apply(op, p, rows8):
    return op(p.reshape(p.shape[0] // 8, 8, p.shape[1]), rows8).reshape(p.shape)


def _features(p):
    e_pos = jnp.exp2(_apply(jnp.subtract, p, _per_head(jnp.maximum, p)))
    e_neg = jnp.exp2(_apply(lambda a, low: low - a, p, _per_head(jnp.minimum, p)))
    pos = _apply(jnp.multiply, e_pos, _recip(_per_head(jnp.add, e_pos)))
    neg = _apply(jnp.multiply, e_neg, _recip(_per_head(jnp.add, e_neg)))
    return jnp.concatenate([pos, neg], axis=0)


def _interleaved_source(row):
    return (row & ~63) + ((row & 1) << 5) + ((row & 63) >> 1)


class _Backlog:
    def __init__(self):
        self.queue = collections.deque()
        self.credit = 0.0

    def defer(self, cost, task):
        self.queue.append((cost, task))

    def spent(self, cycles):
        self.credit += 0.55 * cycles
        while self.queue and self.credit >= self.queue[0][0]:
            cost, task = self.queue.popleft()
            self.credit -= cost
            task()
        if not self.queue:
            self.credit = 0.0

    def drain(self):
        while self.queue:
            self.queue.popleft()[1]()
        self.credit = 0.0


def _follow(plan):
    count = 0

    def step():
        nonlocal count
        count += 1
        for task in plan.pop(count, ()):
            task()

    for task in plan.pop(0, ()):
        task()
    return step


def _kernel(x_hbm, wqkv_hbm, wphi_hbm, wo_hbm, wr_hbm, wg_hbm, wu_hbm, wd_hbm, c_hbm, wmod_hbm,
            out_hbm,
            x_v, wqkv_v, wphi_v, wo_v, wr_v, wg_v, wu_v, wd_v, c_v, wmod_v,
            act_v, column_v, raw_v, mod_v, stat_v, bias_v, fold_v, wot_v, h_v, h0_v,
            phiq_v, phik_v, vt_v, kv_v, summary_v, oa_v, ob_v, norm_v, out_v, fix_v,
            in_sems, out_sems, *terms_v):
    wq_v, wk_v, wv_v = terms_v[:4], terms_v[4:8], terms_v[8:]
    backlog = _Backlog()
    new_plan = lambda: collections.defaultdict(list)

    copies = {}

    def add_copy(name, src, dst, part=Ellipsis):
        if part is not Ellipsis:
            src, dst = src.at[part], dst.at[part]
        copies[name] = pltpu.make_async_copy(src, dst, in_sems.at[len(copies)])

    columns = lambda lo, n: (pl.ds(0, D), pl.ds(lo, n))
    for name, src, dst in (("c", c_hbm, c_v), ("wphi", wphi_hbm, wphi_v), ("wr", wr_hbm, wr_v),
                           ("wo", wo_hbm, wo_v), ("wg", wg_hbm, wg_v), ("wu", wu_hbm, wu_v),
                           ("wd", wd_hbm, wd_v)):
        add_copy(name, src, dst)
    add_copy("wq", wqkv_hbm, wqkv_v, columns(0, D))
    for t in range(NTILE):
        add_copy(("x", t), x_hbm, x_v, pl.ds(t * T, T))
        add_copy(("mod", t), wmod_hbm, wmod_v, columns(2 * D + t * MOD_COLS, MOD_COLS))
    for half in range(2):
        add_copy(("shift", half), wmod_hbm, wmod_v, (pl.ds(half * HD, HD), pl.ds(0, D)))
        for n in range(2):
            add_copy(("scale", n, half), wmod_hbm, wmod_v, columns(D + half * HD + n * 256, 256))
            add_copy(("wk", n, half), wqkv_hbm, wqkv_v, columns(D + half * HD + n * 256, 256))
        for n, (lo, size) in enumerate(((0, 128), (128, 128), (256, 256))):
            add_copy(("wv", n, half), wqkv_hbm, wqkv_v, columns(2 * D + half * HD + lo, size))
    both = lambda *name: ((*name, 0), (*name, 1))

    def start(*names):
        for name in names:
            copies[name].start()

    def wait(*names):
        for name in names:
            copies[name].wait()

    def out_copy(step):
        rows = pl.ds(step * 2 * G, 2 * G)
        return pltpu.make_async_copy(out_v.at[rows], out_hbm.at[rows], out_sems.at[step])

    start("c", ("x", 0), *both("scale", 0), *both("scale", 1), *both("wv", 0), *both("wv", 1),
          *both("wv", 2), *both("shift"), "wphi", *both("wk", 0), *both("wk", 1), ("x", 1), "wq",
          ("x", 2), ("mod", 1), ("x", 3), ("mod", 2), ("mod", 3), ("mod", 0), "wo", "wr")
    wait("c")

    bits = pltpu.bitcast(jnp.broadcast_to(c_v[:, :128].astype(F32), (8, 128)), I32)
    zero = jnp.minimum(jnp.max(bits & 0xFF), 0)

    class Chain:
        def __init__(self, strands):
            self.tokens = collections.deque([None] * strands)

        def enter(self, rows8):
            token = self.tokens.popleft()
            if token is None:
                return rows8
            head = pltpu.bitcast(pltpu.bitcast(rows8[:, :128], I32) | token, F32)
            return jnp.concatenate([head, rows8[:, 128:]], axis=1)

        def leave(self, *values):
            words = [pltpu.bitcast(value, I32) for value in values]
            self.tokens.append(functools.reduce(jnp.bitwise_or, words) & zero)

    clock = 0
    due = collections.defaultdict(list)

    def finish_within(delay, *values):
        parts = [pltpu.bitcast(value, U32)[r:r + 8, l:l + 128] for value in values
                 for r in range(0, value.shape[0], 8) for l in range(0, value.shape[1], 128)]
        due[clock + delay].append(functools.reduce(jnp.bitwise_or, parts) & zero.astype(U32))

    def gated(ref, j, row=0):
        nonlocal clock
        clock += 1
        tokens = [token for when in sorted(due) if when < clock for token in due.pop(when)]
        if tokens:
            corner = (j, pl.ds(row, 8), pl.ds(0, 128))
            ref[corner] = functools.reduce(jnp.bitwise_or, tokens, ref[corner])
        return ref[j]

    def modulation(lo, n, half):
        rows, lanes = pl.ds(half * HD, HD), pl.ds(lo, n)
        m = _dot(_unpack(act_v[:, rows]), wmod_v[rows, lanes])[:8]
        raw_v[:, lanes] = raw_v[:, lanes] + m if half else m

    raw = lambda i: raw_v[:, pl.ds(i * D, D)]

    def store_column(rows):
        column_v[...] = jnp.broadcast_to(rows[:1], (128, D)).T

    def plan_vector_modulation(plan, slots):
        sums = {}

        def unit(i, k):
            total = sums.get(i)
            for r in range(k, k + 64, 8):
                w = wmod_v[pl.ds(r, 8), pl.ds(i * D, D)].astype(F32)
                term = w * jnp.concatenate([column_v[pl.ds(r, 8), :]] * (D // 128), axis=1)
                total = term if total is None else total + term
            sums[i] = total
            finish_within(2, total)
            if k + 64 == D:
                raw_v[:, pl.ds(i * D, D)] = jnp.broadcast_to(jnp.sum(total, axis=0, keepdims=True), (8, D))

        plan[0].append(lambda: store_column(_unpack(act_v[...]).astype(F32)))
        units = [(i, k) for i in range(2, 6) for k in range(0, D, 64)]
        for n, (i, k) in enumerate(units):
            plan[slots[len(slots) * n // len(units)]].append(functools.partial(unit, i, k))

    def output_weights():
        w = wr_v[...].astype(F32)
        w = jnp.concatenate([jnp.broadcast_to(w[j:j + 1], (8, 128)) for j in range(D // 128)], axis=1)
        for i in range(2, 6):
            mod_v[i] = raw(i) + 1.0 if i == 4 else raw(i)
        mod_v[6] = mod_v[4] * w
        mod_v[7] = mod_v[4] * mod_v[5]
        mod_v[8] = mod_v[3] * mod_v[5]
        mod_v[9] = jnp.broadcast_to(jnp.sum(mod_v[3] * w, axis=1, keepdims=True), (8, D))

    def feature_maps():
        row = _interleaved_source(jax.lax.broadcasted_iota(I32, (128, DH), 0))
        col = jax.lax.broadcasted_iota(I32, (128, DH), 1)
        select = jnp.where((row & (DH - 1)) == col, 1.0, 0.0).astype(BF16)
        row_head = _interleaved_source(jax.lax.broadcasted_iota(I32, (128, 128), 0)) >> 5
        col_head = jax.lax.broadcasted_iota(I32, (128, 128), 1) >> 5
        for g in range(D // 128):
            tiled = _dot(select, wphi_v[pl.ds(g * 128, 128), :], NT)
            fold_v[g] = _pack(jnp.where(row_head == col_head, tiled, 0.0))

    def prep_scores(i, g):
        blocks = []
        for group in (g, g + HD // 128):
            for half in range(2):
                w = wqkv_v[pl.ds(half * HD, HD), pl.ds(i * D + group * 128, 128)]
                blocks.append(_dot(_unpack(fold_v[group]), w, NT) * LOG2E)
        for j, term in enumerate(_lhs_terms(*blocks)):
            (wq_v, wk_v)[i][g][j] = _pack(term)

    def prep_values(g):
        chain = Chain(1)
        for r in range(0, HD, 64):
            blocks = [wqkv_v[pl.ds(row + r, 64), pl.ds(2 * D + col + g * 128, 128)].astype(F32)
                      for col in (0, HD) for row in (0, HD)]
            token = chain.tokens.popleft()
            if token is not None:
                head = pltpu.bitcast(pltpu.bitcast(blocks[3][:8], I32) | token, F32)
                blocks[3] = jnp.concatenate([head, blocks[3][8:]], axis=0)
            for j, term in enumerate(_lhs_terms(*blocks)):
                words = _pack(term)
                wv_v[g][j, pl.ds(r // 2, 32), :] = words
            chain.leave(words[:8])

    def prep_output(n):
        lo = wo_v[pl.ds(n * 16, 16), :].astype(F32)
        hi = wo_v[pl.ds(HD + n * 16, 16), :].astype(F32)
        words = [_pack(term) for term in _rhs_terms(lo[:, :HD], lo[:, HD:], hi[:, :HD], hi[:, HD:])]
        for j, w in enumerate(words):
            wot_v[j, pl.ds(n * 8, 8), :] = w
        finish_within(3, *words)

    def row_stats(t, n):
        xx = x_v[pl.ds(t * T + n * 32, 32), :].astype(F32)
        mean = jnp.mean(xx, axis=-1, keepdims=True)
        d = xx - mean
        scale = jax.lax.rsqrt(jnp.mean(d * d, axis=-1, keepdims=True) + EPS)
        stat_v[0, pl.ds(n * 32, 32), :] = jnp.broadcast_to(mean, (32, 128))
        stat_v[1, pl.ds(n * 32, 32), :] = jnp.broadcast_to(scale, (32, 128))

    def normalized(t, offset, lanes):
        wide = lambda k: jnp.concatenate([stat_v[k, pl.ds(offset, 16), :]] * (HD // 128), axis=1)
        return (x_v[pl.ds(t * T + offset, 16), lanes].astype(F32) - wide(0)) * wide(1)

    def norm_terms(rows, n, shift=True, delay=0, lo=0, width=HD):
        blocks = []
        for lanes in (pl.ds(lo, width), pl.ds(HD + lo, width)):
            for offset in (n * 16, HT + n * 16):
                hh = rows(offset, lanes).reshape(2, 8, width) * mod_v[1, :, lanes]
                blocks.append((hh + mod_v[0, :, lanes] if shift else hh).reshape(16, width))
        words = [_pack(term) for term in _rhs_terms(*blocks)]
        if delay:
            finish_within(delay, *words)

        def store(target):
            for j, w in enumerate(words):
                target[j, pl.ds(n * 8, 8), pl.ds(lo, width)] = w

        return store

    def tile_norm(t, n, delay):
        if n % 2 == 0:
            row_stats(t, n // 2)
            row_stats(t, HT // 32 + n // 2)
        return norm_terms(functools.partial(normalized, t), n, delay=delay)

    def products(product, tiles, cycles, hook):
        result = []
        for j in range(7):
            result.append([product(j, k) for k in range(tiles)])
            backlog.spent(cycles)
            hook()
        return result

    def features(weights, source, hook, target, rows):
        for r in range(0, HD, rows):
            m = products(
                lambda j, k: _dot(
                    _unpack(jnp.concatenate([weights[g][j] for g in range(r // 128, (r + rows) // 128)], axis=0)),
                    _unpack(gated(source, j, k * 64)[k * 64:(k + 1) * 64]), NT),
                HT // 128, rows * HT // 128, hook)

            def unit(half, o, m=m, r=r):
                for part in range(2):
                    phi = jnp.concatenate(
                        [_features(_quadrant(2 * half + part, lambda j: m[j][k][o:o + 64]))
                         for k in range(HT // 128)], axis=1)
                    target((half * HD + r + o) // 64, pl.ds(part * HT, HT), phi.astype(BF16))

            for half in range(2):
                for o in range(0, rows, 64):
                    backlog.defer(150 * rows // 256, functools.partial(unit, half, o))

    def store_keys(pair, lanes, phi):
        phik_v[pair, :, lanes] = phi

    def store_queries(t, pair, lanes, phi):
        phiq_v[t, pair, :, lanes] = phi

    def store_values(col, part, v):
        v = v.T.astype(BF16).reshape(2, 64, HT)
        vt_v[pl.ds(col // 64, 2), pl.ds(0, 64), pl.ds(part * HT, HT)] = v

    def values(source, hook, target, cols):
        for r in range(0, HD, cols):
            m = products(
                lambda j, k: _dot(_unpack(source[j]), _unpack(gated(wv_v[r // 128 + k], j))),
                cols // 128, cols * HT // 128, hook)

            def unit(half, part, k, m=m, r=r):
                target(half * HD + r + k * 128, part, _quadrant(2 * half + part, lambda j: m[j][k]))

            for half in range(2):
                for part in range(2):
                    for k in range(cols // 128):
                        backlog.defer(128, functools.partial(unit, half, part, k))

    def accumulate_summary(first):
        backlog.drain()
        for r in range(0, HD, 256):
            for half in range(2):
                for o in range(0, 256, 64):
                    pair = (half * HD + r + o) // 64
                    kv = _dot(vt_v[pair], phik_v[pair], NT)
                    if first:
                        bias = _apply(jnp.multiply, column_v[pl.ds(pair * 64, 64), :], kv[64:72])
                        kv_v[pair] = jnp.concatenate([kv[:64] + bias, kv[64:]], axis=0)
                    else:
                        kv_v[pair] = kv_v[pair] + kv

    def finish_summary(pair):
        row = jax.lax.broadcasted_iota(I32, (80, 128), 0)
        row_head = jnp.where(row < 64, row >> 5, (row >> 3) & 1)
        col_head = jax.lax.broadcasted_iota(I32, (80, 128), 1) & 1
        summary_v[pair] = _pack(jnp.where(row_head == col_head, kv_v[pair], 0.0))

    def attend(step, target):
        t, lanes = step // 2, pl.ds(step % 2 * 2 * G, 2 * G)
        pairs = [[[half * NPAIR // 2 + 2 * i + k for k in range(2)] for half in range(2)] for i in range(4)]
        nums = {p: _dot(_unpack(summary_v[p]), phiq_v[t, p, :, lanes])
                for group in pairs for side in group for p in side}
        sides = []
        for i, group in enumerate(pairs):
            heads = [[_apply(jnp.multiply, nums[p][h * DH:(h + 1) * DH],
                             _recip(nums[p][64 + 8 * h:72 + 8 * h] + 1e-6))
                      for p in side for h in range(2)] for side in group]
            sides.append([jnp.concatenate(side, axis=0).T for side in heads])
            if i % 2:
                lo, hi = (jnp.concatenate([sides[i - 1][s], sides[i][s]], axis=1) for s in range(2))
                for j, term in enumerate(_lhs_terms(lo[:G], hi[:G], lo[G:], hi[G:])):
                    target[j, :, pl.ds((i - 1) * 128, 256)] = term.astype(BF16)

    def project_output(source, lo, n, hook):
        m = products(
            lambda j, k: _dot(source[j, pl.ds(lo, n), :],
                              _unpack(gated(wot_v, j)[:, k * 128:(k + 1) * 128])),
            HD // 128, 4 * n, hook)

        def rows(o):
            part, o = divmod(o, n)
            piece = lambda j: jnp.concatenate([tile[o:o + 32] for tile in m[j]], axis=1)
            return lo + part * G + o, jnp.concatenate(
                [_quadrant(2 * part + half, piece) for half in range(2)], axis=1)

        return rows

    scores = {}

    def finish(step, rows, count, strands, delay):
        chain = Chain(strands)
        lane = jax.lax.broadcasted_iota(I32, (8, 128), 1)
        for start_row in range(0, count, 32):
            row, y = rows(start_row)
            for o in range(0, 32, 8):
                base = step * 2 * G + row + o
                xn = x_v[pl.ds(base, 8), :].astype(F32) + mod_v[2] * chain.enter(y[o:o + 8])
                mean = jnp.mean(xn, axis=-1, keepdims=True)
                d = xn - mean
                scale = jax.lax.rsqrt(jnp.mean(d * d, axis=-1, keepdims=True) + EPS)
                score = jnp.sum(d * mod_v[6], axis=-1, keepdims=True) * scale + mod_v[9, :, :1]
                normed = d * scale
                norm_v[pl.ds(base, 8), :] = normed
                out = normed * mod_v[7] + ((d + mean) + mod_v[8])
                out_v[pl.ds(base, 8), :] = out.astype(BF16)
                held = scores.get(base // 1024, jnp.full((8, 128), -jnp.inf, F32))
                scores[base // 1024] = jnp.where(lane == base % 1024 // 8, score, held)
                chain.leave(*[out[:, l:l + 128] for l in range(128, D, 256)])
        if delay:
            finish_within(delay, *chain.tokens)

    def top_two():
        shape = (S // 1024, 8, 128)
        index = (jax.lax.broadcasted_iota(I32, shape, 0) * 1024 + jax.lax.broadcasted_iota(I32, shape, 2) * 8
                 + jax.lax.broadcasted_iota(I32, shape, 1)).astype(F32)
        left = jnp.stack([scores[b] for b in range(S // 1024)])
        reduce = lambda op, v: op(op(op(v, axis=0), axis=0, keepdims=True), axis=1, keepdims=True)
        top = reduce(jnp.max, left)
        first = reduce(jnp.min, jnp.where(left == top, index, float(S)))
        below = reduce(jnp.max, jnp.where(left == top, -jnp.inf, left))
        tied = reduce(jnp.min, jnp.where((left == top) & (index != first), index, float(S)))
        lower = reduce(jnp.min, jnp.where((left == below) & (left != top), index, float(S)))
        second = jnp.where(tied < S, tied, lower)
        row = lambda v: jnp.clip(jnp.max(v.astype(I32)), 0, S - 1)
        return (row(first), top), (row(second), jnp.where(tied < S, top, below))

    def routed_update():
        (row1, score1), (row2, score2) = top_two()
        sub = jax.lax.broadcasted_iota(I32, (16, D), 0)
        first, second = (jnp.broadcast_to(norm_v[pl.ds(row, 1), :], (16, D)) for row in (row1, row2))
        selected = jnp.where(sub == 0, first, second).reshape(2, 8, D) * mod_v[4] + mod_v[3]
        selected = selected.reshape(16, D).astype(BF16)
        pending = collections.deque()
        parts = []

        def down():
            f, g, u = pending.popleft()
            act = (g * jax.nn.sigmoid(g) * u).astype(BF16)
            part = _dot(act, wd_v[pl.ds(f, FF_CHUNK), :])
            parts.append(parts.pop() + part if parts else part)

        for f in range(0, FF, FF_CHUNK):
            pending.append((f, _dot(selected, wg_v[:, pl.ds(f, FF_CHUNK)]),
                            _dot(selected, wu_v[:, pl.ds(f, FF_CHUNK)])))
            if len(pending) > 2:
                down()
        while pending:
            down()
        y1, y2 = parts[0][0:1] * jax.nn.sigmoid(score1), parts[0][1:2] * jax.nn.sigmoid(score2)
        bases = [pl.multiple_of((row >> 4) * 16, 16) for row in (row1, row2)]
        for n, base in enumerate(bases):
            update = jnp.where(sub == row1 - base, y1, 0.0) + jnp.where(sub == row2 - base, y2, 0.0)
            rows = out_v[pl.ds(base, 16), :].astype(F32).reshape(2, 8, D) + mod_v[5] * update.reshape(2, 8, D)
            fix_v[n] = rows.reshape(16, D).astype(BF16)
        return bases

    cc = c_v[...].astype(F32)
    act_v[...] = _pack(jnp.broadcast_to(cc * jax.nn.sigmoid(cc), (16, D)))
    wait(("x", 0))
    for n in range(T // 32):
        row_stats(0, n)
    for offset in range(0, T, 16):
        for lanes in (pl.ds(0, HD), pl.ds(HD, HD)):
            norm_v[pl.ds(offset, 16), lanes] = normalized(0, offset, lanes)
    first_rows = lambda offset, lanes: norm_v[pl.ds(offset, 16), lanes]
    for piece, lo in enumerate(range(0, HD, 256)):
        wait(*both("scale", piece))
        for column in (lo, HD + lo):
            for half in range(2):
                modulation(D + column, 256, half)
            mod_v[1, :, pl.ds(column, 256)] = raw_v[:, pl.ds(D + column, 256)] + 1.0
        for n in range(NORM_UNITS):
            norm_terms(first_rows, n, shift=False, lo=lo, width=256)(h_v)

    wait(*both("wv", 0))
    prep_values(0)
    plan = new_plan()
    plan[3] += [lambda: wait(*both("wv", 1)), lambda: prep_values(1)]
    plan[12] += [lambda: wait(*both("wv", 2))]
    plan[13] += [lambda: prep_values(2)]
    plan[15] += [lambda: prep_values(3)]
    plan[28] += [lambda: wait("wphi", *both("wk", 0)), feature_maps,
                 lambda: prep_scores(1, 0), lambda: prep_scores(1, 1)]

    def shift_vector():
        wait(*both("shift"))
        for half in range(2):
            modulation(0, D, half)
        mod_v[0] = raw(0)

    def shift_bias():
        shift = jnp.concatenate([raw(0)] * 2, axis=0).astype(BF16)
        bias_v[...] = _dot(shift, wqkv_v[:, pl.ds(2 * D, D)])[:8]

    plan[24] += [shift_vector, shift_bias]
    for n in range(NORM_UNITS):
        plan[25 + 4 * n // NORM_UNITS].append(
            functools.partial(lambda n: norm_terms(first_rows, n, delay=1)(h0_v), n))
    values(h_v, _follow(plan), store_values, 128)
    backlog.drain()

    def ones_rows():
        vt_v[:, pl.ds(64, 16), :] = jnp.ones((NPAIR, 16, T), BF16)

    plan = new_plan()
    plan[0].append(ones_rows)
    plan[4] += [lambda: wait(("x", 1), *both("wk", 1)), lambda: prep_scores(1, 2), lambda: prep_scores(1, 3)]
    plan[1].append(lambda: store_column(bias_v[...]))
    early = 13
    for n in range(early):
        plan[6 + n // 2].append(functools.partial(lambda n: tile_norm(1, n, 3 + n % 2)(h_v), n))
    features(wk_v, h0_v, _follow(plan), store_keys, 256)
    wait("wq")
    for g in range(4):
        prep_scores(0, g)
        backlog.spent(512)
    backlog.drain()
    for n in range(early, NORM_UNITS):
        tile_norm(1, n, 0)(h_v)
    accumulate_summary(first=True)

    for t in range(1, NTILE):
        if t == NTILE - 1:
            wait(*[("mod", i) for i in range(NTILE)])
        plan = new_plan()
        if t + 1 < NTILE:
            wait(("x", t + 1))
        if t == NTILE - 2:
            wait("wo")
        if t + 1 < NTILE:
            stores = []
            for n in range(NORM_UNITS):
                plan[32 + (10 * n) // 16].append(
                    functools.partial(lambda n: stores.append(tile_norm(t + 1, n, 2 + n % 2)), n))
            plan[42].append(lambda: [store(h_v) for store in stores])
        start(("wg", "wu", "wd")[t - 1])
        if t >= NTILE - 2:
            slots = range(4 if t == NTILE - 1 else 1, 32, 2)
            for n in range(16):
                plan[slots[len(slots) * n // 16]].append(functools.partial(prep_output, t % 2 * 16 + n))
        if t == NTILE - 1:
            plan_vector_modulation(plan, (1, 2, 3, 32, 33, 34, 35, 36, 37, 38, 39, 40, 41, 42))
        due.clear()
        hook = _follow(plan)
        features(wk_v, h_v, hook, store_keys, 256)
        features(wq_v, h_v, hook, functools.partial(store_queries, t), 256)
        values(h_v, hook, store_values, 256)
        accumulate_summary(first=False)

    order = [(n + T // (2 * G)) % NSTEP for n in range(NSTEP)]
    wait("wr", "wg", "wu", "wd")
    plan = new_plan()
    plan[0] += [functools.partial(finish_summary, pair) for pair in range(NPAIR)]
    plan[10].append(output_weights)
    due.clear()
    features(wq_v, h0_v, _follow(plan), functools.partial(store_queries, 0), 128)
    attend(order[0], oa_v)

    due.clear()
    rows = None
    for n in range(NSTEP):
        source, target = ((oa_v, ob_v), (ob_v, oa_v))[n % 2]
        if n + 1 < NSTEP:
            attend(order[n + 1], target)
            if rows:
                finish(order[n - 1], rows, 2 * G, 3, 44)
            rows = project_output(source, 0, G, lambda: None)
        else:
            finish(order[n - 1], rows, 2 * G, 6, 26)
            rows = project_output(source, 0, G // 2, lambda: None)
            finish(order[n], rows, G, 8, 24)
            rows = project_output(source, G // 2, G // 2, lambda: None)
        if n > 1:
            out_copy(order[n - 2]).start()
    finish(order[-1], rows, G, G // 8, 0)
    out_copy(order[-2]).start()
    out_copy(order[-1]).start()

    base1, base2 = routed_update()
    for step in order:
        out_copy(step).wait()
    fix = [pltpu.make_async_copy(fix_v.at[n], out_hbm.at[pl.ds(base, 16)], out_sems.at[n])
           for n, base in enumerate((base1, base2))]
    fix[0].start()

    @pl.when(base1 != base2)
    def _():
        fix[1].start()
        fix[1].wait()

    fix[0].wait()


def _scratch():
    vmem = pltpu.VMEM
    return [
        vmem((S, D), BF16), vmem((D, 3 * D), BF16), vmem((D, DH), BF16), vmem((D, D), BF16),
        vmem((8, 128), BF16), vmem((D, FF), BF16), vmem((D, FF), BF16), vmem((FF, D), BF16),
        vmem((1, D), BF16), vmem((D, 6 * D), BF16),
        vmem((8, D), U32), vmem((D, 128), F32), vmem((8, 6 * D), F32), vmem((10, 8, D), F32), vmem((2, T, 128), F32),
        vmem((8, D), F32), vmem((D // 128, 64, 128), U32), vmem((7, HD // 2, HD), U32),
        vmem((7, HT // 2, HD), U32), vmem((7, HT // 2, HD), U32),
        vmem((NTILE, NPAIR, 128, T), BF16), vmem((NPAIR, 128, T), BF16), vmem((NPAIR, 80, T), BF16),
        vmem((NPAIR, 80, 128), F32), vmem((NPAIR, 40, 128), U32),
        vmem((7, G, HD), BF16), vmem((7, G, HD), BF16),
        vmem((S, D), F32), vmem((S, D), BF16), vmem((2, 16, D), BF16),
        pltpu.SemaphoreType.DMA((8 + 2 * NTILE + 16,)), pltpu.SemaphoreType.DMA((NSTEP,)),
    ] + [vmem((7, 64, HD), U32)] * 8 + [vmem((7, HD // 2, 128), U32)] * 4


@jax.jit
def pallas_adaLN_cond__linear_kernel_hedgehog__moe_arch_mod__prompt_kernel(
    A_x: jax.Array,
    A_wqkv: jax.Array,
    A_w_phi: jax.Array,
    A_wo: jax.Array,
    B_x: jax.Array,
    B_w_r: jax.Array,
    B_w_gate: jax.Array,
    B_w_up: jax.Array,
    B_w_down: jax.Array,
    c: jax.Array,
    w_mod: jax.Array,
):
    del B_x
    out = pl.pallas_call(
        _kernel,
        out_shape=jax.ShapeDtypeStruct((S, D), A_x.dtype),
        in_specs=[pl.BlockSpec(memory_space=pl.ANY)] * 10,
        out_specs=pl.BlockSpec(memory_space=pl.ANY),
        scratch_shapes=_scratch(),
        compiler_params=pltpu.CompilerParams(vmem_limit_bytes=120 * 2**20),
    )(A_x.reshape(S, D), A_wqkv, A_w_phi.reshape(D, DH), A_wo, B_w_r.reshape(8, 128),
      B_w_gate, B_w_up, B_w_down, c, w_mod)
    return out.reshape(A_x.shape)
```

```python
import collections
import functools

import jax
import jax.numpy as jnp
import numpy as np
import jax.experimental.pallas as pl
import jax.experimental.pallas.tpu as pltpu

F32, BF16, I32, U32 = jnp.float32, jnp.bfloat16, jnp.int32, jnp.uint32
S, D, HEADS, DH, FF = 2048, 1024, 32, 32, 3584
EPS = 1e-5
LOG2E = float(np.log2(np.e))

HD = D // 2
NPAIR = HEADS // 2
T = 512
HT = T // 2
NTILE = S // T
G = 128
NSTEP = S // (2 * G)
MOD_COLS = 4 * D // NTILE
NORM_UNITS = HT // 16
FF_CHUNK = 256

NN = (((1,), (0,)), ((), ()))
NT = (((1,), (1,)), ((), ()))


def _dot(a, b, dims=NN):
    return jax.lax.dot_general(a, b, dims, preferred_element_type=F32)


def _pack(x):
    n = x.shape[0] // 2
    if x.shape[1] > 128:
        return pltpu.bitcast(x.astype(BF16), U32)
    w = pltpu.bitcast(jnp.concatenate([x[:n], x[n:]], axis=1).astype(BF16), U32)
    return jnp.concatenate([w[:, :128], w[:, 128:]], axis=0)


def _unpack(w):
    return pltpu.bitcast(w, BF16)


def _recip(x):
    r = pl.reciprocal(x, approx=True)
    return r * (2.0 - x * r)


def _lhs_terms(a11, a12, a21, a22):
    return (a11 + a22, a21 + a22, a11, a22, a11 + a12, a21 - a11, a12 - a22)


def _rhs_terms(b11, b12, b21, b22):
    return (b11 + b22, b11, b12 - b22, b21 - b11, b22, b11 + b12, b21 + b22)


_QUADRANTS = (((0, 1), (3, 1), (4, -1), (6, 1)), ((2, 1), (4, 1)), ((1, 1), (3, 1)),
              ((0, 1), (1, -1), (2, 1), (5, 1)))


def _quadrant(q, product):
    total = None
    for j, sign in _QUADRANTS[q]:
        m = product(j)
        total = m if total is None else (total + m if sign > 0 else total - m)
    return total


def _per_head(op, p):
    parts = [p[r:r + 8] for r in range(0, p.shape[0], 8)]
    while len(parts) > 1:
        parts = [op(a, b) for a, b in zip(parts[::2], parts[1::2])]
    out = op(parts[0], pltpu.roll(parts[0], 4, 0))
    return op(out, pltpu.roll(out, 2, 0))


def _apply(op, p, rows8):
    return op(p.reshape(p.shape[0] // 8, 8, p.shape[1]), rows8).reshape(p.shape)


def _features(p):
    e_pos = jnp.exp2(_apply(jnp.subtract, p, _per_head(jnp.maximum, p)))
    e_neg = jnp.exp2(_apply(lambda a, low: low - a, p, _per_head(jnp.minimum, p)))
    pos = _apply(jnp.multiply, e_pos, _recip(_per_head(jnp.add, e_pos)))
    neg = _apply(jnp.multiply, e_neg, _recip(_per_head(jnp.add, e_neg)))
    return jnp.concatenate([pos, neg], axis=0)


def _interleaved_source(row):
    return (row & ~63) + ((row & 1) << 5) + ((row & 63) >> 1)


class _Backlog:
    def __init__(self):
        self.queue = collections.deque()
        self.credit = 0.0

    def defer(self, cost, task):
        self.queue.append((cost, task))

    def spent(self, cycles):
        self.credit += 0.55 * cycles
        while self.queue and self.credit >= self.queue[0][0]:
            cost, task = self.queue.popleft()
            self.credit -= cost
            task()
        if not self.queue:
            self.credit = 0.0

    def drain(self):
        while self.queue:
            self.queue.popleft()[1]()
        self.credit = 0.0


def _follow(plan):
    count = 0

    def step():
        nonlocal count
        count += 1
        for task in plan.pop(count, ()):
            task()

    for task in plan.pop(0, ()):
        task()
    return step


def _kernel(x_hbm, wqkv_hbm, wphi_hbm, wo_hbm, wr_hbm, wg_hbm, wu_hbm, wd_hbm, c_hbm, wmod_hbm,
            out_hbm,
            x_v, wqkv_v, wphi_v, wo_v, wr_v, wg_v, wu_v, wd_v, c_v, wmod_v,
            act_v, column_v, raw_v, mod_v, stat_v, bias_v, fold_v, wot_v, h_v, h0_v,
            phiq_v, phik_v, vt_v, kv_v, summary_v, oa_v, ob_v, norm_v, out_v, fix_v,
            in_sems, out_sems, *terms_v):
    wq_v, wk_v, wv_v = terms_v[:4], terms_v[4:8], terms_v[8:]
    backlog = _Backlog()
    new_plan = lambda: collections.defaultdict(list)

    copies = {}

    def add_copy(name, src, dst, part=Ellipsis):
        if part is not Ellipsis:
            src, dst = src.at[part], dst.at[part]
        copies[name] = pltpu.make_async_copy(src, dst, in_sems.at[len(copies)])

    columns = lambda lo, n: (pl.ds(0, D), pl.ds(lo, n))
    for name, src, dst in (("c", c_hbm, c_v), ("wphi", wphi_hbm, wphi_v), ("wr", wr_hbm, wr_v),
                           ("wo", wo_hbm, wo_v), ("wg", wg_hbm, wg_v), ("wu", wu_hbm, wu_v),
                           ("wd", wd_hbm, wd_v)):
        add_copy(name, src, dst)
    add_copy("wq", wqkv_hbm, wqkv_v, columns(0, D))
    for t in range(NTILE):
        add_copy(("x", t), x_hbm, x_v, pl.ds(t * T, T))
        add_copy(("mod", t), wmod_hbm, wmod_v, columns(2 * D + t * MOD_COLS, MOD_COLS))
    for half in range(2):
        add_copy(("shift", half), wmod_hbm, wmod_v, (pl.ds(half * HD, HD), pl.ds(0, D)))
        for n in range(2):
            add_copy(("scale", n, half), wmod_hbm, wmod_v, columns(D + half * HD + n * 256, 256))
            add_copy(("wk", n, half), wqkv_hbm, wqkv_v, columns(D + half * HD + n * 256, 256))
        for n, (lo, size) in enumerate(((0, 128), (128, 128), (256, 256))):
            add_copy(("wv", n, half), wqkv_hbm, wqkv_v, columns(2 * D + half * HD + lo, size))
    both = lambda *name: ((*name, 0), (*name, 1))

    def start(*names):
        for name in names:
            copies[name].start()

    def wait(*names):
        for name in names:
            copies[name].wait()

    def out_copy(step):
        rows = pl.ds(step * 2 * G, 2 * G)
        return pltpu.make_async_copy(out_v.at[rows], out_hbm.at[rows], out_sems.at[step])

    start("c", ("x", 0), *both("scale", 0), *both("scale", 1), *both("wv", 0), *both("wv", 1),
          *both("wv", 2), *both("shift"), "wphi", *both("wk", 0), *both("wk", 1), ("x", 1), "wq",
          ("x", 2), ("mod", 1), ("x", 3), ("mod", 2), ("mod", 3), ("mod", 0), "wo", "wr")
    wait("c")

    bits = pltpu.bitcast(jnp.broadcast_to(c_v[:, :128].astype(F32), (8, 128)), I32)
    zero = jnp.minimum(jnp.max(bits & 0xFF), 0)

    class Chain:
        def __init__(self, strands):
            self.tokens = collections.deque([None] * strands)

        def enter(self, rows8):
            token = self.tokens.popleft()
            if token is None:
                return rows8
            head = pltpu.bitcast(pltpu.bitcast(rows8[:, :128], I32) | token, F32)
            return jnp.concatenate([head, rows8[:, 128:]], axis=1)

        def leave(self, *values):
            words = [pltpu.bitcast(value, I32) for value in values]
            self.tokens.append(functools.reduce(jnp.bitwise_or, words) & zero)

    clock = 0
    due = collections.defaultdict(list)

    def finish_within(delay, *values):
        parts = [pltpu.bitcast(value, U32)[r:r + 8, l:l + 128] for value in values
                 for r in range(0, value.shape[0], 8) for l in range(0, value.shape[1], 128)]
        due[clock + delay].append(functools.reduce(jnp.bitwise_or, parts) & zero.astype(U32))

    def gated(ref, j, row=0):
        nonlocal clock
        clock += 1
        tokens = [token for when in sorted(due) if when < clock for token in due.pop(when)]
        if tokens:
            corner = (j, pl.ds(row, 8), pl.ds(0, 128))
            ref[corner] = functools.reduce(jnp.bitwise_or, tokens, ref[corner])
        return ref[j]

    def modulation(lo, n, half):
        rows, lanes = pl.ds(half * HD, HD), pl.ds(lo, n)
        m = _dot(_unpack(act_v[:, rows]), wmod_v[rows, lanes])[:8]
        raw_v[:, lanes] = raw_v[:, lanes] + m if half else m

    raw = lambda i: raw_v[:, pl.ds(i * D, D)]

    def store_column(rows):
        column_v[...] = jnp.broadcast_to(rows[:1], (128, D)).T

    def plan_vector_modulation(plan, slots):
        sums = {}

        def unit(i, k):
            total = sums.get(i)
            for r in range(k, k + 64, 8):
                w = wmod_v[pl.ds(r, 8), pl.ds(i * D, D)].astype(F32)
                term = w * jnp.concatenate([column_v[pl.ds(r, 8), :]] * (D // 128), axis=1)
                total = term if total is None else total + term
            sums[i] = total
            finish_within(2, total)
            if k + 64 == D:
                raw_v[:, pl.ds(i * D, D)] = jnp.broadcast_to(jnp.sum(total, axis=0, keepdims=True), (8, D))

        plan[0].append(lambda: store_column(_unpack(act_v[...]).astype(F32)))
        units = [(i, k) for i in range(2, 6) for k in range(0, D, 64)]
        for n, (i, k) in enumerate(units):
            plan[slots[len(slots) * n // len(units)]].append(functools.partial(unit, i, k))

    def output_weights():
        w = wr_v[...].astype(F32)
        w = jnp.concatenate([jnp.broadcast_to(w[j:j + 1], (8, 128)) for j in range(D // 128)], axis=1)
        for i in range(2, 6):
            mod_v[i] = raw(i) + 1.0 if i == 4 else raw(i)
        mod_v[6] = mod_v[4] * w
        mod_v[7] = mod_v[4] * mod_v[5]
        mod_v[8] = mod_v[3] * mod_v[5]
        mod_v[9] = jnp.broadcast_to(jnp.sum(mod_v[3] * w, axis=1, keepdims=True), (8, D))

    def feature_maps():
        row = _interleaved_source(jax.lax.broadcasted_iota(I32, (128, DH), 0))
        col = jax.lax.broadcasted_iota(I32, (128, DH), 1)
        select = jnp.where((row & (DH - 1)) == col, 1.0, 0.0).astype(BF16)
        row_head = _interleaved_source(jax.lax.broadcasted_iota(I32, (128, 128), 0)) >> 5
        col_head = jax.lax.broadcasted_iota(I32, (128, 128), 1) >> 5
        for g in range(D // 128):
            tiled = _dot(select, wphi_v[pl.ds(g * 128, 128), :], NT)
            fold_v[g] = _pack(jnp.where(row_head == col_head, tiled, 0.0))

    def prep_scores(i, g):
        blocks = []
        for group in (g, g + HD // 128):
            for half in range(2):
                w = wqkv_v[pl.ds(half * HD, HD), pl.ds(i * D + group * 128, 128)]
                blocks.append(_dot(_unpack(fold_v[group]), w, NT) * LOG2E)
        for j, term in enumerate(_lhs_terms(*blocks)):
            (wq_v, wk_v)[i][g][j] = _pack(term)

    def prep_values(g):
        chain = Chain(1)
        for r in range(0, HD, 64):
            blocks = [wqkv_v[pl.ds(row + r, 64), pl.ds(2 * D + col + g * 128, 128)].astype(F32)
                      for col in (0, HD) for row in (0, HD)]
            token = chain.tokens.popleft()
            if token is not None:
                head = pltpu.bitcast(pltpu.bitcast(blocks[3][:8], I32) | token, F32)
                blocks[3] = jnp.concatenate([head, blocks[3][8:]], axis=0)
            for j, term in enumerate(_lhs_terms(*blocks)):
                words = _pack(term)
                wv_v[g][j, pl.ds(r // 2, 32), :] = words
            chain.leave(words[:8])

    def prep_output(n):
        lo = wo_v[pl.ds(n * 16, 16), :].astype(F32)
        hi = wo_v[pl.ds(HD + n * 16, 16), :].astype(F32)
        words = [_pack(term) for term in _rhs_terms(lo[:, :HD], lo[:, HD:], hi[:, :HD], hi[:, HD:])]
        for j, w in enumerate(words):
            wot_v[j, pl.ds(n * 8, 8), :] = w
        finish_within(3, *words)

    def row_stats(t, n):
        xx = x_v[pl.ds(t * T + n * 32, 32), :].astype(F32)
        mean = jnp.mean(xx, axis=-1, keepdims=True)
        d = xx - mean
        scale = jax.lax.rsqrt(jnp.mean(d * d, axis=-1, keepdims=True) + EPS)
        stat_v[0, pl.ds(n * 32, 32), :] = jnp.broadcast_to(mean, (32, 128))
        stat_v[1, pl.ds(n * 32, 32), :] = jnp.broadcast_to(scale, (32, 128))

    def normalized(t, offset, lanes):
        wide = lambda k: jnp.concatenate([stat_v[k, pl.ds(offset, 16), :]] * (HD // 128), axis=1)
        return (x_v[pl.ds(t * T + offset, 16), lanes].astype(F32) - wide(0)) * wide(1)

    def norm_terms(rows, n, shift=True, delay=0, lo=0, width=HD):
        blocks = []
        for lanes in (pl.ds(lo, width), pl.ds(HD + lo, width)):
            for offset in (n * 16, HT + n * 16):
                hh = rows(offset, lanes).reshape(2, 8, width) * mod_v[1, :, lanes]
                blocks.append((hh + mod_v[0, :, lanes] if shift else hh).reshape(16, width))
        words = [_pack(term) for term in _rhs_terms(*blocks)]
        if delay:
            finish_within(delay, *words)

        def store(target):
            for j, w in enumerate(words):
                target[j, pl.ds(n * 8, 8), pl.ds(lo, width)] = w

        return store

    def tile_norm(t, n, delay):
        if n % 2 == 0:
            row_stats(t, n // 2)
            row_stats(t, HT // 32 + n // 2)
        return norm_terms(functools.partial(normalized, t), n, delay=delay)

    def products(product, tiles, cycles, hook):
        result = []
        for j in range(7):
            result.append([product(j, k) for k in range(tiles)])
            backlog.spent(cycles)
            hook()
        return result

    def features(weights, source, hook, target, rows):
        for r in range(0, HD, rows):
            m = products(
                lambda j, k: _dot(
                    _unpack(jnp.concatenate([weights[g][j] for g in range(r // 128, (r + rows) // 128)], axis=0)),
                    _unpack(gated(source, j, k * 64)[k * 64:(k + 1) * 64]), NT),
                HT // 128, rows * HT // 128, hook)

            def unit(half, o, m=m, r=r):
                for part in range(2):
                    phi = jnp.concatenate(
                        [_features(_quadrant(2 * half + part, lambda j: m[j][k][o:o + 64]))
                         for k in range(HT // 128)], axis=1)
                    target((half * HD + r + o) // 64, pl.ds(part * HT, HT), phi.astype(BF16))

            for half in range(2):
                for o in range(0, rows, 64):
                    backlog.defer(150 * rows // 256, functools.partial(unit, half, o))

    def store_keys(pair, lanes, phi):
        phik_v[pair, :, lanes] = phi

    def store_queries(t, pair, lanes, phi):
        phiq_v[t, pair, :, lanes] = phi

    def store_values(col, part, v):
        v = v.T.astype(BF16).reshape(2, 64, HT)
        vt_v[pl.ds(col // 64, 2), pl.ds(0, 64), pl.ds(part * HT, HT)] = v

    def values(source, hook, target, cols):
        for r in range(0, HD, cols):
            m = products(
                lambda j, k: _dot(_unpack(source[j]), _unpack(gated(wv_v[r // 128 + k], j))),
                cols // 128, cols * HT // 128, hook)

            def unit(half, part, k, m=m, r=r):
                target(half * HD + r + k * 128, part, _quadrant(2 * half + part, lambda j: m[j][k]))

            for half in range(2):
                for part in range(2):
                    for k in range(cols // 128):
                        backlog.defer(128, functools.partial(unit, half, part, k))

    def accumulate_summary(first):
        backlog.drain()
        for r in range(0, HD, 256):
            for half in range(2):
                for o in range(0, 256, 64):
                    pair = (half * HD + r + o) // 64
                    kv = _dot(vt_v[pair], phik_v[pair], NT)
                    if first:
                        bias = _apply(jnp.multiply, column_v[pl.ds(pair * 64, 64), :], kv[64:72])
                        kv_v[pair] = jnp.concatenate([kv[:64] + bias, kv[64:]], axis=0)
                    else:
                        kv_v[pair] = kv_v[pair] + kv

    def finish_summary(pair):
        row = jax.lax.broadcasted_iota(I32, (80, 128), 0)
        row_head = jnp.where(row < 64, row >> 5, (row >> 3) & 1)
        col_head = jax.lax.broadcasted_iota(I32, (80, 128), 1) & 1
        summary_v[pair] = _pack(jnp.where(row_head == col_head, kv_v[pair], 0.0))

    def attend(step, target):
        t, lanes = step // 2, pl.ds(step % 2 * 2 * G, 2 * G)
        pairs = [[[half * NPAIR // 2 + 2 * i + k for k in range(2)] for half in range(2)] for i in range(4)]
        nums = {p: _dot(_unpack(summary_v[p]), phiq_v[t, p, :, lanes])
                for group in pairs for side in group for p in side}
        sides = []
        for i, group in enumerate(pairs):
            heads = [[_apply(jnp.multiply, nums[p][h * DH:(h + 1) * DH],
                             _recip(nums[p][64 + 8 * h:72 + 8 * h] + 1e-6))
                      for p in side for h in range(2)] for side in group]
            sides.append([jnp.concatenate(side, axis=0).T for side in heads])
            if i % 2:
                lo, hi = (jnp.concatenate([sides[i - 1][s], sides[i][s]], axis=1) for s in range(2))
                for j, term in enumerate(_lhs_terms(lo[:G], hi[:G], lo[G:], hi[G:])):
                    target[j, :, pl.ds((i - 1) * 128, 256)] = term.astype(BF16)

    def project_output(source, lo, n, hook):
        m = products(
            lambda j, k: _dot(source[j, pl.ds(lo, n), :],
                              _unpack(gated(wot_v, j)[:, k * 128:(k + 1) * 128])),
            HD // 128, 4 * n, hook)

        def rows(o):
            part, o = divmod(o, n)
            piece = lambda j: jnp.concatenate([tile[o:o + 32] for tile in m[j]], axis=1)
            return lo + part * G + o, jnp.concatenate(
                [_quadrant(2 * part + half, piece) for half in range(2)], axis=1)

        return rows

    scores = {}

    def finish(step, rows, count, strands, delay):
        chain = Chain(strands)
        lane = jax.lax.broadcasted_iota(I32, (8, 128), 1)
        for start_row in range(0, count, 32):
            row, y = rows(start_row)
            for o in range(0, 32, 8):
                base = step * 2 * G + row + o
                xn = x_v[pl.ds(base, 8), :].astype(F32) + mod_v[2] * chain.enter(y[o:o + 8])
                mean = jnp.mean(xn, axis=-1, keepdims=True)
                d = xn - mean
                scale = jax.lax.rsqrt(jnp.mean(d * d, axis=-1, keepdims=True) + EPS)
                score = jnp.sum(d * mod_v[6], axis=-1, keepdims=True) * scale + mod_v[9, :, :1]
                normed = d * scale
                norm_v[pl.ds(base, 8), :] = normed
                out = normed * mod_v[7] + ((d + mean) + mod_v[8])
                out_v[pl.ds(base, 8), :] = out.astype(BF16)
                held = scores.get(base // 1024, jnp.full((8, 128), -jnp.inf, F32))
                scores[base // 1024] = jnp.where(lane == base % 1024 // 8, score, held)
                chain.leave(*[out[:, l:l + 128] for l in range(128, D, 256)])
        if delay:
            finish_within(delay, *chain.tokens)

    def top_two():
        shape = (S // 1024, 8, 128)
        index = (jax.lax.broadcasted_iota(I32, shape, 0) * 1024 + jax.lax.broadcasted_iota(I32, shape, 2) * 8
                 + jax.lax.broadcasted_iota(I32, shape, 1)).astype(F32)
        left = jnp.stack([scores[b] for b in range(S // 1024)])
        reduce = lambda op, v: op(op(op(v, axis=0), axis=0, keepdims=True), axis=1, keepdims=True)
        top = reduce(jnp.max, left)
        first = reduce(jnp.min, jnp.where(left == top, index, float(S)))
        below = reduce(jnp.max, jnp.where(left == top, -jnp.inf, left))
        tied = reduce(jnp.min, jnp.where((left == top) & (index != first), index, float(S)))
        lower = reduce(jnp.min, jnp.where((left == below) & (left != top), index, float(S)))
        second = jnp.where(tied < S, tied, lower)
        row = lambda v: jnp.clip(jnp.max(v.astype(I32)), 0, S - 1)
        return (row(first), top), (row(second), jnp.where(tied < S, top, below))

    def routed_update():
        (row1, score1), (row2, score2) = top_two()
        sub = jax.lax.broadcasted_iota(I32, (16, D), 0)
        first, second = (jnp.broadcast_to(norm_v[pl.ds(row, 1), :], (16, D)) for row in (row1, row2))
        selected = jnp.where(sub == 0, first, second).reshape(2, 8, D) * mod_v[4] + mod_v[3]
        selected = selected.reshape(16, D).astype(BF16)
        pending = collections.deque()
        parts = []

        def down():
            f, g, u = pending.popleft()
            act = (g * jax.nn.sigmoid(g) * u).astype(BF16)
            part = _dot(act, wd_v[pl.ds(f, FF_CHUNK), :])
            parts.append(parts.pop() + part if parts else part)

        for f in range(0, FF, FF_CHUNK):
            pending.append((f, _dot(selected, wg_v[:, pl.ds(f, FF_CHUNK)]),
                            _dot(selected, wu_v[:, pl.ds(f, FF_CHUNK)])))
            if len(pending) > 2:
                down()
        while pending:
            down()
        y1, y2 = parts[0][0:1] * jax.nn.sigmoid(score1), parts[0][1:2] * jax.nn.sigmoid(score2)
        bases = [pl.multiple_of((row >> 4) * 16, 16) for row in (row1, row2)]
        for n, base in enumerate(bases):
            update = jnp.where(sub == row1 - base, y1, 0.0) + jnp.where(sub == row2 - base, y2, 0.0)
            rows = out_v[pl.ds(base, 16), :].astype(F32).reshape(2, 8, D) + mod_v[5] * update.reshape(2, 8, D)
            fix_v[n] = rows.reshape(16, D).astype(BF16)
        return bases

    cc = c_v[...].astype(F32)
    act_v[...] = _pack(jnp.broadcast_to(cc * jax.nn.sigmoid(cc), (16, D)))
    vt_v[:, pl.ds(64, 16), :] = jnp.ones((NPAIR, 16, T), BF16)
    wait(("x", 0))
    for n in range(T // 32):
        row_stats(0, n)
    for offset in range(0, T, 16):
        for lanes in (pl.ds(0, HD), pl.ds(HD, HD)):
            norm_v[pl.ds(offset, 16), lanes] = normalized(0, offset, lanes)
    first_rows = lambda offset, lanes: norm_v[pl.ds(offset, 16), lanes]
    for piece, lo in enumerate(range(0, HD, 256)):
        wait(*both("scale", piece))
        for column in (lo, HD + lo):
            for half in range(2):
                modulation(D + column, 256, half)
            mod_v[1, :, pl.ds(column, 256)] = raw_v[:, pl.ds(D + column, 256)] + 1.0
        for n in range(NORM_UNITS):
            norm_terms(first_rows, n, shift=False, lo=lo, width=256)(h_v)

    wait(*both("wv", 0))
    prep_values(0)
    plan = new_plan()
    plan[3] += [lambda: wait(*both("wv", 1)), lambda: prep_values(1)]
    plan[12] += [lambda: wait(*both("wv", 2))]
    plan[13] += [lambda: prep_values(2)]
    plan[15] += [lambda: prep_values(3)]
    plan[28] += [lambda: wait("wphi", *both("wk", 0)), feature_maps,
                 lambda: prep_scores(1, 0), lambda: prep_scores(1, 1)]

    def shift_vector():
        wait(*both("shift"))
        for half in range(2):
            modulation(0, D, half)
        mod_v[0] = raw(0)

    def shift_bias():
        shift = jnp.concatenate([raw(0)] * 2, axis=0).astype(BF16)
        bias_v[...] = _dot(shift, wqkv_v[:, pl.ds(2 * D, D)])[:8]

    plan[24] += [shift_vector, shift_bias]
    for n in range(NORM_UNITS):
        plan[25 + 4 * n // NORM_UNITS].append(
            functools.partial(lambda n: norm_terms(first_rows, n, delay=1)(h0_v), n))
    values(h_v, _follow(plan), store_values, 128)
    backlog.drain()

    plan = new_plan()
    plan[1].append(lambda: store_column(bias_v[...]))
    plan[4] += [lambda: wait(("x", 1), *both("wk", 1)), lambda: prep_scores(1, 2), lambda: prep_scores(1, 3)]
    plan[12].append(lambda: wait("wq"))
    for n in range(NORM_UNITS):
        plan[6 + n // 2].append(functools.partial(lambda n: tile_norm(1, n, 2 + n % 2)(h_v), n))
    plan[12].append(lambda: prep_scores(0, 0))
    features(wk_v, h0_v, _follow(plan), store_keys, 256)
    for g in range(1, 4):
        prep_scores(0, g)
        backlog.spent(512)
    backlog.drain()
    accumulate_summary(first=True)

    for t in range(1, NTILE):
        if t == NTILE - 1:
            wait(*[("mod", i) for i in range(NTILE)])
        if t == NTILE - 2:
            wait("wo")
        plan = new_plan()
        if t + 1 < NTILE:
            wait(("x", t + 1))
            stores = []
            for n in range(NORM_UNITS):
                plan[33 + n // 2].append(
                    functools.partial(lambda n: stores.append(tile_norm(t + 1, n, 2 + n % 2)), n))
            plan[42].append(lambda: [store(h_v) for store in stores])
        start(("wg", "wu", "wd")[t - 1])
        if t >= NTILE - 2:
            slots = range(3, 32, 2) if t == NTILE - 1 else range(1, 28, 2)
            for n in range(16):
                plan[slots[len(slots) * n // 16]].append(functools.partial(prep_output, t % 2 * 16 + n))
        if t == NTILE - 1:
            plan_vector_modulation(plan, (1, *range(32, 43)))
        due.clear()
        hook = _follow(plan)
        features(wk_v, h_v, hook, store_keys, 256)
        features(wq_v, h_v, hook, functools.partial(store_queries, t), 256)
        values(h_v, hook, store_values, 256)
        accumulate_summary(first=False)

    order = [(n + T // (2 * G)) % NSTEP for n in range(NSTEP)]
    plan = new_plan()
    plan[0] += [functools.partial(finish_summary, pair) for pair in range(NPAIR)]
    plan[2].append(lambda: wait("wr", "wg", "wu", "wd"))
    plan[10].append(output_weights)
    due.clear()
    features(wq_v, h0_v, _follow(plan), functools.partial(store_queries, 0), 128)
    attend(order[0], oa_v)

    due.clear()
    rows = None
    for n in range(NSTEP):
        source, target = ((oa_v, ob_v), (ob_v, oa_v))[n % 2]
        if n + 1 < NSTEP:
            attend(order[n + 1], target)
            if rows:
                finish(order[n - 1], rows, 2 * G, 3, 44)
            rows = project_output(source, 0, G, lambda: None)
        else:
            finish(order[n - 1], rows, 2 * G, 6, 26)
            rows = project_output(source, 0, G // 2, lambda: None)
            finish(order[n], rows, G, 8, 0)
            rows = project_output(source, G // 2, G // 2, lambda: None)
        if n > 1:
            out_copy(order[n - 2]).start()
    finish(order[-1], rows, G, G // 8, 0)
    out_copy(order[-2]).start()
    out_copy(order[-1]).start()

    base1, base2 = routed_update()
    for step in order:
        out_copy(step).wait()
    fix = [pltpu.make_async_copy(fix_v.at[n], out_hbm.at[pl.ds(base, 16)], out_sems.at[n])
           for n, base in enumerate((base1, base2))]
    fix[0].start()

    @pl.when(base1 != base2)
    def _():
        fix[1].start()
        fix[1].wait()

    fix[0].wait()


def _scratch():
    vmem = pltpu.VMEM
    return [
        vmem((S, D), BF16), vmem((D, 3 * D), BF16), vmem((D, DH), BF16), vmem((D, D), BF16),
        vmem((8, 128), BF16), vmem((D, FF), BF16), vmem((D, FF), BF16), vmem((FF, D), BF16),
        vmem((1, D), BF16), vmem((D, 6 * D), BF16),
        vmem((8, D), U32), vmem((D, 128), F32), vmem((8, 6 * D), F32), vmem((10, 8, D), F32), vmem((2, T, 128), F32),
        vmem((8, D), F32), vmem((D // 128, 64, 128), U32), vmem((7, HD // 2, HD), U32),
        vmem((7, HT // 2, HD), U32), vmem((7, HT // 2, HD), U32),
        vmem((NTILE, NPAIR, 128, T), BF16), vmem((NPAIR, 128, T), BF16), vmem((NPAIR, 80, T), BF16),
        vmem((NPAIR, 80, 128), F32), vmem((NPAIR, 40, 128), U32),
        vmem((7, G, HD), BF16), vmem((7, G, HD), BF16),
        vmem((S, D), F32), vmem((S, D), BF16), vmem((2, 16, D), BF16),
        pltpu.SemaphoreType.DMA((8 + 2 * NTILE + 16,)), pltpu.SemaphoreType.DMA((NSTEP,)),
    ] + [vmem((7, 64, HD), U32)] * 8 + [vmem((7, HD // 2, 128), U32)] * 4


@jax.jit
def pallas_adaLN_cond__linear_kernel_hedgehog__moe_arch_mod__prompt_kernel(
    A_x: jax.Array,
    A_wqkv: jax.Array,
    A_w_phi: jax.Array,
    A_wo: jax.Array,
    B_x: jax.Array,
    B_w_r: jax.Array,
    B_w_gate: jax.Array,
    B_w_up: jax.Array,
    B_w_down: jax.Array,
    c: jax.Array,
    w_mod: jax.Array,
):
    del B_x
    out = pl.pallas_call(
        _kernel,
        out_shape=jax.ShapeDtypeStruct((S, D), A_x.dtype),
        in_specs=[pl.BlockSpec(memory_space=pl.ANY)] * 10,
        out_specs=pl.BlockSpec(memory_space=pl.ANY),
        scratch_shapes=_scratch(),
        compiler_params=pltpu.CompilerParams(vmem_limit_bytes=120 * 2**20),
    )(A_x.reshape(S, D), A_wqkv, A_w_phi.reshape(D, DH), A_wo, B_w_r.reshape(8, 128),
      B_w_gate, B_w_up, B_w_down, c, w_mod)
    return out.reshape(A_x.shape)
```
